```python
import jax
import jax.numpy as jnp

def _softmax(x, axis=-1):
    return jax.nn.softmax(x, axis=axis)

def _gelu(x):
    return jax.nn.gelu(x, approximate=True)

def _silu(x):
    return jax.nn.silu(x)

def _sigmoid(x):
    return jax.nn.sigmoid(x)

def _layernorm(x, axis=-1, eps=1e-05):
    m = jnp.mean(x, axis=axis, keepdims=True)
    v = jnp.var(x, axis=axis, keepdims=True)
    return (x - m) / jnp.sqrt(v + eps)

def _scatter_add(tgt, idx, src, axis=0):
    return tgt.at[idx].add(src)

def _segment_sum(src, seg, n):
    return jax.ops.segment_sum(src, seg, n)

class _Rng:

    def __init__(self, key):
        self._k = key

    def _next(self):
        self._k, sub = jax.random.split(self._k)
        return sub

    def normal(self, shape):
        return jax.random.normal(self._next(), shape, dtype=jnp.bfloat16)

    def randint(self, lo, hi, shape):
        return jax.random.randint(self._next(), shape, lo, hi, dtype=jnp.int32)

    def uniform(self, shape, lo=0.0, hi=1.0):
        return jax.random.uniform(self._next(), shape, jnp.bfloat16, lo, hi)

    def permutation(self, n):
        return jax.random.permutation(self._next(), n)
kernel_name = 'sequential_preLN__memory_aug_recurrent_mem_tr__mixer_s_mlp__prompt'

def setup_inputs():
    _rng = _Rng(jax.random.key(int.from_bytes(__import__("os").urandom(4), "little")))
    _w = lambda a: (lambda t: t.astype(jnp.bfloat16) if jnp.issubdtype(t.dtype, jnp.floating) else t)(jnp.asarray(a))

    def _A_setup():
        B, S, Dm = (1, 2048, 1024)
        H, Dh = (32, 128)
        M, seg = (8, 32)
        seg = min(seg, S)
        S = S // seg * seg
        return {'x': _w((lambda *s: _rng.normal(s) * 0.05)(B, S, Dm)), 'mem0': _w((lambda *s: _rng.normal(s) * 0.05)(B, M, Dm)), 'Wq': _w((lambda *s: _rng.normal(s) * 0.05)(Dm, H, Dh) * Dm ** (-0.5)), 'Wk': _w((lambda *s: _rng.normal(s) * 0.05)(Dm, H, Dh) * Dm ** (-0.5)), 'Wv': _w((lambda *s: _rng.normal(s) * 0.05)(Dm, H, Dh) * Dm ** (-0.5)), 'Wo': _w((lambda *s: _rng.normal(s) * 0.05)(H, Dh, Dm) * (H * Dh) ** (-0.5)), 'seg_len': seg}
    _A_in = _A_setup()

    def _B_setup():
        B, S, D, F = (1, 2048, 1024, 3584)
        return {'x': _w((lambda *s: _rng.normal(s) * 0.05)(B, S, D)), 'w1': _w((lambda *s: _rng.normal(s) * 0.05)(D, D) * D ** (-0.5)), 'w2': _w((lambda *s: _rng.normal(s) * 0.05)(D, D) * D ** (-0.5)), 'w3': _w((lambda *s: _rng.normal(s) * 0.05)(D, F) * D ** (-0.5)), 'w4': _w((lambda *s: _rng.normal(s) * 0.05)(F, D) * F ** (-0.5))}
    _B_in = _B_setup()
    return {'A_x': _A_in['x'], 'A_mem0': _A_in['mem0'], 'A_Wq': _A_in['Wq'], 'A_Wk': _A_in['Wk'], 'A_Wv': _A_in['Wv'], 'A_Wo': _A_in['Wo'], 'A_seg_len': _A_in['seg_len'], 'B_x': _B_in['x'], 'B_w1': _B_in['w1'], 'B_w2': _B_in['w2'], 'B_w3': _B_in['w3'], 'B_w4': _B_in['w4']}

def reference(A_x, A_mem0, A_Wq, A_Wk, A_Wv, A_Wo, A_seg_len, B_x, B_w1, B_w2, B_w3, B_w4):

    def _A_ref(x, mem0, Wq, Wk, Wv, Wo, seg_len):
        B, S, Dm = x.shape
        H, Dh = (Wq.shape[1], Wq.shape[2])
        M = mem0.shape[1]
        scale = Dh ** (-0.5)
        n_seg = S // seg_len
        L = M + seg_len
        idx = jnp.arange(L)
        mask = (idx[:, None] < M) | (idx[:, None] >= idx[None, :])
        mem = mem0
        outs = []
        for s in range(n_seg):
            xs = x[:, s * seg_len:(s + 1) * seg_len, :].copy()
            h = jnp.concatenate([mem, xs], axis=1)
            q = jnp.einsum('btd,dhe->bhte', h, Wq)
            k = jnp.einsum('btd,dhe->bhte', h, Wk)
            v = jnp.einsum('btd,dhe->bhte', h, Wv)
            scores = jnp.einsum('bhqe,bhke->bhqk', q, k) * scale
            scores = jnp.where(mask[None, None], scores, -1000000000.0)
            p = _softmax(scores, axis=-1)
            o = jnp.einsum('bhqk,bhke->bhqe', p, v)
            o = jnp.einsum('bhte,hed->btd', o, Wo)
            mem = o[:, :M, :].copy()
            outs.append(o[:, M:, :])
        return jnp.concatenate(outs, axis=1)

    def _B_ref(x, w1, w2, w3, w4):
        B, S, D = x.shape
        h = _gelu(_layernorm(x, axis=-1) @ w1)
        c = D // 4
        g0 = jnp.pad(h[:, :, 0 * c:1 * c], ((0, 0), (1, 0), (0, 0)))[:, :S, :]
        g1 = jnp.pad(h[:, :, 1 * c:2 * c], ((0, 0), (0, 1), (0, 0)))[:, 1:, :]
        g2 = jnp.pad(h[:, :, 2 * c:3 * c], ((0, 0), (2, 0), (0, 0)))[:, :S, :]
        g3 = jnp.pad(h[:, :, 3 * c:], ((0, 0), (0, 2), (0, 0)))[:, 2:, :]
        hs = jnp.concatenate([g0, g1, g2, g3], axis=-1) @ w2
        x1 = x + hs
        h2 = _gelu(_layernorm(x1, axis=-1) @ w3) @ w4
        return x1 + h2
    x = A_x
    h = x + _A_ref(_layernorm(x, axis=-1), A_mem0, A_Wq, A_Wk, A_Wv, A_Wo, A_seg_len)
    h2 = h + _B_ref(_layernorm(h, axis=-1), B_w1, B_w2, B_w3, B_w4)
    return h2
```

```python
import functools

import jax
import jax.numpy as jnp
from jax.experimental import pallas as pl
from jax.experimental.pallas import tpu as pltpu

BF = jnp.bfloat16
F32 = jnp.float32

SEG = 32
MEM = 8
PAIR = 2 * SEG
LAG = 2
HALO = 8
LN_EPS = 1e-5
CFG = dict(a=True, b=True, att=True)


def _ln(x):
    m = jnp.mean(x, axis=-1, keepdims=True)
    xc = x - m
    v = jnp.mean(xc * xc, axis=-1, keepdims=True)
    return xc * jax.lax.rsqrt(v + LN_EPS)


def _dot(a, b):
    return jnp.dot(a, b, preferred_element_type=F32)


def _gelu(x):
    return jax.nn.gelu(x, approximate=True)


def _make_kernel(S, D, H, E, F):
    n_pairs = S // PAIR
    nD = D // 128
    nF = F // 128
    scale = float(E) ** -0.5
    L = MEM + SEG

    def attend(q, k, v, mask):
        if not CFG['att']:
            return q + k + v
        s = jax.lax.dot_general(q.astype(BF), k.astype(BF), (((1,), (1,)), ((), ())),
                                preferred_element_type=F32) * scale
        s = jnp.where(mask, s, -1000000000.0)
        m = jnp.max(s, axis=-1, keepdims=True)
        p = jnp.exp(s - m)
        l = jnp.sum(p, axis=-1, keepdims=True)
        p = p * pl.reciprocal(l, approx=False)
        return _dot(p.astype(BF), v.astype(BF))

    def kernel(x_ref, mem0_ref, wq_hbm, wk_hbm, wv_hbm, wo_hbm, w1_hbm, w2_hbm, w3_hbm, w4_hbm,
               out_ref,
               raw, wq_t, wk_t, wv_t, wo_t, w1_t, w2_t, w3_t, w4_t,
               lb_e, lb_o, sv, ob, h_buf, a1_buf, sems):
        t = pl.program_id(0)

        def raw_copy(i, src):
            return pltpu.make_async_copy(src, raw.at[i], sems.at[i])

        def col_copies(src, dst, n, sem_idx):
            return [pltpu.make_async_copy(src.at[:, pl.ds(j * 128, 128)], dst.at[j], sems.at[sem_idx])
                    for j in range(n)]

        def relayout(i, dst):
            def body(b, c):
                d0 = pl.multiple_of(b * 16, 16)
                blk = raw[i, pl.ds(d0, 16), :, :]
                dst[:, pl.ds(d0, 16), :] = jnp.swapaxes(blk, 0, 1)
                return c
            jax.lax.fori_loop(0, D // 16, body, 0)

        @pl.when(t == 0)
        def _():
            qkv = [raw_copy(0, wq_hbm), raw_copy(1, wk_hbm), raw_copy(2, wv_hbm)]
            rest = (col_copies(wo_hbm, wo_t, nD, 3) + col_copies(w1_hbm, w1_t, nD, 4)
                    + col_copies(w2_hbm, w2_t, nD, 4) + col_copies(w3_hbm, w3_t, nF, 4)
                    + col_copies(w4_hbm, w4_t, nD, 4))
            for c in qkv + rest:
                c.start()
            h_buf[pl.ds(0, HALO), :] = jnp.zeros((HALO, D), F32)
            h_buf[pl.ds(HALO + S, HALO), :] = jnp.zeros((HALO, D), F32)
            lb_e[pl.ds(40, MEM), :] = mem0_ref[...]
            for i, dst in enumerate((wq_t, wk_t, wv_t)):
                qkv[i].wait()
                relayout(i, dst)
            for c in col_copies(wo_hbm, wo_t, nD, 3):
                c.wait()

        @pl.when(t == LAG)
        def _():
            for c in (col_copies(w1_hbm, w1_t, nD, 4) + col_copies(w2_hbm, w2_t, nD, 4)
                      + col_copies(w3_hbm, w3_t, nF, 4) + col_copies(w4_hbm, w4_t, nD, 4)):
                c.wait()

        def part_a():
            if not CFG['a']:
                return
            row = jax.lax.broadcasted_iota(jnp.int32, (L, L), 0)
            col = jax.lax.broadcasted_iota(jnp.int32, (L, L), 1)
            mask = (col <= row) | (col >= SEG)

            x = x_ref[...].astype(F32)
            xn = _ln(x).astype(BF)
            lb_e[pl.ds(0, 8), :] = xn[32:40]
            lb_e[pl.ds(8, 32), :] = xn[0:32]
            lb_o[pl.ds(0, 24), :] = xn[40:64]

            lhs = lb_e[...]
            for h in range(H):
                q = _dot(lhs, wq_t[h])
                k = _dot(lhs, wk_t[h])
                v = _dot(lhs, wv_t[h])
                cs = pl.ds(h * E, E)
                sv[0, :, cs] = q[0:8]
                sv[1, :, cs] = k[0:8]
                sv[2, :, cs] = v[0:8]
                o = attend(q[8:48], k[8:48], v[8:48], mask).astype(BF)
                ob[pl.ds(32, 8), cs] = o[0:8]
                ob[pl.ds(0, 32), cs] = o[8:40]
            lhs = ob[pl.ds(0, 32), :]
            h0 = t * PAIR + HALO
            for j in range(nD):
                r = _dot(lhs, wo_t[j])
                cs = pl.ds(j * 128, 128)
                lb_o[pl.ds(24, 8), cs] = r[24:32].astype(BF)
                h_buf[pl.ds(pl.multiple_of(h0 + 8, 8), 24), cs] = x[8:32, j * 128:(j + 1) * 128] + r[0:24]

            lhs = lb_o[...]
            for h in range(H):
                cs = pl.ds(h * E, E)
                q = jnp.concatenate([sv[0, :, cs], _dot(lhs, wq_t[h])], axis=0)
                k = jnp.concatenate([sv[1, :, cs], _dot(lhs, wk_t[h])], axis=0)
                v = jnp.concatenate([sv[2, :, cs], _dot(lhs, wv_t[h])], axis=0)
                ob[pl.ds(40, 40), cs] = attend(q, k, v, mask).astype(BF)
            lhs = ob[pl.ds(32, 48), :]
            for j in range(nD):
                r = _dot(lhs, wo_t[j])
                cs = pl.ds(j * 128, 128)
                lb_e[pl.ds(40, 8), cs] = r[40:48].astype(BF)
                h_buf[pl.ds(pl.multiple_of(h0, 8), 8), cs] = x[0:8, j * 128:(j + 1) * 128] + r[0:8]
                h_buf[pl.ds(pl.multiple_of(h0 + 32, 8), 32), cs] = x[32:64, j * 128:(j + 1) * 128] + r[8:40]

        def part_b():
            if not CFG['b']:
                out_ref[...] = h_buf[pl.ds(pl.multiple_of((t - LAG) * PAIR + HALO, 8), PAIR), :].astype(out_ref.dtype)
                return
            c = t - LAG
            r0 = pl.multiple_of(c * PAIR, PAIR)
            R = PAIR + 2 * HALO
            hh = h_buf[pl.ds(r0, R), :]
            y = _ln(hh)
            z = _ln(y).astype(BF)
            tok = jax.lax.broadcasted_iota(jnp.int32, (R, 128), 0) + (r0 - HALO)
            valid = (tok >= 0) & (tok < S)
            for j in range(nD):
                a = _gelu(_dot(z, w1_t[j]))
                a1_buf[:, pl.ds(j * 128, 128)] = jnp.where(valid, a, 0.0)
            cq = D // 4
            g = jnp.concatenate([
                a1_buf[pl.ds(HALO - 1, PAIR), pl.ds(0 * cq, cq)],
                a1_buf[pl.ds(HALO + 1, PAIR), pl.ds(1 * cq, cq)],
                a1_buf[pl.ds(HALO - 2, PAIR), pl.ds(2 * cq, cq)],
                a1_buf[pl.ds(HALO + 2, PAIR), pl.ds(3 * cq, cq)]], axis=1).astype(BF)
            x1 = y[HALO:HALO + PAIR] + jnp.concatenate([_dot(g, w2_t[j]) for j in range(nD)], axis=1)
            z1 = _ln(x1).astype(BF)
            a3 = jnp.concatenate([_gelu(_dot(z1, w3_t[j])).astype(BF) for j in range(nF)], axis=1)
            h2 = jnp.concatenate([_dot(a3, w4_t[j]) for j in range(nD)], axis=1)
            out_ref[...] = (hh[HALO:HALO + PAIR] + (x1 + h2)).astype(out_ref.dtype)

        @pl.when(t < LAG)
        def _():
            part_a()

        @pl.when(jnp.logical_and(t >= LAG, t < n_pairs))
        def _():
            part_a()
            part_b()

        @pl.when(t >= n_pairs)
        def _():
            part_b()

    return kernel


@functools.partial(jax.jit, static_argnames=("A_seg_len",))
def pallas_sequential_preLN__memory_aug_recurrent_mem_tr__mixer_s_mlp__prompt_kernel(
    A_x, A_mem0, A_Wq, A_Wk, A_Wv, A_Wo, A_seg_len, B_x, B_w1, B_w2, B_w3, B_w4,
):
    _, S, D = A_x.shape
    H, E = A_Wq.shape[1], A_Wq.shape[2]
    F = B_w3.shape[1]
    assert A_seg_len == SEG and A_mem0.shape[1] == MEM and S % PAIR == 0
    n_pairs = S // PAIR
    nD, nF = D // 128, F // 128

    x = A_x.reshape(S, D)
    mem0 = A_mem0.reshape(MEM, D)
    wo = A_Wo.reshape(H * E, D)

    any_spec = pl.BlockSpec(memory_space=pl.ANY)
    out = pl.pallas_call(
        _make_kernel(S, D, H, E, F),
        grid=(n_pairs + LAG,),
        in_specs=[
            pl.BlockSpec((PAIR, D), lambda t: (jnp.minimum(t, n_pairs - 1), 0)),
            pl.BlockSpec((MEM, D), lambda t: (0, 0)),
        ] + [any_spec] * 8,
        out_specs=pl.BlockSpec((PAIR, D), lambda t: (jnp.maximum(t - LAG, 0), 0)),
        out_shape=jax.ShapeDtypeStruct((S, D), A_x.dtype),
        scratch_shapes=[
            pltpu.VMEM((3, D, H, E), BF),
            pltpu.VMEM((H, D, E), BF),
            pltpu.VMEM((H, D, E), BF),
            pltpu.VMEM((H, D, E), BF),
            pltpu.VMEM((nD, H * E, 128), BF),
            pltpu.VMEM((nD, D, 128), BF),
            pltpu.VMEM((nD, D, 128), BF),
            pltpu.VMEM((nF, D, 128), BF),
            pltpu.VMEM((nD, F, 128), BF),
            pltpu.VMEM((48, D), BF),
            pltpu.VMEM((32, D), BF),
            pltpu.VMEM((3, 8, H * E), F32),
            pltpu.VMEM((80, H * E), BF),
            pltpu.VMEM((S + 2 * HALO, D), F32),
            pltpu.VMEM((PAIR + 2 * HALO, D), F32),
            pltpu.SemaphoreType.DMA((5,)),
        ],
        compiler_params=pltpu.CompilerParams(
            dimension_semantics=("arbitrary",),
            vmem_limit_bytes=120 * 1024 * 1024,
        ),
    )(x, mem0, A_Wq, A_Wk, A_Wv, wo, B_w1, B_w2, B_w3, B_w4)
    return out.reshape(1, S, D)
```

```python
import functools

import jax
import jax.numpy as jnp
from jax.experimental import pallas as pl
from jax.experimental.pallas import tpu as pltpu

BF = jnp.bfloat16
F32 = jnp.float32
U32 = jnp.uint32

SEG = 32
MEM = 8
PAIR = 2 * SEG
LAG = 2
HALO = 8
LN_EPS = 1e-5
LOG2E = 1.4426950408889634
CFG = dict(a=True, b=True, att=True, G=2, tail_heads=4, fuse=True)


def _ln(x):
    m = jnp.mean(x, axis=-1, keepdims=True)
    xc = x - m
    v = jnp.mean(xc * xc, axis=-1, keepdims=True)
    return xc * jax.lax.rsqrt(v + LN_EPS)


def _dot(a, b):
    return jnp.dot(a, b, preferred_element_type=F32)


def _gelu(x):
    return jax.nn.gelu(x, approximate=True)


def _as_bf(x_u32):
    return pltpu.bitcast(x_u32, BF)


def _as_u32(x_bf):
    return pltpu.bitcast(x_bf, U32)


def _interleave(main, fill):
    out = []
    for i, j in enumerate(main):
        out.extend(fill.get(i, []))
        out.append(j)
    out.extend(fill.get(len(main), []))
    return out


def _make_kernel(S, D, H, E, F):
    n_pairs = S // PAIR
    nD = D // 128
    nF = F // 128
    c_exp = float(E) ** -0.5 * LOG2E
    neg_raw = -1000000000.0 / (float(E) ** -0.5)
    L = MEM + SEG
    G = CFG['G']
    n_slots = H // G
    TH = CFG['tail_heads']
    K1 = (H - TH) * E

    def kernel(x_ref, xn_ref, mem0_ref, wq_hbm, wk_hbm, wv_hbm, wo_hbm, w1_hbm, w2_hbm, w3_hbm, w4_hbm,
               out_ref,
               raw, wq_t, wk_t, wv_t, wo_t, w1_t, w2_t, w3_t, w4_t,
               lb_e, lb_o, sv, ob, h_buf, a1_buf, sems):
        t = pl.program_id(0)

        def raw_copy(i, src):
            return pltpu.make_async_copy(src, raw.at[i], sems.at[i])

        def col_copies(src, dst, n, sem_idx):
            return [pltpu.make_async_copy(src.at[:, pl.ds(j * 128, 128)], dst.at[j], sems.at[sem_idx])
                    for j in range(n)]

        def relayout(i, dst):
            def body(b, c):
                blk = raw[i, pl.ds(pl.multiple_of(b * 16, 16), 16), :, :]
                dst[:, pl.ds(pl.multiple_of(b * 8, 8), 8), :] = _as_u32(jnp.swapaxes(blk, 0, 1))
                return c
            jax.lax.fori_loop(0, D // 16, body, 0)

        def store_xn(x_bf):
            xn = _ln(x_bf.astype(F32))
            lb_e[pl.ds(0, 4), :] = _as_u32(xn[32:40].astype(BF))
            lb_e[pl.ds(4, 4), :] = _as_u32(xn[0:8].astype(BF))
            lb_e[pl.ds(8, 8), :] = _as_u32(xn[8:24].astype(BF))
            lb_e[pl.ds(16, 4), :] = _as_u32(xn[24:32].astype(BF))
            lb_o[pl.ds(0, 8), :] = _as_u32(xn[40:56].astype(BF))
            lb_o[pl.ds(8, 4), :] = _as_u32(xn[56:64].astype(BF))

        @pl.when(t == 0)
        def _():
            qkv = [raw_copy(0, wq_hbm), raw_copy(1, wk_hbm), raw_copy(2, wv_hbm)]
            rest = (col_copies(wo_hbm, wo_t, nD, 3) + col_copies(w1_hbm, w1_t, nD, 4)
                    + col_copies(w2_hbm, w2_t, nD, 4) + col_copies(w3_hbm, w3_t, nF, 4)
                    + col_copies(w4_hbm, w4_t, nD, 4))
            for c in qkv + rest:
                c.start()
            h_buf[pl.ds(0, HALO), :] = jnp.zeros((HALO, D), F32)
            h_buf[pl.ds(HALO + S, HALO), :] = jnp.zeros((HALO, D), F32)
            lb_e[pl.ds(20, 4), :] = _as_u32(mem0_ref[...])
            store_xn(x_ref[...])
            for i, dst in enumerate((wq_t, wk_t, wv_t)):
                qkv[i].wait()
                relayout(i, dst)
            for c in col_copies(wo_hbm, wo_t, nD, 3):
                c.wait()

        @pl.when(t == LAG)
        def _():
            for c in (col_copies(w1_hbm, w1_t, nD, 4) + col_copies(w2_hbm, w2_t, nD, 4)
                      + col_copies(w3_hbm, w3_t, nF, 4) + col_copies(w4_hbm, w4_t, nD, 4)):
                c.wait()

        def a_jobs():
            row = jax.lax.broadcasted_iota(jnp.int32, (L, L), 0)
            col = jax.lax.broadcasted_iota(jnp.int32, (L, L), 1)
            mask = (col <= row) | (col >= SEG)
            h0 = t * PAIR + HALO

            def step_jobs(even):
                lb = lb_e if even else lb_o
                st = {}

                def j_qkv(g):
                    def run():
                        lhs = _as_bf(lb[...])
                        for h in range(g * G, (g + 1) * G):
                            cs = pl.ds(h * E, E)
                            r = [_dot(lhs, _as_bf(w[h])) for w in (wq_t, wk_t, wv_t)]
                            if even:
                                for i in range(3):
                                    sv[i, :, cs] = r[i][0:8]
                                r = [a[8:48] for a in r]
                            else:
                                r = [jnp.concatenate([sv[i, :, cs], r[i]], axis=0) for i in range(3)]
                            st['qkv', h] = [a.astype(BF) for a in r]
                    return run

                def j_s(g):
                    def run():
                        for h in range(g * G, (g + 1) * G):
                            q, k, v = st.pop(('qkv', h))
                            if not CFG['att']:
                                st['p', h] = (q + k, v, None)
                                continue
                            s = jax.lax.dot_general(q, k, (((1,), (1,)), ((), ())),
                                                    preferred_element_type=F32)
                            s = jnp.where(mask, s, neg_raw)
                            m = jnp.max(s, axis=-1, keepdims=True)
                            p = jnp.exp2((s - m) * c_exp)
                            l = jnp.sum(p, axis=-1, keepdims=True)
                            r0 = pl.reciprocal(l, approx=True)
                            st['p', h] = (p.astype(BF), v, r0 * (2.0 - l * r0))
                    return run

                def j_pv(g):
                    def run():
                        for h in range(g * G, (g + 1) * G):
                            p, v, r = st.pop(('p', h))
                            cs = pl.ds(h * E, E)
                            o = (_dot(p, v) * r) if CFG['att'] else (p + v).astype(F32)
                            if even:
                                ob[pl.ds(16, 4), cs] = _as_u32(o[0:8].astype(BF))
                                ob[pl.ds(0, 16), cs] = _as_u32(o[8:40].astype(BF))
                            else:
                                ob[pl.ds(20, 4), cs] = _as_u32(o[0:8].astype(BF))
                                ob[pl.ds(24, 16), cs] = _as_u32(o[8:40].astype(BF))
                    return run

                rows = pl.ds(0, 16) if even else pl.ds(16, 24)

                def j_wo1(j):
                    def run():
                        lhs = _as_bf(ob[rows, pl.ds(0, K1)])
                        st['wo', j] = _dot(lhs, wo_t[j, pl.ds(0, K1), :])
                    return run

                def j_wo2(j):
                    def run():
                        lhs = _as_bf(ob[rows, pl.ds(K1, H * E - K1)])
                        r = st.pop(('wo', j)) + _dot(lhs, wo_t[j, pl.ds(K1, H * E - K1), :])
                        cs = pl.ds(j * 128, 128)
                        xs = x_ref[:, cs].astype(F32)
                        if even:
                            lb_o[pl.ds(12, 4), cs] = _as_u32(r[24:32].astype(BF))
                            h_buf[pl.ds(pl.multiple_of(h0 + 8, 8), 24), cs] = xs[8:32] + r[0:24]
                        else:
                            lb_e[pl.ds(20, 4), cs] = _as_u32(r[40:48].astype(BF))
                            h_buf[pl.ds(pl.multiple_of(h0, 8), 8), cs] = xs[0:8] + r[0:8]
                            h_buf[pl.ds(pl.multiple_of(h0 + 32, 8), 32), cs] = xs[32:64] + r[8:40]
                    return run

                jobs = []
                for g in range(n_slots):
                    jobs.append(j_qkv(g))
                    if g >= 1:
                        jobs.append(j_s(g - 1))
                    if g >= 2:
                        jobs.append(j_pv(g - 2))
                n_main = len(jobs)
                last_need = (H - TH) // G - 1
                pend = [j_s(n_slots - 1), j_pv(n_slots - 2), j_pv(n_slots - 1)]
                if last_need >= n_slots - 2:
                    raise ValueError("tail_heads too small")
                jobs += [j_wo1(0), j_wo1(1), j_wo1(2), pend[0], pend[1],
                         j_wo1(3), j_wo1(4), j_wo1(5), pend[2], j_wo1(6), j_wo1(7)]
                jobs += [j_wo2(j) for j in range(nD)]
                return jobs, n_main

            def j_next_xn():
                store_xn(xn_ref[...])

            ej, e_main = step_jobs(True)
            oj, o_main = step_jobs(False)
            last_qkv = 3 * (n_slots - 1) - 1 if n_slots > 2 else 0
            idx = [i for i in range(o_main)][-3] + 1
            oj = oj[:idx] + [j_next_xn] + oj[idx:]
            return ej, oj

        def b_jobs():
            c = t - LAG
            r0 = pl.multiple_of(c * PAIR, PAIR)
            R = PAIR + 2 * HALO
            st = {}

            def j_pre():
                hh = h_buf[pl.ds(r0, R), :]
                y = _ln(hh)
                st['y'] = y[HALO:HALO + PAIR]
                st['z'] = _ln(y).astype(BF)

            def j_w1(j):
                def run():
                    tok = jax.lax.broadcasted_iota(jnp.int32, (R, 128), 0) + (r0 - HALO)
                    valid = (tok >= 0) & (tok < S)
                    a = _gelu(_dot(st['z'], w1_t[j]))
                    a1_buf[:, pl.ds(j * 128, 128)] = jnp.where(valid, a, 0.0)
                return run

            def j_shift():
                cq = D // 4
                st['g'] = jnp.concatenate([
                    a1_buf[pl.ds(HALO - 1, PAIR), pl.ds(0 * cq, cq)],
                    a1_buf[pl.ds(HALO + 1, PAIR), pl.ds(1 * cq, cq)],
                    a1_buf[pl.ds(HALO - 2, PAIR), pl.ds(2 * cq, cq)],
                    a1_buf[pl.ds(HALO + 2, PAIR), pl.ds(3 * cq, cq)]], axis=1).astype(BF)

            def j_w2(j):
                def run():
                    st['x1', j] = st['y'][:, j * 128:(j + 1) * 128] + _dot(st['g'], w2_t[j])
                return run

            def j_ln3():
                x1 = jnp.concatenate([st['x1', j] for j in range(nD)], axis=1)
                st['z1'] = _ln(x1).astype(BF)

            def j_w3(j):
                def run():
                    st['a3', j] = _gelu(_dot(st['z1'], w3_t[j])).astype(BF)
                return run

            def j_cat():
                st['a3'] = jnp.concatenate([st.pop(('a3', j)) for j in range(nF)], axis=1)

            def j_w4(j):
                def run():
                    cs = pl.ds(j * 128, 128)
                    hh = h_buf[pl.ds(pl.multiple_of(r0 + HALO, 8), PAIR), cs]
                    out_ref[:, cs] = (hh + (st['x1', j] + _dot(st['a3'], w4_t[j]))).astype(out_ref.dtype)
                return run

            return dict(pre=j_pre, w1=[j_w1(j) for j in range(nD)], shift=j_shift,
                        w2=[j_w2(j) for j in range(nD)], ln3=j_ln3,
                        w3=[j_w3(j) for j in range(nF)], cat=j_cat,
                        w4=[j_w4(j) for j in range(nD)])

        def b_flat(b):
            return [b['pre']] + b['w1'] + [b['shift']] + b['w2'] + [b['ln3']] + b['w3'] + [b['cat']] + b['w4']

        def run_jobs(jobs):
            for j in jobs:
                j()

        def part_a():
            if CFG['a']:
                ej, oj = a_jobs()
                run_jobs(ej + oj)

        def part_b():
            if CFG['b']:
                run_jobs(b_flat(b_jobs()))
            else:
                out_ref[...] = h_buf[pl.ds(pl.multiple_of((t - LAG) * PAIR + HALO, 8), PAIR), :].astype(out_ref.dtype)

        def part_ab():
            if not (CFG['a'] and CFG['b'] and CFG['fuse']):
                part_a()
                part_b()
                return
            ej, oj = a_jobs()
            b = b_jobs()
            w3 = b['w3']
            def slot_pos(g):
                return 0 if g == 0 else (1 if g == 1 else 3 * (g - 1))
            fe = {0: [b['pre']]}
            for i in range(nD):
                fe.setdefault(slot_pos(2 + i // 2), []).append(b['w1'][i])
            fe.setdefault(slot_pos(6), []).append(b['shift'])
            for i in range(nD):
                fe.setdefault(slot_pos(8 + i // 2), []).append(b['w2'][i])
            fe.setdefault(slot_pos(12), []).append(b['ln3'])
            fe.setdefault(slot_pos(14), []).extend(w3[0:2])
            fe.setdefault(slot_pos(15), []).extend(w3[2:4])
            fe.setdefault(len(ej), []).extend(w3[4:7])
            fo = {}
            k = 7
            for g in range(1, 11):
                fo.setdefault(slot_pos(g), []).extend(w3[k:k + 2])
                k += 2
            fo.setdefault(slot_pos(11), []).append(w3[27])
            fo.setdefault(slot_pos(12), []).append(b['cat'])
            w4 = b['w4']
            fo.setdefault(slot_pos(13) + 1, []).append(w4[0])
            fo.setdefault(slot_pos(14) + 1, []).append(w4[1])
            fo.setdefault(slot_pos(15) + 1, []).append(w4[2])
            fo.setdefault(len(oj), []).extend(w4[3:])
            run_jobs(_interleave(ej, fe) + _interleave(oj, fo))

        @pl.when(t < LAG)
        def _():
            part_a()

        @pl.when(jnp.logical_and(t >= LAG, t < n_pairs))
        def _():
            part_ab()

        @pl.when(t >= n_pairs)
        def _():
            part_b()

    return kernel


@functools.partial(jax.jit, static_argnames=("A_seg_len",))
def pallas_sequential_preLN__memory_aug_recurrent_mem_tr__mixer_s_mlp__prompt_kernel(
    A_x, A_mem0, A_Wq, A_Wk, A_Wv, A_Wo, A_seg_len, B_x, B_w1, B_w2, B_w3, B_w4,
):
    _, S, D = A_x.shape
    H, E = A_Wq.shape[1], A_Wq.shape[2]
    F = B_w3.shape[1]
    assert A_seg_len == SEG and A_mem0.shape[1] == MEM and S % PAIR == 0
    n_pairs = S // PAIR
    nD, nF = D // 128, F // 128

    x = A_x.reshape(S, D)
    mem0 = A_mem0.reshape(MEM, D)
    wo = A_Wo.reshape(H * E, D)

    any_spec = pl.BlockSpec(memory_space=pl.ANY)
    out = pl.pallas_call(
        _make_kernel(S, D, H, E, F),
        grid=(n_pairs + LAG,),
        in_specs=[
            pl.BlockSpec((PAIR, D), lambda t: (jnp.minimum(t, n_pairs - 1), 0)),
            pl.BlockSpec((PAIR, D), lambda t: (jnp.minimum(t + 1, n_pairs - 1), 0)),
            pl.BlockSpec((MEM, D), lambda t: (0, 0)),
        ] + [any_spec] * 8,
        out_specs=pl.BlockSpec((PAIR, D), lambda t: (jnp.maximum(t - LAG, 0), 0)),
        out_shape=jax.ShapeDtypeStruct((S, D), A_x.dtype),
        scratch_shapes=[
            pltpu.VMEM((3, D, H, E), BF),
            pltpu.VMEM((H, D // 2, E), U32),
            pltpu.VMEM((H, D // 2, E), U32),
            pltpu.VMEM((H, D // 2, E), U32),
            pltpu.VMEM((nD, H * E, 128), BF),
            pltpu.VMEM((nD, D, 128), BF),
            pltpu.VMEM((nD, D, 128), BF),
            pltpu.VMEM((nF, D, 128), BF),
            pltpu.VMEM((nD, F, 128), BF),
            pltpu.VMEM((24, D), U32),
            pltpu.VMEM((16, D), U32),
            pltpu.VMEM((3, 8, H * E), F32),
            pltpu.VMEM((40, H * E), U32),
            pltpu.VMEM((S + 2 * HALO, D), F32),
            pltpu.VMEM((PAIR + 2 * HALO, D), F32),
            pltpu.SemaphoreType.DMA((5,)),
        ],
        compiler_params=pltpu.CompilerParams(
            dimension_semantics=("arbitrary",),
            vmem_limit_bytes=120 * 1024 * 1024,
        ),
    )(x, x, mem0, A_Wq, A_Wk, A_Wv, wo, B_w1, B_w2, B_w3, B_w4)
    return out.reshape(1, S, D)
```

```python
import functools

import jax
import jax.numpy as jnp
from jax.experimental import pallas as pl
from jax.experimental.pallas import tpu as pltpu

BF = jnp.bfloat16
F32 = jnp.float32
U32 = jnp.uint32

SEG = 32
MEM = 8
PAIR = 2 * SEG
LAG = 2
HALO = 8
LN_EPS = 1e-5
LOG2E = 1.4426950408889634
CFG = dict(a=True, b=True, att=True, G=2, tail_heads=4, fuse=True)


def _ln(x):
    m = jnp.mean(x, axis=-1, keepdims=True)
    xc = x - m
    v = jnp.mean(xc * xc, axis=-1, keepdims=True)
    return xc * jax.lax.rsqrt(v + LN_EPS)


_dot = functools.partial(jnp.dot, preferred_element_type=F32)


def _gelu(x):
    return jax.nn.gelu(x, approximate=True)


def _as_bf(x_u32):
    return pltpu.bitcast(x_u32, BF)


def _as_u32(x_bf):
    return pltpu.bitcast(x_bf, U32)


def _interleave(main, fill):
    out = []
    for i, j in enumerate(main):
        out.extend(fill.get(i, []))
        out.append(j)
    out.extend(fill.get(len(main), []))
    return out


def _make_kernel(S, D, H, E, F):
    n_pairs = S // PAIR
    nD = D // 128
    nF = F // 128
    c_exp = float(E) ** -0.5 * LOG2E
    neg_raw = -1000000000.0 / (float(E) ** -0.5)
    L = MEM + SEG
    G = CFG['G']
    n_slots = H // G
    TH = CFG['tail_heads']
    K1 = (H - TH) * E

    def kernel(x_ref, xn_ref, mem0_ref, wq_hbm, wk_hbm, wv_hbm, wo_hbm, w1_hbm, w2_hbm, w3_hbm, w4_hbm,
               out_ref,
               raw, wq_t, wk_t, wv_t, wo_raw, wo_t, w1_t, w2_t, w3_t, w4_t,
               lb_e, lb_o, sv, ob, wacc, h_buf, a1_buf, sems):
        t = pl.program_id(0)

        NCH = 4
        CH = D // NCH

        def raw_copy(i, c, src):
            return pltpu.make_async_copy(src.at[pl.ds(c * CH, CH)], raw.at[i, pl.ds(c * CH, CH)],
                                         sems.at[i * NCH + c])

        def col_copies(src, dst, n, sem_idx):
            return [pltpu.make_async_copy(src.at[:, pl.ds(j * 128, 128)], dst.at[j], sems.at[sem_idx])
                    for j in range(n)]

        WO_SEM = 3 * NCH
        B_SEM = WO_SEM + nD

        def wo_copy(j):
            return pltpu.make_async_copy(wo_hbm.at[:, pl.ds(j * 128, 128)], wo_raw.at[j], sems.at[WO_SEM + j])

        def wo_finish():
            for j in range(nD):
                wo_copy(j).wait()

                def body(b, carry):
                    blk = wo_raw[j, pl.ds(pl.multiple_of(b * 256, 256), 256), :]
                    wo_t[j, pl.ds(pl.multiple_of(b * 128, 128), 128), :] = _as_u32(blk)
                    return carry
                jax.lax.fori_loop(0, H * E // 256, body, 0)

        def b_copies():
            return (col_copies(w1_hbm, w1_t, nD, B_SEM) + col_copies(w2_hbm, w2_t, nD, B_SEM)
                    + col_copies(w3_hbm, w3_t, nF, B_SEM) + col_copies(w4_hbm, w4_t, nD, B_SEM))

        def relayout(i, c, dst):
            def body(b, carry):
                blk = raw[i, pl.ds(pl.multiple_of(b * 16, 16), 16), :, :]
                dst[:, pl.ds(pl.multiple_of(b * 8, 8), 8), :] = _as_u32(jnp.swapaxes(blk, 0, 1))
                return carry
            jax.lax.fori_loop(c * (CH // 16), (c + 1) * (CH // 16), body, 0)

        def store_xn(x_bf):
            xn = _ln(x_bf.astype(F32))
            lb_e[pl.ds(0, 4), :] = _as_u32(xn[32:40].astype(BF))
            lb_e[pl.ds(4, 4), :] = _as_u32(xn[0:8].astype(BF))
            lb_e[pl.ds(8, 8), :] = _as_u32(xn[8:24].astype(BF))
            lb_e[pl.ds(16, 4), :] = _as_u32(xn[24:32].astype(BF))
            lb_o[pl.ds(0, 8), :] = _as_u32(xn[40:56].astype(BF))
            lb_o[pl.ds(8, 4), :] = _as_u32(xn[56:64].astype(BF))

        @pl.when(t == 0)
        def _():
            srcs = (wq_hbm, wk_hbm, wv_hbm)
            qkv = [[raw_copy(i, c, srcs[i]) for c in range(NCH)] for i in range(3)]
            for i in range(3):
                for c in range(NCH):
                    qkv[i][c].start()
            for j in range(nD):
                wo_copy(j).start()
            h_buf[pl.ds(0, HALO), :] = jnp.zeros((HALO, D), F32)
            h_buf[pl.ds(HALO + S, HALO), :] = jnp.zeros((HALO, D), F32)
            lb_e[pl.ds(20, 4), :] = _as_u32(mem0_ref[...])
            store_xn(x_ref[...])
            for i, dst in enumerate((wq_t, wk_t, wv_t)):
                for c in range(NCH):
                    qkv[i][c].wait()
                    relayout(i, c, dst)
            for c in b_copies():
                c.start()
            if not CFG['a']:
                wo_finish()

        @pl.when(t == LAG)
        def _():
            for c in b_copies():
                c.wait()

        def a_jobs():
            row = jax.lax.broadcasted_iota(jnp.int32, (G * L, G * L), 0)
            col = jax.lax.broadcasted_iota(jnp.int32, (G * L, G * L), 1)
            mask = None
            for i in range(G):
                rl, cl = row - i * L, col - i * L
                blk = ((rl >= 0) & (rl < L) & (cl >= 0) & (cl < L)) & ((cl <= rl) | (cl >= SEG))
                mask = blk if mask is None else (mask | blk)
            h0 = t * PAIR + HALO

            def step_jobs(even):
                lb = lb_e if even else lb_o
                st = {}

                def j_qkv(g):
                    def run():
                        lhs = _as_bf(lb[...])
                        parts = [[], [], []]
                        for h in range(g * G, (g + 1) * G):
                            cs = pl.ds(h * E, E)
                            r = [_dot(lhs, _as_bf(w[h])) for w in (wq_t, wk_t, wv_t)]
                            for i in range(3):
                                if even:
                                    sv[i, :, cs] = r[i][0:8]
                                    parts[i].append(r[i][8:48])
                                else:
                                    parts[i] += [sv[i, :, cs], r[i]]
                        st['qkv', g] = [jnp.concatenate(a, axis=0).astype(BF) for a in parts]
                    return run

                def j_s(g):
                    def run():
                        q, k, v = st.pop(('qkv', g))
                        if not CFG['att']:
                            st['p', g] = (q + k, v, None)
                            return
                        s = jax.lax.dot_general(q, k, (((1,), (1,)), ((), ())),
                                                preferred_element_type=F32)
                        s = jnp.where(mask, s, neg_raw)
                        m = jnp.max(s, axis=-1, keepdims=True)
                        p = jnp.exp2((s - m) * c_exp)
                        l = jnp.sum(p, axis=-1, keepdims=True)
                        r0 = pl.reciprocal(l, approx=True)
                        p = p * (r0 * (2.0 - l * r0))
                        st['p', g] = (p.astype(BF), v, None)
                    return run

                def j_pv(g):
                    def run():
                        p, v, r = st.pop(('p', g))
                        o2 = _dot(p, v) if CFG['att'] else (p + v).astype(F32)
                        for i, h in enumerate(range(g * G, (g + 1) * G)):
                            o = o2[i * L:(i + 1) * L]
                            cs = pl.ds(h * E, E)
                            if even:
                                ob[pl.ds(16, 4), cs] = _as_u32(o[0:8].astype(BF))
                                ob[pl.ds(0, 16), cs] = _as_u32(o[8:40].astype(BF))
                            else:
                                ob[pl.ds(20, 4), cs] = _as_u32(o[0:8].astype(BF))
                                ob[pl.ds(24, 16), cs] = _as_u32(o[8:40].astype(BF))
                    return run

                rows = pl.ds(0, 16) if even else pl.ds(16, 24)
                nrows = 32 if even else 48

                def j_wo1(j):
                    def run():
                        lhs = _as_bf(ob[rows, pl.ds(0, K1)])
                        wacc[pl.ds(0, nrows), pl.ds(j * 128, 128)] = _dot(lhs, _as_bf(wo_t[j, pl.ds(0, K1 // 2), :]))
                    return run

                def j_wo2(j):
                    def run():
                        lhs = _as_bf(ob[rows, pl.ds(K1, H * E - K1)])
                        r = wacc[pl.ds(0, nrows), pl.ds(j * 128, 128)] + _dot(lhs, _as_bf(wo_t[j, pl.ds(K1 // 2, (H * E - K1) // 2), :]))
                        cs = pl.ds(j * 128, 128)
                        xs = x_ref[:, cs].astype(F32)
                        if even:
                            lb_o[pl.ds(12, 4), cs] = _as_u32(r[24:32].astype(BF))
                            h_buf[pl.ds(pl.multiple_of(h0 + 8, 8), 24), cs] = xs[8:32] + r[0:24]
                        else:
                            lb_e[pl.ds(20, 4), cs] = _as_u32(r[40:48].astype(BF))
                            h_buf[pl.ds(pl.multiple_of(h0, 8), 8), cs] = xs[0:8] + r[0:8]
                            h_buf[pl.ds(pl.multiple_of(h0 + 32, 8), 32), cs] = xs[32:64] + r[8:40]
                    return run

                jobs = []
                for g in range(n_slots):
                    jobs.append(j_qkv(g))
                    if g >= 1:
                        jobs.append(j_s(g - 1))
                    if g >= 2:
                        jobs.append(j_pv(g - 2))
                n_main = len(jobs)
                last_need = (H - TH) // G - 1
                pend = [j_s(n_slots - 1), j_pv(n_slots - 2), j_pv(n_slots - 1)]
                if last_need >= n_slots - 2:
                    raise ValueError("tail_heads too small")
                jobs += [j_wo1(0), j_wo1(1), j_wo1(2), pend[0], pend[1],
                         j_wo1(3), j_wo1(4), j_wo1(5), pend[2], j_wo1(6), j_wo1(7)]
                jobs += [j_wo2(j) for j in range(nD)]
                return jobs, n_main

            def j_next_xn():
                store_xn(xn_ref[...])

            ej, e_main = step_jobs(True)
            oj, o_main = step_jobs(False)
            last_qkv = 3 * (n_slots - 1) - 1 if n_slots > 2 else 0
            idx = [i for i in range(o_main)][-3] + 1
            oj = oj[:idx] + [j_next_xn] + oj[idx:]
            return ej, oj, e_main

        def b_jobs():
            c = t - LAG
            r0 = pl.multiple_of(c * PAIR, PAIR)
            R = PAIR + 2 * HALO
            st = {}

            def j_pre():
                hh = h_buf[pl.ds(r0, R), :]
                y = _ln(hh)
                st['y'] = y[HALO:HALO + PAIR]
                st['z'] = _ln(y).astype(BF)

            def j_w1(j):
                def run():
                    tok = jax.lax.broadcasted_iota(jnp.int32, (R, 128), 0) + (r0 - HALO)
                    valid = (tok >= 0) & (tok < S)
                    a = _gelu(_dot(st['z'], w1_t[j]))
                    a1_buf[:, pl.ds(j * 128, 128)] = jnp.where(valid, a, 0.0)
                return run

            def j_shift():
                cq = D // 4
                st['g'] = jnp.concatenate([
                    a1_buf[pl.ds(HALO - 1, PAIR), pl.ds(0 * cq, cq)],
                    a1_buf[pl.ds(HALO + 1, PAIR), pl.ds(1 * cq, cq)],
                    a1_buf[pl.ds(HALO - 2, PAIR), pl.ds(2 * cq, cq)],
                    a1_buf[pl.ds(HALO + 2, PAIR), pl.ds(3 * cq, cq)]], axis=1).astype(BF)

            def j_w2(j):
                def run():
                    st['x1', j] = st['y'][:, j * 128:(j + 1) * 128] + _dot(st['g'], w2_t[j])
                return run

            def j_ln3():
                x1 = jnp.concatenate([st['x1', j] for j in range(nD)], axis=1)
                st['z1'] = _ln(x1).astype(BF)

            def j_w3(j):
                def run():
                    st['a3', j] = _gelu(_dot(st['z1'], w3_t[j])).astype(BF)
                return run

            def j_cat():
                st['a3'] = jnp.concatenate([st.pop(('a3', j)) for j in range(nF)], axis=1)

            def j_w4(j):
                def run():
                    cs = pl.ds(j * 128, 128)
                    hh = h_buf[pl.ds(pl.multiple_of(r0 + HALO, 8), PAIR), cs]
                    out_ref[:, cs] = (hh + (st['x1', j] + _dot(st['a3'], w4_t[j]))).astype(out_ref.dtype)
                return run

            return dict(pre=j_pre, w1=[j_w1(j) for j in range(nD)], shift=j_shift,
                        w2=[j_w2(j) for j in range(nD)], ln3=j_ln3,
                        w3=[j_w3(j) for j in range(nF)], cat=j_cat,
                        w4=[j_w4(j) for j in range(nD)])

        def b_flat(b):
            return [b['pre']] + b['w1'] + [b['shift']] + b['w2'] + [b['ln3']] + b['w3'] + [b['cat']] + b['w4']

        def run_jobs(jobs):
            for j in jobs:
                j()

        def part_a():
            if CFG['a']:
                ej, oj, e_main = a_jobs()

                def j_wo_wait():
                    pl.when(t == 0)(wo_finish)
                run_jobs(ej[:e_main] + [j_wo_wait] + ej[e_main:] + oj)

        def part_b():
            if CFG['b']:
                run_jobs(b_flat(b_jobs()))
            else:
                out_ref[...] = h_buf[pl.ds(pl.multiple_of((t - LAG) * PAIR + HALO, 8), PAIR), :].astype(out_ref.dtype)

        def part_ab():
            if not (CFG['a'] and CFG['b'] and CFG['fuse']):
                part_a()
                part_b()
                return
            ej, oj, _ = a_jobs()
            b = b_jobs()
            w3 = b['w3']
            def slot_pos(g):
                return 0 if g == 0 else (1 if g == 1 else 3 * (g - 1))
            fe = {0: [b['pre']]}
            for i in range(nD):
                fe.setdefault(slot_pos(2 + i // 2), []).append(b['w1'][i])
            fe.setdefault(slot_pos(6), []).append(b['shift'])
            for i in range(nD):
                fe.setdefault(slot_pos(8 + i // 2), []).append(b['w2'][i])
            fe.setdefault(slot_pos(12), []).append(b['ln3'])
            fe.setdefault(slot_pos(14), []).extend(w3[0:2])
            fe.setdefault(slot_pos(15), []).extend(w3[2:4])
            fe.setdefault(len(ej), []).extend(w3[4:7])
            fo = {}
            k = 7
            for g in range(1, 11):
                fo.setdefault(slot_pos(g), []).extend(w3[k:k + 2])
                k += 2
            fo.setdefault(slot_pos(11), []).append(w3[27])
            fo.setdefault(slot_pos(12), []).append(b['cat'])
            w4 = b['w4']
            fo.setdefault(slot_pos(13) + 1, []).append(w4[0])
            fo.setdefault(slot_pos(14) + 1, []).append(w4[1])
            fo.setdefault(slot_pos(15) + 1, []).append(w4[2])
            fo.setdefault(len(oj), []).extend(w4[3:])
            run_jobs(_interleave(ej, fe) + _interleave(oj, fo))

        @pl.when(t < LAG)
        def _():
            part_a()

        @pl.when(jnp.logical_and(t >= LAG, t < n_pairs))
        def _():
            part_ab()

        @pl.when(t >= n_pairs)
        def _():
            part_b()

    return kernel


@functools.partial(jax.jit, static_argnames=("A_seg_len",))
def pallas_sequential_preLN__memory_aug_recurrent_mem_tr__mixer_s_mlp__prompt_kernel(
    A_x, A_mem0, A_Wq, A_Wk, A_Wv, A_Wo, A_seg_len, B_x, B_w1, B_w2, B_w3, B_w4,
):
    _, S, D = A_x.shape
    H, E = A_Wq.shape[1], A_Wq.shape[2]
    F = B_w3.shape[1]
    assert A_seg_len == SEG and A_mem0.shape[1] == MEM and S % PAIR == 0
    n_pairs = S // PAIR
    nD, nF = D // 128, F // 128

    x = A_x.reshape(S, D)
    mem0 = A_mem0.reshape(MEM, D)
    wo = A_Wo.reshape(H * E, D)

    any_spec = pl.BlockSpec(memory_space=pl.ANY)
    out = pl.pallas_call(
        _make_kernel(S, D, H, E, F),
        grid=(n_pairs + LAG,),
        in_specs=[
            pl.BlockSpec((PAIR, D), lambda t: (jnp.minimum(t, n_pairs - 1), 0)),
            pl.BlockSpec((PAIR, D), lambda t: (jnp.minimum(t + 1, n_pairs - 1), 0)),
            pl.BlockSpec((MEM, D), lambda t: (0, 0)),
        ] + [any_spec] * 8,
        out_specs=pl.BlockSpec((PAIR, D), lambda t: (jnp.maximum(t - LAG, 0), 0)),
        out_shape=jax.ShapeDtypeStruct((S, D), A_x.dtype),
        scratch_shapes=[
            pltpu.VMEM((3, D, H, E), BF),
            pltpu.VMEM((H, D // 2, E), U32),
            pltpu.VMEM((H, D // 2, E), U32),
            pltpu.VMEM((H, D // 2, E), U32),
            pltpu.VMEM((nD, H * E, 128), BF),
            pltpu.VMEM((nD, H * E // 2, 128), U32),
            pltpu.VMEM((nD, D, 128), BF),
            pltpu.VMEM((nD, D, 128), BF),
            pltpu.VMEM((nF, D, 128), BF),
            pltpu.VMEM((nD, F, 128), BF),
            pltpu.VMEM((24, D), U32),
            pltpu.VMEM((16, D), U32),
            pltpu.VMEM((3, 8, H * E), F32),
            pltpu.VMEM((40, H * E), U32),
            pltpu.VMEM((48, D), F32),
            pltpu.VMEM((S + 2 * HALO, D), F32),
            pltpu.VMEM((PAIR + 2 * HALO, D), F32),
            pltpu.SemaphoreType.DMA((3 * 4 + nD + 1,)),
        ],
        compiler_params=pltpu.CompilerParams(
            dimension_semantics=("arbitrary",),
            vmem_limit_bytes=120 * 1024 * 1024,
        ),
    )(x, x, mem0, A_Wq, A_Wk, A_Wv, wo, B_w1, B_w2, B_w3, B_w4)
    return out.reshape(1, S, D)
```

```python
import functools

import jax
import jax.numpy as jnp
from jax.experimental import pallas as pl
from jax.experimental.pallas import tpu as pltpu

BF = jnp.bfloat16
F32 = jnp.float32
U32 = jnp.uint32

SEG = 32
MEM = 8
PAIR = 2 * SEG
LAG = 2
HALO = 8
LN_EPS = 1e-5
LOG2E = 1.4426950408889634
CFG = dict(a=True, b=True, att=True, G=2, tail_heads=4, fuse=True, bstart='early')


def _ln(x):
    m = jnp.mean(x, axis=-1, keepdims=True)
    xc = x - m
    v = jnp.mean(xc * xc, axis=-1, keepdims=True)
    return xc * jax.lax.rsqrt(v + LN_EPS)


_dot = functools.partial(jnp.dot, preferred_element_type=F32)


def _gelu(x):
    return jax.nn.gelu(x, approximate=True)


def _as_bf(x_u32):
    return pltpu.bitcast(x_u32, BF)


def _as_u32(x_bf):
    return pltpu.bitcast(x_bf, U32)


def _interleave(main, fill):
    out = []
    for i, j in enumerate(main):
        out.extend(fill.get(i, []))
        out.append(j)
    out.extend(fill.get(len(main), []))
    return out


def _make_kernel(S, D, H, E, F):
    n_pairs = S // PAIR
    nD = D // 128
    nF = F // 128
    c_exp = float(E) ** -0.5 * LOG2E
    neg_raw = -1000000000.0 / (float(E) ** -0.5)
    L = MEM + SEG
    G = CFG['G']
    n_slots = H // G
    TH = CFG['tail_heads']
    K1 = (H - TH) * E

    def kernel(x_ref, xn_ref, mem0_ref, wq_hbm, wk_hbm, wv_hbm, wo_hbm, w1_hbm, w2_hbm, w3_hbm, w4_hbm,
               out_ref,
               raw, wq_t, wk_t, wv_t, wo_raw, wo_t, w1_t, w2_t, w3_t, w4_t,
               lb_e, lb_o, sv, ob, wacc, h_buf, a1_buf, sems):
        t = pl.program_id(0)

        NCH = 4
        CH = D // NCH

        def raw_copy(i, c, src):
            return pltpu.make_async_copy(src.at[pl.ds(c * CH, CH)], raw.at[i, pl.ds(c * CH, CH)],
                                         sems.at[i * NCH + c])

        def col_copies(src, dst, n, sem_idx):
            return [pltpu.make_async_copy(src.at[:, pl.ds(j * 128, 128)], dst.at[j], sems.at[sem_idx])
                    for j in range(n)]

        WO_SEM = 3 * NCH
        B_SEM = WO_SEM + nD

        def wo_copy(j):
            rows = pl.ds(j * (H * E // nD), H * E // nD)
            return pltpu.make_async_copy(wo_hbm.at[rows], wo_raw.at[rows], sems.at[WO_SEM + j])

        def wo_finish():
            for j in range(nD):
                wo_copy(j).wait()

                def body(b, carry):
                    r = j * (H * E // nD) + b * 64
                    blk = wo_raw[pl.ds(pl.multiple_of(r, 64), 64), :]
                    for n in range(nD):
                        wo_t[n, pl.ds(pl.multiple_of(r // 2, 32), 32), :] = _as_u32(blk[:, n * 128:(n + 1) * 128])
                    return carry
                jax.lax.fori_loop(0, H * E // nD // 64, body, 0)
                if j == CFG['bstart']:
                    for c in b_copies():
                        c.start()

        def b_copies():
            return (col_copies(w1_hbm, w1_t, nD, B_SEM) + col_copies(w2_hbm, w2_t, nD, B_SEM)
                    + col_copies(w3_hbm, w3_t, nF, B_SEM) + col_copies(w4_hbm, w4_t, nD, B_SEM))

        def relayout(i, c, dst):
            def body(b, carry):
                blk = raw[i, pl.ds(pl.multiple_of(b * 16, 16), 16), :, :]
                dst[:, pl.ds(pl.multiple_of(b * 8, 8), 8), :] = _as_u32(jnp.swapaxes(blk, 0, 1))
                return carry
            jax.lax.fori_loop(c * (CH // 16), (c + 1) * (CH // 16), body, 0)

        def store_xn(x_bf):
            xn = _ln(x_bf.astype(F32))
            lb_e[pl.ds(0, 4), :] = _as_u32(xn[32:40].astype(BF))
            lb_e[pl.ds(4, 4), :] = _as_u32(xn[0:8].astype(BF))
            lb_e[pl.ds(8, 8), :] = _as_u32(xn[8:24].astype(BF))
            lb_e[pl.ds(16, 4), :] = _as_u32(xn[24:32].astype(BF))
            lb_o[pl.ds(0, 8), :] = _as_u32(xn[40:56].astype(BF))
            lb_o[pl.ds(8, 4), :] = _as_u32(xn[56:64].astype(BF))

        @pl.when(t == 0)
        def _():
            srcs = (wq_hbm, wk_hbm, wv_hbm)
            qkv = [[raw_copy(i, c, srcs[i]) for c in range(NCH)] for i in range(3)]
            for i in range(3):
                for c in range(NCH):
                    qkv[i][c].start()
            for j in range(nD):
                wo_copy(j).start()
            h_buf[pl.ds(0, HALO), :] = jnp.zeros((HALO, D), F32)
            h_buf[pl.ds(HALO + S, HALO), :] = jnp.zeros((HALO, D), F32)
            lb_e[pl.ds(20, 4), :] = _as_u32(mem0_ref[...])
            store_xn(x_ref[...])
            for i, dst in enumerate((wq_t, wk_t, wv_t)):
                for c in range(NCH):
                    qkv[i][c].wait()
                    relayout(i, c, dst)
            if CFG['bstart'] == 'early':
                for c in b_copies():
                    c.start()
            if not CFG['a']:
                wo_finish()

        @pl.when(t == LAG)
        def _():
            for c in b_copies():
                c.wait()
            z = _ln(_ln(h_buf[pl.ds(0, 2 * HALO), :])).astype(BF)
            tok = jax.lax.broadcasted_iota(jnp.int32, (2 * HALO, 128), 0) - HALO
            for j in range(nD):
                a1_buf[pl.ds(PAIR, 2 * HALO), pl.ds(j * 128, 128)] = jnp.where(
                    tok >= 0, _gelu(_dot(z, w1_t[j])), 0.0)

        def a_jobs():
            row = jax.lax.broadcasted_iota(jnp.int32, (G * L, G * L), 0)
            col = jax.lax.broadcasted_iota(jnp.int32, (G * L, G * L), 1)
            mask = None
            for i in range(G):
                rl, cl = row - i * L, col - i * L
                blk = ((rl >= 0) & (rl < L) & (cl >= 0) & (cl < L)) & ((cl <= rl) | (cl >= SEG))
                mask = blk if mask is None else (mask | blk)
            h0 = t * PAIR + HALO

            def step_jobs(even):
                lb = lb_e if even else lb_o
                st = {}

                def j_qkv(g):
                    def run():
                        lhs = _as_bf(lb[...])
                        parts = [[], [], []]
                        for h in range(g * G, (g + 1) * G):
                            cs = pl.ds(h * E, E)
                            r = [_dot(lhs, _as_bf(w[h])) for w in (wq_t, wk_t, wv_t)]
                            for i in range(3):
                                if even:
                                    sv[i, :, cs] = r[i][0:8]
                                    parts[i].append(r[i][8:48])
                                else:
                                    parts[i] += [sv[i, :, cs], r[i]]
                        st['qkv', g] = [jnp.concatenate(a, axis=0).astype(BF) for a in parts]
                    return run

                def j_s(g):
                    def run():
                        q, k, v = st.pop(('qkv', g))
                        if not CFG['att']:
                            st['p', g] = (q + k, v, None)
                            return
                        s = jax.lax.dot_general(q, k, (((1,), (1,)), ((), ())),
                                                preferred_element_type=F32)
                        s = jnp.where(mask, s, neg_raw)
                        m = jnp.max(s, axis=-1, keepdims=True)
                        p = jnp.exp2((s - m) * c_exp)
                        l = jnp.sum(p, axis=-1, keepdims=True)
                        r0 = pl.reciprocal(l, approx=True)
                        p = p * (r0 * (2.0 - l * r0))
                        st['p', g] = (p.astype(BF), v, None)
                    return run

                def j_pv(g):
                    def run():
                        p, v, r = st.pop(('p', g))
                        o2 = _dot(p, v) if CFG['att'] else (p + v).astype(F32)
                        for i, h in enumerate(range(g * G, (g + 1) * G)):
                            o = o2[i * L:(i + 1) * L]
                            cs = pl.ds(h * E, E)
                            if even:
                                ob[pl.ds(16, 4), cs] = _as_u32(o[0:8].astype(BF))
                                ob[pl.ds(0, 16), cs] = _as_u32(o[8:40].astype(BF))
                            else:
                                ob[pl.ds(20, 4), cs] = _as_u32(o[0:8].astype(BF))
                                ob[pl.ds(24, 16), cs] = _as_u32(o[8:40].astype(BF))
                    return run

                rows = pl.ds(0, 16) if even else pl.ds(16, 24)
                nrows = 32 if even else 48

                def j_wo1(j):
                    def run():
                        lhs = _as_bf(ob[rows, pl.ds(0, K1)])
                        wacc[pl.ds(0, nrows), pl.ds(j * 128, 128)] = _dot(lhs, _as_bf(wo_t[j, pl.ds(0, K1 // 2), :]))
                    return run

                def j_wo2(j):
                    def run():
                        lhs = _as_bf(ob[rows, pl.ds(K1, H * E - K1)])
                        r = wacc[pl.ds(0, nrows), pl.ds(j * 128, 128)] + _dot(lhs, _as_bf(wo_t[j, pl.ds(K1 // 2, (H * E - K1) // 2), :]))
                        cs = pl.ds(j * 128, 128)
                        xs = x_ref[:, cs].astype(F32)
                        if even:
                            lb_o[pl.ds(12, 4), cs] = _as_u32(r[24:32].astype(BF))
                            h_buf[pl.ds(pl.multiple_of(h0 + 8, 8), 24), cs] = xs[8:32] + r[0:24]
                        else:
                            lb_e[pl.ds(20, 4), cs] = _as_u32(r[40:48].astype(BF))
                            h_buf[pl.ds(pl.multiple_of(h0, 8), 8), cs] = xs[0:8] + r[0:8]
                            h_buf[pl.ds(pl.multiple_of(h0 + 32, 8), 32), cs] = xs[32:64] + r[8:40]
                    return run

                jobs = []
                for g in range(n_slots):
                    jobs.append(j_qkv(g))
                    if g >= 1:
                        jobs.append(j_s(g - 1))
                    if g >= 2:
                        jobs.append(j_pv(g - 2))
                n_main = len(jobs)
                last_need = (H - TH) // G - 1
                pend = [j_s(n_slots - 1), j_pv(n_slots - 2), j_pv(n_slots - 1)]
                if last_need >= n_slots - 2:
                    raise ValueError("tail_heads too small")
                jobs += [j_wo1(0), j_wo1(1), j_wo1(2), pend[0], pend[1],
                         j_wo1(3), j_wo1(4), j_wo1(5), pend[2], j_wo1(6), j_wo1(7)]
                jobs += [j_wo2(j) for j in range(nD)]
                return jobs, n_main

            def j_next_xn():
                store_xn(xn_ref[...])

            ej, e_main = step_jobs(True)
            oj, o_main = step_jobs(False)
            last_qkv = 3 * (n_slots - 1) - 1 if n_slots > 2 else 0
            idx = [i for i in range(o_main)][-3] + 1
            oj = oj[:idx] + [j_next_xn] + oj[idx:]
            return ej, oj, e_main

        def b_jobs():
            c = t - LAG
            r0 = pl.multiple_of(c * PAIR, PAIR)
            st = {}

            def j_pre():
                a1_buf[pl.ds(0, 2 * HALO), :] = a1_buf[pl.ds(PAIR, 2 * HALO), :]
                y = _ln(h_buf[pl.ds(pl.multiple_of(r0 + HALO, 8), PAIR + HALO), :])
                st['y'] = y[0:PAIR]
                st['z'] = _ln(y[HALO:]).astype(BF)

            def j_w1(j):
                def run():
                    tok = jax.lax.broadcasted_iota(jnp.int32, (PAIR, 128), 0) + (r0 + HALO)
                    a = _gelu(_dot(st['z'], w1_t[j]))
                    a1_buf[pl.ds(2 * HALO, PAIR), pl.ds(j * 128, 128)] = jnp.where(tok < S, a, 0.0)
                return run

            def j_shift():
                cq = D // 4
                st['g'] = jnp.concatenate([
                    a1_buf[pl.ds(HALO - 1, PAIR), pl.ds(0 * cq, cq)],
                    a1_buf[pl.ds(HALO + 1, PAIR), pl.ds(1 * cq, cq)],
                    a1_buf[pl.ds(HALO - 2, PAIR), pl.ds(2 * cq, cq)],
                    a1_buf[pl.ds(HALO + 2, PAIR), pl.ds(3 * cq, cq)]], axis=1).astype(BF)

            def j_w2(j):
                def run():
                    st['x1', j] = st['y'][:, j * 128:(j + 1) * 128] + _dot(st['g'], w2_t[j])
                return run

            def j_ln3():
                x1 = jnp.concatenate([st['x1', j] for j in range(nD)], axis=1)
                st['z1'] = _ln(x1).astype(BF)

            def j_w3(j):
                def run():
                    st['a3', j] = _gelu(_dot(st['z1'], w3_t[j])).astype(BF)
                return run

            def j_cat():
                st['a3'] = jnp.concatenate([st.pop(('a3', j)) for j in range(nF)], axis=1)

            def j_w4(j):
                def run():
                    cs = pl.ds(j * 128, 128)
                    hh = h_buf[pl.ds(pl.multiple_of(r0 + HALO, 8), PAIR), cs]
                    out_ref[:, cs] = (hh + (st['x1', j] + _dot(st['a3'], w4_t[j]))).astype(out_ref.dtype)
                return run

            return dict(pre=j_pre, w1=[j_w1(j) for j in range(nD)], shift=j_shift,
                        w2=[j_w2(j) for j in range(nD)], ln3=j_ln3,
                        w3=[j_w3(j) for j in range(nF)], cat=j_cat,
                        w4=[j_w4(j) for j in range(nD)])

        def b_flat(b):
            return [b['pre']] + b['w1'] + [b['shift']] + b['w2'] + [b['ln3']] + b['w3'] + [b['cat']] + b['w4']

        def run_jobs(jobs):
            for j in jobs:
                j()

        def part_a():
            if CFG['a']:
                ej, oj, e_main = a_jobs()

                def j_wo_wait():
                    pl.when(t == 0)(wo_finish)
                run_jobs(ej[:e_main] + [j_wo_wait] + ej[e_main:] + oj)

        def part_b():
            if CFG['b']:
                run_jobs(b_flat(b_jobs()))
            else:
                out_ref[...] = h_buf[pl.ds(pl.multiple_of((t - LAG) * PAIR + HALO, 8), PAIR), :].astype(out_ref.dtype)

        def part_ab():
            if not (CFG['a'] and CFG['b'] and CFG['fuse']):
                part_a()
                part_b()
                return
            ej, oj, _ = a_jobs()
            b = b_jobs()
            w3 = b['w3']
            def slot_pos(g):
                return 0 if g == 0 else (1 if g == 1 else 3 * (g - 1))
            fe = {0: [b['pre']]}
            for i in range(nD):
                fe.setdefault(slot_pos(2 + i // 2), []).append(b['w1'][i])
            fe.setdefault(slot_pos(6), []).append(b['shift'])
            for i in range(nD):
                fe.setdefault(slot_pos(8 + i // 2), []).append(b['w2'][i])
            fe.setdefault(slot_pos(12), []).append(b['ln3'])
            fe.setdefault(slot_pos(14), []).extend(w3[0:2])
            fe.setdefault(slot_pos(15), []).extend(w3[2:4])
            fe.setdefault(len(ej), []).extend(w3[4:7])
            fo = {}
            k = 7
            for g in range(1, 11):
                fo.setdefault(slot_pos(g), []).extend(w3[k:k + 2])
                k += 2
            fo.setdefault(slot_pos(11), []).append(w3[27])
            fo.setdefault(slot_pos(12), []).append(b['cat'])
            w4 = b['w4']
            fo.setdefault(slot_pos(13) + 1, []).append(w4[0])
            fo.setdefault(slot_pos(14) + 1, []).append(w4[1])
            fo.setdefault(slot_pos(15) + 1, []).append(w4[2])
            fo.setdefault(len(oj), []).extend(w4[3:])
            run_jobs(_interleave(ej, fe) + _interleave(oj, fo))

        @pl.when(t < LAG)
        def _():
            part_a()

        @pl.when(jnp.logical_and(t >= LAG, t < n_pairs))
        def _():
            part_ab()

        @pl.when(t >= n_pairs)
        def _():
            part_b()

    return kernel


@functools.partial(jax.jit, static_argnames=("A_seg_len",))
def pallas_sequential_preLN__memory_aug_recurrent_mem_tr__mixer_s_mlp__prompt_kernel(
    A_x, A_mem0, A_Wq, A_Wk, A_Wv, A_Wo, A_seg_len, B_x, B_w1, B_w2, B_w3, B_w4,
):
    _, S, D = A_x.shape
    H, E = A_Wq.shape[1], A_Wq.shape[2]
    F = B_w3.shape[1]
    assert A_seg_len == SEG and A_mem0.shape[1] == MEM and S % PAIR == 0
    n_pairs = S // PAIR
    nD, nF = D // 128, F // 128

    x = A_x.reshape(S, D)
    mem0 = A_mem0.reshape(MEM, D)
    wo = A_Wo.reshape(H * E, D)

    any_spec = pl.BlockSpec(memory_space=pl.ANY)
    out = pl.pallas_call(
        _make_kernel(S, D, H, E, F),
        grid=(n_pairs + LAG,),
        in_specs=[
            pl.BlockSpec((PAIR, D), lambda t: (jnp.minimum(t, n_pairs - 1), 0)),
            pl.BlockSpec((PAIR, D), lambda t: (jnp.minimum(t + 1, n_pairs - 1), 0)),
            pl.BlockSpec((MEM, D), lambda t: (0, 0)),
        ] + [any_spec] * 8,
        out_specs=pl.BlockSpec((PAIR, D), lambda t: (jnp.maximum(t - LAG, 0), 0)),
        out_shape=jax.ShapeDtypeStruct((S, D), A_x.dtype),
        scratch_shapes=[
            pltpu.VMEM((3, D, H, E), BF),
            pltpu.VMEM((H, D // 2, E), U32),
            pltpu.VMEM((H, D // 2, E), U32),
            pltpu.VMEM((H, D // 2, E), U32),
            pltpu.VMEM((H * E, D), BF),
            pltpu.VMEM((nD, H * E // 2, 128), U32),
            pltpu.VMEM((nD, D, 128), BF),
            pltpu.VMEM((nD, D, 128), BF),
            pltpu.VMEM((nF, D, 128), BF),
            pltpu.VMEM((nD, F, 128), BF),
            pltpu.VMEM((24, D), U32),
            pltpu.VMEM((16, D), U32),
            pltpu.VMEM((3, 8, H * E), F32),
            pltpu.VMEM((40, H * E), U32),
            pltpu.VMEM((48, D), F32),
            pltpu.VMEM((S + 2 * HALO, D), F32),
            pltpu.VMEM((PAIR + 2 * HALO, D), F32),
            pltpu.SemaphoreType.DMA((3 * 4 + nD + 1,)),
        ],
        compiler_params=pltpu.CompilerParams(
            dimension_semantics=("arbitrary",),
            vmem_limit_bytes=120 * 1024 * 1024,
        ),
    )(x, x, mem0, A_Wq, A_Wk, A_Wv, wo, B_w1, B_w2, B_w3, B_w4)
    return out.reshape(1, S, D)
```

```python
import functools

import jax
import jax.numpy as jnp
from jax.experimental import pallas as pl
from jax.experimental.pallas import tpu as pltpu

BF = jnp.bfloat16
F32 = jnp.float32
U32 = jnp.uint32

SEG = 32
MEM = 8
PAIR = 2 * SEG
LAG = 2
HALO = 8
LN_EPS = 1e-5
LOG2E = 1.4426950408889634
CFG = dict(a=True, b=True, att=True, G=2, tail_heads=4, fuse=True, U=1, bwait=0, nobc=True)


def _ln(x):
    m = jnp.mean(x, axis=-1, keepdims=True)
    xc = x - m
    v = jnp.mean(xc * xc, axis=-1, keepdims=True)
    return xc * jax.lax.rsqrt(v + LN_EPS)


_dot = functools.partial(jnp.dot, preferred_element_type=F32)


def _gelu(x):
    return jax.nn.gelu(x, approximate=True)


def _as_bf(x_u32):
    return pltpu.bitcast(x_u32, BF)


def _as_u32(x_bf):
    return pltpu.bitcast(x_bf, U32)


def _interleave(main, fill):
    out = []
    for i, j in enumerate(main):
        out.extend(fill.get(i, []))
        out.append(j)
    out.extend(fill.get(len(main), []))
    return out


def _make_kernel(S, D, H, E, F):
    n_pairs = S // PAIR
    nD = D // 128
    nF = F // 128
    c_exp = float(E) ** -0.5 * LOG2E
    neg_raw = -1000000000.0 / (float(E) ** -0.5)
    L = MEM + SEG
    G = CFG['G']
    U = CFG['U']
    assert LAG % U == 0
    n_steps = n_pairs // U
    lag_steps = LAG // U
    n_slots = H // G
    TH = CFG['tail_heads']
    K1 = (H - TH) * E

    def kernel(x_ref, xn_ref, mem0_ref, wq_hbm, wk_hbm, wv_hbm, wo_hbm, w1_hbm, w2_hbm, w3_hbm, w4_hbm,
               out_ref,
               raw, wq_t, wk_t, wv_t, wo_raw, wo_t, w1_t, w2_t, w3_t, w4_t,
               lb_e, lb_o, sv, ob, wacc, h_buf, a1_buf, sems):
        t = pl.program_id(0)

        NCH = 4
        CH = D // NCH

        def raw_copy(i, c, src):
            return pltpu.make_async_copy(src.at[pl.ds(c * CH, CH)], raw.at[i, pl.ds(c * CH, CH)],
                                         sems.at[i * NCH + c])

        def col_copies(src, dst, n, sem_idx):
            return [pltpu.make_async_copy(src.at[:, pl.ds(j * 128, 128)], dst.at[j], sems.at[sem_idx])
                    for j in range(n)]

        WO_SEM = 3 * NCH
        B_SEM = WO_SEM + nD

        def wo_copy(j):
            rows = pl.ds(j * (H * E // nD), H * E // nD)
            return pltpu.make_async_copy(wo_hbm.at[rows], wo_raw.at[rows], sems.at[WO_SEM + j])

        def wo_finish():
            for j in range(nD):
                wo_copy(j).wait()

                def body(b, carry):
                    r = j * (H * E // nD) + b * 64
                    blk = wo_raw[pl.ds(pl.multiple_of(r, 64), 64), :]
                    for n in range(nD):
                        wo_t[n, pl.ds(pl.multiple_of(r // 2, 32), 32), :] = _as_u32(blk[:, n * 128:(n + 1) * 128])
                    return carry
                jax.lax.fori_loop(0, H * E // nD // 64, body, 0)

        def b_copies():
            return (col_copies(w1_hbm, w1_t, nD, B_SEM) + col_copies(w2_hbm, w2_t, nD, B_SEM)
                    + col_copies(w3_hbm, w3_t, nF, B_SEM) + col_copies(w4_hbm, w4_t, nD, B_SEM))

        def relayout(i, c, dst):
            def body(b, carry):
                blk = raw[i, pl.ds(pl.multiple_of(b * 16, 16), 16), :, :]
                dst[:, pl.ds(pl.multiple_of(b * 8, 8), 8), :] = _as_u32(jnp.swapaxes(blk, 0, 1))
                return carry
            jax.lax.fori_loop(c * (CH // 16), (c + 1) * (CH // 16), body, 0)

        def store_xn(x_bf):
            xn = _ln(x_bf.astype(F32))
            lb_e[pl.ds(0, 4), :] = _as_u32(xn[32:40].astype(BF))
            lb_e[pl.ds(4, 4), :] = _as_u32(xn[0:8].astype(BF))
            lb_e[pl.ds(8, 8), :] = _as_u32(xn[8:24].astype(BF))
            lb_e[pl.ds(16, 4), :] = _as_u32(xn[24:32].astype(BF))
            lb_o[pl.ds(0, 8), :] = _as_u32(xn[40:56].astype(BF))
            lb_o[pl.ds(8, 4), :] = _as_u32(xn[56:64].astype(BF))

        @pl.when(t == 0)
        def _():
            srcs = (wq_hbm, wk_hbm, wv_hbm)
            qkv = [[raw_copy(i, c, srcs[i]) for c in range(NCH)] for i in range(3)]
            for i in range(3):
                for c in range(NCH):
                    qkv[i][c].start()
            for j in range(nD):
                wo_copy(j).start()
            h_buf[pl.ds(0, HALO), :] = jnp.zeros((HALO, D), F32)
            h_buf[pl.ds(HALO + S, HALO), :] = jnp.zeros((HALO, D), F32)
            lb_e[pl.ds(20, 4), :] = _as_u32(mem0_ref[...])
            store_xn(x_ref[pl.ds(0, PAIR), :])
            for i, dst in enumerate((wq_t, wk_t, wv_t)):
                for c in range(NCH):
                    qkv[i][c].wait()
                    relayout(i, c, dst)
            for c in b_copies():
                c.start()
            if not CFG['a']:
                wo_finish()

        if CFG['bwait']:
            @pl.when(t == lag_steps + CFG['bwait'])
            def _():
                for c in b_copies():
                    c.wait()

        @pl.when(t == lag_steps)
        def _():
            if not CFG['bwait']:
                for c in b_copies():
                    c.wait()
            z = _ln(_ln(h_buf[pl.ds(0, 2 * HALO), :])).astype(BF)
            tok = jax.lax.broadcasted_iota(jnp.int32, (2 * HALO, 128), 0) - HALO
            for j in range(nD):
                a1_buf[pl.ds(PAIR, 2 * HALO), pl.ds(j * 128, 128)] = jnp.where(
                    tok >= 0, _gelu(_dot(z, w1_t[j])), 0.0)

        def a_jobs(u):
            row = jax.lax.broadcasted_iota(jnp.int32, (G * L, G * L), 0)
            col = jax.lax.broadcasted_iota(jnp.int32, (G * L, G * L), 1)
            mask = None
            for i in range(G):
                rl, cl = row - i * L, col - i * L
                blk = ((rl >= 0) & (rl < L) & (cl >= 0) & (cl < L)) & ((cl <= rl) | (cl >= SEG))
                mask = blk if mask is None else (mask | blk)
            h0 = (t * U + u) * PAIR + HALO

            def step_jobs(even):
                lb = lb_e if even else lb_o
                st = {}

                def j_qkv(g):
                    def run():
                        lhs = _as_bf(lb[...])
                        parts = [[], [], []]
                        for h in range(g * G, (g + 1) * G):
                            cs = pl.ds(h * E, E)
                            r = [_dot(lhs, _as_bf(w[h])) for w in (wq_t, wk_t, wv_t)]
                            for i in range(3):
                                if even:
                                    sv[i, :, cs] = r[i][0:8]
                                    parts[i].append(r[i][8:48])
                                else:
                                    parts[i] += [sv[i, :, cs], r[i]]
                        st['qkv', g] = [jnp.concatenate(a, axis=0).astype(BF) for a in parts]
                    return run

                def j_s(g):
                    def run():
                        q, k, v = st.pop(('qkv', g))
                        if not CFG['att']:
                            st['p', g] = (q + k, v)
                            return
                        s = jax.lax.dot_general(q, k, (((1,), (1,)), ((), ())),
                                                preferred_element_type=F32)
                        s = jnp.where(mask, s, neg_raw)
                        m = jnp.max(s, axis=-1, keepdims=True)
                        p = jnp.exp2((s - m) * c_exp)
                        l = jnp.sum(p, axis=-1, keepdims=True)
                        r0 = pl.reciprocal(l, approx=True)
                        p = p * (r0 * (2.0 - l * r0))
                        st['p', g] = (p.astype(BF), v)
                    return run

                def j_pv(g):
                    def run():
                        p, v = st.pop(('p', g))
                        o2 = _dot(p, v) if CFG['att'] else (p + v).astype(F32)
                        for i, h in enumerate(range(g * G, (g + 1) * G)):
                            o = o2[i * L:(i + 1) * L]
                            cs = pl.ds(h * E, E)
                            if even:
                                ob[pl.ds(16, 4), cs] = _as_u32(o[0:8].astype(BF))
                                ob[pl.ds(0, 16), cs] = _as_u32(o[8:40].astype(BF))
                            else:
                                ob[pl.ds(20, 4), cs] = _as_u32(o[0:8].astype(BF))
                                ob[pl.ds(24, 16), cs] = _as_u32(o[8:40].astype(BF))
                    return run

                rows = pl.ds(0, 16) if even else pl.ds(16, 24)
                nrows = 32 if even else 48

                def j_wo1(j):
                    def run():
                        lhs = _as_bf(ob[rows, pl.ds(0, K1)])
                        wacc[pl.ds(0, nrows), pl.ds(j * 128, 128)] = _dot(
                            lhs, _as_bf(wo_t[j, pl.ds(0, K1 // 2), :]))
                    return run

                def j_wo2(j):
                    def run():
                        lhs = _as_bf(ob[rows, pl.ds(K1, H * E - K1)])
                        r = wacc[pl.ds(0, nrows), pl.ds(j * 128, 128)] + _dot(
                            lhs, _as_bf(wo_t[j, pl.ds(K1 // 2, (H * E - K1) // 2), :]))
                        cs = pl.ds(j * 128, 128)
                        xs = x_ref[pl.ds(u * PAIR, PAIR), cs].astype(F32)
                        if even:
                            lb_o[pl.ds(12, 4), cs] = _as_u32(r[24:32].astype(BF))
                            h_buf[pl.ds(pl.multiple_of(h0 + 8, 8), 24), cs] = xs[8:32] + r[0:24]
                        else:
                            lb_e[pl.ds(20, 4), cs] = _as_u32(r[40:48].astype(BF))
                            h_buf[pl.ds(pl.multiple_of(h0, 8), 8), cs] = xs[0:8] + r[0:8]
                            h_buf[pl.ds(pl.multiple_of(h0 + 32, 8), 32), cs] = xs[32:64] + r[8:40]
                    return run

                jobs = []
                for g in range(n_slots):
                    jobs.append(j_qkv(g))
                    if g >= 1:
                        jobs.append(j_s(g - 1))
                    if g >= 2:
                        jobs.append(j_pv(g - 2))
                n_main = len(jobs)
                assert (H - TH) // G - 1 < n_slots - 2
                jobs += [j_wo1(0), j_wo1(1), j_wo1(2), j_s(n_slots - 1), j_pv(n_slots - 2),
                         j_wo1(3), j_wo1(4), j_wo1(5), j_pv(n_slots - 1), j_wo1(6), j_wo1(7)]
                jobs += [j_wo2(j) for j in range(nD)]
                return jobs, n_main

            def j_next_xn():
                if u + 1 < U:
                    store_xn(x_ref[pl.ds((u + 1) * PAIR, PAIR), :])
                else:
                    store_xn(xn_ref[...])

            ej, e_main = step_jobs(True)
            oj, o_main = step_jobs(False)
            idx = o_main - 2
            oj = oj[:idx] + [j_next_xn] + oj[idx:]
            return ej, oj, e_main

        def b_jobs(u):
            c = (t - lag_steps) * U + u
            r0 = pl.multiple_of(c * PAIR, PAIR)
            st = {}

            def j_pre():
                a1_buf[pl.ds(0, 2 * HALO), :] = a1_buf[pl.ds(PAIR, 2 * HALO), :]
                y = _ln(h_buf[pl.ds(pl.multiple_of(r0 + HALO, 8), PAIR + HALO), :])
                st['y'] = y[0:PAIR]
                st['z'] = _ln(y[HALO:]).astype(BF)

            def j_w1(j):
                def run():
                    tok = jax.lax.broadcasted_iota(jnp.int32, (PAIR, 128), 0) + (r0 + HALO)
                    a = _gelu(_dot(st['z'], w1_t[j]))
                    a1_buf[pl.ds(2 * HALO, PAIR), pl.ds(j * 128, 128)] = jnp.where(tok < S, a, 0.0)
                return run

            def j_shift():
                cq = D // 4
                st['g'] = jnp.concatenate([
                    a1_buf[pl.ds(HALO - 1, PAIR), pl.ds(0 * cq, cq)],
                    a1_buf[pl.ds(HALO + 1, PAIR), pl.ds(1 * cq, cq)],
                    a1_buf[pl.ds(HALO - 2, PAIR), pl.ds(2 * cq, cq)],
                    a1_buf[pl.ds(HALO + 2, PAIR), pl.ds(3 * cq, cq)]], axis=1).astype(BF)

            def j_w2(j):
                def run():
                    st['x1', j] = st['y'][:, j * 128:(j + 1) * 128] + _dot(st['g'], w2_t[j])
                return run

            def j_ln3():
                x1 = jnp.concatenate([st['x1', j] for j in range(nD)], axis=1)
                st['z1'] = _ln(x1).astype(BF)

            def j_w3(j):
                def run():
                    st['a3', j] = _gelu(_dot(st['z1'], w3_t[j])).astype(BF)
                return run

            def j_cat():
                st['a3'] = jnp.concatenate([st.pop(('a3', j)) for j in range(nF)], axis=1)

            def j_w4(j):
                def run():
                    cs = pl.ds(j * 128, 128)
                    hh = h_buf[pl.ds(pl.multiple_of(r0 + HALO, 8), PAIR), cs]
                    out_ref[pl.ds(u * PAIR, PAIR), cs] = (
                        hh + (st['x1', j] + _dot(st['a3'], w4_t[j]))).astype(out_ref.dtype)
                return run

            return dict(pre=j_pre, w1=[j_w1(j) for j in range(nD)], shift=j_shift,
                        w2=[j_w2(j) for j in range(nD)], ln3=j_ln3,
                        w3=[j_w3(j) for j in range(nF)], cat=j_cat,
                        w4=[j_w4(j) for j in range(nD)])

        def b_flat(b):
            return [b['pre']] + b['w1'] + [b['shift']] + b['w2'] + [b['ln3']] + b['w3'] + [b['cat']] + b['w4']

        def run_jobs(jobs):
            for j in jobs:
                j()

        def part_a():
            if not CFG['a']:
                return
            for u in range(U):
                ej, oj, e_main = a_jobs(u)
                if u == 0:
                    def j_wo_wait():
                        pl.when(t == 0)(wo_finish)
                    ej = ej[:e_main] + [j_wo_wait] + ej[e_main:]
                run_jobs(ej + oj)

        def part_b():
            if not CFG['b']:
                out_ref[...] = h_buf[pl.ds(pl.multiple_of((t - lag_steps) * U * PAIR + HALO, 8), U * PAIR), :].astype(out_ref.dtype)
                return
            bs = [b_jobs(u) for u in range(U)]
            if U == 1:
                run_jobs(b_flat(bs[0]))
                return
            b0, b1 = bs
            run_jobs([b0['pre']] + b0['w1'] + [b0['shift'], b1['pre']] + b1['w1'] + b0['w2']
                     + [b1['shift'], b0['ln3']] + b1['w2'] + [b1['ln3']] + b0['w3'] + [b0['cat']]
                     + b1['w3'] + [b1['cat']] + b0['w4'] + b1['w4'])

        def fused_jobs(u):
            ej, oj, _ = a_jobs(u)
            b = b_jobs(u)
            w3, w4 = b['w3'], b['w4']

            def slot_pos(g):
                return 0 if g == 0 else (1 if g == 1 else 3 * (g - 1))
            fe = {0: [b['pre']]}
            for i in range(nD):
                fe.setdefault(slot_pos(2 + i // 2), []).append(b['w1'][i])
            fe.setdefault(slot_pos(6), []).append(b['shift'])
            for i in range(nD):
                fe.setdefault(slot_pos(8 + i // 2), []).append(b['w2'][i])
            fe.setdefault(slot_pos(12), []).append(b['ln3'])
            fe.setdefault(slot_pos(15), []).extend(w3[0:1])
            fe.setdefault(len(ej), []).extend(w3[1:4])
            fo = {}
            k = 4
            for g in range(1, 13):
                fo.setdefault(slot_pos(g), []).extend(w3[k:k + 2])
                k += 2
            off = 1
            fo.setdefault(slot_pos(13), []).append(b['cat'])
            fo.setdefault(slot_pos(14), []).append(w4[0])
            fo.setdefault(slot_pos(15), []).append(w4[1])
            fo.setdefault(slot_pos(15) + 3 + off, []).append(w4[2])
            fo.setdefault(len(oj), []).extend(w4[3:])
            return _interleave(ej, fe) + _interleave(oj, fo)

        def part_ab():
            if not (CFG['a'] and CFG['b'] and CFG['fuse']):
                part_a()
                part_b()
                return
            for u in range(U):
                run_jobs(fused_jobs(u))

        @pl.when(t < lag_steps)
        def _():
            part_a()

        @pl.when(jnp.logical_and(t >= lag_steps, t < n_steps))
        def _():
            part_ab()

        @pl.when(t >= n_steps)
        def _():
            part_b()

    return kernel


@functools.partial(jax.jit, static_argnames=("A_seg_len",))
def pallas_sequential_preLN__memory_aug_recurrent_mem_tr__mixer_s_mlp__prompt_kernel(
    A_x, A_mem0, A_Wq, A_Wk, A_Wv, A_Wo, A_seg_len, B_x, B_w1, B_w2, B_w3, B_w4,
):
    _, S, D = A_x.shape
    H, E = A_Wq.shape[1], A_Wq.shape[2]
    F = B_w3.shape[1]
    U = CFG['U']
    assert A_seg_len == SEG and A_mem0.shape[1] == MEM and S % (U * PAIR) == 0
    n_pairs = S // PAIR
    n_steps, lag_steps = n_pairs // U, LAG // U
    nD, nF = D // 128, F // 128

    x = A_x.reshape(S, D)
    mem0 = A_mem0.reshape(MEM, D)
    wo = A_Wo.reshape(H * E, D)

    any_spec = pl.BlockSpec(memory_space=pl.ANY)
    out = pl.pallas_call(
        _make_kernel(S, D, H, E, F),
        grid=(n_steps + lag_steps,),
        in_specs=[
            pl.BlockSpec((U * PAIR, D), lambda t: (jnp.minimum(t, n_steps - 1), 0)),
            pl.BlockSpec((PAIR, D), lambda t: (jnp.minimum((t + 1) * U, n_pairs - 1), 0)),
            pl.BlockSpec((MEM, D), lambda t: (0, 0)),
        ] + [any_spec] * 8,
        out_specs=pl.BlockSpec((U * PAIR, D), lambda t: (jnp.maximum(t - lag_steps, 0), 0)),
        out_shape=jax.ShapeDtypeStruct((S, D), A_x.dtype),
        scratch_shapes=[
            pltpu.VMEM((3, D, H, E), BF),
            pltpu.VMEM((H, D // 2, E), U32),
            pltpu.VMEM((H, D // 2, E), U32),
            pltpu.VMEM((H, D // 2, E), U32),
            pltpu.VMEM((H * E, D), BF),
            pltpu.VMEM((nD, H * E // 2, 128), U32),
            pltpu.VMEM((nD, D, 128), BF),
            pltpu.VMEM((nD, D, 128), BF),
            pltpu.VMEM((nF, D, 128), BF),
            pltpu.VMEM((nD, F, 128), BF),
            pltpu.VMEM((24, D), U32),
            pltpu.VMEM((16, D), U32),
            pltpu.VMEM((3, 8, H * E), F32),
            pltpu.VMEM((40, H * E), U32),
            pltpu.VMEM((48, D), F32),
            pltpu.VMEM((S + 2 * HALO, D), F32),
            pltpu.VMEM((PAIR + 2 * HALO, D), F32),
            pltpu.SemaphoreType.DMA((3 * 4 + nD + 1,)),
        ],
        compiler_params=pltpu.CompilerParams(
            dimension_semantics=("arbitrary",),
            vmem_limit_bytes=120 * 1024 * 1024,
            disable_bounds_checks=CFG['nobc'],
        ),
    )(x, x, mem0, A_Wq, A_Wk, A_Wv, wo, B_w1, B_w2, B_w3, B_w4)
    return out.reshape(1, S, D)
```

```python
import functools

import jax
import jax.numpy as jnp
from jax.experimental import pallas as pl
from jax.experimental.pallas import tpu as pltpu

BF = jnp.bfloat16
F32 = jnp.float32
U32 = jnp.uint32

SEG = 32
MEM = 8
PAIR = 2 * SEG
LAG = 2
HALO = 8
LN_EPS = 1e-5
LOG2E = 1.4426950408889634
CFG = dict(a=True, b=True, att=True, G=2, tail_heads=4, nobc=True, bcol=True)


def _ln(x):
    m = jnp.mean(x, axis=-1, keepdims=True)
    xc = x - m
    v = jnp.mean(xc * xc, axis=-1, keepdims=True)
    return xc * jax.lax.rsqrt(v + LN_EPS)


_dot = functools.partial(jnp.dot, preferred_element_type=F32)


def _gelu(x):
    return jax.nn.gelu(x, approximate=True)


def _as_bf(x_u32):
    return pltpu.bitcast(x_u32, BF)


def _as_u32(x_bf):
    return pltpu.bitcast(x_bf, U32)


def _interleave(main, fill):
    out = []
    for i, j in enumerate(main):
        out.extend(fill.get(i, []))
        out.append(j)
    out.extend(fill.get(len(main), []))
    return out


def _make_kernel(S, D, H, E, F):
    n_pairs = S // PAIR
    nD = D // 128
    nF = F // 128
    c_exp = float(E) ** -0.5 * LOG2E
    neg_raw = -1000000000.0 / (float(E) ** -0.5)
    L = MEM + SEG
    G = CFG['G']
    assert LAG == 2 and n_pairs >= 6
    n_slots = H // G
    TH = CFG['tail_heads']
    K1 = (H - TH) * E

    X0 = 4 * PAIR

    def kernel(x_hbm, mem0_hbm, wq_hbm, wk_hbm, wv_hbm, wo_hbm, w1_hbm, w2_hbm, w3_hbm, w4_hbm,
               out_hbm,
               raw, wq_t, wk_t, wv_t, wo_raw, wo_t, w1_t, w2_t, w3_t, w4_t,
               x_v, out_v, mem0_v, lb_e, lb_o, sv, ob, wacc, h_buf, a1_buf, sems):
        NCH = 4
        CH = D // NCH

        def raw_copy(i, c, src):
            return pltpu.make_async_copy(src.at[pl.ds(c * CH, CH)], raw.at[i, pl.ds(c * CH, CH)],
                                         sems.at[i * NCH + c])

        def col_copies(src, dst, n, sem_idx):
            return [pltpu.make_async_copy(src.at[:, pl.ds(j * 128, 128)], dst.at[j], sems.at[sem_idx])
                    for j in range(n)]

        WO_SEM = 3 * NCH
        B_SEM = WO_SEM + nD
        X0_SEM, X1_SEM, MEM_SEM, OUT_SEM = B_SEM + 1, B_SEM + 2, B_SEM + 3, B_SEM + 4

        def x_head_copy():
            return pltpu.make_async_copy(x_hbm.at[pl.ds(0, X0)], x_v.at[pl.ds(0, X0)], sems.at[X0_SEM])

        def x_rest_copy():
            return pltpu.make_async_copy(x_hbm.at[pl.ds(X0, S - X0)], x_v.at[pl.ds(X0, S - X0)],
                                         sems.at[X1_SEM])

        def mem_copy():
            return pltpu.make_async_copy(mem0_hbm, mem0_v, sems.at[MEM_SEM])

        def out_copy(c):
            rows = pl.ds(pl.multiple_of(c * PAIR, PAIR), PAIR)
            return pltpu.make_async_copy(out_v.at[rows], out_hbm.at[rows], sems.at[OUT_SEM])

        def wo_copy(j):
            rows = pl.ds(j * (H * E // nD), H * E // nD)
            return pltpu.make_async_copy(wo_hbm.at[rows], wo_raw.at[rows], sems.at[WO_SEM + j])

        def wo_finish():
            for j in range(nD):
                wo_copy(j).wait()

                def body(b, carry):
                    r = j * (H * E // nD) + b * 64
                    blk = wo_raw[pl.ds(pl.multiple_of(r, 64), 64), :]
                    for n in range(nD):
                        wo_t[n, pl.ds(pl.multiple_of(r // 2, 32), 32), :] = _as_u32(blk[:, n * 128:(n + 1) * 128])
                    return carry
                jax.lax.fori_loop(0, H * E // nD // 64, body, 0)

        def b_copies():
            if CFG['bcol']:
                return (col_copies(w1_hbm, w1_t, nD, B_SEM) + col_copies(w2_hbm, w2_t, nD, B_SEM)
                        + col_copies(w3_hbm, w3_t, nF, B_SEM) + col_copies(w4_hbm, w4_t, nD, B_SEM))
            return [pltpu.make_async_copy(src, dst, sems.at[B_SEM])
                    for src, dst in ((w1_hbm, w1_t), (w2_hbm, w2_t), (w3_hbm, w3_t), (w4_hbm, w4_t))]

        def wtile(w, j):
            return w[j] if CFG['bcol'] else w[:, pl.ds(j * 128, 128)]

        def relayout(i, c, dst):
            def body(b, carry):
                blk = raw[i, pl.ds(pl.multiple_of(b * 16, 16), 16), :, :]
                dst[:, pl.ds(pl.multiple_of(b * 8, 8), 8), :] = _as_u32(jnp.swapaxes(blk, 0, 1))
                return carry
            jax.lax.fori_loop(c * (CH // 16), (c + 1) * (CH // 16), body, 0)

        def store_xn(x_bf):
            xn = _ln(x_bf.astype(F32))
            lb_e[pl.ds(0, 4), :] = _as_u32(xn[32:40].astype(BF))
            lb_e[pl.ds(4, 4), :] = _as_u32(xn[0:8].astype(BF))
            lb_e[pl.ds(8, 8), :] = _as_u32(xn[8:24].astype(BF))
            lb_e[pl.ds(16, 4), :] = _as_u32(xn[24:32].astype(BF))
            lb_o[pl.ds(0, 8), :] = _as_u32(xn[40:56].astype(BF))
            lb_o[pl.ds(8, 4), :] = _as_u32(xn[56:64].astype(BF))

        def prologue():
            x_head_copy().start()
            mem_copy().start()
            srcs = (wq_hbm, wk_hbm, wv_hbm)
            qkv = [[raw_copy(i, c, srcs[i]) for c in range(NCH)] for i in range(3)]
            for i in range(3):
                for c in range(NCH):
                    qkv[i][c].start()
            for j in range(nD):
                wo_copy(j).start()
            h_buf[pl.ds(0, HALO), :] = jnp.zeros((HALO, D), F32)
            h_buf[pl.ds(HALO + S, HALO), :] = jnp.zeros((HALO, D), F32)
            x_head_copy().wait()
            mem_copy().wait()
            lb_e[pl.ds(20, 4), :] = _as_u32(mem0_v[...])
            store_xn(x_v[pl.ds(0, PAIR), :])
            for i, dst in enumerate((wq_t, wk_t, wv_t)):
                for c in range(NCH):
                    qkv[i][c].wait()
                    relayout(i, c, dst)
            for c in b_copies():
                c.start()
            x_rest_copy().start()
            if not CFG['a']:
                wo_finish()

        def mlp_prologue():
            for c in b_copies():
                c.wait()
            z = _ln(_ln(h_buf[pl.ds(0, 2 * HALO), :])).astype(BF)
            tok = jax.lax.broadcasted_iota(jnp.int32, (2 * HALO, 128), 0) - HALO
            for j in range(nD):
                a1_buf[pl.ds(PAIR, 2 * HALO), pl.ds(j * 128, 128)] = jnp.where(
                    tok >= 0, _gelu(_dot(z, wtile(w1_t, j))), 0.0)

        def a_jobs(t):
            row = jax.lax.broadcasted_iota(jnp.int32, (G * L, G * L), 0)
            col = jax.lax.broadcasted_iota(jnp.int32, (G * L, G * L), 1)
            mask = None
            for i in range(G):
                rl, cl = row - i * L, col - i * L
                blk = ((rl >= 0) & (rl < L) & (cl >= 0) & (cl < L)) & ((cl <= rl) | (cl >= SEG))
                mask = blk if mask is None else (mask | blk)
            x0 = t * PAIR
            h0 = x0 + HALO

            def step_jobs(even):
                lb = lb_e if even else lb_o
                st = {}

                def j_qkv(g):
                    def run():
                        lhs = _as_bf(lb[...])
                        parts = [[], [], []]
                        for h in range(g * G, (g + 1) * G):
                            cs = pl.ds(h * E, E)
                            r = [_dot(lhs, _as_bf(w[h])) for w in (wq_t, wk_t, wv_t)]
                            for i in range(3):
                                if even:
                                    sv[i, :, cs] = r[i][0:8]
                                    parts[i].append(r[i][8:48])
                                else:
                                    parts[i] += [sv[i, :, cs], r[i]]
                        st['qkv', g] = [jnp.concatenate(a, axis=0).astype(BF) for a in parts]
                    return run

                def j_s(g):
                    def run():
                        q, k, v = st.pop(('qkv', g))
                        if not CFG['att']:
                            st['p', g] = (q + k, v)
                            return
                        s = jax.lax.dot_general(q, k, (((1,), (1,)), ((), ())),
                                                preferred_element_type=F32)
                        s = jnp.where(mask, s, neg_raw)
                        m = jnp.max(s, axis=-1, keepdims=True)
                        p = jnp.exp2((s - m) * c_exp)
                        l = jnp.sum(p, axis=-1, keepdims=True)
                        r0 = pl.reciprocal(l, approx=True)
                        p = p * (r0 * (2.0 - l * r0))
                        st['p', g] = (p.astype(BF), v)
                    return run

                def j_pv(g):
                    def run():
                        p, v = st.pop(('p', g))
                        o2 = _dot(p, v) if CFG['att'] else (p + v).astype(F32)
                        for i, h in enumerate(range(g * G, (g + 1) * G)):
                            o = o2[i * L:(i + 1) * L]
                            cs = pl.ds(h * E, E)
                            if even:
                                ob[pl.ds(16, 4), cs] = _as_u32(o[0:8].astype(BF))
                                ob[pl.ds(0, 16), cs] = _as_u32(o[8:40].astype(BF))
                            else:
                                ob[pl.ds(20, 4), cs] = _as_u32(o[0:8].astype(BF))
                                ob[pl.ds(24, 16), cs] = _as_u32(o[8:40].astype(BF))
                    return run

                rows = pl.ds(0, 16) if even else pl.ds(16, 24)
                nrows = 32 if even else 48

                def j_wo1(j):
                    def run():
                        lhs = _as_bf(ob[rows, pl.ds(0, K1)])
                        wacc[pl.ds(0, nrows), pl.ds(j * 128, 128)] = _dot(
                            lhs, _as_bf(wo_t[j, pl.ds(0, K1 // 2), :]))
                    return run

                def j_wo2(j):
                    def run():
                        lhs = _as_bf(ob[rows, pl.ds(K1, H * E - K1)])
                        r = wacc[pl.ds(0, nrows), pl.ds(j * 128, 128)] + _dot(
                            lhs, _as_bf(wo_t[j, pl.ds(K1 // 2, (H * E - K1) // 2), :]))
                        cs = pl.ds(j * 128, 128)
                        xs = x_v[pl.ds(pl.multiple_of(x0, PAIR), PAIR), cs].astype(F32)
                        if even:
                            lb_o[pl.ds(12, 4), cs] = _as_u32(r[24:32].astype(BF))
                            h_buf[pl.ds(pl.multiple_of(h0 + 8, 8), 24), cs] = xs[8:32] + r[0:24]
                        else:
                            lb_e[pl.ds(20, 4), cs] = _as_u32(r[40:48].astype(BF))
                            h_buf[pl.ds(pl.multiple_of(h0, 8), 8), cs] = xs[0:8] + r[0:8]
                            h_buf[pl.ds(pl.multiple_of(h0 + 32, 8), 32), cs] = xs[32:64] + r[8:40]
                    return run

                jobs = []
                for g in range(n_slots):
                    jobs.append(j_qkv(g))
                    if g >= 1:
                        jobs.append(j_s(g - 1))
                    if g >= 2:
                        jobs.append(j_pv(g - 2))
                n_main = len(jobs)
                assert (H - TH) // G - 1 < n_slots - 2
                jobs += [j_wo1(0), j_wo1(1), j_wo1(2), j_s(n_slots - 1), j_pv(n_slots - 2),
                         j_wo1(3), j_wo1(4), j_wo1(5), j_pv(n_slots - 1), j_wo1(6), j_wo1(7)]
                jobs += [j_wo2(j) for j in range(nD)]
                return jobs, n_main

            def j_next_xn():
                nxt = jnp.minimum(t + 1, n_pairs - 1) * PAIR
                store_xn(x_v[pl.ds(pl.multiple_of(nxt, PAIR), PAIR), :])

            ej, e_main = step_jobs(True)
            oj, o_main = step_jobs(False)
            idx = o_main - 2
            oj = oj[:idx] + [j_next_xn] + oj[idx:]
            return ej, oj, e_main

        def b_jobs(c):
            r0 = pl.multiple_of(c * PAIR, PAIR)
            st = {}

            def j_pre():
                a1_buf[pl.ds(0, 2 * HALO), :] = a1_buf[pl.ds(PAIR, 2 * HALO), :]
                y = _ln(h_buf[pl.ds(pl.multiple_of(r0 + HALO, 8), PAIR + HALO), :])
                st['y'] = y[0:PAIR]
                st['z'] = _ln(y[HALO:]).astype(BF)

            def j_w1(j):
                def run():
                    tok = jax.lax.broadcasted_iota(jnp.int32, (PAIR, 128), 0) + (r0 + HALO)
                    a = _gelu(_dot(st['z'], wtile(w1_t, j)))
                    a1_buf[pl.ds(2 * HALO, PAIR), pl.ds(j * 128, 128)] = jnp.where(tok < S, a, 0.0)
                return run

            def j_shift():
                cq = D // 4
                st['g'] = jnp.concatenate([
                    a1_buf[pl.ds(HALO - 1, PAIR), pl.ds(0 * cq, cq)],
                    a1_buf[pl.ds(HALO + 1, PAIR), pl.ds(1 * cq, cq)],
                    a1_buf[pl.ds(HALO - 2, PAIR), pl.ds(2 * cq, cq)],
                    a1_buf[pl.ds(HALO + 2, PAIR), pl.ds(3 * cq, cq)]], axis=1).astype(BF)

            def j_w2(j):
                def run():
                    st['x1', j] = st['y'][:, j * 128:(j + 1) * 128] + _dot(st['g'], wtile(w2_t, j))
                return run

            def j_ln3():
                x1 = jnp.concatenate([st['x1', j] for j in range(nD)], axis=1)
                st['z1'] = _ln(x1).astype(BF)

            def j_w3(j):
                def run():
                    st['a3', j] = _gelu(_dot(st['z1'], wtile(w3_t, j))).astype(BF)
                return run

            def j_cat():
                st['a3'] = jnp.concatenate([st.pop(('a3', j)) for j in range(nF)], axis=1)

            def j_w4(j):
                def run():
                    cs = pl.ds(j * 128, 128)
                    hh = h_buf[pl.ds(pl.multiple_of(r0 + HALO, 8), PAIR), cs]
                    out_v[pl.ds(r0, PAIR), cs] = (
                        hh + (st['x1', j] + _dot(st['a3'], wtile(w4_t, j)))).astype(out_v.dtype)
                return run

            return dict(pre=j_pre, w1=[j_w1(j) for j in range(nD)], shift=j_shift,
                        w2=[j_w2(j) for j in range(nD)], ln3=j_ln3,
                        w3=[j_w3(j) for j in range(nF)], cat=j_cat,
                        w4=[j_w4(j) for j in range(nD)])

        def run_jobs(jobs):
            for j in jobs:
                j()

        def fused_jobs(t):
            ej, oj, _ = a_jobs(t)
            b = b_jobs(t - LAG)
            w3, w4 = b['w3'], b['w4']

            def slot_pos(g):
                return 0 if g == 0 else (1 if g == 1 else 3 * (g - 1))
            fe = {0: [b['pre']]}
            for i in range(nD):
                fe.setdefault(slot_pos(2 + i // 2), []).append(b['w1'][i])
            fe.setdefault(slot_pos(6), []).append(b['shift'])
            for i in range(nD):
                fe.setdefault(slot_pos(8 + i // 2), []).append(b['w2'][i])
            fe.setdefault(slot_pos(12), []).append(b['ln3'])
            fe.setdefault(slot_pos(15), []).extend(w3[0:1])
            fe.setdefault(len(ej), []).extend(w3[1:4])
            fo = {}
            k = 4
            for g in range(1, 13):
                fo.setdefault(slot_pos(g), []).extend(w3[k:k + 2])
                k += 2
            off = 1
            fo.setdefault(slot_pos(13), []).append(b['cat'])
            fo.setdefault(slot_pos(14), []).append(w4[0])
            fo.setdefault(slot_pos(15), []).append(w4[1])
            fo.setdefault(slot_pos(15) + 3 + off, []).append(w4[2])
            fo.setdefault(len(oj), []).extend(w4[3:])
            return _interleave(ej, fe) + _interleave(oj, fo)

        def a_only(t, carry):
            ej, oj, e_main = a_jobs(t)

            def j_wo_wait():
                with jax.named_scope("sc_wo_finish"):
                    pl.when(t == 0)(wo_finish)
            run_jobs(ej[:e_main] + [j_wo_wait] + ej[e_main:] + oj)
            return carry

        def fused(t, carry):
            with jax.named_scope("sc_xwait"):
                @pl.when(t == X0 // PAIR - 1)
                def _():
                    x_rest_copy().wait()

                @pl.when(t > LAG)
                def _():
                    out_copy(t - LAG - 1).start()
            with jax.named_scope("sc_fused_body"):
                run_jobs(fused_jobs(t))
            return carry

        def b_only(c, carry):
            out_copy(c - 1).start()
            b = b_jobs(c)
            run_jobs([b['pre']] + b['w1'] + [b['shift']] + b['w2'] + [b['ln3']] + b['w3'] + [b['cat']] + b['w4'])
            return carry

        def b_tail():
            jax.lax.fori_loop(n_pairs - LAG, n_pairs, b_only, 0)
            out_copy(n_pairs - 1).start()

        with jax.named_scope("sc_prologue"):
            prologue()
        with jax.named_scope("sc_a_only"):
            jax.lax.fori_loop(0, LAG, a_only, 0)
        with jax.named_scope("sc_mlp_prologue"):
            mlp_prologue()
        with jax.named_scope("sc_fused"):
            jax.lax.fori_loop(LAG, n_pairs, fused, 0)
        with jax.named_scope("sc_b_tail"):
            b_tail()
        with jax.named_scope("sc_out_wait"):
            pltpu.make_async_copy(out_v, out_hbm, sems.at[OUT_SEM]).wait()

    return kernel


@functools.partial(jax.jit, static_argnames=("A_seg_len",))
def pallas_sequential_preLN__memory_aug_recurrent_mem_tr__mixer_s_mlp__prompt_kernel(
    A_x, A_mem0, A_Wq, A_Wk, A_Wv, A_Wo, A_seg_len, B_x, B_w1, B_w2, B_w3, B_w4,
):
    _, S, D = A_x.shape
    H, E = A_Wq.shape[1], A_Wq.shape[2]
    F = B_w3.shape[1]
    assert A_seg_len == SEG and A_mem0.shape[1] == MEM and S % PAIR == 0
    nD, nF = D // 128, F // 128

    x = A_x.reshape(S, D)
    mem0 = A_mem0.reshape(MEM, D)
    wo = A_Wo.reshape(H * E, D)

    any_spec = pl.BlockSpec(memory_space=pl.ANY)
    out = pl.pallas_call(
        _make_kernel(S, D, H, E, F),
        in_specs=[any_spec] * 10,
        out_specs=any_spec,
        out_shape=jax.ShapeDtypeStruct((S, D), A_x.dtype),
        scratch_shapes=[
            pltpu.VMEM((3, D, H, E), BF),
            pltpu.VMEM((H, D // 2, E), U32),
            pltpu.VMEM((H, D // 2, E), U32),
            pltpu.VMEM((H, D // 2, E), U32),
            pltpu.VMEM((H * E, D), BF),
            pltpu.VMEM((nD, H * E // 2, 128), U32),
            pltpu.VMEM((nD, D, 128) if CFG['bcol'] else (D, D), BF),
            pltpu.VMEM((nD, D, 128) if CFG['bcol'] else (D, D), BF),
            pltpu.VMEM((nF, D, 128) if CFG['bcol'] else (D, F), BF),
            pltpu.VMEM((nD, F, 128) if CFG['bcol'] else (F, D), BF),
            pltpu.VMEM((S, D), BF),
            pltpu.VMEM((S, D), BF),
            pltpu.VMEM((MEM, D), BF),
            pltpu.VMEM((24, D), U32),
            pltpu.VMEM((16, D), U32),
            pltpu.VMEM((3, 8, H * E), F32),
            pltpu.VMEM((40, H * E), U32),
            pltpu.VMEM((48, D), F32),
            pltpu.VMEM((S + 2 * HALO, D), F32),
            pltpu.VMEM((PAIR + 2 * HALO, D), F32),
            pltpu.SemaphoreType.DMA((3 * 4 + nD + 5,)),
        ],
        compiler_params=pltpu.CompilerParams(
            vmem_limit_bytes=120 * 1024 * 1024,
            disable_bounds_checks=CFG['nobc'],
        ),
    )(x, mem0, A_Wq, A_Wk, A_Wv, wo, B_w1, B_w2, B_w3, B_w4)
    return out.reshape(1, S, D)
```

```python
import functools

import jax
import jax.numpy as jnp
from jax.experimental import pallas as pl
from jax.experimental.pallas import tpu as pltpu

BF = jnp.bfloat16
F32 = jnp.float32
U32 = jnp.uint32

SEG = 32
MEM = 8
PAIR = 2 * SEG
HALO = 8
LN_EPS = 1e-5
LOG2E = 1.4426950408889634
CFG = dict(a=True, b=True, att=True, G=2, tail_heads=4, nobc=True, bcol=True, lag=3, b_after_wo=False)


def _ln(x):
    m = jnp.mean(x, axis=-1, keepdims=True)
    xc = x - m
    v = jnp.mean(xc * xc, axis=-1, keepdims=True)
    return xc * jax.lax.rsqrt(v + LN_EPS)


_dot = functools.partial(jnp.dot, preferred_element_type=F32)


def _gelu(x):
    return jax.nn.gelu(x, approximate=True)


def _as_bf(x_u32):
    return pltpu.bitcast(x_u32, BF)


def _as_u32(x_bf):
    return pltpu.bitcast(x_bf, U32)


def _interleave(main, fill):
    out = []
    for i, j in enumerate(main):
        out.extend(fill.get(i, []))
        out.append(j)
    out.extend(fill.get(len(main), []))
    return out


def _make_kernel(S, D, H, E, F):
    n_pairs = S // PAIR
    nD = D // 128
    nF = F // 128
    c_exp = float(E) ** -0.5 * LOG2E
    neg_raw = -1000000000.0 / (float(E) ** -0.5)
    L = MEM + SEG
    G = CFG['G']
    LAG = CFG['lag']
    assert 2 <= LAG <= 3 and n_pairs >= 8
    n_slots = H // G
    TH = CFG['tail_heads']
    K1 = (H - TH) * E

    X0 = 4 * PAIR

    def kernel(x_hbm, mem0_hbm, wq_hbm, wk_hbm, wv_hbm, wo_hbm, w1_hbm, w2_hbm, w3_hbm, w4_hbm,
               out_hbm,
               raw, wq_t, wk_t, wv_t, wo_raw, wo_t, w1_t, w2_t, w3_t, w4_t,
               x_v, out_v, mem0_v, lb_e, lb_o, sv, ob, wacc, h_buf, a1_buf, sems):
        NCH = 4
        CH = D // NCH

        def raw_copy(i, c, src):
            return pltpu.make_async_copy(src.at[pl.ds(c * CH, CH)], raw.at[i, pl.ds(c * CH, CH)],
                                         sems.at[i * NCH + c])

        def col_copies(src, dst, n, sem_idx):
            return [pltpu.make_async_copy(src.at[:, pl.ds(j * 128, 128)], dst.at[j], sems.at[sem_idx])
                    for j in range(n)]

        WO_SEM = 3 * NCH
        B_SEM = WO_SEM + nD
        X0_SEM, X1_SEM, MEM_SEM, OUT_SEM = B_SEM + 1, B_SEM + 2, B_SEM + 3, B_SEM + 4

        def x_head_copy():
            return pltpu.make_async_copy(x_hbm.at[pl.ds(0, X0)], x_v.at[pl.ds(0, X0)], sems.at[X0_SEM])

        def x_rest_copy():
            return pltpu.make_async_copy(x_hbm.at[pl.ds(X0, S - X0)], x_v.at[pl.ds(X0, S - X0)],
                                         sems.at[X1_SEM])

        def mem_copy():
            return pltpu.make_async_copy(mem0_hbm, mem0_v, sems.at[MEM_SEM])

        def out_copy(c):
            rows = pl.ds(pl.multiple_of(c * PAIR, PAIR), PAIR)
            return pltpu.make_async_copy(out_v.at[rows], out_hbm.at[rows], sems.at[OUT_SEM])

        def wo_copy(j):
            rows = pl.ds(j * (H * E // nD), H * E // nD)
            return pltpu.make_async_copy(wo_hbm.at[rows], wo_raw.at[rows], sems.at[WO_SEM + j])

        def wo_finish():
            for j in range(nD):
                wo_copy(j).wait()

                def body(b, carry):
                    r = j * (H * E // nD) + b * 64
                    blk = wo_raw[pl.ds(pl.multiple_of(r, 64), 64), :]
                    for n in range(nD):
                        wo_t[n, pl.ds(pl.multiple_of(r // 2, 32), 32), :] = _as_u32(blk[:, n * 128:(n + 1) * 128])
                    return carry
                jax.lax.fori_loop(0, H * E // nD // 64, body, 0)
            if CFG['b_after_wo']:
                start_rest()

        def start_rest():
            for c in b_copies():
                c.start()
            x_rest_copy().start()

        def b_copies():
            if CFG['bcol']:
                return (col_copies(w1_hbm, w1_t, nD, B_SEM) + col_copies(w2_hbm, w2_t, nD, B_SEM)
                        + col_copies(w3_hbm, w3_t, nF, B_SEM) + col_copies(w4_hbm, w4_t, nD, B_SEM))
            return [pltpu.make_async_copy(src, dst, sems.at[B_SEM])
                    for src, dst in ((w1_hbm, w1_t), (w2_hbm, w2_t), (w3_hbm, w3_t), (w4_hbm, w4_t))]

        def wtile(w, j):
            return w[j] if CFG['bcol'] else w[:, pl.ds(j * 128, 128)]

        def relayout(i, c, dst):
            def body(b, carry):
                blk = raw[i, pl.ds(pl.multiple_of(b * 16, 16), 16), :, :]
                dst[:, pl.ds(pl.multiple_of(b * 8, 8), 8), :] = _as_u32(jnp.swapaxes(blk, 0, 1))
                return carry
            jax.lax.fori_loop(c * (CH // 16), (c + 1) * (CH // 16), body, 0)

        def store_xn(x_bf):
            xn = _ln(x_bf.astype(F32))
            lb_e[pl.ds(0, 4), :] = _as_u32(xn[32:40].astype(BF))
            lb_e[pl.ds(4, 4), :] = _as_u32(xn[0:8].astype(BF))
            lb_e[pl.ds(8, 8), :] = _as_u32(xn[8:24].astype(BF))
            lb_e[pl.ds(16, 4), :] = _as_u32(xn[24:32].astype(BF))
            lb_o[pl.ds(0, 8), :] = _as_u32(xn[40:56].astype(BF))
            lb_o[pl.ds(8, 4), :] = _as_u32(xn[56:64].astype(BF))

        def prologue():
            x_head_copy().start()
            mem_copy().start()
            srcs = (wq_hbm, wk_hbm, wv_hbm)
            qkv = [[raw_copy(i, c, srcs[i]) for c in range(NCH)] for i in range(3)]
            for i in range(3):
                for c in range(NCH):
                    qkv[i][c].start()
            for j in range(nD):
                wo_copy(j).start()
            h_buf[pl.ds(0, HALO), :] = jnp.zeros((HALO, D), F32)
            h_buf[pl.ds(HALO + S, HALO), :] = jnp.zeros((HALO, D), F32)
            x_head_copy().wait()
            mem_copy().wait()
            lb_e[pl.ds(20, 4), :] = _as_u32(mem0_v[...])
            store_xn(x_v[pl.ds(0, PAIR), :])
            for i, dst in enumerate((wq_t, wk_t, wv_t)):
                for c in range(NCH):
                    qkv[i][c].wait()
                    relayout(i, c, dst)
            if not CFG['b_after_wo']:
                start_rest()
            if not CFG['a']:
                wo_finish()

        def mlp_prologue():
            for c in b_copies():
                c.wait()
            z = _ln(_ln(h_buf[pl.ds(0, 2 * HALO), :])).astype(BF)
            tok = jax.lax.broadcasted_iota(jnp.int32, (2 * HALO, 128), 0) - HALO
            for j in range(nD):
                a1_buf[pl.ds(PAIR, 2 * HALO), pl.ds(j * 128, 128)] = jnp.where(
                    tok >= 0, _gelu(_dot(z, wtile(w1_t, j))), 0.0)

        def a_jobs(t):
            row = jax.lax.broadcasted_iota(jnp.int32, (G * L, G * L), 0)
            col = jax.lax.broadcasted_iota(jnp.int32, (G * L, G * L), 1)
            mask = None
            for i in range(G):
                rl, cl = row - i * L, col - i * L
                blk = ((rl >= 0) & (rl < L) & (cl >= 0) & (cl < L)) & ((cl <= rl) | (cl >= SEG))
                mask = blk if mask is None else (mask | blk)
            x0 = t * PAIR
            h0 = x0 + HALO

            def step_jobs(even):
                lb = lb_e if even else lb_o
                st = {}

                def j_qkv(g):
                    def run():
                        lhs = _as_bf(lb[...])
                        parts = [[], [], []]
                        for h in range(g * G, (g + 1) * G):
                            cs = pl.ds(h * E, E)
                            r = [_dot(lhs, _as_bf(w[h])) for w in (wq_t, wk_t, wv_t)]
                            for i in range(3):
                                if even:
                                    sv[i, :, cs] = r[i][0:8]
                                    parts[i].append(r[i][8:48])
                                else:
                                    parts[i] += [sv[i, :, cs], r[i]]
                        st['qkv', g] = [jnp.concatenate(a, axis=0).astype(BF) for a in parts]
                    return run

                def j_s(g):
                    def run():
                        q, k, v = st.pop(('qkv', g))
                        if not CFG['att']:
                            st['p', g] = (q + k, v)
                            return
                        s = jax.lax.dot_general(q, k, (((1,), (1,)), ((), ())),
                                                preferred_element_type=F32)
                        s = jnp.where(mask, s, neg_raw)
                        m = jnp.max(s, axis=-1, keepdims=True)
                        p = jnp.exp2((s - m) * c_exp)
                        l = jnp.sum(p, axis=-1, keepdims=True)
                        r0 = pl.reciprocal(l, approx=True)
                        p = p * (r0 * (2.0 - l * r0))
                        st['p', g] = (p.astype(BF), v)
                    return run

                def j_pv(g):
                    def run():
                        p, v = st.pop(('p', g))
                        o2 = _dot(p, v) if CFG['att'] else (p + v).astype(F32)
                        for i, h in enumerate(range(g * G, (g + 1) * G)):
                            o = o2[i * L:(i + 1) * L]
                            cs = pl.ds(h * E, E)
                            if even:
                                ob[pl.ds(16, 4), cs] = _as_u32(o[0:8].astype(BF))
                                ob[pl.ds(0, 16), cs] = _as_u32(o[8:40].astype(BF))
                            else:
                                ob[pl.ds(20, 4), cs] = _as_u32(o[0:8].astype(BF))
                                ob[pl.ds(24, 16), cs] = _as_u32(o[8:40].astype(BF))
                    return run

                rows = pl.ds(0, 16) if even else pl.ds(16, 24)
                nrows = 32 if even else 48

                def j_wo1(j):
                    def run():
                        lhs = _as_bf(ob[rows, pl.ds(0, K1)])
                        wacc[pl.ds(0, nrows), pl.ds(j * 128, 128)] = _dot(
                            lhs, _as_bf(wo_t[j, pl.ds(0, K1 // 2), :]))
                    return run

                def j_wo2(j):
                    def run():
                        lhs = _as_bf(ob[rows, pl.ds(K1, H * E - K1)])
                        r = wacc[pl.ds(0, nrows), pl.ds(j * 128, 128)] + _dot(
                            lhs, _as_bf(wo_t[j, pl.ds(K1 // 2, (H * E - K1) // 2), :]))
                        cs = pl.ds(j * 128, 128)
                        xs = x_v[pl.ds(pl.multiple_of(x0, PAIR), PAIR), cs].astype(F32)
                        if even:
                            lb_o[pl.ds(12, 4), cs] = _as_u32(r[24:32].astype(BF))
                            h_buf[pl.ds(pl.multiple_of(h0 + 8, 8), 24), cs] = xs[8:32] + r[0:24]
                        else:
                            lb_e[pl.ds(20, 4), cs] = _as_u32(r[40:48].astype(BF))
                            h_buf[pl.ds(pl.multiple_of(h0, 8), 8), cs] = xs[0:8] + r[0:8]
                            h_buf[pl.ds(pl.multiple_of(h0 + 32, 8), 32), cs] = xs[32:64] + r[8:40]
                    return run

                jobs = []
                for g in range(n_slots):
                    jobs.append(j_qkv(g))
                    if g >= 1:
                        jobs.append(j_s(g - 1))
                    if g >= 2:
                        jobs.append(j_pv(g - 2))
                n_main = len(jobs)
                assert (H - TH) // G - 1 < n_slots - 2
                jobs += [j_wo1(0), j_wo1(1), j_wo1(2), j_s(n_slots - 1), j_pv(n_slots - 2),
                         j_wo1(3), j_wo1(4), j_wo1(5), j_pv(n_slots - 1), j_wo1(6), j_wo1(7)]
                jobs += [j_wo2(j) for j in range(nD)]
                return jobs, n_main

            def j_next_xn():
                nxt = jnp.minimum(t + 1, n_pairs - 1) * PAIR
                store_xn(x_v[pl.ds(pl.multiple_of(nxt, PAIR), PAIR), :])

            ej, e_main = step_jobs(True)
            oj, o_main = step_jobs(False)
            idx = o_main - 2
            oj = oj[:idx] + [j_next_xn] + oj[idx:]
            return ej, oj, e_main

        def b_jobs(c):
            r0 = pl.multiple_of(c * PAIR, PAIR)
            st = {}

            def j_pre():
                a1_buf[pl.ds(0, 2 * HALO), :] = a1_buf[pl.ds(PAIR, 2 * HALO), :]
                y = _ln(h_buf[pl.ds(pl.multiple_of(r0 + HALO, 8), PAIR + HALO), :])
                st['y'] = y[0:PAIR]
                st['z'] = _ln(y[HALO:]).astype(BF)

            def j_w1(j):
                def run():
                    tok = jax.lax.broadcasted_iota(jnp.int32, (PAIR, 128), 0) + (r0 + HALO)
                    a = _gelu(_dot(st['z'], wtile(w1_t, j)))
                    a1_buf[pl.ds(2 * HALO, PAIR), pl.ds(j * 128, 128)] = jnp.where(tok < S, a, 0.0)
                return run

            def j_shift():
                cq = D // 4
                st['g'] = jnp.concatenate([
                    a1_buf[pl.ds(HALO - 1, PAIR), pl.ds(0 * cq, cq)],
                    a1_buf[pl.ds(HALO + 1, PAIR), pl.ds(1 * cq, cq)],
                    a1_buf[pl.ds(HALO - 2, PAIR), pl.ds(2 * cq, cq)],
                    a1_buf[pl.ds(HALO + 2, PAIR), pl.ds(3 * cq, cq)]], axis=1).astype(BF)

            def j_w2(j):
                def run():
                    st['x1', j] = st['y'][:, j * 128:(j + 1) * 128] + _dot(st['g'], wtile(w2_t, j))
                return run

            def j_ln3():
                x1 = jnp.concatenate([st['x1', j] for j in range(nD)], axis=1)
                st['z1'] = _ln(x1).astype(BF)

            def j_w3(j):
                def run():
                    st['a3', j] = _gelu(_dot(st['z1'], wtile(w3_t, j))).astype(BF)
                return run

            def j_cat():
                st['a3'] = jnp.concatenate([st.pop(('a3', j)) for j in range(nF)], axis=1)

            def j_w4(j):
                def run():
                    cs = pl.ds(j * 128, 128)
                    hh = h_buf[pl.ds(pl.multiple_of(r0 + HALO, 8), PAIR), cs]
                    out_v[pl.ds(r0, PAIR), cs] = (
                        hh + (st['x1', j] + _dot(st['a3'], wtile(w4_t, j)))).astype(out_v.dtype)
                return run

            return dict(pre=j_pre, w1=[j_w1(j) for j in range(nD)], shift=j_shift,
                        w2=[j_w2(j) for j in range(nD)], ln3=j_ln3,
                        w3=[j_w3(j) for j in range(nF)], cat=j_cat,
                        w4=[j_w4(j) for j in range(nD)])

        def run_jobs(jobs):
            for j in jobs:
                j()

        def fused_jobs(t):
            ej, oj, _ = a_jobs(t)
            b = b_jobs(t - LAG)
            w3, w4 = b['w3'], b['w4']

            def slot_pos(g):
                return 0 if g == 0 else (1 if g == 1 else 3 * (g - 1))
            fe = {0: [b['pre']]}
            for i in range(nD):
                fe.setdefault(slot_pos(2 + i // 2), []).append(b['w1'][i])
            fe.setdefault(slot_pos(6), []).append(b['shift'])
            for i in range(nD):
                fe.setdefault(slot_pos(8 + i // 2), []).append(b['w2'][i])
            fe.setdefault(slot_pos(12), []).append(b['ln3'])
            fe.setdefault(slot_pos(15), []).extend(w3[0:1])
            fe.setdefault(len(ej), []).extend(w3[1:4])
            fo = {}
            k = 4
            for g in range(1, 13):
                fo.setdefault(slot_pos(g), []).extend(w3[k:k + 2])
                k += 2
            off = 1
            fo.setdefault(slot_pos(13), []).append(b['cat'])
            fo.setdefault(slot_pos(14), []).append(w4[0])
            fo.setdefault(slot_pos(15), []).append(w4[1])
            fo.setdefault(slot_pos(15) + 3 + off, []).append(w4[2])
            fo.setdefault(len(oj), []).extend(w4[3:])
            return _interleave(ej, fe) + _interleave(oj, fo)

        def a_only(t, carry):
            ej, oj, e_main = a_jobs(t)

            def j_wo_wait():
                with jax.named_scope("sc_wo_finish"):
                    pl.when(t == 0)(wo_finish)
            run_jobs(ej[:e_main] + [j_wo_wait] + ej[e_main:] + oj)
            return carry

        def fused(t, carry):
            with jax.named_scope("sc_xwait"):
                @pl.when(t == X0 // PAIR - 1)
                def _():
                    x_rest_copy().wait()

                @pl.when(t > LAG)
                def _():
                    out_copy(t - LAG - 1).start()
            with jax.named_scope("sc_fused_body"):
                run_jobs(fused_jobs(t))
            return carry

        def b_only(c, carry):
            out_copy(c - 1).start()
            b = b_jobs(c)
            run_jobs([b['pre']] + b['w1'] + [b['shift']] + b['w2'] + [b['ln3']] + b['w3'] + [b['cat']] + b['w4'])
            return carry

        def b_tail():
            jax.lax.fori_loop(n_pairs - LAG, n_pairs, b_only, 0)
            out_copy(n_pairs - 1).start()

        with jax.named_scope("sc_prologue"):
            prologue()
        with jax.named_scope("sc_a_only"):
            jax.lax.fori_loop(0, LAG, a_only, 0)
        with jax.named_scope("sc_mlp_prologue"):
            mlp_prologue()
        with jax.named_scope("sc_fused"):
            jax.lax.fori_loop(LAG, n_pairs, fused, 0)
        with jax.named_scope("sc_b_tail"):
            b_tail()
        with jax.named_scope("sc_out_wait"):
            pltpu.make_async_copy(out_v, out_hbm, sems.at[OUT_SEM]).wait()

    return kernel


@functools.partial(jax.jit, static_argnames=("A_seg_len",))
def pallas_sequential_preLN__memory_aug_recurrent_mem_tr__mixer_s_mlp__prompt_kernel(
    A_x, A_mem0, A_Wq, A_Wk, A_Wv, A_Wo, A_seg_len, B_x, B_w1, B_w2, B_w3, B_w4,
):
    _, S, D = A_x.shape
    H, E = A_Wq.shape[1], A_Wq.shape[2]
    F = B_w3.shape[1]
    assert A_seg_len == SEG and A_mem0.shape[1] == MEM and S % PAIR == 0
    nD, nF = D // 128, F // 128

    x = A_x.reshape(S, D)
    mem0 = A_mem0.reshape(MEM, D)
    wo = A_Wo.reshape(H * E, D)

    any_spec = pl.BlockSpec(memory_space=pl.ANY)
    out = pl.pallas_call(
        _make_kernel(S, D, H, E, F),
        in_specs=[any_spec] * 10,
        out_specs=any_spec,
        out_shape=jax.ShapeDtypeStruct((S, D), A_x.dtype),
        scratch_shapes=[
            pltpu.VMEM((3, D, H, E), BF),
            pltpu.VMEM((H, D // 2, E), U32),
            pltpu.VMEM((H, D // 2, E), U32),
            pltpu.VMEM((H, D // 2, E), U32),
            pltpu.VMEM((H * E, D), BF),
            pltpu.VMEM((nD, H * E // 2, 128), U32),
            pltpu.VMEM((nD, D, 128) if CFG['bcol'] else (D, D), BF),
            pltpu.VMEM((nD, D, 128) if CFG['bcol'] else (D, D), BF),
            pltpu.VMEM((nF, D, 128) if CFG['bcol'] else (D, F), BF),
            pltpu.VMEM((nD, F, 128) if CFG['bcol'] else (F, D), BF),
            pltpu.VMEM((S, D), BF),
            pltpu.VMEM((S, D), BF),
            pltpu.VMEM((MEM, D), BF),
            pltpu.VMEM((24, D), U32),
            pltpu.VMEM((16, D), U32),
            pltpu.VMEM((3, 8, H * E), F32),
            pltpu.VMEM((40, H * E), U32),
            pltpu.VMEM((48, D), F32),
            pltpu.VMEM((S + 2 * HALO, D), F32),
            pltpu.VMEM((PAIR + 2 * HALO, D), F32),
            pltpu.SemaphoreType.DMA((3 * 4 + nD + 5,)),
        ],
        compiler_params=pltpu.CompilerParams(
            vmem_limit_bytes=120 * 1024 * 1024,
            disable_bounds_checks=CFG['nobc'],
        ),
    )(x, mem0, A_Wq, A_Wk, A_Wv, wo, B_w1, B_w2, B_w3, B_w4)
    return out.reshape(1, S, D)
```

```python
import functools

import jax
import jax.numpy as jnp
from jax.experimental import pallas as pl
from jax.experimental.pallas import tpu as pltpu

BF = jnp.bfloat16
F32 = jnp.float32
U32 = jnp.uint32

SEG = 32
MEM = 8
PAIR = 2 * SEG
HALO = 8
LN_EPS = 1e-5
LOG2E = 1.4426950408889634
CFG = dict(a=True, b=True, att=True, G=2, tail_heads=4, nobc=True, bcol=True, lag=3, b_after_wo=False, w4_last=True, fine=True, etail=0)


def _ln(x):
    m = jnp.mean(x, axis=-1, keepdims=True)
    xc = x - m
    v = jnp.mean(xc * xc, axis=-1, keepdims=True)
    return xc * jax.lax.rsqrt(v + LN_EPS)


_dot = functools.partial(jnp.dot, preferred_element_type=F32)


def _gelu(x):
    return jax.nn.gelu(x, approximate=True)


def _as_bf(x_u32):
    return pltpu.bitcast(x_u32, BF)


def _as_u32(x_bf):
    return pltpu.bitcast(x_bf, U32)


def _interleave(main, fill):
    fill = dict(fill)
    out = []
    for label, job in main:
        out.extend(fill.pop(label, []))
        out.append(job)
    out.extend(fill.pop('end', []))
    assert not fill, fill
    return out


def _make_kernel(S, D, H, E, F):
    n_pairs = S // PAIR
    nD = D // 128
    nF = F // 128
    c_exp = float(E) ** -0.5 * LOG2E
    neg_raw = -1000000000.0 / (float(E) ** -0.5)
    L = MEM + SEG
    G = CFG['G']
    LAG = CFG['lag']
    assert 2 <= LAG <= 3 and n_pairs >= 8
    n_slots = H // G
    TH = CFG['tail_heads']
    K1 = (H - TH) * E

    X0 = 4 * PAIR

    def kernel(x_hbm, mem0_hbm, wq_hbm, wk_hbm, wv_hbm, wo_hbm, w1_hbm, w2_hbm, w3_hbm, w4_hbm,
               out_hbm,
               raw, wq_t, wk_t, wv_t, wo_raw, wo_t, w1_t, w2_t, w3_t, w4_t,
               x_v, out_v, mem0_v, lb_e, lb_o, sv, ob, wacc, h_buf, a1_buf, sems):
        NCH = 4
        CH = D // NCH

        def raw_copy(i, c, src):
            return pltpu.make_async_copy(src.at[pl.ds(c * CH, CH)], raw.at[i, pl.ds(c * CH, CH)],
                                         sems.at[i * NCH + c])

        def col_copies(src, dst, n, sem_idx):
            return [pltpu.make_async_copy(src.at[:, pl.ds(j * 128, 128)], dst.at[j], sems.at[sem_idx])
                    for j in range(n)]

        WO_SEM = 3 * NCH
        B_SEM = WO_SEM + nD
        X0_SEM, X1_SEM, MEM_SEM, OUT_SEM = B_SEM + 1, B_SEM + 2, B_SEM + 3, B_SEM + 4

        def x_head_copy():
            return pltpu.make_async_copy(x_hbm.at[pl.ds(0, X0)], x_v.at[pl.ds(0, X0)], sems.at[X0_SEM])

        def x_rest_copy():
            return pltpu.make_async_copy(x_hbm.at[pl.ds(X0, S - X0)], x_v.at[pl.ds(X0, S - X0)],
                                         sems.at[X1_SEM])

        def mem_copy():
            return pltpu.make_async_copy(mem0_hbm, mem0_v, sems.at[MEM_SEM])

        def out_copy(c):
            rows = pl.ds(pl.multiple_of(c * PAIR, PAIR), PAIR)
            return pltpu.make_async_copy(out_v.at[rows], out_hbm.at[rows], sems.at[OUT_SEM])

        def wo_copy(j):
            rows = pl.ds(j * (H * E // nD), H * E // nD)
            return pltpu.make_async_copy(wo_hbm.at[rows], wo_raw.at[rows], sems.at[WO_SEM + j])

        def wo_finish():
            for j in range(nD):
                wo_copy(j).wait()

                def body(b, carry):
                    r = j * (H * E // nD) + b * 64
                    blk = wo_raw[pl.ds(pl.multiple_of(r, 64), 64), :]
                    for n in range(nD):
                        wo_t[n, pl.ds(pl.multiple_of(r // 2, 32), 32), :] = _as_u32(blk[:, n * 128:(n + 1) * 128])
                    return carry
                jax.lax.fori_loop(0, H * E // nD // 64, body, 0)
            if CFG['b_after_wo']:
                start_rest()

        def start_rest():
            for c in b_copies():
                c.start()
            x_rest_copy().start()

        def b_copies():
            if CFG['bcol']:
                return (col_copies(w1_hbm, w1_t, nD, B_SEM) + col_copies(w2_hbm, w2_t, nD, B_SEM)
                        + col_copies(w3_hbm, w3_t, nF, B_SEM) + col_copies(w4_hbm, w4_t, nD, B_SEM))
            return [pltpu.make_async_copy(src, dst, sems.at[B_SEM])
                    for src, dst in ((w1_hbm, w1_t), (w2_hbm, w2_t), (w3_hbm, w3_t), (w4_hbm, w4_t))]

        def wtile(w, j):
            return w[j] if CFG['bcol'] else w[:, pl.ds(j * 128, 128)]

        def relayout(i, c, dst):
            def body(b, carry):
                blk = raw[i, pl.ds(pl.multiple_of(b * 16, 16), 16), :, :]
                dst[:, pl.ds(pl.multiple_of(b * 8, 8), 8), :] = _as_u32(jnp.swapaxes(blk, 0, 1))
                return carry
            jax.lax.fori_loop(c * (CH // 16), (c + 1) * (CH // 16), body, 0)

        def store_xn(x_bf):
            xn = _ln(x_bf.astype(F32))
            lb_e[pl.ds(0, 4), :] = _as_u32(xn[32:40].astype(BF))
            lb_e[pl.ds(4, 4), :] = _as_u32(xn[0:8].astype(BF))
            lb_e[pl.ds(8, 8), :] = _as_u32(xn[8:24].astype(BF))
            lb_e[pl.ds(16, 4), :] = _as_u32(xn[24:32].astype(BF))
            lb_o[pl.ds(0, 8), :] = _as_u32(xn[40:56].astype(BF))
            lb_o[pl.ds(8, 4), :] = _as_u32(xn[56:64].astype(BF))

        def prologue():
            x_head_copy().start()
            mem_copy().start()
            srcs = (wq_hbm, wk_hbm, wv_hbm)
            qkv = [[raw_copy(i, c, srcs[i]) for c in range(NCH)] for i in range(3)]
            for i in range(3):
                for c in range(NCH):
                    qkv[i][c].start()
            for j in range(nD):
                wo_copy(j).start()
            h_buf[pl.ds(0, HALO), :] = jnp.zeros((HALO, D), F32)
            h_buf[pl.ds(HALO + S, HALO), :] = jnp.zeros((HALO, D), F32)
            x_head_copy().wait()
            mem_copy().wait()
            lb_e[pl.ds(20, 4), :] = _as_u32(mem0_v[...])
            store_xn(x_v[pl.ds(0, PAIR), :])
            for i, dst in enumerate((wq_t, wk_t, wv_t)):
                for c in range(NCH):
                    qkv[i][c].wait()
                    if not CFG.get('norelayout'):
                        relayout(i, c, dst)
            if not CFG['b_after_wo']:
                start_rest()
            if not CFG['a']:
                wo_finish()

        def mlp_prologue():
            for c in b_copies():
                c.wait()
            z = _ln(_ln(h_buf[pl.ds(0, 2 * HALO), :])).astype(BF)
            tok = jax.lax.broadcasted_iota(jnp.int32, (2 * HALO, 128), 0) - HALO
            for j in range(nD):
                a1_buf[pl.ds(PAIR, 2 * HALO), pl.ds(j * 128, 128)] = jnp.where(
                    tok >= 0, _gelu(_dot(z, wtile(w1_t, j))), 0.0)

        def a_jobs(t):
            row = jax.lax.broadcasted_iota(jnp.int32, (G * L, G * L), 0)
            col = jax.lax.broadcasted_iota(jnp.int32, (G * L, G * L), 1)
            mask = None
            for i in range(G):
                rl, cl = row - i * L, col - i * L
                blk = ((rl >= 0) & (rl < L) & (cl >= 0) & (cl < L)) & ((cl <= rl) | (cl >= SEG))
                mask = blk if mask is None else (mask | blk)
            x0 = t * PAIR
            h0 = x0 + HALO

            def step_jobs(even):
                lb = lb_e if even else lb_o
                st = {}

                def j_qkv(g, i):
                    def run():
                        h = g * G + i
                        lhs = _as_bf(lb[...])
                        cs = pl.ds(h * E, E)
                        r = [_dot(lhs, _as_bf(w[h])) for w in (wq_t, wk_t, wv_t)]
                        parts = st.setdefault(('parts', g), [[], [], []])
                        for n in range(3):
                            if even:
                                sv[n, :, cs] = r[n][0:8]
                                parts[n].append(r[n][8:48])
                            else:
                                parts[n] += [sv[n, :, cs], r[n]]
                        if i == G - 1:
                            st['qkv', g] = [jnp.concatenate(a, axis=0).astype(BF)
                                            for a in st.pop(('parts', g))]
                    return run

                def j_s(g):
                    def run():
                        q, k, v = st.pop(('qkv', g))
                        if not CFG['att']:
                            st['p', g] = (q + k, v)
                            return
                        s = jax.lax.dot_general(q, k, (((1,), (1,)), ((), ())),
                                                preferred_element_type=F32)
                        s = jnp.where(mask, s, neg_raw)
                        m = jnp.max(s, axis=-1, keepdims=True)
                        p = jnp.exp2((s - m) * c_exp)
                        l = jnp.sum(p, axis=-1, keepdims=True)
                        r0 = pl.reciprocal(l, approx=True)
                        p = p * (r0 * (2.0 - l * r0))
                        st['p', g] = (p.astype(BF), v)
                    return run

                def j_pv(g):
                    def run():
                        p, v = st.pop(('p', g))
                        o2 = _dot(p, v) if CFG['att'] else (p + v).astype(F32)
                        for i, h in enumerate(range(g * G, (g + 1) * G)):
                            o = o2[i * L:(i + 1) * L]
                            cs = pl.ds(h * E, E)
                            if even:
                                ob[pl.ds(16, 4), cs] = _as_u32(o[0:8].astype(BF))
                                ob[pl.ds(0, 16), cs] = _as_u32(o[8:40].astype(BF))
                            else:
                                ob[pl.ds(20, 4), cs] = _as_u32(o[0:8].astype(BF))
                                ob[pl.ds(24, 16), cs] = _as_u32(o[8:40].astype(BF))
                    return run

                rows = pl.ds(0, 16) if even else pl.ds(16, 24)
                nrows = 32 if even else 48

                def j_wo1(j):
                    def run():
                        lhs = _as_bf(ob[rows, pl.ds(0, K1)])
                        wacc[pl.ds(0, nrows), pl.ds(j * 128, 128)] = _dot(
                            lhs, _as_bf(wo_t[j, pl.ds(0, K1 // 2), :]))
                    return run

                def j_wo2(j):
                    def run():
                        lhs = _as_bf(ob[rows, pl.ds(K1, H * E - K1)])
                        r = wacc[pl.ds(0, nrows), pl.ds(j * 128, 128)] + _dot(
                            lhs, _as_bf(wo_t[j, pl.ds(K1 // 2, (H * E - K1) // 2), :]))
                        cs = pl.ds(j * 128, 128)
                        xs = x_v[pl.ds(pl.multiple_of(x0, PAIR), PAIR), cs].astype(F32)
                        if even:
                            lb_o[pl.ds(12, 4), cs] = _as_u32(r[24:32].astype(BF))
                            h_buf[pl.ds(pl.multiple_of(h0 + 8, 8), 24), cs] = xs[8:32] + r[0:24]
                        else:
                            lb_e[pl.ds(20, 4), cs] = _as_u32(r[40:48].astype(BF))
                            h_buf[pl.ds(pl.multiple_of(h0, 8), 8), cs] = xs[0:8] + r[0:8]
                            h_buf[pl.ds(pl.multiple_of(h0 + 32, 8), 32), cs] = xs[32:64] + r[8:40]
                    return run

                jobs = []
                for g in range(n_slots):
                    for i in range(G):
                        jobs.append((('qkv', g, i), j_qkv(g, i)))
                    if g >= 1:
                        jobs.append((('s', g - 1), j_s(g - 1)))
                    if g >= 2:
                        jobs.append((('pv', g - 2), j_pv(g - 2)))
                assert (H - TH) // G - 1 < n_slots - 2
                wo1 = [(('wo1', j), j_wo1(j)) for j in range(nD)]
                jobs += (wo1[0:3] + [(('s', n_slots - 1), j_s(n_slots - 1)),
                                     (('pv', n_slots - 2), j_pv(n_slots - 2))]
                         + wo1[3:6] + [(('pv', n_slots - 1), j_pv(n_slots - 1))] + wo1[6:8])
                jobs += [(('wo2', j), j_wo2(j)) for j in range(nD)]
                return jobs

            def j_next_xn():
                nxt = jnp.minimum(t + 1, n_pairs - 1) * PAIR
                store_xn(x_v[pl.ds(pl.multiple_of(nxt, PAIR), PAIR), :])

            return step_jobs(True), step_jobs(False), j_next_xn

        def b_jobs(c):
            r0 = pl.multiple_of(c * PAIR, PAIR)
            st = {}

            def j_pre():
                a1_buf[pl.ds(0, 2 * HALO), :] = a1_buf[pl.ds(PAIR, 2 * HALO), :]
                y = _ln(h_buf[pl.ds(pl.multiple_of(r0 + HALO, 8), PAIR + HALO), :])
                st['y'] = y[0:PAIR]
                st['z'] = _ln(y[HALO:]).astype(BF)

            def j_w1(j):
                def run():
                    tok = jax.lax.broadcasted_iota(jnp.int32, (PAIR, 128), 0) + (r0 + HALO)
                    a = _gelu(_dot(st['z'], wtile(w1_t, j)))
                    a1_buf[pl.ds(2 * HALO, PAIR), pl.ds(j * 128, 128)] = jnp.where(tok < S, a, 0.0)
                return run

            def j_shift():
                cq = D // 4
                st['g'] = jnp.concatenate([
                    a1_buf[pl.ds(HALO - 1, PAIR), pl.ds(0 * cq, cq)],
                    a1_buf[pl.ds(HALO + 1, PAIR), pl.ds(1 * cq, cq)],
                    a1_buf[pl.ds(HALO - 2, PAIR), pl.ds(2 * cq, cq)],
                    a1_buf[pl.ds(HALO + 2, PAIR), pl.ds(3 * cq, cq)]], axis=1).astype(BF)

            def j_w2(j):
                def run():
                    st['x1', j] = st['y'][:, j * 128:(j + 1) * 128] + _dot(st['g'], wtile(w2_t, j))
                return run

            def j_ln3():
                x1 = jnp.concatenate([st['x1', j] for j in range(nD)], axis=1)
                st['z1'] = _ln(x1).astype(BF)

            def j_w3(j):
                def run():
                    st['a3', j] = _gelu(_dot(st['z1'], wtile(w3_t, j))).astype(BF)
                return run

            def j_cat():
                st['a3'] = jnp.concatenate([st.pop(('a3', j)) for j in range(nF)], axis=1)

            def j_w4(j):
                def run():
                    cs = pl.ds(j * 128, 128)
                    hh = h_buf[pl.ds(pl.multiple_of(r0 + HALO, 8), PAIR), cs]
                    out_v[pl.ds(r0, PAIR), cs] = (
                        hh + (st['x1', j] + _dot(st['a3'], wtile(w4_t, j)))).astype(out_v.dtype)
                return run

            return dict(pre=j_pre, w1=[j_w1(j) for j in range(nD)], shift=j_shift,
                        w2=[j_w2(j) for j in range(nD)], ln3=j_ln3,
                        w3=[j_w3(j) for j in range(nF)], cat=j_cat,
                        w4=[j_w4(j) for j in range(nD)])

        def run_jobs(jobs):
            for j in jobs:
                j()

        last_s = ('s', n_slots - 2)

        def fused_jobs(t):
            ej, oj, j_next_xn = a_jobs(t)
            b = b_jobs(t - LAG)
            w3, w4 = b['w3'], b['w4']
            fe, fo = {}, {}

            def put(d, label, *jobs):
                d.setdefault(label, []).extend(jobs)
            put(fe, ('qkv', 0, 0), b['pre'])
            for i in range(nD):
                put(fe, ('qkv', 2 + i // 2, i % 2), b['w1'][i])
                put(fe, ('qkv', 8 + i // 2, i % 2), b['w2'][i])
            put(fe, ('qkv', 6, 0), b['shift'])
            put(fe, ('qkv', 12, 0), b['ln3'])
            if CFG['etail'] == 0:
                put(fe, ('qkv', 15, 0), w3[0])
                put(fe, 'end', *w3[1:4])
            elif CFG['etail'] == 1:
                put(fe, ('wo1', 1), w3[0])
                put(fe, ('wo1', 4), w3[1])
                put(fe, 'end', *w3[2:4])
            elif CFG['etail'] == 2:
                put(fe, ('wo1', 1), w3[0])
                put(fe, ('wo1', 4), w3[1])
                put(fe, ('wo1', 7), w3[2])
                put(fe, 'end', w3[3])
            if CFG['fine']:
                for k in range(4, nF):
                    put(fo, ('qkv', 1 + (k - 4) // 2, (k - 4) % 2), w3[k])
            else:
                for k in range(4, nF):
                    put(fo, ('qkv', 1 + (k - 4) // 2, 0), w3[k])
            put(fo, ('qkv', 13, 0), b['cat'])
            put(fo, ('qkv', 14, 0), w4[0])
            put(fo, ('qkv', 15, 0), w4[1])
            put(fo, last_s, j_next_xn)
            put(fo, ('s', n_slots - 1), w4[2])
            put(fo, 'end' if CFG['w4_last'] else ('wo2', 0), *w4[3:])
            return _interleave(ej, fe) + _interleave(oj, fo)

        def a_only(t, carry):
            ej, oj, j_next_xn = a_jobs(t)

            def j_wo_wait():
                with jax.named_scope("sc_wo_finish"):
                    pl.when(t == 0)(wo_finish)
            run_jobs(_interleave(ej, {('wo1', 0): [j_wo_wait]}) + _interleave(oj, {last_s: [j_next_xn]}))
            return carry

        def fused(t, carry):
            with jax.named_scope("sc_xwait"):
                @pl.when(t == X0 // PAIR - 1)
                def _():
                    x_rest_copy().wait()

                @pl.when(t > LAG)
                def _():
                    out_copy(t - LAG - 1).start()
            with jax.named_scope("sc_fused_body"):
                run_jobs(fused_jobs(t))
            return carry

        def b_only(c, carry):
            out_copy(c - 1).start()
            b = b_jobs(c)
            run_jobs([b['pre']] + b['w1'] + [b['shift']] + b['w2'] + [b['ln3']] + b['w3'] + [b['cat']] + b['w4'])
            return carry

        def b_tail():
            jax.lax.fori_loop(n_pairs - LAG, n_pairs, b_only, 0)
            out_copy(n_pairs - 1).start()

        with jax.named_scope("sc_prologue"):
            prologue()
        with jax.named_scope("sc_a_only"):
            jax.lax.fori_loop(0, LAG, a_only, 0)
        with jax.named_scope("sc_mlp_prologue"):
            mlp_prologue()
        with jax.named_scope("sc_fused"):
            jax.lax.fori_loop(LAG, n_pairs, fused, 0)
        with jax.named_scope("sc_b_tail"):
            b_tail()
        with jax.named_scope("sc_out_wait"):
            pltpu.make_async_copy(out_v, out_hbm, sems.at[OUT_SEM]).wait()

    return kernel


@functools.partial(jax.jit, static_argnames=("A_seg_len",))
def pallas_sequential_preLN__memory_aug_recurrent_mem_tr__mixer_s_mlp__prompt_kernel(
    A_x, A_mem0, A_Wq, A_Wk, A_Wv, A_Wo, A_seg_len, B_x, B_w1, B_w2, B_w3, B_w4,
):
    _, S, D = A_x.shape
    H, E = A_Wq.shape[1], A_Wq.shape[2]
    F = B_w3.shape[1]
    assert A_seg_len == SEG and A_mem0.shape[1] == MEM and S % PAIR == 0
    nD, nF = D // 128, F // 128

    x = A_x.reshape(S, D)
    mem0 = A_mem0.reshape(MEM, D)
    wo = A_Wo.reshape(H * E, D)

    any_spec = pl.BlockSpec(memory_space=pl.ANY)
    out = pl.pallas_call(
        _make_kernel(S, D, H, E, F),
        in_specs=[any_spec] * 10,
        out_specs=any_spec,
        out_shape=jax.ShapeDtypeStruct((S, D), A_x.dtype),
        scratch_shapes=[
            pltpu.VMEM((3, D, H, E), BF),
            pltpu.VMEM((H, D // 2, E), U32),
            pltpu.VMEM((H, D // 2, E), U32),
            pltpu.VMEM((H, D // 2, E), U32),
            pltpu.VMEM((H * E, D), BF),
            pltpu.VMEM((nD, H * E // 2, 128), U32),
            pltpu.VMEM((nD, D, 128) if CFG['bcol'] else (D, D), BF),
            pltpu.VMEM((nD, D, 128) if CFG['bcol'] else (D, D), BF),
            pltpu.VMEM((nF, D, 128) if CFG['bcol'] else (D, F), BF),
            pltpu.VMEM((nD, F, 128) if CFG['bcol'] else (F, D), BF),
            pltpu.VMEM((S, D), BF),
            pltpu.VMEM((S, D), BF),
            pltpu.VMEM((MEM, D), BF),
            pltpu.VMEM((24, D), U32),
            pltpu.VMEM((16, D), U32),
            pltpu.VMEM((3, 8, H * E), F32),
            pltpu.VMEM((40, H * E), U32),
            pltpu.VMEM((48, D), F32),
            pltpu.VMEM((S + 2 * HALO, D), F32),
            pltpu.VMEM((PAIR + 2 * HALO, D), F32),
            pltpu.SemaphoreType.DMA((3 * 4 + nD + 5,)),
        ],
        compiler_params=pltpu.CompilerParams(
            vmem_limit_bytes=120 * 1024 * 1024,
            disable_bounds_checks=CFG['nobc'],
        ),
    )(x, mem0, A_Wq, A_Wk, A_Wv, wo, B_w1, B_w2, B_w3, B_w4)
    return out.reshape(1, S, D)
```

```python
import functools

import jax
import jax.numpy as jnp
from jax.experimental import pallas as pl
from jax.experimental.pallas import tpu as pltpu

BF = jnp.bfloat16
F32 = jnp.float32
U32 = jnp.uint32

SEG = 32
MEM = 8
PAIR = 2 * SEG
HALO = 8
LN_EPS = 1e-5
LOG2E = 1.4426950408889634
CFG = dict(a=True, b=True, att=True, G=2, tail_heads=4, nobc=True, bcol=True, lag=3, b_after_wo=False, w4_last=True, fine=True, etail=0)


def _ln(x):
    m = jnp.mean(x, axis=-1, keepdims=True)
    xc = x - m
    v = jnp.mean(xc * xc, axis=-1, keepdims=True)
    return xc * jax.lax.rsqrt(v + LN_EPS)


_dot = functools.partial(jnp.dot, preferred_element_type=F32)


def _gelu(x):
    return jax.nn.gelu(x, approximate=True)


def _as_bf(x_u32):
    return pltpu.bitcast(x_u32, BF)


def _as_u32(x_bf):
    return pltpu.bitcast(x_bf, U32)


def _interleave(main, fill):
    fill = dict(fill)
    out = []
    for label, job in main:
        out.extend(fill.pop(label, []))
        out.append(job)
    out.extend(fill.pop('end', []))
    assert not fill, fill
    return out


def _make_kernel(S, D, H, E, F):
    n_pairs = S // PAIR
    nD = D // 128
    nF = F // 128
    c_exp = float(E) ** -0.5 * LOG2E
    neg_raw = -1000000000.0 / (float(E) ** -0.5)
    L = MEM + SEG
    G = CFG['G']
    LAG = CFG['lag']
    assert 2 <= LAG <= 3 and n_pairs >= 8
    n_slots = H // G
    TH = CFG['tail_heads']
    K1 = (H - TH) * E

    X0 = 4 * PAIR

    def kernel(x_hbm, mem0_hbm, wq_hbm, wk_hbm, wv_hbm, wo_hbm, w1_hbm, w2_hbm, w3_hbm, w4_hbm,
               out_hbm,
               raw, wq_t, wk_t, wv_t, wo_raw, wo_t, w1_t, w2_t, w3_t, w4_t,
               x_v, out_v, mem0_v, lb_e, lb_o, sv, ob, wacc, h_buf, a1_buf, sems):
        NCH = 4
        CH = D // NCH

        def raw_copy(i, c, src):
            return pltpu.make_async_copy(src.at[pl.ds(c * CH, CH)], raw.at[i, pl.ds(c * CH, CH)],
                                         sems.at[i * NCH + c])

        def col_copies(src, dst, n, sem_idx):
            return [pltpu.make_async_copy(src.at[:, pl.ds(j * 128, 128)], dst.at[j], sems.at[sem_idx])
                    for j in range(n)]

        WO_SEM = 3 * NCH
        B_SEM = WO_SEM + nD
        X0_SEM, X1_SEM, MEM_SEM, OUT_SEM, XM_SEM = (B_SEM + i for i in range(1, 6))

        def x_head_copy():
            return pltpu.make_async_copy(x_hbm.at[pl.ds(0, PAIR)], x_v.at[pl.ds(0, PAIR)], sems.at[X0_SEM])

        def x_mid_copy():
            return pltpu.make_async_copy(x_hbm.at[pl.ds(PAIR, X0 - PAIR)], x_v.at[pl.ds(PAIR, X0 - PAIR)],
                                         sems.at[XM_SEM])

        def x_rest_copy():
            return pltpu.make_async_copy(x_hbm.at[pl.ds(X0, S - X0)], x_v.at[pl.ds(X0, S - X0)],
                                         sems.at[X1_SEM])

        def mem_copy():
            return pltpu.make_async_copy(mem0_hbm, mem0_v, sems.at[MEM_SEM])

        def out_copy(c):
            rows = pl.ds(pl.multiple_of(c * PAIR, PAIR), PAIR)
            return pltpu.make_async_copy(out_v.at[rows], out_hbm.at[rows], sems.at[OUT_SEM])

        def wo_copy(j):
            rows = pl.ds(j * (H * E // nD), H * E // nD)
            return pltpu.make_async_copy(wo_hbm.at[rows], wo_raw.at[rows], sems.at[WO_SEM + j])

        def wo_finish():
            for j in range(nD):
                wo_copy(j).wait()

                def body(b, carry):
                    r = j * (H * E // nD) + b * 64
                    blk = wo_raw[pl.ds(pl.multiple_of(r, 64), 64), :]
                    for n in range(nD):
                        wo_t[n, pl.ds(pl.multiple_of(r // 2, 32), 32), :] = _as_u32(blk[:, n * 128:(n + 1) * 128])
                    return carry
                jax.lax.fori_loop(0, H * E // nD // 64, body, 0)
            x_mid_copy().wait()
            if CFG['b_after_wo']:
                start_rest()

        def start_rest():
            for c in b_copies():
                c.start()
            x_rest_copy().start()

        def b_copies():
            if CFG['bcol']:
                return (col_copies(w1_hbm, w1_t, nD, B_SEM) + col_copies(w2_hbm, w2_t, nD, B_SEM)
                        + col_copies(w3_hbm, w3_t, nF, B_SEM) + col_copies(w4_hbm, w4_t, nD, B_SEM))
            return [pltpu.make_async_copy(src, dst, sems.at[B_SEM])
                    for src, dst in ((w1_hbm, w1_t), (w2_hbm, w2_t), (w3_hbm, w3_t), (w4_hbm, w4_t))]

        def wtile(w, j):
            return w[j] if CFG['bcol'] else w[:, pl.ds(j * 128, 128)]

        def relayout(i, c, dst):
            def body(b, carry):
                blk = raw[i, pl.ds(pl.multiple_of(b * 16, 16), 16), :, :]
                dst[:, pl.ds(pl.multiple_of(b * 8, 8), 8), :] = _as_u32(jnp.swapaxes(blk, 0, 1))
                return carry
            jax.lax.fori_loop(c * (CH // 16), (c + 1) * (CH // 16), body, 0)

        def store_xn(x_bf):
            xn = _ln(x_bf.astype(F32))
            lb_e[pl.ds(0, 4), :] = _as_u32(xn[32:40].astype(BF))
            lb_e[pl.ds(4, 4), :] = _as_u32(xn[0:8].astype(BF))
            lb_e[pl.ds(8, 8), :] = _as_u32(xn[8:24].astype(BF))
            lb_e[pl.ds(16, 4), :] = _as_u32(xn[24:32].astype(BF))
            lb_o[pl.ds(0, 8), :] = _as_u32(xn[40:56].astype(BF))
            lb_o[pl.ds(8, 4), :] = _as_u32(xn[56:64].astype(BF))

        def prologue():
            x_head_copy().start()
            mem_copy().start()
            srcs = (wq_hbm, wk_hbm, wv_hbm)
            qkv = [[raw_copy(i, c, srcs[i]) for c in range(NCH)] for i in range(3)]
            for i in range(3):
                for c in range(NCH):
                    qkv[i][c].start()
            for j in range(nD):
                wo_copy(j).start()
            x_mid_copy().start()
            h_buf[pl.ds(0, HALO), :] = jnp.zeros((HALO, D), F32)
            h_buf[pl.ds(HALO + S, HALO), :] = jnp.zeros((HALO, D), F32)
            x_head_copy().wait()
            mem_copy().wait()
            lb_e[pl.ds(20, 4), :] = _as_u32(mem0_v[...])
            store_xn(x_v[pl.ds(0, PAIR), :])
            for i, dst in enumerate((wq_t, wk_t, wv_t)):
                for c in range(NCH):
                    qkv[i][c].wait()
                    if not CFG.get('norelayout'):
                        relayout(i, c, dst)
            if not CFG['b_after_wo']:
                start_rest()
            if not CFG['a']:
                wo_finish()

        def mlp_prologue():
            for c in b_copies():
                c.wait()
            z = _ln(_ln(h_buf[pl.ds(0, 2 * HALO), :])).astype(BF)
            tok = jax.lax.broadcasted_iota(jnp.int32, (2 * HALO, 128), 0) - HALO
            for j in range(nD):
                a1_buf[pl.ds(PAIR, 2 * HALO), pl.ds(j * 128, 128)] = jnp.where(
                    tok >= 0, _gelu(_dot(z, wtile(w1_t, j))), 0.0)

        def a_jobs(t):
            row = jax.lax.broadcasted_iota(jnp.int32, (G * L, G * L), 0)
            col = jax.lax.broadcasted_iota(jnp.int32, (G * L, G * L), 1)
            mask = None
            for i in range(G):
                rl, cl = row - i * L, col - i * L
                blk = ((rl >= 0) & (rl < L) & (cl >= 0) & (cl < L)) & ((cl <= rl) | (cl >= SEG))
                mask = blk if mask is None else (mask | blk)
            x0 = t * PAIR
            h0 = x0 + HALO

            def step_jobs(even):
                lb = lb_e if even else lb_o
                st = {}

                def j_qkv(g, i):
                    def run():
                        h = g * G + i
                        lhs = _as_bf(lb[...])
                        cs = pl.ds(h * E, E)
                        r = [_dot(lhs, _as_bf(w[h])) for w in (wq_t, wk_t, wv_t)]
                        parts = st.setdefault(('parts', g), [[], [], []])
                        for n in range(3):
                            if even:
                                sv[n, :, cs] = r[n][0:8]
                                parts[n].append(r[n][8:48])
                            else:
                                parts[n] += [sv[n, :, cs], r[n]]
                        if i == G - 1:
                            st['qkv', g] = [jnp.concatenate(a, axis=0).astype(BF)
                                            for a in st.pop(('parts', g))]
                    return run

                def j_s(g):
                    def run():
                        q, k, v = st.pop(('qkv', g))
                        if not CFG['att']:
                            st['p', g] = (q + k, v)
                            return
                        s = jax.lax.dot_general(q, k, (((1,), (1,)), ((), ())),
                                                preferred_element_type=F32)
                        s = jnp.where(mask, s, neg_raw)
                        m = jnp.max(s, axis=-1, keepdims=True)
                        p = jnp.exp2((s - m) * c_exp)
                        l = jnp.sum(p, axis=-1, keepdims=True)
                        r0 = pl.reciprocal(l, approx=True)
                        p = p * (r0 * (2.0 - l * r0))
                        st['p', g] = (p.astype(BF), v)
                    return run

                def j_pv(g):
                    def run():
                        p, v = st.pop(('p', g))
                        o2 = _dot(p, v) if CFG['att'] else (p + v).astype(F32)
                        for i, h in enumerate(range(g * G, (g + 1) * G)):
                            o = o2[i * L:(i + 1) * L]
                            cs = pl.ds(h * E, E)
                            if even:
                                ob[pl.ds(16, 4), cs] = _as_u32(o[0:8].astype(BF))
                                ob[pl.ds(0, 16), cs] = _as_u32(o[8:40].astype(BF))
                            else:
                                ob[pl.ds(20, 4), cs] = _as_u32(o[0:8].astype(BF))
                                ob[pl.ds(24, 16), cs] = _as_u32(o[8:40].astype(BF))
                    return run

                rows = pl.ds(0, 16) if even else pl.ds(16, 24)
                nrows = 32 if even else 48

                def j_wo1(j):
                    def run():
                        lhs = _as_bf(ob[rows, pl.ds(0, K1)])
                        wacc[pl.ds(0, nrows), pl.ds(j * 128, 128)] = _dot(
                            lhs, _as_bf(wo_t[j, pl.ds(0, K1 // 2), :]))
                    return run

                def j_wo2(j):
                    def run():
                        lhs = _as_bf(ob[rows, pl.ds(K1, H * E - K1)])
                        r = wacc[pl.ds(0, nrows), pl.ds(j * 128, 128)] + _dot(
                            lhs, _as_bf(wo_t[j, pl.ds(K1 // 2, (H * E - K1) // 2), :]))
                        cs = pl.ds(j * 128, 128)
                        xs = x_v[pl.ds(pl.multiple_of(x0, PAIR), PAIR), cs].astype(F32)
                        if even:
                            lb_o[pl.ds(12, 4), cs] = _as_u32(r[24:32].astype(BF))
                            h_buf[pl.ds(pl.multiple_of(h0 + 8, 8), 24), cs] = xs[8:32] + r[0:24]
                        else:
                            lb_e[pl.ds(20, 4), cs] = _as_u32(r[40:48].astype(BF))
                            h_buf[pl.ds(pl.multiple_of(h0, 8), 8), cs] = xs[0:8] + r[0:8]
                            h_buf[pl.ds(pl.multiple_of(h0 + 32, 8), 32), cs] = xs[32:64] + r[8:40]
                    return run

                jobs = []
                for g in range(n_slots):
                    for i in range(G):
                        jobs.append((('qkv', g, i), j_qkv(g, i)))
                    if g >= 1:
                        jobs.append((('s', g - 1), j_s(g - 1)))
                    if g >= 2:
                        jobs.append((('pv', g - 2), j_pv(g - 2)))
                assert (H - TH) // G - 1 < n_slots - 2
                wo1 = [(('wo1', j), j_wo1(j)) for j in range(nD)]
                jobs += (wo1[0:3] + [(('s', n_slots - 1), j_s(n_slots - 1)),
                                     (('pv', n_slots - 2), j_pv(n_slots - 2))]
                         + wo1[3:6] + [(('pv', n_slots - 1), j_pv(n_slots - 1))] + wo1[6:8])
                jobs += [(('wo2', j), j_wo2(j)) for j in range(nD)]
                return jobs

            def j_next_xn():
                nxt = jnp.minimum(t + 1, n_pairs - 1) * PAIR
                store_xn(x_v[pl.ds(pl.multiple_of(nxt, PAIR), PAIR), :])

            return step_jobs(True), step_jobs(False), j_next_xn

        def b_jobs(c):
            r0 = pl.multiple_of(c * PAIR, PAIR)
            st = {}

            def j_pre():
                a1_buf[pl.ds(0, 2 * HALO), :] = a1_buf[pl.ds(PAIR, 2 * HALO), :]
                y = _ln(h_buf[pl.ds(pl.multiple_of(r0 + HALO, 8), PAIR + HALO), :])
                st['y'] = y[0:PAIR]
                st['z'] = _ln(y[HALO:]).astype(BF)

            def j_w1(j):
                def run():
                    tok = jax.lax.broadcasted_iota(jnp.int32, (PAIR, 128), 0) + (r0 + HALO)
                    a = _gelu(_dot(st['z'], wtile(w1_t, j)))
                    a1_buf[pl.ds(2 * HALO, PAIR), pl.ds(j * 128, 128)] = jnp.where(tok < S, a, 0.0)
                return run

            def j_shift():
                cq = D // 4
                st['g'] = jnp.concatenate([
                    a1_buf[pl.ds(HALO - 1, PAIR), pl.ds(0 * cq, cq)],
                    a1_buf[pl.ds(HALO + 1, PAIR), pl.ds(1 * cq, cq)],
                    a1_buf[pl.ds(HALO - 2, PAIR), pl.ds(2 * cq, cq)],
                    a1_buf[pl.ds(HALO + 2, PAIR), pl.ds(3 * cq, cq)]], axis=1).astype(BF)

            def j_w2(j):
                def run():
                    st['x1', j] = st['y'][:, j * 128:(j + 1) * 128] + _dot(st['g'], wtile(w2_t, j))
                return run

            def j_ln3():
                x1 = jnp.concatenate([st['x1', j] for j in range(nD)], axis=1)
                st['z1'] = _ln(x1).astype(BF)

            def j_w3(j):
                def run():
                    st['a3', j] = _gelu(_dot(st['z1'], wtile(w3_t, j))).astype(BF)
                return run

            def j_cat():
                st['a3'] = jnp.concatenate([st.pop(('a3', j)) for j in range(nF)], axis=1)

            def j_w4(j):
                def run():
                    cs = pl.ds(j * 128, 128)
                    hh = h_buf[pl.ds(pl.multiple_of(r0 + HALO, 8), PAIR), cs]
                    out_v[pl.ds(r0, PAIR), cs] = (
                        hh + (st['x1', j] + _dot(st['a3'], wtile(w4_t, j)))).astype(out_v.dtype)
                return run

            return dict(pre=j_pre, w1=[j_w1(j) for j in range(nD)], shift=j_shift,
                        w2=[j_w2(j) for j in range(nD)], ln3=j_ln3,
                        w3=[j_w3(j) for j in range(nF)], cat=j_cat,
                        w4=[j_w4(j) for j in range(nD)])

        def run_jobs(jobs):
            for j in jobs:
                j()

        last_s = ('s', n_slots - 2)

        def fused_jobs(t):
            ej, oj, j_next_xn = a_jobs(t)
            b = b_jobs(t - LAG)
            w3, w4 = b['w3'], b['w4']
            fe, fo = {}, {}

            def put(d, label, *jobs):
                d.setdefault(label, []).extend(jobs)
            put(fe, ('qkv', 0, 0), b['pre'])
            for i in range(nD):
                put(fe, ('qkv', 2 + i // 2, i % 2), b['w1'][i])
                put(fe, ('qkv', 8 + i // 2, i % 2), b['w2'][i])
            put(fe, ('qkv', 6, 0), b['shift'])
            put(fe, ('qkv', 12, 0), b['ln3'])
            if CFG['etail'] == 0:
                put(fe, ('qkv', 15, 0), w3[0])
                put(fe, 'end', *w3[1:4])
            elif CFG['etail'] == 1:
                put(fe, ('wo1', 1), w3[0])
                put(fe, ('wo1', 4), w3[1])
                put(fe, 'end', *w3[2:4])
            elif CFG['etail'] == 2:
                put(fe, ('wo1', 1), w3[0])
                put(fe, ('wo1', 4), w3[1])
                put(fe, ('wo1', 7), w3[2])
                put(fe, 'end', w3[3])
            if CFG['fine']:
                for k in range(4, nF):
                    put(fo, ('qkv', 1 + (k - 4) // 2, (k - 4) % 2), w3[k])
            else:
                for k in range(4, nF):
                    put(fo, ('qkv', 1 + (k - 4) // 2, 0), w3[k])
            put(fo, ('qkv', 13, 0), b['cat'])
            put(fo, ('qkv', 14, 0), w4[0])
            put(fo, ('qkv', 15, 0), w4[1])
            put(fo, last_s, j_next_xn)
            put(fo, ('s', n_slots - 1), w4[2])
            put(fo, 'end' if CFG['w4_last'] else ('wo2', 0), *w4[3:])
            return _interleave(ej, fe) + _interleave(oj, fo)

        def a_only(t, carry):
            ej, oj, j_next_xn = a_jobs(t)

            def j_wo_wait():
                with jax.named_scope("sc_wo_finish"):
                    pl.when(t == 0)(wo_finish)
            run_jobs(_interleave(ej, {last_s: [j_wo_wait]}) + _interleave(oj, {last_s: [j_next_xn]}))
            return carry

        def fused(t, carry):
            with jax.named_scope("sc_xwait"):
                @pl.when(t == X0 // PAIR - 1)
                def _():
                    x_rest_copy().wait()

                @pl.when(t > LAG)
                def _():
                    out_copy(t - LAG - 1).start()
            with jax.named_scope("sc_fused_body"):
                run_jobs(fused_jobs(t))
            return carry

        def b_only(c, carry):
            out_copy(c - 1).start()
            b = b_jobs(c)
            run_jobs([b['pre']] + b['w1'] + [b['shift']] + b['w2'] + [b['ln3']] + b['w3'] + [b['cat']] + b['w4'])
            return carry

        def b_tail():
            jax.lax.fori_loop(n_pairs - LAG, n_pairs, b_only, 0)
            out_copy(n_pairs - 1).start()

        with jax.named_scope("sc_prologue"):
            prologue()
        with jax.named_scope("sc_a_only"):
            jax.lax.fori_loop(0, LAG, a_only, 0)
        with jax.named_scope("sc_mlp_prologue"):
            mlp_prologue()
        with jax.named_scope("sc_fused"):
            jax.lax.fori_loop(LAG, n_pairs, fused, 0)
        with jax.named_scope("sc_b_tail"):
            b_tail()
        with jax.named_scope("sc_out_wait"):
            pltpu.make_async_copy(out_v, out_hbm, sems.at[OUT_SEM]).wait()

    return kernel


@functools.partial(jax.jit, static_argnames=("A_seg_len",))
def pallas_sequential_preLN__memory_aug_recurrent_mem_tr__mixer_s_mlp__prompt_kernel(
    A_x, A_mem0, A_Wq, A_Wk, A_Wv, A_Wo, A_seg_len, B_x, B_w1, B_w2, B_w3, B_w4,
):
    _, S, D = A_x.shape
    H, E = A_Wq.shape[1], A_Wq.shape[2]
    F = B_w3.shape[1]
    assert A_seg_len == SEG and A_mem0.shape[1] == MEM and S % PAIR == 0
    nD, nF = D // 128, F // 128

    x = A_x.reshape(S, D)
    mem0 = A_mem0.reshape(MEM, D)
    wo = A_Wo.reshape(H * E, D)

    any_spec = pl.BlockSpec(memory_space=pl.ANY)
    out = pl.pallas_call(
        _make_kernel(S, D, H, E, F),
        in_specs=[any_spec] * 10,
        out_specs=any_spec,
        out_shape=jax.ShapeDtypeStruct((S, D), A_x.dtype),
        scratch_shapes=[
            pltpu.VMEM((3, D, H, E), BF),
            pltpu.VMEM((H, D // 2, E), U32),
            pltpu.VMEM((H, D // 2, E), U32),
            pltpu.VMEM((H, D // 2, E), U32),
            pltpu.VMEM((H * E, D), BF),
            pltpu.VMEM((nD, H * E // 2, 128), U32),
            pltpu.VMEM((nD, D, 128) if CFG['bcol'] else (D, D), BF),
            pltpu.VMEM((nD, D, 128) if CFG['bcol'] else (D, D), BF),
            pltpu.VMEM((nF, D, 128) if CFG['bcol'] else (D, F), BF),
            pltpu.VMEM((nD, F, 128) if CFG['bcol'] else (F, D), BF),
            pltpu.VMEM((S, D), BF),
            pltpu.VMEM((S, D), BF),
            pltpu.VMEM((MEM, D), BF),
            pltpu.VMEM((24, D), U32),
            pltpu.VMEM((16, D), U32),
            pltpu.VMEM((3, 8, H * E), F32),
            pltpu.VMEM((40, H * E), U32),
            pltpu.VMEM((48, D), F32),
            pltpu.VMEM((S + 2 * HALO, D), F32),
            pltpu.VMEM((PAIR + 2 * HALO, D), F32),
            pltpu.SemaphoreType.DMA((3 * 4 + nD + 6,)),
        ],
        compiler_params=pltpu.CompilerParams(
            vmem_limit_bytes=120 * 1024 * 1024,
            disable_bounds_checks=CFG['nobc'],
        ),
    )(x, mem0, A_Wq, A_Wk, A_Wv, wo, B_w1, B_w2, B_w3, B_w4)
    return out.reshape(1, S, D)
```

```python
import functools

import jax
import jax.numpy as jnp
from jax.experimental import pallas as pl
from jax.experimental.pallas import tpu as pltpu

BF = jnp.bfloat16
F32 = jnp.float32
U32 = jnp.uint32

SEG = 32
MEM = 8
PAIR = 2 * SEG
HALO = 8
LN_EPS = 1e-5
LOG2E = 1.4426950408889634
CFG = dict(a=True, b=True, att=True, G=2, tail_heads=6, nobc=True, bcol=True, lag=3, b_after_wo=False, w4_last=True, fine=True, etail=0, prepos=('o', ('qkv', 0, 1)), w1slot=2, w4pos=[('qkv', 14, 0), ('qkv', 15, 0), ('s', 15)])


def _ln(x):
    m = jnp.mean(x, axis=-1, keepdims=True)
    xc = x - m
    v = jnp.mean(xc * xc, axis=-1, keepdims=True)
    return xc * jax.lax.rsqrt(v + LN_EPS)


_dot = functools.partial(jnp.dot, preferred_element_type=F32)


def _gelu(x):
    return jax.nn.gelu(x, approximate=True)


def _as_bf(x_u32):
    return pltpu.bitcast(x_u32, BF)


def _as_u32(x_bf):
    return pltpu.bitcast(x_bf, U32)


def _interleave(main, fill):
    fill = dict(fill)
    out = []
    for label, job in main:
        out.extend(fill.pop(label, []))
        out.append(job)
    out.extend(fill.pop('end', []))
    assert not fill, fill
    return out


def _make_kernel(S, D, H, E, F):
    n_pairs = S // PAIR
    nD = D // 128
    nF = F // 128
    c_exp = float(E) ** -0.5 * LOG2E
    neg_raw = -1000000000.0 / (float(E) ** -0.5)
    L = MEM + SEG
    G = CFG['G']
    LAG = CFG['lag']
    assert 2 <= LAG <= 3 and n_pairs >= 8
    n_slots = H // G
    TH = CFG['tail_heads']
    K1 = (H - TH) * E

    X0 = 4 * PAIR

    def kernel(x_hbm, mem0_hbm, wq_hbm, wk_hbm, wv_hbm, wo_hbm, w1_hbm, w2_hbm, w3_hbm, w4_hbm,
               out_hbm,
               raw, wq_t, wk_t, wv_t, wo_raw, wo_t, w1_t, w2_t, w3_t, w4_t,
               x_v, out_v, mem0_v, lb_e, lb_o, sv, ob, wacc, h_buf, a1_buf, y_buf, z_buf, sems):
        NCH = 4
        CH = D // NCH

        def raw_copy(i, c, src):
            return pltpu.make_async_copy(src.at[pl.ds(c * CH, CH)], raw.at[i, pl.ds(c * CH, CH)],
                                         sems.at[i * NCH + c])

        def col_copies(src, dst, n, sem_idx):
            return [pltpu.make_async_copy(src.at[:, pl.ds(j * 128, 128)], dst.at[j], sems.at[sem_idx])
                    for j in range(n)]

        WO_SEM = 3 * NCH
        B_SEM = WO_SEM + nD
        X0_SEM, X1_SEM, MEM_SEM, OUT_SEM, XM_SEM = (B_SEM + i for i in range(1, 6))

        def x_head_copy():
            return pltpu.make_async_copy(x_hbm.at[pl.ds(0, PAIR)], x_v.at[pl.ds(0, PAIR)], sems.at[X0_SEM])

        def x_mid_copy():
            return pltpu.make_async_copy(x_hbm.at[pl.ds(PAIR, X0 - PAIR)], x_v.at[pl.ds(PAIR, X0 - PAIR)],
                                         sems.at[XM_SEM])

        def x_rest_copy():
            return pltpu.make_async_copy(x_hbm.at[pl.ds(X0, S - X0)], x_v.at[pl.ds(X0, S - X0)],
                                         sems.at[X1_SEM])

        def mem_copy():
            return pltpu.make_async_copy(mem0_hbm, mem0_v, sems.at[MEM_SEM])

        def out_copy(c):
            rows = pl.ds(pl.multiple_of(c * PAIR, PAIR), PAIR)
            return pltpu.make_async_copy(out_v.at[rows], out_hbm.at[rows], sems.at[OUT_SEM])

        def wo_copy(j):
            rows = pl.ds(j * (H * E // nD), H * E // nD)
            return pltpu.make_async_copy(wo_hbm.at[rows], wo_raw.at[rows], sems.at[WO_SEM + j])

        def wo_finish():
            for j in range(nD):
                wo_copy(j).wait()

                def body(b, carry):
                    r = j * (H * E // nD) + b * 64
                    blk = wo_raw[pl.ds(pl.multiple_of(r, 64), 64), :]
                    for n in range(nD):
                        wo_t[n, pl.ds(pl.multiple_of(r // 2, 32), 32), :] = _as_u32(blk[:, n * 128:(n + 1) * 128])
                    return carry
                jax.lax.fori_loop(0, H * E // nD // 64, body, 0)
            x_mid_copy().wait()
            if CFG['b_after_wo']:
                start_rest()

        def start_rest():
            for c in b_copies():
                c.start()
            x_rest_copy().start()

        def b_copies():
            if CFG['bcol']:
                return (col_copies(w1_hbm, w1_t, nD, B_SEM) + col_copies(w2_hbm, w2_t, nD, B_SEM)
                        + col_copies(w3_hbm, w3_t, nF, B_SEM) + col_copies(w4_hbm, w4_t, nD, B_SEM))
            return [pltpu.make_async_copy(src, dst, sems.at[B_SEM])
                    for src, dst in ((w1_hbm, w1_t), (w2_hbm, w2_t), (w3_hbm, w3_t), (w4_hbm, w4_t))]

        def wtile(w, j):
            return w[j] if CFG['bcol'] else w[:, pl.ds(j * 128, 128)]

        def relayout(i, c, dst):
            def body(b, carry):
                blk = raw[i, pl.ds(pl.multiple_of(b * 16, 16), 16), :, :]
                dst[:, pl.ds(pl.multiple_of(b * 8, 8), 8), :] = _as_u32(jnp.swapaxes(blk, 0, 1))
                return carry
            jax.lax.fori_loop(c * (CH // 16), (c + 1) * (CH // 16), body, 0)

        def store_xn(x_bf):
            xn = _ln(x_bf.astype(F32))
            lb_e[pl.ds(0, 4), :] = _as_u32(xn[32:40].astype(BF))
            lb_e[pl.ds(4, 4), :] = _as_u32(xn[0:8].astype(BF))
            lb_e[pl.ds(8, 8), :] = _as_u32(xn[8:24].astype(BF))
            lb_e[pl.ds(16, 4), :] = _as_u32(xn[24:32].astype(BF))
            lb_o[pl.ds(0, 8), :] = _as_u32(xn[40:56].astype(BF))
            lb_o[pl.ds(8, 4), :] = _as_u32(xn[56:64].astype(BF))

        def prologue():
            x_head_copy().start()
            mem_copy().start()
            srcs = (wq_hbm, wk_hbm, wv_hbm)
            qkv = [[raw_copy(i, c, srcs[i]) for c in range(NCH)] for i in range(3)]
            for i in range(3):
                for c in range(NCH):
                    qkv[i][c].start()
            for j in range(nD):
                wo_copy(j).start()
            x_mid_copy().start()
            h_buf[pl.ds(0, HALO), :] = jnp.zeros((HALO, D), F32)
            h_buf[pl.ds(HALO + S, HALO), :] = jnp.zeros((HALO, D), F32)
            x_head_copy().wait()
            mem_copy().wait()
            lb_e[pl.ds(20, 4), :] = _as_u32(mem0_v[...])
            store_xn(x_v[pl.ds(0, PAIR), :])
            for i, dst in enumerate((wq_t, wk_t, wv_t)):
                for c in range(NCH):
                    qkv[i][c].wait()
                    if not CFG.get('norelayout'):
                        relayout(i, c, dst)
            if not CFG['b_after_wo']:
                start_rest()
            if not CFG['a']:
                wo_finish()

        def mlp_pre(c):
            a1_buf[pl.ds(0, 2 * HALO), :] = a1_buf[pl.ds(PAIR, 2 * HALO), :]
            y = _ln(h_buf[pl.ds(pl.multiple_of(c * PAIR + HALO, 8), PAIR + HALO), :])
            y_buf[...] = y[0:PAIR]
            z_buf[...] = _as_u32(_ln(y[HALO:]).astype(BF))

        def mlp_prologue():
            for c in b_copies():
                c.wait()
            z = _ln(_ln(h_buf[pl.ds(0, 2 * HALO), :])).astype(BF)
            tok = jax.lax.broadcasted_iota(jnp.int32, (2 * HALO, 128), 0) - HALO
            for j in range(nD):
                a1_buf[pl.ds(PAIR, 2 * HALO), pl.ds(j * 128, 128)] = jnp.where(
                    tok >= 0, _gelu(_dot(z, wtile(w1_t, j))), 0.0)
            mlp_pre(0)

        def a_jobs(t):
            row = jax.lax.broadcasted_iota(jnp.int32, (G * L, G * L), 0)
            col = jax.lax.broadcasted_iota(jnp.int32, (G * L, G * L), 1)
            mask = None
            for i in range(G):
                rl, cl = row - i * L, col - i * L
                blk = ((rl >= 0) & (rl < L) & (cl >= 0) & (cl < L)) & ((cl <= rl) | (cl >= SEG))
                mask = blk if mask is None else (mask | blk)
            x0 = t * PAIR
            h0 = x0 + HALO

            def step_jobs(even):
                lb = lb_e if even else lb_o
                st = {}

                def j_qkv(g, i):
                    def run():
                        h = g * G + i
                        lhs = _as_bf(lb[...])
                        cs = pl.ds(h * E, E)
                        r = [_dot(lhs, _as_bf(w[h])) for w in (wq_t, wk_t, wv_t)]
                        parts = st.setdefault(('parts', g), [[], [], []])
                        for n in range(3):
                            if even:
                                sv[n, :, cs] = r[n][0:8]
                                parts[n].append(r[n][8:48])
                            else:
                                parts[n] += [sv[n, :, cs], r[n]]
                        if i == G - 1:
                            st['qkv', g] = [jnp.concatenate(a, axis=0).astype(BF)
                                            for a in st.pop(('parts', g))]
                    return run

                def j_s(g):
                    def run():
                        q, k, v = st.pop(('qkv', g))
                        if not CFG['att']:
                            st['p', g] = (q + k, v)
                            return
                        s = jax.lax.dot_general(q, k, (((1,), (1,)), ((), ())),
                                                preferred_element_type=F32)
                        s = jnp.where(mask, s, neg_raw)
                        m = jnp.max(s, axis=-1, keepdims=True)
                        p = jnp.exp2((s - m) * c_exp)
                        l = jnp.sum(p, axis=-1, keepdims=True)
                        r0 = pl.reciprocal(l, approx=True)
                        p = p * (r0 * (2.0 - l * r0))
                        st['p', g] = (p.astype(BF), v)
                    return run

                def j_pv(g):
                    def run():
                        p, v = st.pop(('p', g))
                        o2 = _dot(p, v) if CFG['att'] else (p + v).astype(F32)
                        for i, h in enumerate(range(g * G, (g + 1) * G)):
                            o = o2[i * L:(i + 1) * L]
                            cs = pl.ds(h * E, E)
                            if even:
                                ob[pl.ds(16, 4), cs] = _as_u32(o[0:8].astype(BF))
                                ob[pl.ds(0, 16), cs] = _as_u32(o[8:40].astype(BF))
                            else:
                                ob[pl.ds(20, 4), cs] = _as_u32(o[0:8].astype(BF))
                                ob[pl.ds(24, 16), cs] = _as_u32(o[8:40].astype(BF))
                    return run

                rows = pl.ds(0, 16) if even else pl.ds(16, 24)
                nrows = 32 if even else 48

                def j_wo1(j):
                    def run():
                        lhs = _as_bf(ob[rows, pl.ds(0, K1)])
                        wacc[pl.ds(0, nrows), pl.ds(j * 128, 128)] = _dot(
                            lhs, _as_bf(wo_t[j, pl.ds(0, K1 // 2), :]))
                    return run

                def j_wo2(j):
                    def run():
                        lhs = _as_bf(ob[rows, pl.ds(K1, H * E - K1)])
                        r = wacc[pl.ds(0, nrows), pl.ds(j * 128, 128)] + _dot(
                            lhs, _as_bf(wo_t[j, pl.ds(K1 // 2, (H * E - K1) // 2), :]))
                        cs = pl.ds(j * 128, 128)
                        xs = x_v[pl.ds(pl.multiple_of(x0, PAIR), PAIR), cs].astype(F32)
                        if even:
                            lb_o[pl.ds(12, 4), cs] = _as_u32(r[24:32].astype(BF))
                            h_buf[pl.ds(pl.multiple_of(h0 + 8, 8), 24), cs] = xs[8:32] + r[0:24]
                        else:
                            lb_e[pl.ds(20, 4), cs] = _as_u32(r[40:48].astype(BF))
                            h_buf[pl.ds(pl.multiple_of(h0, 8), 8), cs] = xs[0:8] + r[0:8]
                            h_buf[pl.ds(pl.multiple_of(h0 + 32, 8), 32), cs] = xs[32:64] + r[8:40]
                    return run

                jobs = []
                for g in range(n_slots):
                    for i in range(G):
                        jobs.append((('qkv', g, i), j_qkv(g, i)))
                    if g >= 1:
                        jobs.append((('s', g - 1), j_s(g - 1)))
                    if g >= 2:
                        jobs.append((('pv', g - 2), j_pv(g - 2)))
                assert (H - TH) // G - 1 < n_slots - 2
                wo1 = [(('wo1', j), j_wo1(j)) for j in range(nD)]
                jobs += (wo1[0:3] + [(('s', n_slots - 1), j_s(n_slots - 1)),
                                     (('pv', n_slots - 2), j_pv(n_slots - 2))]
                         + wo1[3:6] + [(('pv', n_slots - 1), j_pv(n_slots - 1))] + wo1[6:8])
                jobs += [(('wo2', j), j_wo2(j)) for j in range(nD)]
                return jobs

            def j_next_xn():
                nxt = jnp.minimum(t + 1, n_pairs - 1) * PAIR
                store_xn(x_v[pl.ds(pl.multiple_of(nxt, PAIR), PAIR), :])

            return step_jobs(True), step_jobs(False), j_next_xn

        def b_jobs(c):
            r0 = pl.multiple_of(c * PAIR, PAIR)
            st = {}

            def j_pre_next():
                mlp_pre(jnp.minimum(c + 1, n_pairs - 1))

            def j_w1(j):
                def run():
                    tok = jax.lax.broadcasted_iota(jnp.int32, (PAIR, 128), 0) + (r0 + HALO)
                    a = _gelu(_dot(_as_bf(z_buf[...]), wtile(w1_t, j)))
                    a1_buf[pl.ds(2 * HALO, PAIR), pl.ds(j * 128, 128)] = jnp.where(tok < S, a, 0.0)
                return run

            def j_shift():
                cq = D // 4
                st['g'] = jnp.concatenate([
                    a1_buf[pl.ds(HALO - 1, PAIR), pl.ds(0 * cq, cq)],
                    a1_buf[pl.ds(HALO + 1, PAIR), pl.ds(1 * cq, cq)],
                    a1_buf[pl.ds(HALO - 2, PAIR), pl.ds(2 * cq, cq)],
                    a1_buf[pl.ds(HALO + 2, PAIR), pl.ds(3 * cq, cq)]], axis=1).astype(BF)

            def j_w2(j):
                def run():
                    st['x1', j] = y_buf[:, pl.ds(j * 128, 128)] + _dot(st['g'], wtile(w2_t, j))
                return run

            def j_ln3():
                x1 = jnp.concatenate([st['x1', j] for j in range(nD)], axis=1)
                st['z1'] = _ln(x1).astype(BF)

            def j_w3(j):
                def run():
                    st['a3', j] = _gelu(_dot(st['z1'], wtile(w3_t, j))).astype(BF)
                return run

            def j_cat():
                st['a3'] = jnp.concatenate([st.pop(('a3', j)) for j in range(nF)], axis=1)

            def j_w4(j):
                def run():
                    cs = pl.ds(j * 128, 128)
                    hh = h_buf[pl.ds(pl.multiple_of(r0 + HALO, 8), PAIR), cs]
                    out_v[pl.ds(r0, PAIR), cs] = (
                        hh + (st['x1', j] + _dot(st['a3'], wtile(w4_t, j)))).astype(out_v.dtype)
                return run

            return dict(pre_next=j_pre_next, w1=[j_w1(j) for j in range(nD)], shift=j_shift,
                        w2=[j_w2(j) for j in range(nD)], ln3=j_ln3,
                        w3=[j_w3(j) for j in range(nF)], cat=j_cat,
                        w4=[j_w4(j) for j in range(nD)])

        def run_jobs(jobs):
            for j in jobs:
                j()

        last_s = ('s', n_slots - 2)

        def fused_jobs(t):
            ej, oj, j_next_xn = a_jobs(t)
            b = b_jobs(t - LAG)
            w3, w4 = b['w3'], b['w4']
            fe, fo = {}, {}

            def put(d, label, *jobs):
                d.setdefault(label, []).extend(jobs)
            for i in range(nD):
                put(fe, ('qkv', CFG['w1slot'] + i // 2, i % 2), b['w1'][i])
                put(fe, ('qkv', 8 + i // 2, i % 2), b['w2'][i])
            put(fe, ('qkv', 6, 0), b['shift'])
            put(fe, ('qkv', 12, 0), b['ln3'])
            put(fe if CFG['prepos'][0] == 'e' else fo, CFG['prepos'][1], b['pre_next'])
            if CFG['etail'] == 0:
                put(fe, ('qkv', 15, 0), w3[0])
                put(fe, 'end', *w3[1:4])
            elif CFG['etail'] == 1:
                put(fe, ('wo1', 1), w3[0])
                put(fe, ('wo1', 4), w3[1])
                put(fe, 'end', *w3[2:4])
            elif CFG['etail'] == 2:
                put(fe, ('wo1', 1), w3[0])
                put(fe, ('wo1', 4), w3[1])
                put(fe, ('wo1', 7), w3[2])
                put(fe, 'end', w3[3])
            if CFG['fine']:
                for k in range(4, nF):
                    put(fo, ('qkv', 1 + (k - 4) // 2, (k - 4) % 2), w3[k])
            else:
                for k in range(4, nF):
                    put(fo, ('qkv', 1 + (k - 4) // 2, 0), w3[k])
            put(fo, ('qkv', 13, 0), b['cat'])
            for lab, job in zip(CFG['w4pos'], w4):
                put(fo, lab, job)
            put(fo, last_s, j_next_xn)
            put(fo, 'end' if CFG['w4_last'] else ('wo2', 0), *w4[len(CFG['w4pos']):])
            return _interleave(ej, fe) + _interleave(oj, fo)

        def a_only(t, carry):
            ej, oj, j_next_xn = a_jobs(t)

            def j_wo_wait():
                with jax.named_scope("sc_wo_finish"):
                    pl.when(t == 0)(wo_finish)
            run_jobs(_interleave(ej, {last_s: [j_wo_wait]}) + _interleave(oj, {last_s: [j_next_xn]}))
            return carry

        def fused(t, carry):
            with jax.named_scope("sc_xwait"):
                @pl.when(t == X0 // PAIR - 1)
                def _():
                    x_rest_copy().wait()

                @pl.when(t > LAG)
                def _():
                    out_copy(t - LAG - 1).start()
            with jax.named_scope("sc_fused_body"):
                run_jobs(fused_jobs(t))
            return carry

        def b_only(c, carry):
            out_copy(c - 1).start()
            b = b_jobs(c)
            run_jobs(b['w1'] + [b['shift']] + b['w2'] + [b['ln3'], b['pre_next']] + b['w3'] + [b['cat']] + b['w4'])
            return carry

        def b_tail():
            jax.lax.fori_loop(n_pairs - LAG, n_pairs, b_only, 0)
            out_copy(n_pairs - 1).start()

        with jax.named_scope("sc_prologue"):
            prologue()
        with jax.named_scope("sc_a_only"):
            jax.lax.fori_loop(0, LAG, a_only, 0)
        with jax.named_scope("sc_mlp_prologue"):
            mlp_prologue()
        with jax.named_scope("sc_fused"):
            jax.lax.fori_loop(LAG, n_pairs, fused, 0)
        with jax.named_scope("sc_b_tail"):
            b_tail()
        with jax.named_scope("sc_out_wait"):
            pltpu.make_async_copy(out_v, out_hbm, sems.at[OUT_SEM]).wait()

    return kernel


@functools.partial(jax.jit, static_argnames=("A_seg_len",))
def pallas_sequential_preLN__memory_aug_recurrent_mem_tr__mixer_s_mlp__prompt_kernel(
    A_x, A_mem0, A_Wq, A_Wk, A_Wv, A_Wo, A_seg_len, B_x, B_w1, B_w2, B_w3, B_w4,
):
    _, S, D = A_x.shape
    H, E = A_Wq.shape[1], A_Wq.shape[2]
    F = B_w3.shape[1]
    assert A_seg_len == SEG and A_mem0.shape[1] == MEM and S % PAIR == 0
    nD, nF = D // 128, F // 128

    x = A_x.reshape(S, D)
    mem0 = A_mem0.reshape(MEM, D)
    wo = A_Wo.reshape(H * E, D)

    any_spec = pl.BlockSpec(memory_space=pl.ANY)
    out = pl.pallas_call(
        _make_kernel(S, D, H, E, F),
        in_specs=[any_spec] * 10,
        out_specs=any_spec,
        out_shape=jax.ShapeDtypeStruct((S, D), A_x.dtype),
        scratch_shapes=[
            pltpu.VMEM((3, D, H, E), BF),
            pltpu.VMEM((H, D // 2, E), U32),
            pltpu.VMEM((H, D // 2, E), U32),
            pltpu.VMEM((H, D // 2, E), U32),
            pltpu.VMEM((H * E, D), BF),
            pltpu.VMEM((nD, H * E // 2, 128), U32),
            pltpu.VMEM((nD, D, 128) if CFG['bcol'] else (D, D), BF),
            pltpu.VMEM((nD, D, 128) if CFG['bcol'] else (D, D), BF),
            pltpu.VMEM((nF, D, 128) if CFG['bcol'] else (D, F), BF),
            pltpu.VMEM((nD, F, 128) if CFG['bcol'] else (F, D), BF),
            pltpu.VMEM((S, D), BF),
            pltpu.VMEM((S, D), BF),
            pltpu.VMEM((MEM, D), BF),
            pltpu.VMEM((24, D), U32),
            pltpu.VMEM((16, D), U32),
            pltpu.VMEM((3, 8, H * E), F32),
            pltpu.VMEM((40, H * E), U32),
            pltpu.VMEM((48, D), F32),
            pltpu.VMEM((S + 2 * HALO, D), F32),
            pltpu.VMEM((PAIR + 2 * HALO, D), F32),
            pltpu.VMEM((PAIR, D), F32),
            pltpu.VMEM((PAIR // 2, D), U32),
            pltpu.SemaphoreType.DMA((3 * 4 + nD + 6,)),
        ],
        compiler_params=pltpu.CompilerParams(
            vmem_limit_bytes=120 * 1024 * 1024,
            disable_bounds_checks=CFG['nobc'],
        ),
    )(x, mem0, A_Wq, A_Wk, A_Wv, wo, B_w1, B_w2, B_w3, B_w4)
    return out.reshape(1, S, D)
```

```python
import functools

import jax
import jax.numpy as jnp
from jax.experimental import pallas as pl
from jax.experimental.pallas import tpu as pltpu

BF = jnp.bfloat16
F32 = jnp.float32
U32 = jnp.uint32

SEG = 32
MEM = 8
PAIR = 2 * SEG
LAG = 3
HALO = 8
G = 2
TAIL_HEADS = 6
X0 = 4 * PAIR
NCH = 4
LN_EPS = 1e-5
LOG2E = 1.4426950408889634


def _ln(x):
    m = jnp.mean(x, axis=-1, keepdims=True)
    xc = x - m
    v = jnp.mean(xc * xc, axis=-1, keepdims=True)
    return xc * jax.lax.rsqrt(v + LN_EPS)


_dot = functools.partial(jnp.dot, preferred_element_type=F32)


def _gelu(x):
    return jax.nn.gelu(x, approximate=True)


def _as_bf(x_u32):
    return pltpu.bitcast(x_u32, BF)


def _as_u32(x_bf):
    return pltpu.bitcast(x_bf, U32)


def _interleave(main, fill):
    fill = dict(fill)
    out = []
    for label, job in main:
        out.extend(fill.pop(label, []))
        out.append(job)
    out.extend(fill.pop('end', []))
    assert not fill, fill
    return out


def _run(jobs):
    for job in jobs:
        job()


def _make_kernel(S, D, H, E, F):
    n_pairs = S // PAIR
    nD = D // 128
    nF = F // 128
    scale = float(E) ** -0.5
    L = MEM + SEG
    n_slots = H // G
    K1 = (H - TAIL_HEADS) * E
    CH = D // NCH
    WO_CH = H * E // nD
    assert n_pairs >= 8 and X0 // PAIR - 1 >= LAG and G == 2 and n_slots == 16 and nF == 28 and nD == 8
    assert (H - TAIL_HEADS) // G - 1 < n_slots - 2

    WO_SEM = 3 * NCH
    B_SEM, X0_SEM, XM_SEM, X1_SEM, MEM_SEM, OUT_SEM = (WO_SEM + nD + i for i in range(6))

    def kernel(x_hbm, mem0_hbm, wq_hbm, wk_hbm, wv_hbm, wo_hbm, w1_hbm, w2_hbm, w3_hbm, w4_hbm,
               out_hbm,
               raw, wq_t, wk_t, wv_t, wo_raw, wo_t, w1_t, w2_t, w3_t, w4_t,
               x_v, out_v, mem0_v, lb_e, lb_o, sv, ob, wacc, h_buf, a1_buf, y_buf, z_buf, sems):

        def rows_copy(src, dst, start, size, sem):
            return pltpu.make_async_copy(src.at[pl.ds(start, size)], dst.at[pl.ds(start, size)], sems.at[sem])

        def raw_copy(i, c):
            src = (wq_hbm, wk_hbm, wv_hbm)[i]
            return rows_copy(src, raw.at[i], c * CH, CH, i * NCH + c)

        def wo_copy(j):
            return rows_copy(wo_hbm, wo_raw, j * WO_CH, WO_CH, WO_SEM + j)

        def mlp_weight_copies():
            return [pltpu.make_async_copy(src.at[:, pl.ds(j * 128, 128)], dst.at[j], sems.at[B_SEM])
                    for src, dst, n in ((w1_hbm, w1_t, nD), (w2_hbm, w2_t, nD),
                                        (w3_hbm, w3_t, nF), (w4_hbm, w4_t, nD))
                    for j in range(n)]

        def x_head_copy():
            return rows_copy(x_hbm, x_v, 0, PAIR, X0_SEM)

        def x_mid_copy():
            return rows_copy(x_hbm, x_v, PAIR, X0 - PAIR, XM_SEM)

        def x_rest_copy():
            return rows_copy(x_hbm, x_v, X0, S - X0, X1_SEM)

        def mem_copy():
            return pltpu.make_async_copy(mem0_hbm, mem0_v, sems.at[MEM_SEM])

        def out_copy(c):
            return rows_copy(out_v, out_hbm, pl.multiple_of(c * PAIR, PAIR), PAIR, OUT_SEM)

        def relayout(i, c, dst):
            def body(b, carry):
                blk = raw[i, pl.ds(pl.multiple_of(b * 16, 16), 16), :, :]
                dst[:, pl.ds(pl.multiple_of(b * 8, 8), 8), :] = _as_u32(jnp.swapaxes(blk, 0, 1))
                return carry
            jax.lax.fori_loop(c * (CH // 16), (c + 1) * (CH // 16), body, 0)

        def wo_finish():
            for j in range(nD):
                wo_copy(j).wait()

                def body(b, carry):
                    r = j * WO_CH + b * 64
                    blk = wo_raw[pl.ds(pl.multiple_of(r, 64), 64), :]
                    for n in range(nD):
                        wo_t[n, pl.ds(pl.multiple_of(r // 2, 32), 32), :] = _as_u32(blk[:, n * 128:(n + 1) * 128])
                    return carry
                jax.lax.fori_loop(0, WO_CH // 64, body, 0)
            x_mid_copy().wait()

        def store_xn(x_bf):
            xn = _ln(x_bf.astype(F32))
            lb_e[pl.ds(0, 4), :] = _as_u32(xn[32:40].astype(BF))
            lb_e[pl.ds(4, 4), :] = _as_u32(xn[0:8].astype(BF))
            lb_e[pl.ds(8, 8), :] = _as_u32(xn[8:24].astype(BF))
            lb_e[pl.ds(16, 4), :] = _as_u32(xn[24:32].astype(BF))
            lb_o[pl.ds(0, 8), :] = _as_u32(xn[40:56].astype(BF))
            lb_o[pl.ds(8, 4), :] = _as_u32(xn[56:64].astype(BF))

        def prologue():
            x_head_copy().start()
            mem_copy().start()
            for i in range(3):
                for c in range(NCH):
                    raw_copy(i, c).start()
            for j in range(nD):
                wo_copy(j).start()
            x_mid_copy().start()
            h_buf[pl.ds(0, HALO), :] = jnp.zeros((HALO, D), F32)
            h_buf[pl.ds(HALO + S, HALO), :] = jnp.zeros((HALO, D), F32)
            x_head_copy().wait()
            mem_copy().wait()
            lb_e[pl.ds(20, 4), :] = _as_u32(mem0_v[...])
            store_xn(x_v[pl.ds(0, PAIR), :])
            for i, dst in enumerate((wq_t, wk_t, wv_t)):
                for c in range(NCH):
                    raw_copy(i, c).wait()
                    relayout(i, c, dst)
            for c in mlp_weight_copies():
                c.start()
            x_rest_copy().start()

        def mlp_pre(c):
            a1_buf[pl.ds(0, 2 * HALO), :] = a1_buf[pl.ds(PAIR, 2 * HALO), :]
            y = _ln(h_buf[pl.ds(pl.multiple_of(c * PAIR + HALO, 8), PAIR + HALO), :])
            y_buf[...] = y[0:PAIR]
            z_buf[...] = _as_u32(_ln(y[HALO:]).astype(BF))

        def mlp_prologue():
            for c in mlp_weight_copies():
                c.wait()
            z = _ln(_ln(h_buf[pl.ds(0, 2 * HALO), :])).astype(BF)
            tok = jax.lax.broadcasted_iota(jnp.int32, (2 * HALO, 128), 0) - HALO
            for j in range(nD):
                a1_buf[pl.ds(PAIR, 2 * HALO), pl.ds(j * 128, 128)] = jnp.where(
                    tok >= 0, _gelu(_dot(z, w1_t[j])), 0.0)
            mlp_pre(0)

        def attention_jobs(t):
            row = jax.lax.broadcasted_iota(jnp.int32, (G * L, G * L), 0)
            col = jax.lax.broadcasted_iota(jnp.int32, (G * L, G * L), 1)
            mask = None
            for i in range(G):
                rl, cl = row - i * L, col - i * L
                blk = ((rl >= 0) & (rl < L) & (cl >= 0) & (cl < L)) & ((cl <= rl) | (cl >= SEG))
                mask = blk if mask is None else (mask | blk)
            x0 = t * PAIR
            h0 = x0 + HALO

            def step_jobs(even):
                lb = lb_e if even else lb_o
                st = {}

                def j_qkv(g, i):
                    def run():
                        h = g * G + i
                        lhs = _as_bf(lb[...])
                        cs = pl.ds(h * E, E)
                        r = [_dot(lhs, _as_bf(w[h])) for w in (wq_t, wk_t, wv_t)]
                        parts = st.setdefault(('parts', g), [[], [], []])
                        for n in range(3):
                            if even:
                                sv[n, :, cs] = r[n][0:8]
                                parts[n].append(r[n][8:48])
                            else:
                                parts[n] += [sv[n, :, cs], r[n]]
                        if i == G - 1:
                            st['qkv', g] = [jnp.concatenate(a, axis=0).astype(BF)
                                            for a in st.pop(('parts', g))]
                    return run

                def j_scores(g):
                    def run():
                        q, k, v = st.pop(('qkv', g))
                        s = jax.lax.dot_general(q, k, (((1,), (1,)), ((), ())),
                                                preferred_element_type=F32)
                        s = jnp.where(mask, s, -1000000000.0 / scale)
                        m = jnp.max(s, axis=-1, keepdims=True)
                        p = jnp.exp2((s - m) * (scale * LOG2E))
                        l = jnp.sum(p, axis=-1, keepdims=True)
                        r0 = pl.reciprocal(l, approx=True)
                        p = p * (r0 * (2.0 - l * r0))
                        st['p', g] = (p.astype(BF), v)
                    return run

                def j_pv(g):
                    def run():
                        p, v = st.pop(('p', g))
                        o2 = _dot(p, v)
                        for i, h in enumerate(range(g * G, (g + 1) * G)):
                            o = o2[i * L:(i + 1) * L]
                            cs = pl.ds(h * E, E)
                            if even:
                                ob[pl.ds(16, 4), cs] = _as_u32(o[0:8].astype(BF))
                                ob[pl.ds(0, 16), cs] = _as_u32(o[8:40].astype(BF))
                            else:
                                ob[pl.ds(20, 4), cs] = _as_u32(o[0:8].astype(BF))
                                ob[pl.ds(24, 16), cs] = _as_u32(o[8:40].astype(BF))
                    return run

                rows = pl.ds(0, 16) if even else pl.ds(16, 24)
                nrows = 32 if even else 48

                def j_wo1(j):
                    def run():
                        lhs = _as_bf(ob[rows, pl.ds(0, K1)])
                        wacc[pl.ds(0, nrows), pl.ds(j * 128, 128)] = _dot(
                            lhs, _as_bf(wo_t[j, pl.ds(0, K1 // 2), :]))
                    return run

                def j_wo2(j):
                    def run():
                        lhs = _as_bf(ob[rows, pl.ds(K1, H * E - K1)])
                        r = wacc[pl.ds(0, nrows), pl.ds(j * 128, 128)] + _dot(
                            lhs, _as_bf(wo_t[j, pl.ds(K1 // 2, (H * E - K1) // 2), :]))
                        cs = pl.ds(j * 128, 128)
                        xs = x_v[pl.ds(pl.multiple_of(x0, PAIR), PAIR), cs].astype(F32)
                        if even:
                            lb_o[pl.ds(12, 4), cs] = _as_u32(r[24:32].astype(BF))
                            h_buf[pl.ds(pl.multiple_of(h0 + 8, 8), 24), cs] = xs[8:32] + r[0:24]
                        else:
                            lb_e[pl.ds(20, 4), cs] = _as_u32(r[40:48].astype(BF))
                            h_buf[pl.ds(pl.multiple_of(h0, 8), 8), cs] = xs[0:8] + r[0:8]
                            h_buf[pl.ds(pl.multiple_of(h0 + 32, 8), 32), cs] = xs[32:64] + r[8:40]
                    return run

                last = n_slots - 1
                jobs = []
                for g in range(n_slots):
                    for i in range(G):
                        jobs.append((('qkv', g, i), j_qkv(g, i)))
                    if g >= 1:
                        jobs.append((('s', g - 1), j_scores(g - 1)))
                    if g >= 2:
                        jobs.append((('pv', g - 2), j_pv(g - 2)))
                wo1 = [(('wo1', j), j_wo1(j)) for j in range(nD)]
                jobs += (wo1[0:3] + [(('s', last), j_scores(last)), (('pv', last - 1), j_pv(last - 1))]
                         + wo1[3:6] + [(('pv', last), j_pv(last))] + wo1[6:8])
                jobs += [(('wo2', j), j_wo2(j)) for j in range(nD)]
                return jobs

            def j_next_xn():
                nxt = jnp.minimum(t + 1, n_pairs - 1) * PAIR
                store_xn(x_v[pl.ds(pl.multiple_of(nxt, PAIR), PAIR), :])

            return step_jobs(True), step_jobs(False), j_next_xn

        after_qkv = ('s', n_slots - 2)

        def mlp_jobs(c):
            r0 = pl.multiple_of(c * PAIR, PAIR)
            st = {}

            def j_pre_next():
                mlp_pre(jnp.minimum(c + 1, n_pairs - 1))

            def j_w1(j):
                def run():
                    tok = jax.lax.broadcasted_iota(jnp.int32, (PAIR, 128), 0) + (r0 + HALO)
                    a = _gelu(_dot(_as_bf(z_buf[...]), w1_t[j]))
                    a1_buf[pl.ds(2 * HALO, PAIR), pl.ds(j * 128, 128)] = jnp.where(tok < S, a, 0.0)
                return run

            def j_shift():
                cq = D // 4
                st['g'] = jnp.concatenate([
                    a1_buf[pl.ds(HALO - 1, PAIR), pl.ds(0 * cq, cq)],
                    a1_buf[pl.ds(HALO + 1, PAIR), pl.ds(1 * cq, cq)],
                    a1_buf[pl.ds(HALO - 2, PAIR), pl.ds(2 * cq, cq)],
                    a1_buf[pl.ds(HALO + 2, PAIR), pl.ds(3 * cq, cq)]], axis=1).astype(BF)

            def j_w2(j):
                def run():
                    st['x1', j] = y_buf[:, pl.ds(j * 128, 128)] + _dot(st['g'], w2_t[j])
                return run

            def j_ln3():
                x1 = jnp.concatenate([st['x1', j] for j in range(nD)], axis=1)
                st['z1'] = _ln(x1).astype(BF)

            def j_w3(j):
                def run():
                    st['a3', j] = _gelu(_dot(st['z1'], w3_t[j])).astype(BF)
                return run

            def j_cat():
                st['a3'] = jnp.concatenate([st.pop(('a3', j)) for j in range(nF)], axis=1)

            def j_w4(j):
                def run():
                    cs = pl.ds(j * 128, 128)
                    hh = h_buf[pl.ds(pl.multiple_of(r0 + HALO, 8), PAIR), cs]
                    out_v[pl.ds(r0, PAIR), cs] = (
                        hh + (st['x1', j] + _dot(st['a3'], w4_t[j]))).astype(out_v.dtype)
                return run

            return dict(pre_next=j_pre_next, w1=[j_w1(j) for j in range(nD)], shift=j_shift,
                        w2=[j_w2(j) for j in range(nD)], ln3=j_ln3,
                        w3=[j_w3(j) for j in range(nF)], cat=j_cat,
                        w4=[j_w4(j) for j in range(nD)])

        def attention_only(t, carry):
            ej, oj, j_next_xn = attention_jobs(t)

            def j_wo_wait():
                pl.when(t == 0)(wo_finish)
            _run(_interleave(ej, {after_qkv: [j_wo_wait]}) + _interleave(oj, {after_qkv: [j_next_xn]}))
            return carry

        def fused(t, carry):
            @pl.when(t == X0 // PAIR - 1)
            def _():
                x_rest_copy().wait()

            @pl.when(t > LAG)
            def _():
                out_copy(t - LAG - 1).start()

            ej, oj, j_next_xn = attention_jobs(t)
            b = mlp_jobs(t - LAG)
            w3, w4 = b['w3'], b['w4']
            fe, fo = {}, {}

            def put(d, label, *jobs):
                d.setdefault(label, []).extend(jobs)
            for i in range(nD):
                put(fe, ('qkv', 2 + i // 2, i % 2), b['w1'][i])
                put(fe, ('qkv', 8 + i // 2, i % 2), b['w2'][i])
            put(fe, ('qkv', 6, 0), b['shift'])
            put(fe, ('qkv', 12, 0), b['ln3'])
            put(fe, ('qkv', 15, 0), w3[0])
            put(fe, 'end', *w3[1:4])
            put(fo, ('qkv', 0, 1), b['pre_next'])
            for k in range(4, nF):
                put(fo, ('qkv', 1 + (k - 4) // 2, (k - 4) % 2), w3[k])
            put(fo, ('qkv', 13, 0), b['cat'])
            put(fo, ('qkv', 14, 0), w4[0])
            put(fo, ('qkv', 15, 0), w4[1])
            put(fo, after_qkv, j_next_xn)
            put(fo, ('s', n_slots - 1), w4[2])
            put(fo, 'end', *w4[3:])
            _run(_interleave(ej, fe) + _interleave(oj, fo))
            return carry

        def mlp_only(c, carry):
            out_copy(c - 1).start()
            b = mlp_jobs(c)
            _run(b['w1'] + [b['shift']] + b['w2'] + [b['ln3'], b['pre_next']] + b['w3'] + [b['cat']] + b['w4'])
            return carry

        prologue()
        jax.lax.fori_loop(0, LAG, attention_only, 0)
        mlp_prologue()
        jax.lax.fori_loop(LAG, n_pairs, fused, 0)
        jax.lax.fori_loop(n_pairs - LAG, n_pairs, mlp_only, 0)
        out_copy(n_pairs - 1).start()
        pltpu.make_async_copy(out_v, out_hbm, sems.at[OUT_SEM]).wait()

    return kernel, WO_SEM + nD + 6


@functools.partial(jax.jit, static_argnames=("A_seg_len",))
def pallas_sequential_preLN__memory_aug_recurrent_mem_tr__mixer_s_mlp__prompt_kernel(
    A_x, A_mem0, A_Wq, A_Wk, A_Wv, A_Wo, A_seg_len, B_x, B_w1, B_w2, B_w3, B_w4,
):
    _, S, D = A_x.shape
    H, E = A_Wq.shape[1], A_Wq.shape[2]
    F = B_w3.shape[1]
    assert A_seg_len == SEG and A_mem0.shape[1] == MEM and S % PAIR == 0
    nD, nF = D // 128, F // 128

    x = A_x.reshape(S, D)
    mem0 = A_mem0.reshape(MEM, D)
    wo = A_Wo.reshape(H * E, D)

    kernel, n_sems = _make_kernel(S, D, H, E, F)
    any_spec = pl.BlockSpec(memory_space=pl.ANY)
    out = pl.pallas_call(
        kernel,
        in_specs=[any_spec] * 10,
        out_specs=any_spec,
        out_shape=jax.ShapeDtypeStruct((S, D), A_x.dtype),
        scratch_shapes=[
            pltpu.VMEM((3, D, H, E), BF),
            pltpu.VMEM((H, D // 2, E), U32),
            pltpu.VMEM((H, D // 2, E), U32),
            pltpu.VMEM((H, D // 2, E), U32),
            pltpu.VMEM((H * E, D), BF),
            pltpu.VMEM((nD, H * E // 2, 128), U32),
            pltpu.VMEM((nD, D, 128), BF),
            pltpu.VMEM((nD, D, 128), BF),
            pltpu.VMEM((nF, D, 128), BF),
            pltpu.VMEM((nD, F, 128), BF),
            pltpu.VMEM((S, D), BF),
            pltpu.VMEM((S, D), BF),
            pltpu.VMEM((MEM, D), BF),
            pltpu.VMEM((24, D), U32),
            pltpu.VMEM((16, D), U32),
            pltpu.VMEM((3, 8, H * E), F32),
            pltpu.VMEM((40, H * E), U32),
            pltpu.VMEM((48, D), F32),
            pltpu.VMEM((S + 2 * HALO, D), F32),
            pltpu.VMEM((PAIR + 2 * HALO, D), F32),
            pltpu.VMEM((PAIR, D), F32),
            pltpu.VMEM((PAIR // 2, D), U32),
            pltpu.SemaphoreType.DMA((n_sems,)),
        ],
        compiler_params=pltpu.CompilerParams(
            vmem_limit_bytes=120 * 1024 * 1024,
            disable_bounds_checks=True,
        ),
    )(x, mem0, A_Wq, A_Wk, A_Wv, wo, B_w1, B_w2, B_w3, B_w4)
    return out.reshape(1, S, D)
```

```python
import functools

import jax
import jax.numpy as jnp
from jax.experimental import pallas as pl
from jax.experimental.pallas import tpu as pltpu

BF = jnp.bfloat16
F32 = jnp.float32
U32 = jnp.uint32

SEG = 32
MEM = 8
PAIR = 2 * SEG
LAG = 3
HALO = 8
G = 2
TAIL_HEADS = 6
QR = 24
NCH = 4
LN_EPS = 1e-5
LOG2E = 1.4426950408889634


def _ln(x):
    m = jnp.mean(x, axis=-1, keepdims=True)
    xc = x - m
    v = jnp.mean(xc * xc, axis=-1, keepdims=True)
    return xc * jax.lax.rsqrt(v + LN_EPS)


_dot = functools.partial(jnp.dot, preferred_element_type=F32)


def _gelu(x):
    return jax.nn.gelu(x, approximate=True)


def _as_bf(x_u32):
    return pltpu.bitcast(x_u32, BF)


def _as_u32(x_bf):
    return pltpu.bitcast(x_bf, U32)


def _interleave(main, fill):
    fill = dict(fill)
    out = []
    for label, job in main:
        out.extend(fill.pop(label, []))
        out.append(job)
    out.extend(fill.pop('end', []))
    assert not fill, fill
    return out


def _run(jobs):
    for job in jobs:
        job()


def _make_kernel(S, D, H, E, F):
    n_pairs = S // PAIR
    nD = D // 128
    nF = F // 128
    scale = float(E) ** -0.5
    L = MEM + SEG
    n_slots = H // G
    K1 = (H - TAIL_HEADS) * E
    CH = D // NCH
    WO_CH = H * E // nD
    X0 = S - 2 * QR * n_pairs
    assert X0 % PAIR == 0 and X0 // PAIR - 1 >= LAG and X0 < S
    assert G == 2 and n_slots == 16 and nF == 28 and nD == 8 and H == 2 * NCH * 4
    assert (H - TAIL_HEADS) // G - 1 < n_slots - 2

    WO_SEM = 3 * NCH
    B_SEM, X0_SEM, XM_SEM, X1_SEM, MEM_SEM, OUT_SEM = (WO_SEM + nD + i for i in range(6))
    XA = X0 + 2 * QR
    XB = X0 + 2 * QR * (LAG + 1)

    def kernel(x_hbm, mem0_hbm, wq_hbm, wk_hbm, wv_hbm, wo_hbm, w1_hbm, w2_hbm, w3_hbm, w4_hbm,
               out_hbm,
               raw, w_t, wo_raw, wo_t, w1_t, w2_t, w3_t, w4_t,
               x_v, out_v, mem0_v, xn0, q_buf, lq_e, lq_o, lb_e, lb_o, sv, ob, wacc,
               h_buf, a1_buf, y_buf, z_buf, sems):

        def rows_copy(src, dst, start, size, sem):
            return pltpu.make_async_copy(src.at[pl.ds(start, size)], dst.at[pl.ds(start, size)], sems.at[sem])

        def raw_copy(i, c):
            src = (wq_hbm, wk_hbm, wv_hbm)[i]
            return rows_copy(src, raw.at[i], c * CH, CH, i * NCH + c)

        def wo_copy(j):
            return rows_copy(wo_hbm, wo_raw, j * WO_CH, WO_CH, WO_SEM + j)

        def mlp_weight_copies():
            return [pltpu.make_async_copy(src.at[:, pl.ds(j * 128, 128)], dst.at[j], sems.at[B_SEM])
                    for src, dst, n in ((w1_hbm, w1_t, nD), (w2_hbm, w2_t, nD),
                                        (w3_hbm, w3_t, nF), (w4_hbm, w4_t, nD))
                    for j in range(n)]

        def x_head_copy():
            return rows_copy(x_hbm, x_v, 0, XA, X0_SEM)

        def x_mid_copy():
            return rows_copy(x_hbm, x_v, XA, XB - XA, XM_SEM)

        def x_rest_copy():
            return rows_copy(x_hbm, x_v, XB, S - XB, X1_SEM)

        def mem_copy():
            return pltpu.make_async_copy(mem0_hbm, mem0_v, sems.at[MEM_SEM])

        def out_copy(c):
            return rows_copy(out_v, out_hbm, pl.multiple_of(c * PAIR, PAIR), PAIR, OUT_SEM)

        def relayout_block(i, b):
            blk = raw[i, pl.ds(pl.multiple_of(b * 16, 16), 16), :, :]
            w_t[i, :, pl.ds(pl.multiple_of(b * 8, 8), 8), :] = _as_u32(jnp.swapaxes(blk, 0, 1))

        def wo_finish():
            for j in range(nD):
                wo_copy(j).wait()

                def body(b, carry):
                    r = j * WO_CH + b * 64
                    blk = wo_raw[pl.ds(pl.multiple_of(r, 64), 64), :]
                    for n in range(nD):
                        wo_t[n, pl.ds(pl.multiple_of(r // 2, 32), 32), :] = _as_u32(blk[:, n * 128:(n + 1) * 128])
                    return carry
                jax.lax.fori_loop(0, WO_CH // 64, body, 0)
            x_mid_copy().wait()

        def store_xn(t):
            xn = _ln(x_v[pl.ds(pl.multiple_of(t * PAIR, PAIR), PAIR), :].astype(F32))
            lb_e[pl.ds(0, 4), :] = _as_u32(xn[32:40].astype(BF))
            lb_e[pl.ds(4, 4), :] = _as_u32(xn[0:8].astype(BF))
            lb_e[pl.ds(8, 8), :] = _as_u32(xn[8:24].astype(BF))
            lb_e[pl.ds(16, 4), :] = _as_u32(xn[24:32].astype(BF))
            lb_o[pl.ds(0, 8), :] = _as_u32(xn[40:56].astype(BF))
            lb_o[pl.ds(8, 4), :] = _as_u32(xn[56:64].astype(BF))
            xq = _ln(x_v[pl.ds(pl.multiple_of(X0 + t * 2 * QR, 16), 2 * QR), :].astype(F32))
            lq_e[pl.ds(0, 8), :] = _as_u32(xq[0:16].astype(BF))
            lq_e[pl.ds(8, 4), :] = _as_u32(xq[16:24].astype(BF))
            for n in range(3):
                lq_o[pl.ds(4 * n, 4), :] = _as_u32(xq[24 + 8 * n:32 + 8 * n].astype(BF))

        def prologue():
            x_head_copy().start()
            mem_copy().start()
            for i in range(3):
                for c in range(NCH):
                    raw_copy(i, c).start()
            for j in range(nD):
                wo_copy(j).start()
            x_mid_copy().start()
            h_buf[pl.ds(0, HALO), :] = jnp.zeros((HALO, D), F32)
            h_buf[pl.ds(HALO + S, HALO), :] = jnp.zeros((HALO, D), F32)
            x_head_copy().wait()
            mem_copy().wait()
            lb_e[pl.ds(20, 4), :] = _as_u32(mem0_v[...])
            lq_e[pl.ds(12, 4), :] = _as_u32(mem0_v[...])

            def ln_body(b, carry):
                rows = x_v[pl.ds(pl.multiple_of(b * 64, 64), 64), :].astype(F32)
                xn0[pl.ds(pl.multiple_of(b * 32, 32), 32), :] = _as_u32(_ln(rows).astype(BF))
                return carry
            jax.lax.fori_loop(0, X0 // 64, ln_body, 0)

            for c in range(NCH):
                raw_copy(0, c).wait()

                def q_body(b, carry):
                    relayout_block(0, b)
                    return carry
                jax.lax.fori_loop(c * (CH // 16), (c + 1) * (CH // 16), q_body, 0)

            per_it = 2 * (D // 16) // H
            it_per_chunk = H // (2 * NCH)

            def kv_body(h, carry):
                i = 1 + h // (H // 2)

                @pl.when(h % it_per_chunk == 0)
                def _():
                    n = h // it_per_chunk
                    dst = raw.at[i, pl.ds((n % NCH) * CH, CH)]
                    pltpu.make_async_copy(dst, dst, sems.at[NCH + n]).wait()
                q = _dot(_as_bf(xn0[...]), _as_bf(w_t[0, h]))
                q_buf[pl.ds(0, X0 // 2), pl.ds(pl.multiple_of(h * E, E), E)] = _as_u32(q.astype(BF))
                for n in range(per_it):
                    relayout_block(i, (h % (H // 2)) * per_it + n)
                return carry
            jax.lax.fori_loop(0, H, kv_body, 0)

            for c in mlp_weight_copies():
                c.start()
            x_rest_copy().start()

        def mlp_pre(c):
            a1_buf[pl.ds(0, 2 * HALO), :] = a1_buf[pl.ds(PAIR, 2 * HALO), :]
            y = _ln(h_buf[pl.ds(pl.multiple_of(c * PAIR + HALO, 8), PAIR + HALO), :])
            y_buf[...] = y[0:PAIR]
            z_buf[...] = _as_u32(_ln(y[HALO:]).astype(BF))

        def mlp_prologue():
            for c in mlp_weight_copies():
                c.wait()
            z = _ln(_ln(h_buf[pl.ds(0, 2 * HALO), :])).astype(BF)
            tok = jax.lax.broadcasted_iota(jnp.int32, (2 * HALO, 128), 0) - HALO
            for j in range(nD):
                a1_buf[pl.ds(PAIR, 2 * HALO), pl.ds(j * 128, 128)] = jnp.where(
                    tok >= 0, _gelu(_dot(z, w1_t[j])), 0.0)
            mlp_pre(0)

        def attention_jobs(t):
            row = jax.lax.broadcasted_iota(jnp.int32, (G * L, G * L), 0)
            col = jax.lax.broadcasted_iota(jnp.int32, (G * L, G * L), 1)

            def head_of(r):
                return jnp.where(r < G * SEG, r // SEG, (r - G * SEG) // MEM)
            mask = (head_of(row) == head_of(col)) & ((col >= G * SEG) | (row >= G * SEG) | (col <= row))
            x0 = t * PAIR
            h0 = x0 + HALO

            def step_jobs(even):
                lb = lb_e if even else lb_o
                st = {}

                lq = lq_e if even else lq_o
                q_new = pl.multiple_of(X0 // 2 + t * QR, 8)
                q_use = t * SEG + (0 if even else SEG // 2)

                def j_qkv(g, i):
                    def run():
                        h = g * G + i
                        cs = pl.ds(h * E, E)
                        q = _dot(_as_bf(lq[...]), _as_bf(w_t[0, h]))
                        if even:
                            q_buf[pl.ds(q_new, 8), cs] = _as_u32(q[0:16].astype(BF))
                            sv[2, :, cs] = q[16:24]
                        else:
                            q_buf[pl.ds(q_new + 8, 16), cs] = _as_u32(
                                jnp.concatenate([sv[2, :, cs], q[0:QR]], axis=0).astype(BF))
                        lhs = _as_bf(lb[...])
                        kv = [_dot(lhs, _as_bf(w_t[n, h])) for n in (1, 2)]
                        parts = st.setdefault(('parts', g), dict(qx=[], qm=[], x=[[], []], m=[[], []]))
                        parts['qx'].append(_as_bf(q_buf[pl.ds(pl.multiple_of(q_use, 16), SEG // 2), cs]))
                        parts['qm'].append(q[QR:QR + MEM])
                        for n in range(2):
                            if even:
                                sv[n, :, cs] = kv[n][0:8]
                                parts['x'][n].append(kv[n][8:40])
                                parts['m'][n].append(kv[n][40:48])
                            else:
                                parts['x'][n] += [sv[n, :, cs], kv[n][0:24]]
                                parts['m'][n].append(kv[n][24:32])
                        if i == G - 1:
                            parts = st.pop(('parts', g))
                            q2 = jnp.concatenate(
                                parts['qx'] + [jnp.concatenate(parts['qm'], axis=0).astype(BF)], axis=0)
                            st['qkv', g] = [q2] + [
                                jnp.concatenate(parts['x'][n] + parts['m'][n], axis=0).astype(BF)
                                for n in range(2)]
                    return run

                def j_scores(g):
                    def run():
                        q, k, v = st.pop(('qkv', g))
                        s = jax.lax.dot_general(q, k, (((1,), (1,)), ((), ())),
                                                preferred_element_type=F32)
                        s = jnp.where(mask, s, -1000000000.0 / scale)
                        m = jnp.max(s, axis=-1, keepdims=True)
                        p = jnp.exp2((s - m) * (scale * LOG2E))
                        l = jnp.sum(p, axis=-1, keepdims=True)
                        r0 = pl.reciprocal(l, approx=True)
                        p = p * (r0 * (2.0 - l * r0))
                        st['p', g] = (p.astype(BF), v)
                    return run

                def j_pv(g):
                    def run():
                        p, v = st.pop(('p', g))
                        o2 = _dot(p, v)
                        for i, h in enumerate(range(g * G, (g + 1) * G)):
                            ox = o2[i * SEG:(i + 1) * SEG]
                            om = o2[G * SEG + i * MEM:G * SEG + (i + 1) * MEM]
                            cs = pl.ds(h * E, E)
                            if even:
                                ob[pl.ds(16, 4), cs] = _as_u32(ox[0:8].astype(BF))
                                ob[pl.ds(0, 16), cs] = _as_u32(
                                    jnp.concatenate([ox[8:32], om], axis=0).astype(BF))
                            else:
                                ob[pl.ds(20, 4), cs] = _as_u32(ox[0:8].astype(BF))
                                ob[pl.ds(24, 16), cs] = _as_u32(
                                    jnp.concatenate([ox[8:32], om], axis=0).astype(BF))
                    return run

                rows = pl.ds(0, 16) if even else pl.ds(16, 24)
                nrows = 32 if even else 48

                def j_wo1(j):
                    def run():
                        lhs = _as_bf(ob[rows, pl.ds(0, K1)])
                        wacc[pl.ds(0, nrows), pl.ds(j * 128, 128)] = _dot(
                            lhs, _as_bf(wo_t[j, pl.ds(0, K1 // 2), :]))
                    return run

                def j_wo2(j):
                    def run():
                        lhs = _as_bf(ob[rows, pl.ds(K1, H * E - K1)])
                        r = wacc[pl.ds(0, nrows), pl.ds(j * 128, 128)] + _dot(
                            lhs, _as_bf(wo_t[j, pl.ds(K1 // 2, (H * E - K1) // 2), :]))
                        cs = pl.ds(j * 128, 128)
                        xs = x_v[pl.ds(pl.multiple_of(x0, PAIR), PAIR), cs].astype(F32)
                        if even:
                            mem = _as_u32(r[24:32].astype(BF))
                            lb_o[pl.ds(12, 4), cs] = mem
                            lq_o[pl.ds(12, 4), cs] = mem
                            h_buf[pl.ds(pl.multiple_of(h0 + 8, 8), 24), cs] = xs[8:32] + r[0:24]
                        else:
                            mem = _as_u32(r[40:48].astype(BF))
                            lb_e[pl.ds(20, 4), cs] = mem
                            lq_e[pl.ds(12, 4), cs] = mem
                            h_buf[pl.ds(pl.multiple_of(h0, 8), 8), cs] = xs[0:8] + r[0:8]
                            h_buf[pl.ds(pl.multiple_of(h0 + 32, 8), 32), cs] = xs[32:64] + r[8:40]
                    return run

                last = n_slots - 1
                jobs = []
                for g in range(n_slots):
                    for i in range(G):
                        jobs.append((('qkv', g, i), j_qkv(g, i)))
                    if g >= 1:
                        jobs.append((('s', g - 1), j_scores(g - 1)))
                    if g >= 2:
                        jobs.append((('pv', g - 2), j_pv(g - 2)))
                wo1 = [(('wo1', j), j_wo1(j)) for j in range(nD)]
                jobs += (wo1[0:3] + [(('s', last), j_scores(last)), (('pv', last - 1), j_pv(last - 1))]
                         + wo1[3:6] + [(('pv', last), j_pv(last))] + wo1[6:8])
                jobs += [(('wo2', j), j_wo2(j)) for j in range(nD)]
                return jobs

            def j_next_xn():
                store_xn(jnp.minimum(t + 1, n_pairs - 1))

            return step_jobs(True), step_jobs(False), j_next_xn

        after_qkv = ('s', n_slots - 2)

        def mlp_jobs(c):
            r0 = pl.multiple_of(c * PAIR, PAIR)
            st = {}

            def j_pre_next():
                mlp_pre(jnp.minimum(c + 1, n_pairs - 1))

            def j_w1(j):
                def run():
                    tok = jax.lax.broadcasted_iota(jnp.int32, (PAIR, 128), 0) + (r0 + HALO)
                    a = _gelu(_dot(_as_bf(z_buf[...]), w1_t[j]))
                    a1_buf[pl.ds(2 * HALO, PAIR), pl.ds(j * 128, 128)] = jnp.where(tok < S, a, 0.0)
                return run

            def j_shift():
                cq = D // 4
                st['g'] = jnp.concatenate([
                    a1_buf[pl.ds(HALO - 1, PAIR), pl.ds(0 * cq, cq)],
                    a1_buf[pl.ds(HALO + 1, PAIR), pl.ds(1 * cq, cq)],
                    a1_buf[pl.ds(HALO - 2, PAIR), pl.ds(2 * cq, cq)],
                    a1_buf[pl.ds(HALO + 2, PAIR), pl.ds(3 * cq, cq)]], axis=1).astype(BF)

            def j_w2(j):
                def run():
                    st['x1', j] = y_buf[:, pl.ds(j * 128, 128)] + _dot(st['g'], w2_t[j])
                return run

            def j_ln3():
                x1 = jnp.concatenate([st['x1', j] for j in range(nD)], axis=1)
                st['z1'] = _ln(x1).astype(BF)

            def j_w3(j):
                def run():
                    st['a3', j] = _gelu(_dot(st['z1'], w3_t[j])).astype(BF)
                return run

            def j_cat():
                st['a3'] = jnp.concatenate([st.pop(('a3', j)) for j in range(nF)], axis=1)

            def j_w4(j):
                def run():
                    cs = pl.ds(j * 128, 128)
                    hh = h_buf[pl.ds(pl.multiple_of(r0 + HALO, 8), PAIR), cs]
                    out_v[pl.ds(r0, PAIR), cs] = (
                        hh + (st['x1', j] + _dot(st['a3'], w4_t[j]))).astype(out_v.dtype)
                return run

            return dict(pre_next=j_pre_next, w1=[j_w1(j) for j in range(nD)], shift=j_shift,
                        w2=[j_w2(j) for j in range(nD)], ln3=j_ln3,
                        w3=[j_w3(j) for j in range(nF)], cat=j_cat,
                        w4=[j_w4(j) for j in range(nD)])

        def attention_only(t, carry):
            ej, oj, j_next_xn = attention_jobs(t)

            def j_wo_wait():
                pl.when(t == 0)(wo_finish)
            _run(_interleave(ej, {after_qkv: [j_wo_wait]}) + _interleave(oj, {after_qkv: [j_next_xn]}))
            return carry

        def fused(t, carry):
            @pl.when(t == LAG)
            def _():
                x_rest_copy().wait()

            @pl.when(t > LAG)
            def _():
                out_copy(t - LAG - 1).start()

            ej, oj, j_next_xn = attention_jobs(t)
            b = mlp_jobs(t - LAG)
            w3, w4 = b['w3'], b['w4']
            fe, fo = {}, {}

            def put(d, label, *jobs):
                d.setdefault(label, []).extend(jobs)
            for i in range(nD):
                put(fe, ('qkv', 2 + i // 2, i % 2), b['w1'][i])
                put(fe, ('qkv', 8 + i // 2, i % 2), b['w2'][i])
            put(fe, ('qkv', 6, 0), b['shift'])
            put(fe, ('qkv', 12, 0), b['ln3'])
            put(fe, ('qkv', 15, 0), w3[0])
            put(fe, 'end', *w3[1:4])
            put(fo, ('qkv', 0, 1), b['pre_next'])
            for k in range(4, nF):
                put(fo, ('qkv', 1 + (k - 4) // 2, (k - 4) % 2), w3[k])
            put(fo, ('qkv', 13, 0), b['cat'])
            put(fo, ('qkv', 14, 0), w4[0])
            put(fo, ('qkv', 15, 0), w4[1])
            put(fo, after_qkv, j_next_xn)
            put(fo, ('s', n_slots - 1), w4[2])
            put(fo, 'end', *w4[3:])
            _run(_interleave(ej, fe) + _interleave(oj, fo))
            return carry

        def mlp_only(c, carry):
            out_copy(c - 1).start()
            b = mlp_jobs(c)
            _run(b['w1'] + [b['shift']] + b['w2'] + [b['ln3'], b['pre_next']] + b['w3'] + [b['cat']] + b['w4'])
            return carry

        prologue()
        store_xn(0)
        jax.lax.fori_loop(0, LAG, attention_only, 0)
        mlp_prologue()
        jax.lax.fori_loop(LAG, n_pairs, fused, 0)
        jax.lax.fori_loop(n_pairs - LAG, n_pairs, mlp_only, 0)
        out_copy(n_pairs - 1).start()
        pltpu.make_async_copy(out_v, out_hbm, sems.at[OUT_SEM]).wait()

    return kernel, WO_SEM + nD + 6, X0


@functools.partial(jax.jit, static_argnames=("A_seg_len",))
def pallas_sequential_preLN__memory_aug_recurrent_mem_tr__mixer_s_mlp__prompt_kernel(
    A_x, A_mem0, A_Wq, A_Wk, A_Wv, A_Wo, A_seg_len, B_x, B_w1, B_w2, B_w3, B_w4,
):
    _, S, D = A_x.shape
    H, E = A_Wq.shape[1], A_Wq.shape[2]
    F = B_w3.shape[1]
    assert A_seg_len == SEG and A_mem0.shape[1] == MEM and S % PAIR == 0
    nD, nF = D // 128, F // 128

    x = A_x.reshape(S, D)
    mem0 = A_mem0.reshape(MEM, D)
    wo = A_Wo.reshape(H * E, D)

    kernel, n_sems, x0 = _make_kernel(S, D, H, E, F)
    any_spec = pl.BlockSpec(memory_space=pl.ANY)
    out = pl.pallas_call(
        kernel,
        in_specs=[any_spec] * 10,
        out_specs=any_spec,
        out_shape=jax.ShapeDtypeStruct((S, D), A_x.dtype),
        scratch_shapes=[
            pltpu.VMEM((3, D, H, E), BF),
            pltpu.VMEM((3, H, D // 2, E), U32),
            pltpu.VMEM((H * E, D), BF),
            pltpu.VMEM((nD, H * E // 2, 128), U32),
            pltpu.VMEM((nD, D, 128), BF),
            pltpu.VMEM((nD, D, 128), BF),
            pltpu.VMEM((nF, D, 128), BF),
            pltpu.VMEM((nD, F, 128), BF),
            pltpu.VMEM((S, D), BF),
            pltpu.VMEM((S, D), BF),
            pltpu.VMEM((MEM, D), BF),
            pltpu.VMEM((x0 // 2, D), U32),
            pltpu.VMEM((S // 2, H * E), U32),
            pltpu.VMEM((16, D), U32),
            pltpu.VMEM((16, D), U32),
            pltpu.VMEM((24, D), U32),
            pltpu.VMEM((16, D), U32),
            pltpu.VMEM((3, 8, H * E), F32),
            pltpu.VMEM((40, H * E), U32),
            pltpu.VMEM((48, D), F32),
            pltpu.VMEM((S + 2 * HALO, D), F32),
            pltpu.VMEM((PAIR + 2 * HALO, D), F32),
            pltpu.VMEM((PAIR, D), F32),
            pltpu.VMEM((PAIR // 2, D), U32),
            pltpu.SemaphoreType.DMA((n_sems,)),
        ],
        compiler_params=pltpu.CompilerParams(
            vmem_limit_bytes=124 * 1024 * 1024,
            disable_bounds_checks=True,
        ),
    )(x, mem0, A_Wq, A_Wk, A_Wv, wo, B_w1, B_w2, B_w3, B_w4)
    return out.reshape(1, S, D)
```

```python
import functools

import jax
import jax.numpy as jnp
from jax.experimental import pallas as pl
from jax.experimental.pallas import tpu as pltpu

BF = jnp.bfloat16
F32 = jnp.float32
U32 = jnp.uint32

SEG = 32
MEM = 8
PAIR = 2 * SEG
LAG = 3
HALO = 8
G = 2
TAIL_HEADS = 6
QR = 24
NCH = 4
LN_EPS = 1e-5
LOG2E = 1.4426950408889634


def _ln(x):
    m = jnp.mean(x, axis=-1, keepdims=True)
    xc = x - m
    v = jnp.mean(xc * xc, axis=-1, keepdims=True)
    return xc * jax.lax.rsqrt(v + LN_EPS)


_dot = functools.partial(jnp.dot, preferred_element_type=F32)


def _gelu(x):
    return jax.nn.gelu(x, approximate=True)


def _as_bf(x_u32):
    return pltpu.bitcast(x_u32, BF)


def _as_u32(x_bf):
    return pltpu.bitcast(x_bf, U32)


def _interleave(main, fill):
    fill = dict(fill)
    out = []
    for label, job in main:
        out.extend(fill.pop(label, []))
        out.append(job)
    out.extend(fill.pop('end', []))
    assert not fill, fill
    return out


def _run(jobs):
    for job in jobs:
        job()


def _make_kernel(S, D, H, E, F):
    n_pairs = S // PAIR
    nD = D // 128
    nF = F // 128
    scale = float(E) ** -0.5
    L = MEM + SEG
    n_slots = H // G
    K1 = (H - TAIL_HEADS) * E
    CH = D // NCH
    WO_CH = H * E // nD
    X0 = S - 2 * QR * n_pairs
    assert X0 % PAIR == 0 and X0 // PAIR - 1 >= LAG and X0 < S
    assert G == 2 and n_slots == 16 and nF == 28 and nD == 8 and H == 2 * NCH * 4
    assert (H - TAIL_HEADS) // G - 1 < n_slots - 2

    WO_SEM = 3 * NCH
    B_SEM, X0_SEM, XM_SEM, X1_SEM, MEM_SEM, OUT_SEM = (WO_SEM + nD + i for i in range(6))
    XA = X0 + 2 * QR
    XB = X0 + 2 * QR * (LAG + 1)

    def kernel(x_hbm, mem0_hbm, wq_hbm, wk_hbm, wv_hbm, wo_hbm, w1_hbm, w2_hbm, w3_hbm, w4_hbm,
               out_hbm,
               raw, w_t, wo_raw, wo_t, w1_t, w2_t, w3_t, w4_t,
               x_v, out_v, mem0_v, xn0, q_buf, lq_e, lq_o, lb_e, lb_o, sv, ob, wacc,
               h_buf, a1_buf, y_buf, z_buf, sems):

        def rows_copy(src, dst, start, size, sem):
            return pltpu.make_async_copy(src.at[pl.ds(start, size)], dst.at[pl.ds(start, size)], sems.at[sem])

        def raw_copy(i, c):
            src = (wq_hbm, wk_hbm, wv_hbm)[i]
            return rows_copy(src, raw.at[i], c * CH, CH, i * NCH + c)

        def wo_copy(j):
            return rows_copy(wo_hbm, wo_raw, j * WO_CH, WO_CH, WO_SEM + j)

        def mlp_weight_copies():
            return [pltpu.make_async_copy(src.at[:, pl.ds(j * 128, 128)], dst.at[j], sems.at[B_SEM])
                    for src, dst, n in ((w1_hbm, w1_t, nD), (w2_hbm, w2_t, nD),
                                        (w3_hbm, w3_t, nF), (w4_hbm, w4_t, nD))
                    for j in range(n)]

        def x_head_copy():
            return rows_copy(x_hbm, x_v, 0, XA, X0_SEM)

        def x_mid_copy():
            return rows_copy(x_hbm, x_v, XA, XB - XA, XM_SEM)

        def x_rest_copy():
            return rows_copy(x_hbm, x_v, XB, S - XB, X1_SEM)

        def mem_copy():
            return pltpu.make_async_copy(mem0_hbm, mem0_v, sems.at[MEM_SEM])

        def out_copy(c):
            return rows_copy(out_v, out_hbm, pl.multiple_of(c * PAIR, PAIR), PAIR, OUT_SEM)

        def relayout_block(i, b):
            x = _as_u32(raw[i, pl.ds(pl.multiple_of(b * 16, 16), 16), :, :]).reshape(8, 2, H // 2, E)
            ev, od = x[:, 0], x[:, 1]
            lo = jnp.swapaxes((ev & 0xFFFF) | (od << 16), 0, 1)
            hi = jnp.swapaxes((ev >> 16) | (od & jnp.uint32(0xFFFF0000)), 0, 1)
            rows = pl.ds(pl.multiple_of(b * 8, 8), 8)
            for p in range(H // 2):
                w_t[i, 2 * p, rows, :] = lo[p]
                w_t[i, 2 * p + 1, rows, :] = hi[p]

        def wo_finish():
            for j in range(nD):
                wo_copy(j).wait()

                def body(b, carry):
                    r = j * WO_CH + b * 64
                    blk = wo_raw[pl.ds(pl.multiple_of(r, 64), 64), :]
                    for n in range(nD):
                        wo_t[n, pl.ds(pl.multiple_of(r // 2, 32), 32), :] = _as_u32(blk[:, n * 128:(n + 1) * 128])
                    return carry
                jax.lax.fori_loop(0, WO_CH // 64, body, 0)
            x_mid_copy().wait()

        def store_xn(t):
            xn = _ln(x_v[pl.ds(pl.multiple_of(t * PAIR, PAIR), PAIR), :].astype(F32))
            lb_e[pl.ds(0, 4), :] = _as_u32(xn[32:40].astype(BF))
            lb_e[pl.ds(4, 4), :] = _as_u32(xn[0:8].astype(BF))
            lb_e[pl.ds(8, 8), :] = _as_u32(xn[8:24].astype(BF))
            lb_e[pl.ds(16, 4), :] = _as_u32(xn[24:32].astype(BF))
            lb_o[pl.ds(0, 8), :] = _as_u32(xn[40:56].astype(BF))
            lb_o[pl.ds(8, 4), :] = _as_u32(xn[56:64].astype(BF))
            xq = _ln(x_v[pl.ds(pl.multiple_of(X0 + t * 2 * QR, 16), 2 * QR), :].astype(F32))
            lq_e[pl.ds(0, 8), :] = _as_u32(xq[0:16].astype(BF))
            lq_e[pl.ds(8, 4), :] = _as_u32(xq[16:24].astype(BF))
            for n in range(3):
                lq_o[pl.ds(4 * n, 4), :] = _as_u32(xq[24 + 8 * n:32 + 8 * n].astype(BF))

        def prologue():
            x_head_copy().start()
            mem_copy().start()
            for i in range(3):
                for c in range(NCH):
                    raw_copy(i, c).start()
            for j in range(nD):
                wo_copy(j).start()
            x_mid_copy().start()
            h_buf[pl.ds(0, HALO), :] = jnp.zeros((HALO, D), F32)
            h_buf[pl.ds(HALO + S, HALO), :] = jnp.zeros((HALO, D), F32)
            x_head_copy().wait()
            mem_copy().wait()
            lb_e[pl.ds(20, 4), :] = _as_u32(mem0_v[...])
            lq_e[pl.ds(12, 4), :] = _as_u32(mem0_v[...])

            def ln_body(b, carry):
                rows = x_v[pl.ds(pl.multiple_of(b * 64, 64), 64), :].astype(F32)
                xn0[pl.ds(pl.multiple_of(b * 32, 32), 32), :] = _as_u32(_ln(rows).astype(BF))
                return carry
            jax.lax.fori_loop(0, X0 // 64, ln_body, 0)

            with jax.named_scope("sc_wq"):
                for c in range(NCH):
                    raw_copy(0, c).wait()

                    def q_body(b, carry):
                        relayout_block(0, b)
                        return carry
                    jax.lax.fori_loop(c * (CH // 16), (c + 1) * (CH // 16), q_body, 0)

            per_it = 2 * (D // 16) // H
            it_per_chunk = H // (2 * NCH)

            def kv_body(h, carry):
                i = 1 + h // (H // 2)

                @pl.when(h % it_per_chunk == 0)
                def _():
                    n = h // it_per_chunk
                    dst = raw.at[i, pl.ds((n % NCH) * CH, CH)]
                    pltpu.make_async_copy(dst, dst, sems.at[NCH + n]).wait()
                rows = X0 // 2 // per_it
                for n in range(per_it):
                    q = _dot(_as_bf(xn0[pl.ds(n * rows, rows), :]), _as_bf(w_t[0, h]))
                    q_buf[pl.ds(n * rows, rows), pl.ds(pl.multiple_of(h * E, E), E)] = _as_u32(q.astype(BF))
                    relayout_block(i, (h % (H // 2)) * per_it + n)
                return carry
            with jax.named_scope("sc_kv"):
                jax.lax.fori_loop(0, H, kv_body, 0)

            for c in mlp_weight_copies():
                c.start()
            x_rest_copy().start()

        def mlp_pre(c):
            a1_buf[pl.ds(0, 2 * HALO), :] = a1_buf[pl.ds(PAIR, 2 * HALO), :]
            y = _ln(h_buf[pl.ds(pl.multiple_of(c * PAIR + HALO, 8), PAIR + HALO), :])
            y_buf[...] = y[0:PAIR]
            z_buf[...] = _as_u32(_ln(y[HALO:]).astype(BF))

        def mlp_prologue():
            for c in mlp_weight_copies():
                c.wait()
            z = _ln(_ln(h_buf[pl.ds(0, 2 * HALO), :])).astype(BF)
            tok = jax.lax.broadcasted_iota(jnp.int32, (2 * HALO, 128), 0) - HALO
            for j in range(nD):
                a1_buf[pl.ds(PAIR, 2 * HALO), pl.ds(j * 128, 128)] = jnp.where(
                    tok >= 0, _gelu(_dot(z, w1_t[j])), 0.0)
            mlp_pre(0)

        def attention_jobs(t):
            row = jax.lax.broadcasted_iota(jnp.int32, (G * L, G * L), 0)
            col = jax.lax.broadcasted_iota(jnp.int32, (G * L, G * L), 1)

            def head_of(r):
                return jnp.where(r < G * SEG, r // SEG, (r - G * SEG) // MEM)
            mask = (head_of(row) == head_of(col)) & ((col >= G * SEG) | (row >= G * SEG) | (col <= row))
            x0 = t * PAIR
            h0 = x0 + HALO

            def step_jobs(even):
                lb = lb_e if even else lb_o
                st = {}

                lq = lq_e if even else lq_o
                q_new = pl.multiple_of(X0 // 2 + t * QR, 8)
                q_use = t * SEG + (0 if even else SEG // 2)

                def j_qkv(g, i):
                    def run():
                        h = g * G + i
                        cs = pl.ds(h * E, E)
                        q = _dot(_as_bf(lq[...]), _as_bf(w_t[0, h]))
                        if even:
                            q_buf[pl.ds(q_new, 8), cs] = _as_u32(q[0:16].astype(BF))
                            sv[2, :, cs] = q[16:24]
                        else:
                            q_buf[pl.ds(q_new + 8, 16), cs] = _as_u32(
                                jnp.concatenate([sv[2, :, cs], q[0:QR]], axis=0).astype(BF))
                        lhs = _as_bf(lb[...])
                        kv = [_dot(lhs, _as_bf(w_t[n, h])) for n in (1, 2)]
                        parts = st.setdefault(('parts', g), dict(qx=[], qm=[], x=[[], []], m=[[], []]))
                        parts['qx'].append(_as_bf(q_buf[pl.ds(pl.multiple_of(q_use, 16), SEG // 2), cs]))
                        parts['qm'].append(q[QR:QR + MEM])
                        for n in range(2):
                            if even:
                                sv[n, :, cs] = kv[n][0:8]
                                parts['x'][n].append(kv[n][8:40])
                                parts['m'][n].append(kv[n][40:48])
                            else:
                                parts['x'][n] += [sv[n, :, cs], kv[n][0:24]]
                                parts['m'][n].append(kv[n][24:32])
                        if i == G - 1:
                            parts = st.pop(('parts', g))
                            q2 = jnp.concatenate(
                                parts['qx'] + [jnp.concatenate(parts['qm'], axis=0).astype(BF)], axis=0)
                            st['qkv', g] = [q2] + [
                                jnp.concatenate(parts['x'][n] + parts['m'][n], axis=0).astype(BF)
                                for n in range(2)]
                    return run

                def j_scores(g):
                    def run():
                        q, k, v = st.pop(('qkv', g))
                        s = jax.lax.dot_general(q, k, (((1,), (1,)), ((), ())),
                                                preferred_element_type=F32)
                        s = jnp.where(mask, s, -1000000000.0 / scale)
                        m = jnp.max(s, axis=-1, keepdims=True)
                        p = jnp.exp2((s - m) * (scale * LOG2E))
                        l = jnp.sum(p, axis=-1, keepdims=True)
                        r0 = pl.reciprocal(l, approx=True)
                        p = p * (r0 * (2.0 - l * r0))
                        st['p', g] = (p.astype(BF), v)
                    return run

                def j_pv(g):
                    def run():
                        p, v = st.pop(('p', g))
                        o2 = _dot(p, v)
                        for i, h in enumerate(range(g * G, (g + 1) * G)):
                            ox = o2[i * SEG:(i + 1) * SEG]
                            om = o2[G * SEG + i * MEM:G * SEG + (i + 1) * MEM]
                            cs = pl.ds(h * E, E)
                            if even:
                                ob[pl.ds(16, 4), cs] = _as_u32(ox[0:8].astype(BF))
                                ob[pl.ds(0, 16), cs] = _as_u32(
                                    jnp.concatenate([ox[8:32], om], axis=0).astype(BF))
                            else:
                                ob[pl.ds(20, 4), cs] = _as_u32(ox[0:8].astype(BF))
                                ob[pl.ds(24, 16), cs] = _as_u32(
                                    jnp.concatenate([ox[8:32], om], axis=0).astype(BF))
                    return run

                rows = pl.ds(0, 16) if even else pl.ds(16, 24)
                nrows = 32 if even else 48

                def j_wo1(j):
                    def run():
                        lhs = _as_bf(ob[rows, pl.ds(0, K1)])
                        wacc[pl.ds(0, nrows), pl.ds(j * 128, 128)] = _dot(
                            lhs, _as_bf(wo_t[j, pl.ds(0, K1 // 2), :]))
                    return run

                def j_wo2(j):
                    def run():
                        lhs = _as_bf(ob[rows, pl.ds(K1, H * E - K1)])
                        r = wacc[pl.ds(0, nrows), pl.ds(j * 128, 128)] + _dot(
                            lhs, _as_bf(wo_t[j, pl.ds(K1 // 2, (H * E - K1) // 2), :]))
                        cs = pl.ds(j * 128, 128)
                        xs = x_v[pl.ds(pl.multiple_of(x0, PAIR), PAIR), cs].astype(F32)
                        if even:
                            mem = _as_u32(r[24:32].astype(BF))
                            lb_o[pl.ds(12, 4), cs] = mem
                            lq_o[pl.ds(12, 4), cs] = mem
                            h_buf[pl.ds(pl.multiple_of(h0 + 8, 8), 24), cs] = xs[8:32] + r[0:24]
                        else:
                            mem = _as_u32(r[40:48].astype(BF))
                            lb_e[pl.ds(20, 4), cs] = mem
                            lq_e[pl.ds(12, 4), cs] = mem
                            h_buf[pl.ds(pl.multiple_of(h0, 8), 8), cs] = xs[0:8] + r[0:8]
                            h_buf[pl.ds(pl.multiple_of(h0 + 32, 8), 32), cs] = xs[32:64] + r[8:40]
                    return run

                last = n_slots - 1
                jobs = []
                for g in range(n_slots):
                    for i in range(G):
                        jobs.append((('qkv', g, i), j_qkv(g, i)))
                    if g >= 1:
                        jobs.append((('s', g - 1), j_scores(g - 1)))
                    if g >= 2:
                        jobs.append((('pv', g - 2), j_pv(g - 2)))
                wo1 = [(('wo1', j), j_wo1(j)) for j in range(nD)]
                jobs += (wo1[0:3] + [(('s', last), j_scores(last)), (('pv', last - 1), j_pv(last - 1))]
                         + wo1[3:6] + [(('pv', last), j_pv(last))] + wo1[6:8])
                jobs += [(('wo2', j), j_wo2(j)) for j in range(nD)]
                return jobs

            def j_next_xn():
                store_xn(jnp.minimum(t + 1, n_pairs - 1))

            return step_jobs(True), step_jobs(False), j_next_xn

        after_qkv = ('s', n_slots - 2)

        def mlp_jobs(c):
            r0 = pl.multiple_of(c * PAIR, PAIR)
            st = {}

            def j_pre_next():
                mlp_pre(jnp.minimum(c + 1, n_pairs - 1))

            def j_w1(j):
                def run():
                    tok = jax.lax.broadcasted_iota(jnp.int32, (PAIR, 128), 0) + (r0 + HALO)
                    a = _gelu(_dot(_as_bf(z_buf[...]), w1_t[j]))
                    a1_buf[pl.ds(2 * HALO, PAIR), pl.ds(j * 128, 128)] = jnp.where(tok < S, a, 0.0)
                return run

            def j_shift():
                cq = D // 4
                st['g'] = jnp.concatenate([
                    a1_buf[pl.ds(HALO - 1, PAIR), pl.ds(0 * cq, cq)],
                    a1_buf[pl.ds(HALO + 1, PAIR), pl.ds(1 * cq, cq)],
                    a1_buf[pl.ds(HALO - 2, PAIR), pl.ds(2 * cq, cq)],
                    a1_buf[pl.ds(HALO + 2, PAIR), pl.ds(3 * cq, cq)]], axis=1).astype(BF)

            def j_w2(j):
                def run():
                    st['x1', j] = y_buf[:, pl.ds(j * 128, 128)] + _dot(st['g'], w2_t[j])
                return run

            def j_ln3():
                x1 = jnp.concatenate([st['x1', j] for j in range(nD)], axis=1)
                st['z1'] = _ln(x1).astype(BF)

            def j_w3(j):
                def run():
                    st['a3', j] = _gelu(_dot(st['z1'], w3_t[j])).astype(BF)
                return run

            def j_cat():
                st['a3'] = jnp.concatenate([st.pop(('a3', j)) for j in range(nF)], axis=1)

            def j_w4(j):
                def run():
                    cs = pl.ds(j * 128, 128)
                    hh = h_buf[pl.ds(pl.multiple_of(r0 + HALO, 8), PAIR), cs]
                    out_v[pl.ds(r0, PAIR), cs] = (
                        hh + (st['x1', j] + _dot(st['a3'], w4_t[j]))).astype(out_v.dtype)
                return run

            return dict(pre_next=j_pre_next, w1=[j_w1(j) for j in range(nD)], shift=j_shift,
                        w2=[j_w2(j) for j in range(nD)], ln3=j_ln3,
                        w3=[j_w3(j) for j in range(nF)], cat=j_cat,
                        w4=[j_w4(j) for j in range(nD)])

        def attention_only(t, carry):
            ej, oj, j_next_xn = attention_jobs(t)

            def j_wo_wait():
                with jax.named_scope("sc_wo_finish"):
                    pl.when(t == 0)(wo_finish)
            _run(_interleave(ej, {after_qkv: [j_wo_wait]}) + _interleave(oj, {after_qkv: [j_next_xn]}))
            return carry

        def fused(t, carry):
            @pl.when(t == LAG)
            def _():
                x_rest_copy().wait()

            @pl.when(t > LAG)
            def _():
                out_copy(t - LAG - 1).start()

            ej, oj, j_next_xn = attention_jobs(t)
            b = mlp_jobs(t - LAG)
            w3, w4 = b['w3'], b['w4']
            fe, fo = {}, {}

            def put(d, label, *jobs):
                d.setdefault(label, []).extend(jobs)
            for i in range(nD):
                put(fe, ('qkv', 2 + i // 2, i % 2), b['w1'][i])
                put(fe, ('qkv', 8 + i // 2, i % 2), b['w2'][i])
            put(fe, ('qkv', 6, 0), b['shift'])
            put(fe, ('qkv', 12, 0), b['ln3'])
            put(fe, ('qkv', 15, 0), w3[0])
            put(fe, 'end', *w3[1:4])
            put(fo, ('qkv', 0, 1), b['pre_next'])
            for k in range(4, nF):
                put(fo, ('qkv', 1 + (k - 4) // 2, (k - 4) % 2), w3[k])
            put(fo, ('qkv', 13, 0), b['cat'])
            put(fo, ('qkv', 14, 0), w4[0])
            put(fo, ('qkv', 15, 0), w4[1])
            put(fo, after_qkv, j_next_xn)
            put(fo, ('s', n_slots - 1), w4[2])
            put(fo, 'end', *w4[3:])
            with jax.named_scope("sc_fused_body"):
                _run(_interleave(ej, fe) + _interleave(oj, fo))
            return carry

        def mlp_only(c, carry):
            out_copy(c - 1).start()
            b = mlp_jobs(c)
            _run(b['w1'] + [b['shift']] + b['w2'] + [b['ln3'], b['pre_next']] + b['w3'] + [b['cat']] + b['w4'])
            return carry

        with jax.named_scope("sc_prologue"):
            prologue()
            store_xn(0)
        with jax.named_scope("sc_a_only"):
            jax.lax.fori_loop(0, LAG, attention_only, 0)
        with jax.named_scope("sc_mlp_prologue"):
            mlp_prologue()
        with jax.named_scope("sc_fused"):
            jax.lax.fori_loop(LAG, n_pairs, fused, 0)
        with jax.named_scope("sc_b_tail"):
            jax.lax.fori_loop(n_pairs - LAG, n_pairs, mlp_only, 0)
        out_copy(n_pairs - 1).start()
        pltpu.make_async_copy(out_v, out_hbm, sems.at[OUT_SEM]).wait()

    return kernel, WO_SEM + nD + 6, X0


@functools.partial(jax.jit, static_argnames=("A_seg_len",))
def pallas_sequential_preLN__memory_aug_recurrent_mem_tr__mixer_s_mlp__prompt_kernel(
    A_x, A_mem0, A_Wq, A_Wk, A_Wv, A_Wo, A_seg_len, B_x, B_w1, B_w2, B_w3, B_w4,
):
    _, S, D = A_x.shape
    H, E = A_Wq.shape[1], A_Wq.shape[2]
    F = B_w3.shape[1]
    assert A_seg_len == SEG and A_mem0.shape[1] == MEM and S % PAIR == 0
    nD, nF = D // 128, F // 128

    x = A_x.reshape(S, D)
    mem0 = A_mem0.reshape(MEM, D)
    wo = A_Wo.reshape(H * E, D)

    kernel, n_sems, x0 = _make_kernel(S, D, H, E, F)
    any_spec = pl.BlockSpec(memory_space=pl.ANY)
    out = pl.pallas_call(
        kernel,
        in_specs=[any_spec] * 10,
        out_specs=any_spec,
        out_shape=jax.ShapeDtypeStruct((S, D), A_x.dtype),
        scratch_shapes=[
            pltpu.VMEM((3, D, H, E), BF),
            pltpu.VMEM((3, H, D // 2, E), U32),
            pltpu.VMEM((H * E, D), BF),
            pltpu.VMEM((nD, H * E // 2, 128), U32),
            pltpu.VMEM((nD, D, 128), BF),
            pltpu.VMEM((nD, D, 128), BF),
            pltpu.VMEM((nF, D, 128), BF),
            pltpu.VMEM((nD, F, 128), BF),
            pltpu.VMEM((S, D), BF),
            pltpu.VMEM((S, D), BF),
            pltpu.VMEM((MEM, D), BF),
            pltpu.VMEM((x0 // 2, D), U32),
            pltpu.VMEM((S // 2, H * E), U32),
            pltpu.VMEM((16, D), U32),
            pltpu.VMEM((16, D), U32),
            pltpu.VMEM((24, D), U32),
            pltpu.VMEM((16, D), U32),
            pltpu.VMEM((3, 8, H * E), F32),
            pltpu.VMEM((40, H * E), U32),
            pltpu.VMEM((48, D), F32),
            pltpu.VMEM((S + 2 * HALO, D), F32),
            pltpu.VMEM((PAIR + 2 * HALO, D), F32),
            pltpu.VMEM((PAIR, D), F32),
            pltpu.VMEM((PAIR // 2, D), U32),
            pltpu.SemaphoreType.DMA((n_sems,)),
        ],
        compiler_params=pltpu.CompilerParams(
            vmem_limit_bytes=124 * 1024 * 1024,
            disable_bounds_checks=True,
        ),
    )(x, mem0, A_Wq, A_Wk, A_Wv, wo, B_w1, B_w2, B_w3, B_w4)
    return out.reshape(1, S, D)
```

```python
import functools

import jax
import jax.numpy as jnp
from jax.experimental import pallas as pl
from jax.experimental.pallas import tpu as pltpu

BF = jnp.bfloat16
F32 = jnp.float32
U32 = jnp.uint32

SEG = 32
MEM = 8
PAIR = 2 * SEG
LAG = 3
HALO = 8
G = 2
TAIL_HEADS = 6
QR = 24
NCH = 4
LN_EPS = 1e-5
LOG2E = 1.4426950408889634


def _ln(x):
    m = jnp.mean(x, axis=-1, keepdims=True)
    xc = x - m
    v = jnp.mean(xc * xc, axis=-1, keepdims=True)
    return xc * jax.lax.rsqrt(v + LN_EPS)


_dot = functools.partial(jnp.dot, preferred_element_type=F32)


def _gelu(x):
    return jax.nn.gelu(x, approximate=True)


def _as_bf(x_u32):
    return pltpu.bitcast(x_u32, BF)


def _as_u32(x_bf):
    return pltpu.bitcast(x_bf, U32)


def _interleave(main, fill):
    fill = dict(fill)
    out = []
    for label, job in main:
        out.extend(fill.pop(label, []))
        out.append(job)
    out.extend(fill.pop('end', []))
    assert not fill, fill
    return out


def _run(jobs):
    for job in jobs:
        job()


def _make_kernel(S, D, H, E, F):
    n_pairs = S // PAIR
    nD = D // 128
    nF = F // 128
    scale = float(E) ** -0.5
    L = MEM + SEG
    n_slots = H // G
    K1 = (H - TAIL_HEADS) * E
    CH = D // NCH
    WO_CH = H * E // nD
    X0 = S - 2 * QR * n_pairs
    assert X0 % PAIR == 0 and X0 // PAIR - 1 >= LAG and X0 < S
    assert G == 2 and n_slots == 16 and nF == 28 and nD == 8 and H == 2 * NCH * 4
    assert (H - TAIL_HEADS) // G - 1 < n_slots - 2

    WO_SEM = 3 * NCH
    B_SEM, X0_SEM, XM_SEM, X1_SEM, MEM_SEM, OUT_SEM = (WO_SEM + nD + i for i in range(6))
    XA = X0 + 2 * QR
    XB = X0 + 2 * QR * (LAG + 1)

    def kernel(x_hbm, mem0_hbm, wq_hbm, wk_hbm, wv_hbm, wo_hbm, w1_hbm, w2_hbm, w3_hbm, w4_hbm,
               out_hbm,
               raw, w_t, wo_raw, wo_t, w1_t, w2_t, w3_t, w4_t,
               x_v, out_v, mem0_v, xn0, q_buf, lq_e, lq_o, lb_e, lb_o, sv, ob, wacc,
               h_buf, a1_buf, y_buf, z_buf, sems):

        def rows_copy(src, dst, start, size, sem):
            return pltpu.make_async_copy(src.at[pl.ds(start, size)], dst.at[pl.ds(start, size)], sems.at[sem])

        def raw_copy(i, c):
            src = (wq_hbm, wk_hbm, wv_hbm)[i]
            return rows_copy(src, raw.at[i], c * CH, CH, i * NCH + c)

        def wo_copy(j):
            return rows_copy(wo_hbm, wo_raw, j * WO_CH, WO_CH, WO_SEM + j)

        def mlp_weight_copies():
            return [pltpu.make_async_copy(src.at[:, pl.ds(j * 128, 128)], dst.at[j], sems.at[B_SEM])
                    for src, dst, n in ((w1_hbm, w1_t, nD), (w2_hbm, w2_t, nD),
                                        (w3_hbm, w3_t, nF), (w4_hbm, w4_t, nD))
                    for j in range(n)]

        def x_head_copy():
            return rows_copy(x_hbm, x_v, 0, XA, X0_SEM)

        def x_mid_copy():
            return rows_copy(x_hbm, x_v, XA, XB - XA, XM_SEM)

        def x_rest_copy():
            return rows_copy(x_hbm, x_v, XB, S - XB, X1_SEM)

        def mem_copy():
            return pltpu.make_async_copy(mem0_hbm, mem0_v, sems.at[MEM_SEM])

        def out_copy(c):
            return rows_copy(out_v, out_hbm, pl.multiple_of(c * PAIR, PAIR), PAIR, OUT_SEM)

        def relayout_block(i, b):
            x = _as_u32(raw[i, pl.ds(pl.multiple_of(b * 16, 16), 16), :, :]).reshape(8, 2, H // 2, E)
            ev, od = x[:, 0], x[:, 1]
            lo = jnp.swapaxes((ev & 0xFFFF) | (od << 16), 0, 1)
            hi = jnp.swapaxes((ev >> 16) | (od & jnp.uint32(0xFFFF0000)), 0, 1)
            rows = pl.ds(pl.multiple_of(b * 8, 8), 8)
            for p in range(H // 2):
                w_t[i, 2 * p, rows, :] = lo[p]
                w_t[i, 2 * p + 1, rows, :] = hi[p]

        def wo_finish():
            for j in range(nD):
                wo_copy(j).wait()

                def body(b, carry):
                    r = j * WO_CH + b * 64
                    blk = wo_raw[pl.ds(pl.multiple_of(r, 64), 64), :]
                    for n in range(nD):
                        wo_t[n, pl.ds(pl.multiple_of(r // 2, 32), 32), :] = _as_u32(blk[:, n * 128:(n + 1) * 128])
                    return carry
                jax.lax.fori_loop(0, WO_CH // 64, body, 0)
            x_mid_copy().wait()

        def store_xn(t):
            xn = _ln(x_v[pl.ds(pl.multiple_of(t * PAIR, PAIR), PAIR), :].astype(F32))
            lb_e[pl.ds(0, 4), :] = _as_u32(xn[32:40].astype(BF))
            lb_e[pl.ds(4, 4), :] = _as_u32(xn[0:8].astype(BF))
            lb_e[pl.ds(8, 8), :] = _as_u32(xn[8:24].astype(BF))
            lb_e[pl.ds(16, 4), :] = _as_u32(xn[24:32].astype(BF))
            lb_o[pl.ds(0, 8), :] = _as_u32(xn[40:56].astype(BF))
            lb_o[pl.ds(8, 4), :] = _as_u32(xn[56:64].astype(BF))
            xq = _ln(x_v[pl.ds(pl.multiple_of(X0 + t * 2 * QR, 16), 2 * QR), :].astype(F32))
            lq_e[pl.ds(0, 8), :] = _as_u32(xq[0:16].astype(BF))
            lq_e[pl.ds(8, 4), :] = _as_u32(xq[16:24].astype(BF))
            for n in range(3):
                lq_o[pl.ds(4 * n, 4), :] = _as_u32(xq[24 + 8 * n:32 + 8 * n].astype(BF))

        def prologue():
            x_head_copy().start()
            mem_copy().start()
            for i in range(3):
                for c in range(NCH):
                    raw_copy(i, c).start()
            for j in range(nD):
                wo_copy(j).start()
            x_mid_copy().start()
            h_buf[pl.ds(0, HALO), :] = jnp.zeros((HALO, D), F32)
            h_buf[pl.ds(HALO + S, HALO), :] = jnp.zeros((HALO, D), F32)
            x_head_copy().wait()
            mem_copy().wait()
            lb_e[pl.ds(20, 4), :] = _as_u32(mem0_v[...])
            lq_e[pl.ds(12, 4), :] = _as_u32(mem0_v[...])

            def ln_body(b, carry):
                rows = x_v[pl.ds(pl.multiple_of(b * 64, 64), 64), :].astype(F32)
                xn0[pl.ds(pl.multiple_of(b * 32, 32), 32), :] = _as_u32(_ln(rows).astype(BF))
                return carry
            jax.lax.fori_loop(0, X0 // 64, ln_body, 0)

            with jax.named_scope("sc_wq"):
                for c in range(NCH):
                    raw_copy(0, c).wait()

                    def q_body(b, carry):
                        relayout_block(0, b)
                        return carry
                    jax.lax.fori_loop(c * (CH // 16), (c + 1) * (CH // 16), q_body, 0)

            HP = 2
            per_head = 2 * (D // 16) // H
            it_per_chunk = H // HP // (2 * NCH)

            def kv_body(it, carry):
                i = 1 + it // (H // HP // 2)

                @pl.when(it % it_per_chunk == 0)
                def _():
                    n = it // it_per_chunk
                    dst = raw.at[i, pl.ds((n % NCH) * CH, CH)]
                    pltpu.make_async_copy(dst, dst, sems.at[NCH + n]).wait()
                rows = X0 // 2 // per_head
                for k in range(HP):
                    h = it * HP + k
                    for n in range(per_head):
                        q = _dot(_as_bf(xn0[pl.ds(n * rows, rows), :]), _as_bf(w_t[0, h]))
                        q_buf[pl.ds(n * rows, rows), pl.ds(pl.multiple_of(h * E, E), E)] = _as_u32(q.astype(BF))
                        relayout_block(i, (h % (H // 2)) * per_head + n)
                return carry
            with jax.named_scope("sc_kv"):
                jax.lax.fori_loop(0, H // HP, kv_body, 0)

            for c in mlp_weight_copies():
                c.start()
            x_rest_copy().start()

        def mlp_pre(c):
            a1_buf[pl.ds(0, 2 * HALO), :] = a1_buf[pl.ds(PAIR, 2 * HALO), :]
            y = _ln(h_buf[pl.ds(pl.multiple_of(c * PAIR + HALO, 8), PAIR + HALO), :])
            y_buf[...] = y[0:PAIR]
            z_buf[...] = _as_u32(_ln(y[HALO:]).astype(BF))

        def mlp_prologue():
            for c in mlp_weight_copies():
                c.wait()
            z = _ln(_ln(h_buf[pl.ds(0, 2 * HALO), :])).astype(BF)
            tok = jax.lax.broadcasted_iota(jnp.int32, (2 * HALO, 128), 0) - HALO
            for j in range(nD):
                a1_buf[pl.ds(PAIR, 2 * HALO), pl.ds(j * 128, 128)] = jnp.where(
                    tok >= 0, _gelu(_dot(z, w1_t[j])), 0.0)
            mlp_pre(0)

        def attention_jobs(t):
            row = jax.lax.broadcasted_iota(jnp.int32, (G * L, G * L), 0)
            col = jax.lax.broadcasted_iota(jnp.int32, (G * L, G * L), 1)

            def head_of(r):
                return jnp.where(r < G * SEG, r // SEG, (r - G * SEG) // MEM)
            mask = (head_of(row) == head_of(col)) & ((col >= G * SEG) | (row >= G * SEG) | (col <= row))
            x0 = t * PAIR
            h0 = x0 + HALO

            def step_jobs(even):
                lb = lb_e if even else lb_o
                st = {}

                lq = lq_e if even else lq_o
                q_new = pl.multiple_of(X0 // 2 + t * QR, 8)
                q_use = t * SEG + (0 if even else SEG // 2)

                def j_qkv(g, i):
                    def run():
                        h = g * G + i
                        cs = pl.ds(h * E, E)
                        q = _dot(_as_bf(lq[...]), _as_bf(w_t[0, h]))
                        if even:
                            q_buf[pl.ds(q_new, 8), cs] = _as_u32(q[0:16].astype(BF))
                            sv[2, :, cs] = q[16:24]
                        else:
                            q_buf[pl.ds(q_new + 8, 16), cs] = _as_u32(
                                jnp.concatenate([sv[2, :, cs], q[0:QR]], axis=0).astype(BF))
                        lhs = _as_bf(lb[...])
                        kv = [_dot(lhs, _as_bf(w_t[n, h])) for n in (1, 2)]
                        parts = st.setdefault(('parts', g), dict(qx=[], qm=[], x=[[], []], m=[[], []]))
                        parts['qx'].append(_as_bf(q_buf[pl.ds(pl.multiple_of(q_use, 16), SEG // 2), cs]))
                        parts['qm'].append(q[QR:QR + MEM])
                        for n in range(2):
                            if even:
                                sv[n, :, cs] = kv[n][0:8]
                                parts['x'][n].append(kv[n][8:40])
                                parts['m'][n].append(kv[n][40:48])
                            else:
                                parts['x'][n] += [sv[n, :, cs], kv[n][0:24]]
                                parts['m'][n].append(kv[n][24:32])
                        if i == G - 1:
                            parts = st.pop(('parts', g))
                            q2 = jnp.concatenate(
                                parts['qx'] + [jnp.concatenate(parts['qm'], axis=0).astype(BF)], axis=0)
                            st['qkv', g] = [q2] + [
                                jnp.concatenate(parts['x'][n] + parts['m'][n], axis=0).astype(BF)
                                for n in range(2)]
                    return run

                def j_scores(g):
                    def run():
                        q, k, v = st.pop(('qkv', g))
                        s = jax.lax.dot_general(q, k, (((1,), (1,)), ((), ())),
                                                preferred_element_type=F32)
                        s = jnp.where(mask, s, -1000000000.0 / scale)
                        m = jnp.max(s, axis=-1, keepdims=True)
                        p = jnp.exp2((s - m) * (scale * LOG2E))
                        l = jnp.sum(p, axis=-1, keepdims=True)
                        r0 = pl.reciprocal(l, approx=True)
                        p = p * (r0 * (2.0 - l * r0))
                        st['p', g] = (p.astype(BF), v)
                    return run

                def j_pv(g):
                    def run():
                        p, v = st.pop(('p', g))
                        o2 = _dot(p, v)
                        for i, h in enumerate(range(g * G, (g + 1) * G)):
                            ox = o2[i * SEG:(i + 1) * SEG]
                            om = o2[G * SEG + i * MEM:G * SEG + (i + 1) * MEM]
                            cs = pl.ds(h * E, E)
                            if even:
                                ob[pl.ds(16, 4), cs] = _as_u32(ox[0:8].astype(BF))
                                ob[pl.ds(0, 16), cs] = _as_u32(
                                    jnp.concatenate([ox[8:32], om], axis=0).astype(BF))
                            else:
                                ob[pl.ds(20, 4), cs] = _as_u32(ox[0:8].astype(BF))
                                ob[pl.ds(24, 16), cs] = _as_u32(
                                    jnp.concatenate([ox[8:32], om], axis=0).astype(BF))
                    return run

                rows = pl.ds(0, 16) if even else pl.ds(16, 24)
                nrows = 32 if even else 48

                def j_wo1(j):
                    def run():
                        lhs = _as_bf(ob[rows, pl.ds(0, K1)])
                        wacc[pl.ds(0, nrows), pl.ds(j * 128, 128)] = _dot(
                            lhs, _as_bf(wo_t[j, pl.ds(0, K1 // 2), :]))
                    return run

                def j_wo2(j):
                    def run():
                        lhs = _as_bf(ob[rows, pl.ds(K1, H * E - K1)])
                        r = wacc[pl.ds(0, nrows), pl.ds(j * 128, 128)] + _dot(
                            lhs, _as_bf(wo_t[j, pl.ds(K1 // 2, (H * E - K1) // 2), :]))
                        cs = pl.ds(j * 128, 128)
                        xs = x_v[pl.ds(pl.multiple_of(x0, PAIR), PAIR), cs].astype(F32)
                        if even:
                            mem = _as_u32(r[24:32].astype(BF))
                            lb_o[pl.ds(12, 4), cs] = mem
                            lq_o[pl.ds(12, 4), cs] = mem
                            h_buf[pl.ds(pl.multiple_of(h0 + 8, 8), 24), cs] = xs[8:32] + r[0:24]
                        else:
                            mem = _as_u32(r[40:48].astype(BF))
                            lb_e[pl.ds(20, 4), cs] = mem
                            lq_e[pl.ds(12, 4), cs] = mem
                            h_buf[pl.ds(pl.multiple_of(h0, 8), 8), cs] = xs[0:8] + r[0:8]
                            h_buf[pl.ds(pl.multiple_of(h0 + 32, 8), 32), cs] = xs[32:64] + r[8:40]
                    return run

                last = n_slots - 1
                jobs = []
                for g in range(n_slots):
                    for i in range(G):
                        jobs.append((('qkv', g, i), j_qkv(g, i)))
                    if g >= 1:
                        jobs.append((('s', g - 1), j_scores(g - 1)))
                    if g >= 2:
                        jobs.append((('pv', g - 2), j_pv(g - 2)))
                wo1 = [(('wo1', j), j_wo1(j)) for j in range(nD)]
                jobs += (wo1[0:3] + [(('s', last), j_scores(last)), (('pv', last - 1), j_pv(last - 1))]
                         + wo1[3:6] + [(('pv', last), j_pv(last))] + wo1[6:8])
                jobs += [(('wo2', j), j_wo2(j)) for j in range(nD)]
                return jobs

            def j_next_xn():
                store_xn(jnp.minimum(t + 1, n_pairs - 1))

            return step_jobs(True), step_jobs(False), j_next_xn

        after_qkv = ('s', n_slots - 2)

        def mlp_jobs(c):
            r0 = pl.multiple_of(c * PAIR, PAIR)
            st = {}

            def j_pre_next():
                mlp_pre(jnp.minimum(c + 1, n_pairs - 1))

            def j_w1(j):
                def run():
                    tok = jax.lax.broadcasted_iota(jnp.int32, (PAIR, 128), 0) + (r0 + HALO)
                    a = _gelu(_dot(_as_bf(z_buf[...]), w1_t[j]))
                    a1_buf[pl.ds(2 * HALO, PAIR), pl.ds(j * 128, 128)] = jnp.where(tok < S, a, 0.0)
                return run

            def j_shift():
                cq = D // 4
                st['g'] = jnp.concatenate([
                    a1_buf[pl.ds(HALO - 1, PAIR), pl.ds(0 * cq, cq)],
                    a1_buf[pl.ds(HALO + 1, PAIR), pl.ds(1 * cq, cq)],
                    a1_buf[pl.ds(HALO - 2, PAIR), pl.ds(2 * cq, cq)],
                    a1_buf[pl.ds(HALO + 2, PAIR), pl.ds(3 * cq, cq)]], axis=1).astype(BF)

            def j_w2(j):
                def run():
                    st['x1', j] = y_buf[:, pl.ds(j * 128, 128)] + _dot(st['g'], w2_t[j])
                return run

            def j_ln3():
                x1 = jnp.concatenate([st['x1', j] for j in range(nD)], axis=1)
                st['z1'] = _ln(x1).astype(BF)

            def j_w3(j):
                def run():
                    st['a3', j] = _gelu(_dot(st['z1'], w3_t[j])).astype(BF)
                return run

            def j_cat():
                st['a3'] = jnp.concatenate([st.pop(('a3', j)) for j in range(nF)], axis=1)

            def j_w4(j):
                def run():
                    cs = pl.ds(j * 128, 128)
                    hh = h_buf[pl.ds(pl.multiple_of(r0 + HALO, 8), PAIR), cs]
                    out_v[pl.ds(r0, PAIR), cs] = (
                        hh + (st['x1', j] + _dot(st['a3'], w4_t[j]))).astype(out_v.dtype)
                return run

            return dict(pre_next=j_pre_next, w1=[j_w1(j) for j in range(nD)], shift=j_shift,
                        w2=[j_w2(j) for j in range(nD)], ln3=j_ln3,
                        w3=[j_w3(j) for j in range(nF)], cat=j_cat,
                        w4=[j_w4(j) for j in range(nD)])

        def attention_only(t, carry):
            ej, oj, j_next_xn = attention_jobs(t)

            def j_wo_wait():
                with jax.named_scope("sc_wo_finish"):
                    pl.when(t == 0)(wo_finish)
            _run(_interleave(ej, {after_qkv: [j_wo_wait]}) + _interleave(oj, {after_qkv: [j_next_xn]}))
            return carry

        def fused(t, carry):
            @pl.when(t == LAG)
            def _():
                x_rest_copy().wait()

            @pl.when(t > LAG)
            def _():
                out_copy(t - LAG - 1).start()

            ej, oj, j_next_xn = attention_jobs(t)
            b = mlp_jobs(t - LAG)
            w3, w4 = b['w3'], b['w4']
            fe, fo = {}, {}

            def put(d, label, *jobs):
                d.setdefault(label, []).extend(jobs)
            for i in range(nD):
                put(fe, ('qkv', 2 + i // 2, i % 2), b['w1'][i])
                put(fe, ('qkv', 8 + i // 2, i % 2), b['w2'][i])
            put(fe, ('qkv', 6, 0), b['shift'])
            put(fe, ('qkv', 12, 0), b['ln3'])
            put(fe, ('qkv', 15, 0), w3[0])
            put(fe, 'end', *w3[1:4])
            put(fo, ('qkv', 0, 1), b['pre_next'])
            for k in range(4, nF):
                put(fo, ('qkv', 1 + (k - 4) // 2, (k - 4) % 2), w3[k])
            put(fo, ('qkv', 13, 0), b['cat'])
            put(fo, ('qkv', 14, 0), w4[0])
            put(fo, ('qkv', 15, 0), w4[1])
            put(fo, after_qkv, j_next_xn)
            put(fo, ('s', n_slots - 1), w4[2])
            put(fo, 'end', *w4[3:])
            with jax.named_scope("sc_fused_body"):
                _run(_interleave(ej, fe) + _interleave(oj, fo))
            return carry

        def mlp_only(c, carry):
            out_copy(c - 1).start()
            b = mlp_jobs(c)
            _run(b['w1'] + [b['shift']] + b['w2'] + [b['ln3'], b['pre_next']] + b['w3'] + [b['cat']] + b['w4'])
            return carry

        with jax.named_scope("sc_prologue"):
            prologue()
            store_xn(0)
        with jax.named_scope("sc_a_only"):
            jax.lax.fori_loop(0, LAG, attention_only, 0)
        with jax.named_scope("sc_mlp_prologue"):
            mlp_prologue()
        with jax.named_scope("sc_fused"):
            jax.lax.fori_loop(LAG, n_pairs, fused, 0)
        with jax.named_scope("sc_b_tail"):
            jax.lax.fori_loop(n_pairs - LAG, n_pairs, mlp_only, 0)
        out_copy(n_pairs - 1).start()
        pltpu.make_async_copy(out_v, out_hbm, sems.at[OUT_SEM]).wait()

    return kernel, WO_SEM + nD + 6, X0


@functools.partial(jax.jit, static_argnames=("A_seg_len",))
def pallas_sequential_preLN__memory_aug_recurrent_mem_tr__mixer_s_mlp__prompt_kernel(
    A_x, A_mem0, A_Wq, A_Wk, A_Wv, A_Wo, A_seg_len, B_x, B_w1, B_w2, B_w3, B_w4,
):
    _, S, D = A_x.shape
    H, E = A_Wq.shape[1], A_Wq.shape[2]
    F = B_w3.shape[1]
    assert A_seg_len == SEG and A_mem0.shape[1] == MEM and S % PAIR == 0
    nD, nF = D // 128, F // 128

    x = A_x.reshape(S, D)
    mem0 = A_mem0.reshape(MEM, D)
    wo = A_Wo.reshape(H * E, D)

    kernel, n_sems, x0 = _make_kernel(S, D, H, E, F)
    any_spec = pl.BlockSpec(memory_space=pl.ANY)
    out = pl.pallas_call(
        kernel,
        in_specs=[any_spec] * 10,
        out_specs=any_spec,
        out_shape=jax.ShapeDtypeStruct((S, D), A_x.dtype),
        scratch_shapes=[
            pltpu.VMEM((3, D, H, E), BF),
            pltpu.VMEM((3, H, D // 2, E), U32),
            pltpu.VMEM((H * E, D), BF),
            pltpu.VMEM((nD, H * E // 2, 128), U32),
            pltpu.VMEM((nD, D, 128), BF),
            pltpu.VMEM((nD, D, 128), BF),
            pltpu.VMEM((nF, D, 128), BF),
            pltpu.VMEM((nD, F, 128), BF),
            pltpu.VMEM((S, D), BF),
            pltpu.VMEM((S, D), BF),
            pltpu.VMEM((MEM, D), BF),
            pltpu.VMEM((x0 // 2, D), U32),
            pltpu.VMEM((S // 2, H * E), U32),
            pltpu.VMEM((16, D), U32),
            pltpu.VMEM((16, D), U32),
            pltpu.VMEM((24, D), U32),
            pltpu.VMEM((16, D), U32),
            pltpu.VMEM((3, 8, H * E), F32),
            pltpu.VMEM((40, H * E), U32),
            pltpu.VMEM((48, D), F32),
            pltpu.VMEM((S + 2 * HALO, D), F32),
            pltpu.VMEM((PAIR + 2 * HALO, D), F32),
            pltpu.VMEM((PAIR, D), F32),
            pltpu.VMEM((PAIR // 2, D), U32),
            pltpu.SemaphoreType.DMA((n_sems,)),
        ],
        compiler_params=pltpu.CompilerParams(
            vmem_limit_bytes=124 * 1024 * 1024,
            disable_bounds_checks=True,
        ),
    )(x, mem0, A_Wq, A_Wk, A_Wv, wo, B_w1, B_w2, B_w3, B_w4)
    return out.reshape(1, S, D)
```

```python
import functools

import jax
import jax.numpy as jnp
from jax.experimental import pallas as pl
from jax.experimental.pallas import tpu as pltpu

BF = jnp.bfloat16
F32 = jnp.float32
U32 = jnp.uint32

SEG = 32
MEM = 8
PAIR = 2 * SEG
LAG = 3
HALO = 8
G = 2
TAIL_HEADS = 6
QR = 24
NCH = 8
LN_EPS = 1e-5
LOG2E = 1.4426950408889634


def _ln(x):
    m = jnp.mean(x, axis=-1, keepdims=True)
    xc = x - m
    v = jnp.mean(xc * xc, axis=-1, keepdims=True)
    return xc * jax.lax.rsqrt(v + LN_EPS)


_dot = functools.partial(jnp.dot, preferred_element_type=F32)


def _gelu(x):
    return jax.nn.gelu(x, approximate=True)


def _as_bf(x_u32):
    return pltpu.bitcast(x_u32, BF)


def _as_u32(x_bf):
    return pltpu.bitcast(x_bf, U32)


def _interleave(main, fill):
    fill = dict(fill)
    out = []
    for label, job in main:
        out.extend(fill.pop(label, []))
        out.append(job)
    out.extend(fill.pop('end', []))
    assert not fill, fill
    return out


def _run(jobs):
    for job in jobs:
        job()


def _make_kernel(S, D, H, E, F):
    n_pairs = S // PAIR
    nD = D // 128
    nF = F // 128
    scale = float(E) ** -0.5
    L = MEM + SEG
    n_slots = H // G
    K1 = (H - TAIL_HEADS) * E
    CH = D // NCH
    WO_CH = H * E // nD
    X0 = S - 2 * QR * n_pairs
    assert X0 % PAIR == 0 and X0 // PAIR - 1 >= LAG and X0 < S
    assert G == 2 and n_slots == 16 and nF == 28 and nD == 8
    assert (H - TAIL_HEADS) // G - 1 < n_slots - 2

    WO_SEM = 3 * NCH
    B_SEM, X0_SEM, XM_SEM, X1_SEM, MEM_SEM, OUT_SEM = (WO_SEM + nD + i for i in range(6))
    XA = X0 + 2 * QR
    XB = X0 + 2 * QR * (LAG + 1)

    def kernel(x_hbm, mem0_hbm, wq_hbm, wk_hbm, wv_hbm, wo_hbm, w1_hbm, w2_hbm, w3_hbm, w4_hbm,
               out_hbm,
               raw, w_t, wo_raw, wo_t, w1_t, w2_t, w3_t, w4_t,
               x_v, out_v, mem0_v, xn0, q_buf, lq_e, lq_o, lb_e, lb_o, sv, ob, wacc,
               h_buf, a1_buf, y_buf, z_buf, sems):

        def rows_copy(src, dst, start, size, sem):
            return pltpu.make_async_copy(src.at[pl.ds(start, size)], dst.at[pl.ds(start, size)], sems.at[sem])

        def raw_copy(i, c):
            src = (wq_hbm, wk_hbm, wv_hbm)[i]
            return rows_copy(src, raw.at[i], c * CH, CH, i * NCH + c)

        def wo_copy(j):
            return rows_copy(wo_hbm, wo_raw, j * WO_CH, WO_CH, WO_SEM + j)

        def mlp_weight_copies():
            return [pltpu.make_async_copy(src.at[:, pl.ds(j * 128, 128)], dst.at[j], sems.at[B_SEM])
                    for src, dst, n in ((w1_hbm, w1_t, nD), (w2_hbm, w2_t, nD),
                                        (w3_hbm, w3_t, nF), (w4_hbm, w4_t, nD))
                    for j in range(n)]

        def x_head_copy():
            return rows_copy(x_hbm, x_v, 0, XA, X0_SEM)

        def x_mid_copy():
            return rows_copy(x_hbm, x_v, XA, XB - XA, XM_SEM)

        def x_rest_copy():
            return rows_copy(x_hbm, x_v, XB, S - XB, X1_SEM)

        def mem_copy():
            return pltpu.make_async_copy(mem0_hbm, mem0_v, sems.at[MEM_SEM])

        def out_copy(c):
            return rows_copy(out_v, out_hbm, pl.multiple_of(c * PAIR, PAIR), PAIR, OUT_SEM)

        def relayout_block(i, b):
            x = _as_u32(raw[i, pl.ds(pl.multiple_of(b * 16, 16), 16), :, :]).reshape(8, 2, H // 2, E)
            ev, od = x[:, 0], x[:, 1]
            lo = jnp.swapaxes((ev & 0xFFFF) | (od << 16), 0, 1)
            hi = jnp.swapaxes((ev >> 16) | (od & jnp.uint32(0xFFFF0000)), 0, 1)
            rows = pl.ds(pl.multiple_of(b * 8, 8), 8)
            for p in range(H // 2):
                w_t[i, 2 * p, rows, :] = lo[p]
                w_t[i, 2 * p + 1, rows, :] = hi[p]

        def wo_finish():
            for j in range(nD):
                wo_copy(j).wait()

                def body(b, carry):
                    r = j * WO_CH + b * 64
                    blk = wo_raw[pl.ds(pl.multiple_of(r, 64), 64), :]
                    for n in range(nD):
                        wo_t[n, pl.ds(pl.multiple_of(r // 2, 32), 32), :] = _as_u32(blk[:, n * 128:(n + 1) * 128])
                    return carry
                jax.lax.fori_loop(0, WO_CH // 64, body, 0)
            x_mid_copy().wait()

        def store_xn(t):
            xn = _ln(x_v[pl.ds(pl.multiple_of(t * PAIR, PAIR), PAIR), :].astype(F32))
            lb_e[pl.ds(0, 4), :] = _as_u32(xn[32:40].astype(BF))
            lb_e[pl.ds(4, 4), :] = _as_u32(xn[0:8].astype(BF))
            lb_e[pl.ds(8, 8), :] = _as_u32(xn[8:24].astype(BF))
            lb_e[pl.ds(16, 4), :] = _as_u32(xn[24:32].astype(BF))
            lb_o[pl.ds(0, 8), :] = _as_u32(xn[40:56].astype(BF))
            lb_o[pl.ds(8, 4), :] = _as_u32(xn[56:64].astype(BF))
            xq = _ln(x_v[pl.ds(pl.multiple_of(X0 + t * 2 * QR, 16), 2 * QR), :].astype(F32))
            lq_e[pl.ds(0, 8), :] = _as_u32(xq[0:16].astype(BF))
            lq_e[pl.ds(8, 4), :] = _as_u32(xq[16:24].astype(BF))
            for n in range(3):
                lq_o[pl.ds(4 * n, 4), :] = _as_u32(xq[24 + 8 * n:32 + 8 * n].astype(BF))

        def prologue():
            x_head_copy().start()
            mem_copy().start()
            for i in range(3):
                for c in range(NCH):
                    raw_copy(i, c).start()
            for j in range(nD):
                wo_copy(j).start()
            x_mid_copy().start()
            h_buf[pl.ds(0, HALO), :] = jnp.zeros((HALO, D), F32)
            h_buf[pl.ds(HALO + S, HALO), :] = jnp.zeros((HALO, D), F32)
            x_head_copy().wait()
            mem_copy().wait()
            lb_e[pl.ds(20, 4), :] = _as_u32(mem0_v[...])
            lq_e[pl.ds(12, 4), :] = _as_u32(mem0_v[...])

            def ln_body(b, carry):
                rows = x_v[pl.ds(pl.multiple_of(b * 64, 64), 64), :].astype(F32)
                xn0[pl.ds(pl.multiple_of(b * 32, 32), 32), :] = _as_u32(_ln(rows).astype(BF))
                return carry
            jax.lax.fori_loop(0, X0 // 64, ln_body, 0)

            with jax.named_scope("sc_wq"):
                def q_chunk(c, carry):
                    dst = raw.at[0, pl.ds(c * CH, CH)]
                    pltpu.make_async_copy(dst, dst, sems.at[c]).wait()

                    def q_body(b, carry):
                        relayout_block(0, b)
                        return carry
                    return jax.lax.fori_loop(c * (CH // 16), (c + 1) * (CH // 16), q_body, carry)
                jax.lax.fori_loop(0, NCH, q_chunk, 0)

            HP = 2
            per_head = 2 * (D // 16) // H
            it_per_chunk = H // HP // (2 * NCH)
            assert it_per_chunk * HP * per_head * 16 == CH

            def kv_body(it, carry):
                i = 1 + it // (H // HP // 2)

                @pl.when(it % it_per_chunk == 0)
                def _():
                    n = it // it_per_chunk
                    dst = raw.at[i, pl.ds((n % NCH) * CH, CH)]
                    pltpu.make_async_copy(dst, dst, sems.at[NCH + n]).wait()
                rows = X0 // 2 // per_head
                for k in range(HP):
                    h = it * HP + k
                    for n in range(per_head):
                        q = _dot(_as_bf(xn0[pl.ds(n * rows, rows), :]), _as_bf(w_t[0, h]))
                        q_buf[pl.ds(n * rows, rows), pl.ds(pl.multiple_of(h * E, E), E)] = _as_u32(q.astype(BF))
                        relayout_block(i, (h % (H // 2)) * per_head + n)
                return carry
            with jax.named_scope("sc_kv"):
                jax.lax.fori_loop(0, H // HP, kv_body, 0)

            for c in mlp_weight_copies():
                c.start()
            x_rest_copy().start()

        def mlp_pre(c):
            a1_buf[pl.ds(0, 2 * HALO), :] = a1_buf[pl.ds(PAIR, 2 * HALO), :]
            y = _ln(h_buf[pl.ds(pl.multiple_of(c * PAIR + HALO, 8), PAIR + HALO), :])
            y_buf[...] = y[0:PAIR]
            z_buf[...] = _as_u32(_ln(y[HALO:]).astype(BF))

        def mlp_prologue():
            for c in mlp_weight_copies():
                c.wait()
            z = _ln(_ln(h_buf[pl.ds(0, 2 * HALO), :])).astype(BF)
            tok = jax.lax.broadcasted_iota(jnp.int32, (2 * HALO, 128), 0) - HALO
            for j in range(nD):
                a1_buf[pl.ds(PAIR, 2 * HALO), pl.ds(j * 128, 128)] = jnp.where(
                    tok >= 0, _gelu(_dot(z, w1_t[j])), 0.0)
            mlp_pre(0)

        def attention_jobs(t):
            row = jax.lax.broadcasted_iota(jnp.int32, (G * L, G * L), 0)
            col = jax.lax.broadcasted_iota(jnp.int32, (G * L, G * L), 1)

            def head_of(r):
                return jnp.where(r < G * SEG, r // SEG, (r - G * SEG) // MEM)
            mask = (head_of(row) == head_of(col)) & ((col >= G * SEG) | (row >= G * SEG) | (col <= row))
            x0 = t * PAIR
            h0 = x0 + HALO

            def step_jobs(even):
                lb = lb_e if even else lb_o
                st = {}

                lq = lq_e if even else lq_o
                q_new = pl.multiple_of(X0 // 2 + t * QR, 8)
                q_use = t * SEG + (0 if even else SEG // 2)

                def j_qkv(g, i):
                    def run():
                        h = g * G + i
                        cs = pl.ds(h * E, E)
                        q = _dot(_as_bf(lq[...]), _as_bf(w_t[0, h]))
                        if even:
                            q_buf[pl.ds(q_new, 8), cs] = _as_u32(q[0:16].astype(BF))
                            sv[2, :, cs] = q[16:24]
                        else:
                            q_buf[pl.ds(q_new + 8, 16), cs] = _as_u32(
                                jnp.concatenate([sv[2, :, cs], q[0:QR]], axis=0).astype(BF))
                        lhs = _as_bf(lb[...])
                        kv = [_dot(lhs, _as_bf(w_t[n, h])) for n in (1, 2)]
                        parts = st.setdefault(('parts', g), dict(qx=[], qm=[], x=[[], []], m=[[], []]))
                        parts['qx'].append(_as_bf(q_buf[pl.ds(pl.multiple_of(q_use, 16), SEG // 2), cs]))
                        parts['qm'].append(q[QR:QR + MEM])
                        for n in range(2):
                            if even:
                                sv[n, :, cs] = kv[n][0:8]
                                parts['x'][n].append(kv[n][8:40])
                                parts['m'][n].append(kv[n][40:48])
                            else:
                                parts['x'][n] += [sv[n, :, cs], kv[n][0:24]]
                                parts['m'][n].append(kv[n][24:32])
                        if i == G - 1:
                            parts = st.pop(('parts', g))
                            q2 = jnp.concatenate(
                                parts['qx'] + [jnp.concatenate(parts['qm'], axis=0).astype(BF)], axis=0)
                            st['qkv', g] = [q2] + [
                                jnp.concatenate(parts['x'][n] + parts['m'][n], axis=0).astype(BF)
                                for n in range(2)]
                    return run

                def j_scores(g):
                    def run():
                        q, k, v = st.pop(('qkv', g))
                        s = jax.lax.dot_general(q, k, (((1,), (1,)), ((), ())),
                                                preferred_element_type=F32)
                        s = jnp.where(mask, s, -1000000000.0 / scale)
                        m = jnp.max(s, axis=-1, keepdims=True)
                        p = jnp.exp2((s - m) * (scale * LOG2E))
                        l = jnp.sum(p, axis=-1, keepdims=True)
                        r0 = pl.reciprocal(l, approx=True)
                        p = p * (r0 * (2.0 - l * r0))
                        st['p', g] = (p.astype(BF), v)
                    return run

                def j_pv(g):
                    def run():
                        p, v = st.pop(('p', g))
                        o2 = _dot(p, v)
                        for i, h in enumerate(range(g * G, (g + 1) * G)):
                            ox = o2[i * SEG:(i + 1) * SEG]
                            om = o2[G * SEG + i * MEM:G * SEG + (i + 1) * MEM]
                            cs = pl.ds(h * E, E)
                            if even:
                                ob[pl.ds(16, 4), cs] = _as_u32(ox[0:8].astype(BF))
                                ob[pl.ds(0, 16), cs] = _as_u32(
                                    jnp.concatenate([ox[8:32], om], axis=0).astype(BF))
                            else:
                                ob[pl.ds(20, 4), cs] = _as_u32(ox[0:8].astype(BF))
                                ob[pl.ds(24, 16), cs] = _as_u32(
                                    jnp.concatenate([ox[8:32], om], axis=0).astype(BF))
                    return run

                rows = pl.ds(0, 16) if even else pl.ds(16, 24)
                nrows = 32 if even else 48

                def j_wo1(j):
                    def run():
                        lhs = _as_bf(ob[rows, pl.ds(0, K1)])
                        wacc[pl.ds(0, nrows), pl.ds(j * 128, 128)] = _dot(
                            lhs, _as_bf(wo_t[j, pl.ds(0, K1 // 2), :]))
                    return run

                def j_wo2(j):
                    def run():
                        lhs = _as_bf(ob[rows, pl.ds(K1, H * E - K1)])
                        r = wacc[pl.ds(0, nrows), pl.ds(j * 128, 128)] + _dot(
                            lhs, _as_bf(wo_t[j, pl.ds(K1 // 2, (H * E - K1) // 2), :]))
                        cs = pl.ds(j * 128, 128)
                        xs = x_v[pl.ds(pl.multiple_of(x0, PAIR), PAIR), cs].astype(F32)
                        if even:
                            mem = _as_u32(r[24:32].astype(BF))
                            lb_o[pl.ds(12, 4), cs] = mem
                            lq_o[pl.ds(12, 4), cs] = mem
                            h_buf[pl.ds(pl.multiple_of(h0 + 8, 8), 24), cs] = xs[8:32] + r[0:24]
                        else:
                            mem = _as_u32(r[40:48].astype(BF))
                            lb_e[pl.ds(20, 4), cs] = mem
                            lq_e[pl.ds(12, 4), cs] = mem
                            h_buf[pl.ds(pl.multiple_of(h0, 8), 8), cs] = xs[0:8] + r[0:8]
                            h_buf[pl.ds(pl.multiple_of(h0 + 32, 8), 32), cs] = xs[32:64] + r[8:40]
                    return run

                last = n_slots - 1
                jobs = []
                for g in range(n_slots):
                    for i in range(G):
                        jobs.append((('qkv', g, i), j_qkv(g, i)))
                    if g >= 1:
                        jobs.append((('s', g - 1), j_scores(g - 1)))
                    if g >= 2:
                        jobs.append((('pv', g - 2), j_pv(g - 2)))
                wo1 = [(('wo1', j), j_wo1(j)) for j in range(nD)]
                jobs += (wo1[0:3] + [(('s', last), j_scores(last)), (('pv', last - 1), j_pv(last - 1))]
                         + wo1[3:6] + [(('pv', last), j_pv(last))] + wo1[6:8])
                jobs += [(('wo2', j), j_wo2(j)) for j in range(nD)]
                return jobs

            def j_next_xn():
                store_xn(jnp.minimum(t + 1, n_pairs - 1))

            return step_jobs(True), step_jobs(False), j_next_xn

        after_qkv = ('s', n_slots - 2)

        def mlp_jobs(c):
            r0 = pl.multiple_of(c * PAIR, PAIR)
            st = {}

            def j_pre_next():
                mlp_pre(jnp.minimum(c + 1, n_pairs - 1))

            def j_w1(j):
                def run():
                    tok = jax.lax.broadcasted_iota(jnp.int32, (PAIR, 128), 0) + (r0 + HALO)
                    a = _gelu(_dot(_as_bf(z_buf[...]), w1_t[j]))
                    a1_buf[pl.ds(2 * HALO, PAIR), pl.ds(j * 128, 128)] = jnp.where(tok < S, a, 0.0)
                return run

            def j_shift():
                cq = D // 4
                st['g'] = jnp.concatenate([
                    a1_buf[pl.ds(HALO - 1, PAIR), pl.ds(0 * cq, cq)],
                    a1_buf[pl.ds(HALO + 1, PAIR), pl.ds(1 * cq, cq)],
                    a1_buf[pl.ds(HALO - 2, PAIR), pl.ds(2 * cq, cq)],
                    a1_buf[pl.ds(HALO + 2, PAIR), pl.ds(3 * cq, cq)]], axis=1).astype(BF)

            def j_w2(j):
                def run():
                    st['x1', j] = y_buf[:, pl.ds(j * 128, 128)] + _dot(st['g'], w2_t[j])
                return run

            def j_ln3():
                x1 = jnp.concatenate([st['x1', j] for j in range(nD)], axis=1)
                st['z1'] = _ln(x1).astype(BF)

            def j_w3(j):
                def run():
                    st['a3', j] = _gelu(_dot(st['z1'], w3_t[j])).astype(BF)
                return run

            def j_cat():
                st['a3'] = jnp.concatenate([st.pop(('a3', j)) for j in range(nF)], axis=1)

            def j_w4(j):
                def run():
                    cs = pl.ds(j * 128, 128)
                    hh = h_buf[pl.ds(pl.multiple_of(r0 + HALO, 8), PAIR), cs]
                    out_v[pl.ds(r0, PAIR), cs] = (
                        hh + (st['x1', j] + _dot(st['a3'], w4_t[j]))).astype(out_v.dtype)
                return run

            return dict(pre_next=j_pre_next, w1=[j_w1(j) for j in range(nD)], shift=j_shift,
                        w2=[j_w2(j) for j in range(nD)], ln3=j_ln3,
                        w3=[j_w3(j) for j in range(nF)], cat=j_cat,
                        w4=[j_w4(j) for j in range(nD)])

        def attention_only(t, carry):
            ej, oj, j_next_xn = attention_jobs(t)

            def j_wo_wait():
                with jax.named_scope("sc_wo_finish"):
                    pl.when(t == 0)(wo_finish)
            _run(_interleave(ej, {after_qkv: [j_wo_wait]}) + _interleave(oj, {after_qkv: [j_next_xn]}))
            return carry

        def fused(t, carry):
            @pl.when(t == LAG)
            def _():
                x_rest_copy().wait()

            @pl.when(t > LAG)
            def _():
                out_copy(t - LAG - 1).start()

            ej, oj, j_next_xn = attention_jobs(t)
            b = mlp_jobs(t - LAG)
            w3, w4 = b['w3'], b['w4']
            fe, fo = {}, {}

            def put(d, label, *jobs):
                d.setdefault(label, []).extend(jobs)
            for i in range(nD):
                put(fe, ('qkv', 2 + i // 2, i % 2), b['w1'][i])
                put(fe, ('qkv', 8 + i // 2, i % 2), b['w2'][i])
            put(fe, ('qkv', 6, 0), b['shift'])
            put(fe, ('qkv', 12, 0), b['ln3'])
            put(fe, ('qkv', 15, 0), w3[0])
            put(fe, 'end', *w3[1:4])
            put(fo, ('qkv', 0, 1), b['pre_next'])
            for k in range(4, nF):
                put(fo, ('qkv', 1 + (k - 4) // 2, (k - 4) % 2), w3[k])
            put(fo, ('qkv', 13, 0), b['cat'])
            put(fo, ('qkv', 14, 0), w4[0])
            put(fo, ('qkv', 15, 0), w4[1])
            put(fo, after_qkv, j_next_xn)
            put(fo, ('s', n_slots - 1), w4[2])
            put(fo, 'end', *w4[3:])
            with jax.named_scope("sc_fused_body"):
                _run(_interleave(ej, fe) + _interleave(oj, fo))
            return carry

        def mlp_only(c, carry):
            out_copy(c - 1).start()
            b = mlp_jobs(c)
            _run(b['w1'] + [b['shift']] + b['w2'] + [b['ln3'], b['pre_next']] + b['w3'] + [b['cat']] + b['w4'])
            return carry

        with jax.named_scope("sc_prologue"):
            prologue()
            store_xn(0)
        with jax.named_scope("sc_a_only"):
            jax.lax.fori_loop(0, LAG, attention_only, 0)
        with jax.named_scope("sc_mlp_prologue"):
            mlp_prologue()
        with jax.named_scope("sc_fused"):
            jax.lax.fori_loop(LAG, n_pairs, fused, 0)
        with jax.named_scope("sc_b_tail"):
            jax.lax.fori_loop(n_pairs - LAG, n_pairs, mlp_only, 0)
        out_copy(n_pairs - 1).start()
        pltpu.make_async_copy(out_v, out_hbm, sems.at[OUT_SEM]).wait()

    return kernel, WO_SEM + nD + 6, X0


@functools.partial(jax.jit, static_argnames=("A_seg_len",))
def pallas_sequential_preLN__memory_aug_recurrent_mem_tr__mixer_s_mlp__prompt_kernel(
    A_x, A_mem0, A_Wq, A_Wk, A_Wv, A_Wo, A_seg_len, B_x, B_w1, B_w2, B_w3, B_w4,
):
    _, S, D = A_x.shape
    H, E = A_Wq.shape[1], A_Wq.shape[2]
    F = B_w3.shape[1]
    assert A_seg_len == SEG and A_mem0.shape[1] == MEM and S % PAIR == 0
    nD, nF = D // 128, F // 128

    x = A_x.reshape(S, D)
    mem0 = A_mem0.reshape(MEM, D)
    wo = A_Wo.reshape(H * E, D)

    kernel, n_sems, x0 = _make_kernel(S, D, H, E, F)
    any_spec = pl.BlockSpec(memory_space=pl.ANY)
    out = pl.pallas_call(
        kernel,
        in_specs=[any_spec] * 10,
        out_specs=any_spec,
        out_shape=jax.ShapeDtypeStruct((S, D), A_x.dtype),
        scratch_shapes=[
            pltpu.VMEM((3, D, H, E), BF),
            pltpu.VMEM((3, H, D // 2, E), U32),
            pltpu.VMEM((H * E, D), BF),
            pltpu.VMEM((nD, H * E // 2, 128), U32),
            pltpu.VMEM((nD, D, 128), BF),
            pltpu.VMEM((nD, D, 128), BF),
            pltpu.VMEM((nF, D, 128), BF),
            pltpu.VMEM((nD, F, 128), BF),
            pltpu.VMEM((S, D), BF),
            pltpu.VMEM((S, D), BF),
            pltpu.VMEM((MEM, D), BF),
            pltpu.VMEM((x0 // 2, D), U32),
            pltpu.VMEM((S // 2, H * E), U32),
            pltpu.VMEM((16, D), U32),
            pltpu.VMEM((16, D), U32),
            pltpu.VMEM((24, D), U32),
            pltpu.VMEM((16, D), U32),
            pltpu.VMEM((3, 8, H * E), F32),
            pltpu.VMEM((40, H * E), U32),
            pltpu.VMEM((48, D), F32),
            pltpu.VMEM((S + 2 * HALO, D), F32),
            pltpu.VMEM((PAIR + 2 * HALO, D), F32),
            pltpu.VMEM((PAIR, D), F32),
            pltpu.VMEM((PAIR // 2, D), U32),
            pltpu.SemaphoreType.DMA((n_sems,)),
        ],
        compiler_params=pltpu.CompilerParams(
            vmem_limit_bytes=124 * 1024 * 1024,
            disable_bounds_checks=True,
        ),
    )(x, mem0, A_Wq, A_Wk, A_Wv, wo, B_w1, B_w2, B_w3, B_w4)
    return out.reshape(1, S, D)
```

```python
import functools

import jax
import jax.numpy as jnp
from jax.experimental import pallas as pl
from jax.experimental.pallas import tpu as pltpu

BF = jnp.bfloat16
F32 = jnp.float32
U32 = jnp.uint32

SEG = 32
MEM = 8
PAIR = 2 * SEG
LAG = 3
HALO = 8
G = 2
TAIL_HEADS = 6
QR = 24
NCH = 8
LN_EPS = 1e-5
LOG2E = 1.4426950408889634


def _ln(x):
    m = jnp.mean(x, axis=-1, keepdims=True)
    xc = x - m
    v = jnp.mean(xc * xc, axis=-1, keepdims=True)
    return xc * jax.lax.rsqrt(v + LN_EPS)


_dot = functools.partial(jnp.dot, preferred_element_type=F32)


def _gelu(x):
    return jax.nn.gelu(x, approximate=True)


def _as_bf(x_u32):
    return pltpu.bitcast(x_u32, BF)


def _as_u32(x_bf):
    return pltpu.bitcast(x_bf, U32)


def _interleave(main, fill):
    fill = dict(fill)
    out = []
    for label, job in main:
        out.extend(fill.pop(label, []))
        out.append(job)
    out.extend(fill.pop('end', []))
    assert not fill, fill
    return out


def _run(jobs):
    for job in jobs:
        job()


def _make_kernel(S, D, H, E, F):
    n_pairs = S // PAIR
    nD = D // 128
    nF = F // 128
    scale = float(E) ** -0.5
    L = MEM + SEG
    n_slots = H // G
    K1 = (H - TAIL_HEADS) * E
    CH = D // NCH
    WO_CH = H * E // nD
    X0 = S - 2 * QR * n_pairs
    assert X0 % PAIR == 0 and X0 // PAIR - 1 >= LAG and X0 < S
    assert G == 2 and n_slots == 16 and nF == 28 and nD == 8
    assert (H - TAIL_HEADS) // G - 1 < n_slots - 2

    WO_SEM = 3 * NCH
    B_SEM, X0_SEM, XM_SEM, X1_SEM, MEM_SEM, OUT_SEM = (WO_SEM + nD + i for i in range(6))
    XA = X0 + 2 * QR
    XB = X0 + 2 * QR * (LAG + 1)

    def kernel(x_hbm, mem0_hbm, wq_hbm, wk_hbm, wv_hbm, wo_hbm, w1_hbm, w2_hbm, w3_hbm, w4_hbm,
               out_hbm,
               raw, w_t, wo_raw, wo_t, w1_t, w2_t, w3_t, w4_t,
               x_v, out_v, mem0_v, xn0, q_buf, lq_e, lq_o, lb_e, lb_o, sv, ob, wacc,
               h_buf, a1_buf, y_buf, z_buf, sems):

        def rows_copy(src, dst, start, size, sem):
            return pltpu.make_async_copy(src.at[pl.ds(start, size)], dst.at[pl.ds(start, size)], sems.at[sem])

        def raw_copy(i, c):
            src = (wq_hbm, wk_hbm, wv_hbm)[i]
            return rows_copy(src, raw.at[i], c * CH, CH, i * NCH + c)

        def wo_copy(j):
            return rows_copy(wo_hbm, wo_raw, j * WO_CH, WO_CH, WO_SEM + j)

        def mlp_weight_copies():
            return [pltpu.make_async_copy(src.at[:, pl.ds(j * 128, 128)], dst.at[j], sems.at[B_SEM])
                    for src, dst, n in ((w1_hbm, w1_t, nD), (w2_hbm, w2_t, nD),
                                        (w3_hbm, w3_t, nF), (w4_hbm, w4_t, nD))
                    for j in range(n)]

        def x_head_copy():
            return rows_copy(x_hbm, x_v, 0, XA, X0_SEM)

        def x_mid_copy():
            return rows_copy(x_hbm, x_v, XA, XB - XA, XM_SEM)

        def x_rest_copy():
            return rows_copy(x_hbm, x_v, XB, S - XB, X1_SEM)

        def mem_copy():
            return pltpu.make_async_copy(mem0_hbm, mem0_v, sems.at[MEM_SEM])

        def out_copy(c):
            return rows_copy(out_v, out_hbm, pl.multiple_of(c * PAIR, PAIR), PAIR, OUT_SEM)

        def relayout_part(i, b, h0, nh):
            x = raw[i, pl.ds(pl.multiple_of(b * 16, 16), 16), pl.ds(h0, nh), :]
            x = _as_u32(x).reshape(8, 2, nh // 2, E)
            ev, od = x[:, 0], x[:, 1]
            lo = jnp.swapaxes((ev & 0xFFFF) | (od << 16), 0, 1)
            hi = jnp.swapaxes((ev >> 16) | (od & jnp.uint32(0xFFFF0000)), 0, 1)
            rows = pl.ds(pl.multiple_of(b * 8, 8), 8)
            for p in range(nh // 2):
                w_t[i, h0 + 2 * p, rows, :] = lo[p]
                w_t[i, h0 + 2 * p + 1, rows, :] = hi[p]

        def relayout_block(i, b):
            relayout_part(i, b, 0, H)

        def wo_finish():
            for j in range(nD):
                wo_copy(j).wait()

                def body(b, carry):
                    r = j * WO_CH + b * 64
                    blk = wo_raw[pl.ds(pl.multiple_of(r, 64), 64), :]
                    for n in range(nD):
                        wo_t[n, pl.ds(pl.multiple_of(r // 2, 32), 32), :] = _as_u32(blk[:, n * 128:(n + 1) * 128])
                    return carry
                jax.lax.fori_loop(0, WO_CH // 64, body, 0)
            x_mid_copy().wait()

        def store_xn(t):
            xn = _ln(x_v[pl.ds(pl.multiple_of(t * PAIR, PAIR), PAIR), :].astype(F32))
            lb_e[pl.ds(0, 4), :] = _as_u32(xn[32:40].astype(BF))
            lb_e[pl.ds(4, 4), :] = _as_u32(xn[0:8].astype(BF))
            lb_e[pl.ds(8, 8), :] = _as_u32(xn[8:24].astype(BF))
            lb_e[pl.ds(16, 4), :] = _as_u32(xn[24:32].astype(BF))
            lb_o[pl.ds(0, 8), :] = _as_u32(xn[40:56].astype(BF))
            lb_o[pl.ds(8, 4), :] = _as_u32(xn[56:64].astype(BF))
            xq = _ln(x_v[pl.ds(pl.multiple_of(X0 + t * 2 * QR, 16), 2 * QR), :].astype(F32))
            lq_e[pl.ds(0, 8), :] = _as_u32(xq[0:16].astype(BF))
            lq_e[pl.ds(8, 4), :] = _as_u32(xq[16:24].astype(BF))
            for n in range(3):
                lq_o[pl.ds(4 * n, 4), :] = _as_u32(xq[24 + 8 * n:32 + 8 * n].astype(BF))

        def prologue():
            x_head_copy().start()
            mem_copy().start()
            for i in range(3):
                for c in range(NCH):
                    raw_copy(i, c).start()
            for j in range(nD):
                wo_copy(j).start()
            x_mid_copy().start()
            h_buf[pl.ds(0, HALO), :] = jnp.zeros((HALO, D), F32)
            h_buf[pl.ds(HALO + S, HALO), :] = jnp.zeros((HALO, D), F32)
            x_head_copy().wait()
            mem_copy().wait()
            lb_e[pl.ds(20, 4), :] = _as_u32(mem0_v[...])
            lq_e[pl.ds(12, 4), :] = _as_u32(mem0_v[...])

            def ln_body(b, carry):
                rows = x_v[pl.ds(pl.multiple_of(b * 64, 64), 64), :].astype(F32)
                xn0[pl.ds(pl.multiple_of(b * 32, 32), 32), :] = _as_u32(_ln(rows).astype(BF))
                return carry
            jax.lax.fori_loop(0, X0 // 64, ln_body, 0)

            with jax.named_scope("sc_wq"):
                def q_chunk(c, carry):
                    dst = raw.at[0, pl.ds(c * CH, CH)]
                    pltpu.make_async_copy(dst, dst, sems.at[c]).wait()

                    def q_body(b, carry):
                        relayout_block(0, b)
                        return carry
                    return jax.lax.fori_loop(c * (CH // 16), (c + 1) * (CH // 16), q_body, carry)
                jax.lax.fori_loop(0, NCH, q_chunk, 0)

            HP = 2
            per_head = 2 * (D // 16) // H
            it_per_chunk = H // HP // (2 * NCH)
            assert it_per_chunk * HP * per_head * 16 == CH

            def kv_body(it, carry):
                i = 1 + it // (H // HP // 2)

                @pl.when(it % it_per_chunk == 0)
                def _():
                    n = it // it_per_chunk
                    dst = raw.at[i, pl.ds((n % NCH) * CH, CH)]
                    pltpu.make_async_copy(dst, dst, sems.at[NCH + n]).wait()
                NPC = 8
                rows = X0 // 2 // NPC
                for k in range(HP):
                    h = it * HP + k
                    for n in range(NPC):
                        q = _dot(_as_bf(xn0[pl.ds(n * rows, rows), :]), _as_bf(w_t[0, h]))
                        q_buf[pl.ds(n * rows, rows), pl.ds(pl.multiple_of(h * E, E), E)] = _as_u32(q.astype(BF))
                        relayout_part(i, (h % (H // 2)) * per_head + n // 2, (n % 2) * (H // 2), H // 2)
                return carry
            with jax.named_scope("sc_kv"):
                jax.lax.fori_loop(0, H // HP, kv_body, 0)

            for c in mlp_weight_copies():
                c.start()
            x_rest_copy().start()

        def mlp_pre(c):
            a1_buf[pl.ds(0, 2 * HALO), :] = a1_buf[pl.ds(PAIR, 2 * HALO), :]
            y = _ln(h_buf[pl.ds(pl.multiple_of(c * PAIR + HALO, 8), PAIR + HALO), :])
            y_buf[...] = y[0:PAIR]
            z_buf[...] = _as_u32(_ln(y[HALO:]).astype(BF))

        def mlp_prologue():
            for c in mlp_weight_copies():
                c.wait()
            z = _ln(_ln(h_buf[pl.ds(0, 2 * HALO), :])).astype(BF)
            tok = jax.lax.broadcasted_iota(jnp.int32, (2 * HALO, 128), 0) - HALO
            for j in range(nD):
                a1_buf[pl.ds(PAIR, 2 * HALO), pl.ds(j * 128, 128)] = jnp.where(
                    tok >= 0, _gelu(_dot(z, w1_t[j])), 0.0)
            mlp_pre(0)

        def attention_jobs(t):
            row = jax.lax.broadcasted_iota(jnp.int32, (G * L, G * L), 0)
            col = jax.lax.broadcasted_iota(jnp.int32, (G * L, G * L), 1)

            def head_of(r):
                return jnp.where(r < G * SEG, r // SEG, (r - G * SEG) // MEM)
            mask = (head_of(row) == head_of(col)) & ((col >= G * SEG) | (row >= G * SEG) | (col <= row))
            x0 = t * PAIR
            h0 = x0 + HALO

            def step_jobs(even):
                lb = lb_e if even else lb_o
                st = {}

                lq = lq_e if even else lq_o
                q_new = pl.multiple_of(X0 // 2 + t * QR, 8)
                q_use = t * SEG + (0 if even else SEG // 2)

                def j_qkv(g, i):
                    def run():
                        h = g * G + i
                        cs = pl.ds(h * E, E)
                        q = _dot(_as_bf(lq[...]), _as_bf(w_t[0, h]))
                        if even:
                            q_buf[pl.ds(q_new, 8), cs] = _as_u32(q[0:16].astype(BF))
                            sv[2, :, cs] = q[16:24]
                        else:
                            q_buf[pl.ds(q_new + 8, 16), cs] = _as_u32(
                                jnp.concatenate([sv[2, :, cs], q[0:QR]], axis=0).astype(BF))
                        lhs = _as_bf(lb[...])
                        kv = [_dot(lhs, _as_bf(w_t[n, h])) for n in (1, 2)]
                        parts = st.setdefault(('parts', g), dict(qx=[], qm=[], x=[[], []], m=[[], []]))
                        parts['qx'].append(_as_bf(q_buf[pl.ds(pl.multiple_of(q_use, 16), SEG // 2), cs]))
                        parts['qm'].append(q[QR:QR + MEM])
                        for n in range(2):
                            if even:
                                sv[n, :, cs] = kv[n][0:8]
                                parts['x'][n].append(kv[n][8:40])
                                parts['m'][n].append(kv[n][40:48])
                            else:
                                parts['x'][n] += [sv[n, :, cs], kv[n][0:24]]
                                parts['m'][n].append(kv[n][24:32])
                        if i == G - 1:
                            parts = st.pop(('parts', g))
                            q2 = jnp.concatenate(
                                parts['qx'] + [jnp.concatenate(parts['qm'], axis=0).astype(BF)], axis=0)
                            st['qkv', g] = [q2] + [
                                jnp.concatenate(parts['x'][n] + parts['m'][n], axis=0).astype(BF)
                                for n in range(2)]
                    return run

                def j_scores(g):
                    def run():
                        q, k, v = st.pop(('qkv', g))
                        s = jax.lax.dot_general(q, k, (((1,), (1,)), ((), ())),
                                                preferred_element_type=F32)
                        s = jnp.where(mask, s, -1000000000.0 / scale)
                        m = jnp.max(s, axis=-1, keepdims=True)
                        p = jnp.exp2((s - m) * (scale * LOG2E))
                        l = jnp.sum(p, axis=-1, keepdims=True)
                        r0 = pl.reciprocal(l, approx=True)
                        p = p * (r0 * (2.0 - l * r0))
                        st['p', g] = (p.astype(BF), v)
                    return run

                def j_pv(g):
                    def run():
                        p, v = st.pop(('p', g))
                        o2 = _dot(p, v)
                        for i, h in enumerate(range(g * G, (g + 1) * G)):
                            ox = o2[i * SEG:(i + 1) * SEG]
                            om = o2[G * SEG + i * MEM:G * SEG + (i + 1) * MEM]
                            cs = pl.ds(h * E, E)
                            if even:
                                ob[pl.ds(16, 4), cs] = _as_u32(ox[0:8].astype(BF))
                                ob[pl.ds(0, 16), cs] = _as_u32(
                                    jnp.concatenate([ox[8:32], om], axis=0).astype(BF))
                            else:
                                ob[pl.ds(20, 4), cs] = _as_u32(ox[0:8].astype(BF))
                                ob[pl.ds(24, 16), cs] = _as_u32(
                                    jnp.concatenate([ox[8:32], om], axis=0).astype(BF))
                    return run

                rows = pl.ds(0, 16) if even else pl.ds(16, 24)
                nrows = 32 if even else 48

                def j_wo1(j):
                    def run():
                        lhs = _as_bf(ob[rows, pl.ds(0, K1)])
                        wacc[pl.ds(0, nrows), pl.ds(j * 128, 128)] = _dot(
                            lhs, _as_bf(wo_t[j, pl.ds(0, K1 // 2), :]))
                    return run

                def j_wo2(j):
                    def run():
                        lhs = _as_bf(ob[rows, pl.ds(K1, H * E - K1)])
                        r = wacc[pl.ds(0, nrows), pl.ds(j * 128, 128)] + _dot(
                            lhs, _as_bf(wo_t[j, pl.ds(K1 // 2, (H * E - K1) // 2), :]))
                        cs = pl.ds(j * 128, 128)
                        xs = x_v[pl.ds(pl.multiple_of(x0, PAIR), PAIR), cs].astype(F32)
                        if even:
                            mem = _as_u32(r[24:32].astype(BF))
                            lb_o[pl.ds(12, 4), cs] = mem
                            lq_o[pl.ds(12, 4), cs] = mem
                            h_buf[pl.ds(pl.multiple_of(h0 + 8, 8), 24), cs] = xs[8:32] + r[0:24]
                        else:
                            mem = _as_u32(r[40:48].astype(BF))
                            lb_e[pl.ds(20, 4), cs] = mem
                            lq_e[pl.ds(12, 4), cs] = mem
                            h_buf[pl.ds(pl.multiple_of(h0, 8), 8), cs] = xs[0:8] + r[0:8]
                            h_buf[pl.ds(pl.multiple_of(h0 + 32, 8), 32), cs] = xs[32:64] + r[8:40]
                    return run

                last = n_slots - 1
                jobs = []
                for g in range(n_slots):
                    for i in range(G):
                        jobs.append((('qkv', g, i), j_qkv(g, i)))
                    if g >= 1:
                        jobs.append((('s', g - 1), j_scores(g - 1)))
                    if g >= 2:
                        jobs.append((('pv', g - 2), j_pv(g - 2)))
                wo1 = [(('wo1', j), j_wo1(j)) for j in range(nD)]
                jobs += (wo1[0:3] + [(('s', last), j_scores(last)), (('pv', last - 1), j_pv(last - 1))]
                         + wo1[3:6] + [(('pv', last), j_pv(last))] + wo1[6:8])
                jobs += [(('wo2', j), j_wo2(j)) for j in range(nD)]
                return jobs

            def j_next_xn():
                store_xn(jnp.minimum(t + 1, n_pairs - 1))

            return step_jobs(True), step_jobs(False), j_next_xn

        after_qkv = ('s', n_slots - 2)

        def mlp_jobs(c):
            r0 = pl.multiple_of(c * PAIR, PAIR)
            st = {}

            def j_pre_next():
                mlp_pre(jnp.minimum(c + 1, n_pairs - 1))

            def j_w1(j):
                def run():
                    tok = jax.lax.broadcasted_iota(jnp.int32, (PAIR, 128), 0) + (r0 + HALO)
                    a = _gelu(_dot(_as_bf(z_buf[...]), w1_t[j]))
                    a1_buf[pl.ds(2 * HALO, PAIR), pl.ds(j * 128, 128)] = jnp.where(tok < S, a, 0.0)
                return run

            def j_shift():
                cq = D // 4
                st['g'] = jnp.concatenate([
                    a1_buf[pl.ds(HALO - 1, PAIR), pl.ds(0 * cq, cq)],
                    a1_buf[pl.ds(HALO + 1, PAIR), pl.ds(1 * cq, cq)],
                    a1_buf[pl.ds(HALO - 2, PAIR), pl.ds(2 * cq, cq)],
                    a1_buf[pl.ds(HALO + 2, PAIR), pl.ds(3 * cq, cq)]], axis=1).astype(BF)

            def j_w2(j):
                def run():
                    st['x1', j] = y_buf[:, pl.ds(j * 128, 128)] + _dot(st['g'], w2_t[j])
                return run

            def j_ln3():
                x1 = jnp.concatenate([st['x1', j] for j in range(nD)], axis=1)
                st['z1'] = _ln(x1).astype(BF)

            def j_w3(j):
                def run():
                    st['a3', j] = _gelu(_dot(st['z1'], w3_t[j])).astype(BF)
                return run

            def j_cat():
                st['a3'] = jnp.concatenate([st.pop(('a3', j)) for j in range(nF)], axis=1)

            def j_w4(j):
                def run():
                    cs = pl.ds(j * 128, 128)
                    hh = h_buf[pl.ds(pl.multiple_of(r0 + HALO, 8), PAIR), cs]
                    out_v[pl.ds(r0, PAIR), cs] = (
                        hh + (st['x1', j] + _dot(st['a3'], w4_t[j]))).astype(out_v.dtype)
                return run

            return dict(pre_next=j_pre_next, w1=[j_w1(j) for j in range(nD)], shift=j_shift,
                        w2=[j_w2(j) for j in range(nD)], ln3=j_ln3,
                        w3=[j_w3(j) for j in range(nF)], cat=j_cat,
                        w4=[j_w4(j) for j in range(nD)])

        def attention_only(t, carry):
            ej, oj, j_next_xn = attention_jobs(t)

            def j_wo_wait():
                with jax.named_scope("sc_wo_finish"):
                    pl.when(t == 0)(wo_finish)
            _run(_interleave(ej, {after_qkv: [j_wo_wait]}) + _interleave(oj, {after_qkv: [j_next_xn]}))
            return carry

        def fused(t, carry):
            @pl.when(t == LAG)
            def _():
                x_rest_copy().wait()

            @pl.when(t > LAG)
            def _():
                out_copy(t - LAG - 1).start()

            ej, oj, j_next_xn = attention_jobs(t)
            b = mlp_jobs(t - LAG)
            w3, w4 = b['w3'], b['w4']
            fe, fo = {}, {}

            def put(d, label, *jobs):
                d.setdefault(label, []).extend(jobs)
            for i in range(nD):
                put(fe, ('qkv', 2 + i // 2, i % 2), b['w1'][i])
                put(fe, ('qkv', 8 + i // 2, i % 2), b['w2'][i])
            put(fe, ('qkv', 6, 0), b['shift'])
            put(fe, ('qkv', 12, 0), b['ln3'])
            put(fe, ('qkv', 15, 0), w3[0])
            put(fe, 'end', *w3[1:4])
            put(fo, ('qkv', 0, 1), b['pre_next'])
            for k in range(4, nF):
                put(fo, ('qkv', 1 + (k - 4) // 2, (k - 4) % 2), w3[k])
            put(fo, ('qkv', 13, 0), b['cat'])
            put(fo, ('qkv', 14, 0), w4[0])
            put(fo, ('qkv', 15, 0), w4[1])
            put(fo, after_qkv, j_next_xn)
            put(fo, ('s', n_slots - 1), w4[2])
            put(fo, 'end', *w4[3:])
            with jax.named_scope("sc_fused_body"):
                _run(_interleave(ej, fe) + _interleave(oj, fo))
            return carry

        def mlp_only(c, carry):
            out_copy(c - 1).start()
            b = mlp_jobs(c)
            _run(b['w1'] + [b['shift']] + b['w2'] + [b['ln3'], b['pre_next']] + b['w3'] + [b['cat']] + b['w4'])
            return carry

        with jax.named_scope("sc_prologue"):
            prologue()
            store_xn(0)
        with jax.named_scope("sc_a_only"):
            jax.lax.fori_loop(0, LAG, attention_only, 0)
        with jax.named_scope("sc_mlp_prologue"):
            mlp_prologue()
        with jax.named_scope("sc_fused"):
            jax.lax.fori_loop(LAG, n_pairs, fused, 0)
        with jax.named_scope("sc_b_tail"):
            jax.lax.fori_loop(n_pairs - LAG, n_pairs, mlp_only, 0)
        out_copy(n_pairs - 1).start()
        pltpu.make_async_copy(out_v, out_hbm, sems.at[OUT_SEM]).wait()

    return kernel, WO_SEM + nD + 6, X0


@functools.partial(jax.jit, static_argnames=("A_seg_len",))
def pallas_sequential_preLN__memory_aug_recurrent_mem_tr__mixer_s_mlp__prompt_kernel(
    A_x, A_mem0, A_Wq, A_Wk, A_Wv, A_Wo, A_seg_len, B_x, B_w1, B_w2, B_w3, B_w4,
):
    _, S, D = A_x.shape
    H, E = A_Wq.shape[1], A_Wq.shape[2]
    F = B_w3.shape[1]
    assert A_seg_len == SEG and A_mem0.shape[1] == MEM and S % PAIR == 0
    nD, nF = D // 128, F // 128

    x = A_x.reshape(S, D)
    mem0 = A_mem0.reshape(MEM, D)
    wo = A_Wo.reshape(H * E, D)

    kernel, n_sems, x0 = _make_kernel(S, D, H, E, F)
    any_spec = pl.BlockSpec(memory_space=pl.ANY)
    out = pl.pallas_call(
        kernel,
        in_specs=[any_spec] * 10,
        out_specs=any_spec,
        out_shape=jax.ShapeDtypeStruct((S, D), A_x.dtype),
        scratch_shapes=[
            pltpu.VMEM((3, D, H, E), BF),
            pltpu.VMEM((3, H, D // 2, E), U32),
            pltpu.VMEM((H * E, D), BF),
            pltpu.VMEM((nD, H * E // 2, 128), U32),
            pltpu.VMEM((nD, D, 128), BF),
            pltpu.VMEM((nD, D, 128), BF),
            pltpu.VMEM((nF, D, 128), BF),
            pltpu.VMEM((nD, F, 128), BF),
            pltpu.VMEM((S, D), BF),
            pltpu.VMEM((S, D), BF),
            pltpu.VMEM((MEM, D), BF),
            pltpu.VMEM((x0 // 2, D), U32),
            pltpu.VMEM((S // 2, H * E), U32),
            pltpu.VMEM((16, D), U32),
            pltpu.VMEM((16, D), U32),
            pltpu.VMEM((24, D), U32),
            pltpu.VMEM((16, D), U32),
            pltpu.VMEM((3, 8, H * E), F32),
            pltpu.VMEM((40, H * E), U32),
            pltpu.VMEM((48, D), F32),
            pltpu.VMEM((S + 2 * HALO, D), F32),
            pltpu.VMEM((PAIR + 2 * HALO, D), F32),
            pltpu.VMEM((PAIR, D), F32),
            pltpu.VMEM((PAIR // 2, D), U32),
            pltpu.SemaphoreType.DMA((n_sems,)),
        ],
        compiler_params=pltpu.CompilerParams(
            vmem_limit_bytes=124 * 1024 * 1024,
            disable_bounds_checks=True,
        ),
    )(x, mem0, A_Wq, A_Wk, A_Wv, wo, B_w1, B_w2, B_w3, B_w4)
    return out.reshape(1, S, D)
```

```python
import functools

import jax
import jax.numpy as jnp
from jax.experimental import pallas as pl
from jax.experimental.pallas import tpu as pltpu

BF = jnp.bfloat16
F32 = jnp.float32
U32 = jnp.uint32

SEG = 32
MEM = 8
PAIR = 2 * SEG
LAG = 3
HALO = 8
G = 2
TAIL_HEADS = 6
QR = 24
NCH = 8
LN_EPS = 1e-5
LOG2E = 1.4426950408889634


def _ln(x):
    m = jnp.mean(x, axis=-1, keepdims=True)
    xc = x - m
    v = jnp.mean(xc * xc, axis=-1, keepdims=True)
    return xc * jax.lax.rsqrt(v + LN_EPS)


_dot = functools.partial(jnp.dot, preferred_element_type=F32)


def _gelu(x):
    return jax.nn.gelu(x, approximate=True)


def _as_bf(x_u32):
    return pltpu.bitcast(x_u32, BF)


def _as_u32(x_bf):
    return pltpu.bitcast(x_bf, U32)


def _interleave(main, fill):
    fill = dict(fill)
    out = []
    for label, job in main:
        out.extend(fill.pop(label, []))
        out.append(job)
    out.extend(fill.pop('end', []))
    assert not fill, fill
    return out


def _run(jobs):
    for job in jobs:
        job()


def _make_kernel(S, D, H, E, F):
    n_pairs = S // PAIR
    nD = D // 128
    nF = F // 128
    scale = float(E) ** -0.5
    L = MEM + SEG
    n_slots = H // G
    K1 = (H - TAIL_HEADS) * E
    CH = D // NCH
    WO_CH = H * E // nD
    X0 = S - 2 * QR * n_pairs
    assert X0 % PAIR == 0 and X0 // PAIR - 1 >= LAG and X0 < S
    assert G == 2 and n_slots == 16 and nF == 28 and nD == 8
    assert (H - TAIL_HEADS) // G - 1 < n_slots - 2

    WO_SEM = 3 * NCH
    B_SEM, X0_SEM, XM_SEM, X1_SEM, MEM_SEM, OUT_SEM = (WO_SEM + nD + i for i in range(6))
    XA = X0 + 2 * QR
    XB = X0 + 2 * QR * (LAG + 1)

    def kernel(x_hbm, mem0_hbm, wq_hbm, wk_hbm, wv_hbm, wo_hbm, w1_hbm, w2_hbm, w3_hbm, w4_hbm,
               out_hbm,
               raw, w_t, wo_raw, wo_t, w1_t, w2_t, w3_t, w4_t,
               x_v, out_v, mem0_v, xn0, q_buf, lq_e, lq_o, lb_e, lb_o, sv, ob, wacc,
               h_buf, a1_buf, y_buf, z_buf, sems):

        def rows_copy(src, dst, start, size, sem):
            return pltpu.make_async_copy(src.at[pl.ds(start, size)], dst.at[pl.ds(start, size)], sems.at[sem])

        def raw_copy(i, c):
            src = (wq_hbm, wk_hbm, wv_hbm)[i]
            return rows_copy(src, raw.at[i], c * CH, CH, i * NCH + c)

        def wo_copy(j):
            return rows_copy(wo_hbm, wo_raw, j * WO_CH, WO_CH, WO_SEM + j)

        def mlp_weight_copies():
            return [pltpu.make_async_copy(src.at[:, pl.ds(j * 128, 128)], dst.at[j], sems.at[B_SEM])
                    for src, dst, n in ((w1_hbm, w1_t, nD), (w2_hbm, w2_t, nD),
                                        (w3_hbm, w3_t, nF), (w4_hbm, w4_t, nD))
                    for j in range(n)]

        def x_head_copy():
            return rows_copy(x_hbm, x_v, 0, XA, X0_SEM)

        def x_mid_copy():
            return rows_copy(x_hbm, x_v, XA, XB - XA, XM_SEM)

        def x_rest_copy():
            return rows_copy(x_hbm, x_v, XB, S - XB, X1_SEM)

        def mem_copy():
            return pltpu.make_async_copy(mem0_hbm, mem0_v, sems.at[MEM_SEM])

        def out_copy(c):
            return rows_copy(out_v, out_hbm, pl.multiple_of(c * PAIR, PAIR), PAIR, OUT_SEM)

        def relayout_part(i, b, h0, nh):
            x = raw[i, pl.ds(pl.multiple_of(b * 16, 16), 16), pl.ds(h0, nh), :]
            x = _as_u32(x).reshape(8, 2, nh // 2, E)
            ev, od = x[:, 0], x[:, 1]
            lo = jnp.swapaxes((ev & 0xFFFF) | (od << 16), 0, 1)
            hi = jnp.swapaxes((ev >> 16) | (od & jnp.uint32(0xFFFF0000)), 0, 1)
            rows = pl.ds(pl.multiple_of(b * 8, 8), 8)
            for p in range(nh // 2):
                w_t[i, h0 + 2 * p, rows, :] = lo[p]
                w_t[i, h0 + 2 * p + 1, rows, :] = hi[p]

        def relayout_block(i, b):
            relayout_part(i, b, 0, H)

        def wo_finish():
            for j in range(nD):
                wo_copy(j).wait()

                def body(b, carry):
                    r = j * WO_CH + b * 256
                    for m in range(4):
                        blk = wo_raw[pl.ds(pl.multiple_of(r + m * 64, 64), 64), :]
                        for n in range(nD):
                            wo_t[n, pl.ds(pl.multiple_of((r + m * 64) // 2, 32), 32), :] = _as_u32(
                                blk[:, n * 128:(n + 1) * 128])
                    return carry
                jax.lax.fori_loop(0, WO_CH // 256, body, 0)
            x_mid_copy().wait()

        def store_xn(t):
            xn = _ln(x_v[pl.ds(pl.multiple_of(t * PAIR, PAIR), PAIR), :].astype(F32))
            lb_e[pl.ds(0, 4), :] = _as_u32(xn[32:40].astype(BF))
            lb_e[pl.ds(4, 4), :] = _as_u32(xn[0:8].astype(BF))
            lb_e[pl.ds(8, 8), :] = _as_u32(xn[8:24].astype(BF))
            lb_e[pl.ds(16, 4), :] = _as_u32(xn[24:32].astype(BF))
            lb_o[pl.ds(0, 8), :] = _as_u32(xn[40:56].astype(BF))
            lb_o[pl.ds(8, 4), :] = _as_u32(xn[56:64].astype(BF))
            xq = _ln(x_v[pl.ds(pl.multiple_of(X0 + t * 2 * QR, 16), 2 * QR), :].astype(F32))
            lq_e[pl.ds(0, 8), :] = _as_u32(xq[0:16].astype(BF))
            lq_e[pl.ds(8, 4), :] = _as_u32(xq[16:24].astype(BF))
            for n in range(3):
                lq_o[pl.ds(4 * n, 4), :] = _as_u32(xq[24 + 8 * n:32 + 8 * n].astype(BF))

        def prologue():
            x_head_copy().start()
            mem_copy().start()
            for i in range(3):
                for c in range(NCH):
                    raw_copy(i, c).start()
            for j in range(nD):
                wo_copy(j).start()
            x_mid_copy().start()
            h_buf[pl.ds(0, HALO), :] = jnp.zeros((HALO, D), F32)
            h_buf[pl.ds(HALO + S, HALO), :] = jnp.zeros((HALO, D), F32)
            x_head_copy().wait()
            mem_copy().wait()
            lb_e[pl.ds(20, 4), :] = _as_u32(mem0_v[...])
            lq_e[pl.ds(12, 4), :] = _as_u32(mem0_v[...])

            def ln_body(b, carry):
                rows = x_v[pl.ds(pl.multiple_of(b * 64, 64), 64), :].astype(F32)
                xn0[pl.ds(pl.multiple_of(b * 32, 32), 32), :] = _as_u32(_ln(rows).astype(BF))
                return carry
            jax.lax.fori_loop(0, X0 // 64, ln_body, 0)

            with jax.named_scope("sc_wq"):
                def q_chunk(c, carry):
                    dst = raw.at[0, pl.ds(c * CH, CH)]
                    pltpu.make_async_copy(dst, dst, sems.at[c]).wait()

                    def q_body(b, carry):
                        relayout_block(0, b)
                        return carry
                    return jax.lax.fori_loop(c * (CH // 16), (c + 1) * (CH // 16), q_body, carry)
                jax.lax.fori_loop(0, NCH, q_chunk, 0)

            HP = 2
            per_head = 2 * (D // 16) // H
            it_per_chunk = H // HP // (2 * NCH)
            assert it_per_chunk * HP * per_head * 16 == CH

            def kv_body(it, carry):
                i = 1 + it // (H // HP // 2)

                @pl.when(it % it_per_chunk == 0)
                def _():
                    n = it // it_per_chunk
                    dst = raw.at[i, pl.ds((n % NCH) * CH, CH)]
                    pltpu.make_async_copy(dst, dst, sems.at[NCH + n]).wait()
                NPC = 8
                rows = X0 // 2 // NPC
                for k in range(HP):
                    h = it * HP + k
                    for n in range(NPC):
                        q = _dot(_as_bf(xn0[pl.ds(n * rows, rows), :]), _as_bf(w_t[0, h]))
                        q_buf[pl.ds(n * rows, rows), pl.ds(pl.multiple_of(h * E, E), E)] = _as_u32(q.astype(BF))
                        relayout_part(i, (h % (H // 2)) * per_head + n // 2, (n % 2) * (H // 2), H // 2)
                return carry
            with jax.named_scope("sc_kv"):
                jax.lax.fori_loop(0, H // HP, kv_body, 0)

            for c in mlp_weight_copies():
                c.start()
            x_rest_copy().start()

        def mlp_pre(c):
            a1_buf[pl.ds(0, 2 * HALO), :] = a1_buf[pl.ds(PAIR, 2 * HALO), :]
            y = _ln(h_buf[pl.ds(pl.multiple_of(c * PAIR + HALO, 8), PAIR + HALO), :])
            y_buf[...] = y[0:PAIR]
            z_buf[...] = _as_u32(_ln(y[HALO:]).astype(BF))

        def mlp_prologue():
            for c in mlp_weight_copies():
                c.wait()
            z = _ln(_ln(h_buf[pl.ds(0, 2 * HALO), :])).astype(BF)
            tok = jax.lax.broadcasted_iota(jnp.int32, (2 * HALO, 128), 0) - HALO
            for j in range(nD):
                a1_buf[pl.ds(PAIR, 2 * HALO), pl.ds(j * 128, 128)] = jnp.where(
                    tok >= 0, _gelu(_dot(z, w1_t[j])), 0.0)
            mlp_pre(0)

        def attention_jobs(t):
            row = jax.lax.broadcasted_iota(jnp.int32, (G * L, G * L), 0)
            col = jax.lax.broadcasted_iota(jnp.int32, (G * L, G * L), 1)

            def head_of(r):
                return jnp.where(r < G * SEG, r // SEG, (r - G * SEG) // MEM)
            mask = (head_of(row) == head_of(col)) & ((col >= G * SEG) | (row >= G * SEG) | (col <= row))
            x0 = t * PAIR
            h0 = x0 + HALO

            def step_jobs(even):
                lb = lb_e if even else lb_o
                st = {}

                lq = lq_e if even else lq_o
                q_new = pl.multiple_of(X0 // 2 + t * QR, 8)
                q_use = t * SEG + (0 if even else SEG // 2)

                def j_qkv(g, i):
                    def run():
                        h = g * G + i
                        cs = pl.ds(h * E, E)
                        q = _dot(_as_bf(lq[...]), _as_bf(w_t[0, h]))
                        if even:
                            q_buf[pl.ds(q_new, 8), cs] = _as_u32(q[0:16].astype(BF))
                            sv[2, :, cs] = q[16:24]
                        else:
                            q_buf[pl.ds(q_new + 8, 16), cs] = _as_u32(
                                jnp.concatenate([sv[2, :, cs], q[0:QR]], axis=0).astype(BF))
                        lhs = _as_bf(lb[...])
                        kv = [_dot(lhs, _as_bf(w_t[n, h])) for n in (1, 2)]
                        parts = st.setdefault(('parts', g), dict(qx=[], qm=[], x=[[], []], m=[[], []]))
                        parts['qx'].append(_as_bf(q_buf[pl.ds(pl.multiple_of(q_use, 16), SEG // 2), cs]))
                        parts['qm'].append(q[QR:QR + MEM])
                        for n in range(2):
                            if even:
                                sv[n, :, cs] = kv[n][0:8]
                                parts['x'][n].append(kv[n][8:40])
                                parts['m'][n].append(kv[n][40:48])
                            else:
                                parts['x'][n] += [sv[n, :, cs], kv[n][0:24]]
                                parts['m'][n].append(kv[n][24:32])
                        if i == G - 1:
                            parts = st.pop(('parts', g))
                            q2 = jnp.concatenate(
                                parts['qx'] + [jnp.concatenate(parts['qm'], axis=0).astype(BF)], axis=0)
                            st['qkv', g] = [q2] + [
                                jnp.concatenate(parts['x'][n] + parts['m'][n], axis=0).astype(BF)
                                for n in range(2)]
                    return run

                def j_scores(g):
                    def run():
                        q, k, v = st.pop(('qkv', g))
                        s = jax.lax.dot_general(q, k, (((1,), (1,)), ((), ())),
                                                preferred_element_type=F32)
                        s = jnp.where(mask, s, -1000000000.0 / scale)
                        m = jnp.max(s, axis=-1, keepdims=True)
                        p = jnp.exp2((s - m) * (scale * LOG2E))
                        l = jnp.sum(p, axis=-1, keepdims=True)
                        r0 = pl.reciprocal(l, approx=True)
                        p = p * (r0 * (2.0 - l * r0))
                        st['p', g] = (p.astype(BF), v)
                    return run

                def j_pv(g):
                    def run():
                        p, v = st.pop(('p', g))
                        o2 = _dot(p, v)
                        for i, h in enumerate(range(g * G, (g + 1) * G)):
                            ox = o2[i * SEG:(i + 1) * SEG]
                            om = o2[G * SEG + i * MEM:G * SEG + (i + 1) * MEM]
                            cs = pl.ds(h * E, E)
                            if even:
                                ob[pl.ds(16, 4), cs] = _as_u32(ox[0:8].astype(BF))
                                ob[pl.ds(0, 16), cs] = _as_u32(
                                    jnp.concatenate([ox[8:32], om], axis=0).astype(BF))
                            else:
                                ob[pl.ds(20, 4), cs] = _as_u32(ox[0:8].astype(BF))
                                ob[pl.ds(24, 16), cs] = _as_u32(
                                    jnp.concatenate([ox[8:32], om], axis=0).astype(BF))
                    return run

                rows = pl.ds(0, 16) if even else pl.ds(16, 24)
                nrows = 32 if even else 48

                def j_wo1(j):
                    def run():
                        lhs = _as_bf(ob[rows, pl.ds(0, K1)])
                        wacc[pl.ds(0, nrows), pl.ds(j * 128, 128)] = _dot(
                            lhs, _as_bf(wo_t[j, pl.ds(0, K1 // 2), :]))
                    return run

                def j_wo2(j):
                    def run():
                        lhs = _as_bf(ob[rows, pl.ds(K1, H * E - K1)])
                        r = wacc[pl.ds(0, nrows), pl.ds(j * 128, 128)] + _dot(
                            lhs, _as_bf(wo_t[j, pl.ds(K1 // 2, (H * E - K1) // 2), :]))
                        cs = pl.ds(j * 128, 128)
                        xs = x_v[pl.ds(pl.multiple_of(x0, PAIR), PAIR), cs].astype(F32)
                        if even:
                            mem = _as_u32(r[24:32].astype(BF))
                            lb_o[pl.ds(12, 4), cs] = mem
                            lq_o[pl.ds(12, 4), cs] = mem
                            h_buf[pl.ds(pl.multiple_of(h0 + 8, 8), 24), cs] = xs[8:32] + r[0:24]
                        else:
                            mem = _as_u32(r[40:48].astype(BF))
                            lb_e[pl.ds(20, 4), cs] = mem
                            lq_e[pl.ds(12, 4), cs] = mem
                            h_buf[pl.ds(pl.multiple_of(h0, 8), 8), cs] = xs[0:8] + r[0:8]
                            h_buf[pl.ds(pl.multiple_of(h0 + 32, 8), 32), cs] = xs[32:64] + r[8:40]
                    return run

                last = n_slots - 1
                jobs = []
                for g in range(n_slots):
                    for i in range(G):
                        jobs.append((('qkv', g, i), j_qkv(g, i)))
                    if g >= 1:
                        jobs.append((('s', g - 1), j_scores(g - 1)))
                    if g >= 2:
                        jobs.append((('pv', g - 2), j_pv(g - 2)))
                wo1 = [(('wo1', j), j_wo1(j)) for j in range(nD)]
                jobs += (wo1[0:3] + [(('s', last), j_scores(last)), (('pv', last - 1), j_pv(last - 1))]
                         + wo1[3:6] + [(('pv', last), j_pv(last))] + wo1[6:8])
                jobs += [(('wo2', j), j_wo2(j)) for j in range(nD)]
                return jobs

            def j_next_xn():
                store_xn(jnp.minimum(t + 1, n_pairs - 1))

            return step_jobs(True), step_jobs(False), j_next_xn

        after_qkv = ('s', n_slots - 2)

        def mlp_jobs(c):
            r0 = pl.multiple_of(c * PAIR, PAIR)
            st = {}

            def j_pre_next():
                mlp_pre(jnp.minimum(c + 1, n_pairs - 1))

            def j_w1(j):
                def run():
                    tok = jax.lax.broadcasted_iota(jnp.int32, (PAIR, 128), 0) + (r0 + HALO)
                    a = _gelu(_dot(_as_bf(z_buf[...]), w1_t[j]))
                    a1_buf[pl.ds(2 * HALO, PAIR), pl.ds(j * 128, 128)] = jnp.where(tok < S, a, 0.0)
                return run

            def j_shift():
                cq = D // 4
                st['g'] = jnp.concatenate([
                    a1_buf[pl.ds(HALO - 1, PAIR), pl.ds(0 * cq, cq)],
                    a1_buf[pl.ds(HALO + 1, PAIR), pl.ds(1 * cq, cq)],
                    a1_buf[pl.ds(HALO - 2, PAIR), pl.ds(2 * cq, cq)],
                    a1_buf[pl.ds(HALO + 2, PAIR), pl.ds(3 * cq, cq)]], axis=1).astype(BF)

            def j_w2(j):
                def run():
                    st['x1', j] = y_buf[:, pl.ds(j * 128, 128)] + _dot(st['g'], w2_t[j])
                return run

            def j_ln3():
                x1 = jnp.concatenate([st['x1', j] for j in range(nD)], axis=1)
                st['z1'] = _ln(x1).astype(BF)

            def j_w3(j):
                def run():
                    st['a3', j] = _gelu(_dot(st['z1'], w3_t[j])).astype(BF)
                return run

            def j_cat():
                st['a3'] = jnp.concatenate([st.pop(('a3', j)) for j in range(nF)], axis=1)

            def j_w4(j):
                def run():
                    cs = pl.ds(j * 128, 128)
                    hh = h_buf[pl.ds(pl.multiple_of(r0 + HALO, 8), PAIR), cs]
                    out_v[pl.ds(r0, PAIR), cs] = (
                        hh + (st['x1', j] + _dot(st['a3'], w4_t[j]))).astype(out_v.dtype)
                return run

            return dict(pre_next=j_pre_next, w1=[j_w1(j) for j in range(nD)], shift=j_shift,
                        w2=[j_w2(j) for j in range(nD)], ln3=j_ln3,
                        w3=[j_w3(j) for j in range(nF)], cat=j_cat,
                        w4=[j_w4(j) for j in range(nD)])

        def attention_only(t, carry):
            ej, oj, j_next_xn = attention_jobs(t)

            def j_wo_wait():
                with jax.named_scope("sc_wo_finish"):
                    pl.when(t == 0)(wo_finish)
            _run(_interleave(ej, {after_qkv: [j_wo_wait]}) + _interleave(oj, {after_qkv: [j_next_xn]}))
            return carry

        def fused(t, carry):
            @pl.when(t == LAG)
            def _():
                x_rest_copy().wait()

            @pl.when(t > LAG)
            def _():
                out_copy(t - LAG - 1).start()

            ej, oj, j_next_xn = attention_jobs(t)
            b = mlp_jobs(t - LAG)
            w3, w4 = b['w3'], b['w4']
            fe, fo = {}, {}

            def put(d, label, *jobs):
                d.setdefault(label, []).extend(jobs)
            for i in range(nD):
                put(fe, ('qkv', 2 + i // 2, i % 2), b['w1'][i])
                put(fe, ('qkv', 8 + i // 2, i % 2), b['w2'][i])
            put(fe, ('qkv', 6, 0), b['shift'])
            put(fe, ('qkv', 12, 0), b['ln3'])
            put(fe, ('qkv', 15, 0), w3[0])
            put(fe, 'end', *w3[1:4])
            put(fo, ('qkv', 0, 1), b['pre_next'])
            for k in range(4, nF):
                put(fo, ('qkv', 1 + (k - 4) // 2, (k - 4) % 2), w3[k])
            put(fo, ('qkv', 13, 0), b['cat'])
            put(fo, ('qkv', 14, 0), w4[0])
            put(fo, ('qkv', 15, 0), w4[1])
            put(fo, after_qkv, j_next_xn)
            put(fo, ('s', n_slots - 1), w4[2])
            put(fo, 'end', *w4[3:])
            with jax.named_scope("sc_fused_body"):
                _run(_interleave(ej, fe) + _interleave(oj, fo))
            return carry

        def mlp_only(c, carry):
            out_copy(c - 1).start()
            b = mlp_jobs(c)
            _run(b['w1'] + [b['shift']] + b['w2'] + [b['ln3'], b['pre_next']] + b['w3'] + [b['cat']] + b['w4'])
            return carry

        with jax.named_scope("sc_prologue"):
            prologue()
            store_xn(0)
        with jax.named_scope("sc_a_only"):
            jax.lax.fori_loop(0, LAG, attention_only, 0)
        with jax.named_scope("sc_mlp_prologue"):
            mlp_prologue()
        with jax.named_scope("sc_fused"):
            jax.lax.fori_loop(LAG, n_pairs, fused, 0)
        with jax.named_scope("sc_b_tail"):
            jax.lax.fori_loop(n_pairs - LAG, n_pairs, mlp_only, 0)
        out_copy(n_pairs - 1).start()
        pltpu.make_async_copy(out_v, out_hbm, sems.at[OUT_SEM]).wait()

    return kernel, WO_SEM + nD + 6, X0


@functools.partial(jax.jit, static_argnames=("A_seg_len",))
def pallas_sequential_preLN__memory_aug_recurrent_mem_tr__mixer_s_mlp__prompt_kernel(
    A_x, A_mem0, A_Wq, A_Wk, A_Wv, A_Wo, A_seg_len, B_x, B_w1, B_w2, B_w3, B_w4,
):
    _, S, D = A_x.shape
    H, E = A_Wq.shape[1], A_Wq.shape[2]
    F = B_w3.shape[1]
    assert A_seg_len == SEG and A_mem0.shape[1] == MEM and S % PAIR == 0
    nD, nF = D // 128, F // 128

    x = A_x.reshape(S, D)
    mem0 = A_mem0.reshape(MEM, D)
    wo = A_Wo.reshape(H * E, D)

    kernel, n_sems, x0 = _make_kernel(S, D, H, E, F)
    any_spec = pl.BlockSpec(memory_space=pl.ANY)
    out = pl.pallas_call(
        kernel,
        in_specs=[any_spec] * 10,
        out_specs=any_spec,
        out_shape=jax.ShapeDtypeStruct((S, D), A_x.dtype),
        scratch_shapes=[
            pltpu.VMEM((3, D, H, E), BF),
            pltpu.VMEM((3, H, D // 2, E), U32),
            pltpu.VMEM((H * E, D), BF),
            pltpu.VMEM((nD, H * E // 2, 128), U32),
            pltpu.VMEM((nD, D, 128), BF),
            pltpu.VMEM((nD, D, 128), BF),
            pltpu.VMEM((nF, D, 128), BF),
            pltpu.VMEM((nD, F, 128), BF),
            pltpu.VMEM((S, D), BF),
            pltpu.VMEM((S, D), BF),
            pltpu.VMEM((MEM, D), BF),
            pltpu.VMEM((x0 // 2, D), U32),
            pltpu.VMEM((S // 2, H * E), U32),
            pltpu.VMEM((16, D), U32),
            pltpu.VMEM((16, D), U32),
            pltpu.VMEM((24, D), U32),
            pltpu.VMEM((16, D), U32),
            pltpu.VMEM((3, 8, H * E), F32),
            pltpu.VMEM((40, H * E), U32),
            pltpu.VMEM((48, D), F32),
            pltpu.VMEM((S + 2 * HALO, D), F32),
            pltpu.VMEM((PAIR + 2 * HALO, D), F32),
            pltpu.VMEM((PAIR, D), F32),
            pltpu.VMEM((PAIR // 2, D), U32),
            pltpu.SemaphoreType.DMA((n_sems,)),
        ],
        compiler_params=pltpu.CompilerParams(
            vmem_limit_bytes=124 * 1024 * 1024,
            disable_bounds_checks=True,
        ),
    )(x, mem0, A_Wq, A_Wk, A_Wv, wo, B_w1, B_w2, B_w3, B_w4)
    return out.reshape(1, S, D)
```

```python
import functools

import jax
import jax.numpy as jnp
from jax.experimental import pallas as pl
from jax.experimental.pallas import tpu as pltpu

BF = jnp.bfloat16
F32 = jnp.float32
U32 = jnp.uint32

SEG = 32
MEM = 8
PAIR = 2 * SEG
LAG = 3
HALO = 8
G = 2
TAIL_HEADS = 6
QR = 24
NK = 8
NCH = 8
LN_EPS = 1e-5
LOG2E = 1.4426950408889634


def _ln(x):
    m = jnp.mean(x, axis=-1, keepdims=True)
    xc = x - m
    v = jnp.mean(xc * xc, axis=-1, keepdims=True)
    return xc * jax.lax.rsqrt(v + LN_EPS)


_dot = functools.partial(jnp.dot, preferred_element_type=F32)


def _gelu(x):
    return jax.nn.gelu(x, approximate=True)


def _as_bf(x_u32):
    return pltpu.bitcast(x_u32, BF)


def _as_u32(x_bf):
    return pltpu.bitcast(x_bf, U32)


def _interleave(main, fill):
    fill = dict(fill)
    out = []
    for label, job in main:
        out.extend(fill.pop(label, []))
        out.append(job)
    out.extend(fill.pop('end', []))
    assert not fill, fill
    return out


def _run(jobs):
    for job in jobs:
        job()


def _make_kernel(S, D, H, E, F):
    n_pairs = S // PAIR
    nD = D // 128
    nF = F // 128
    scale = float(E) ** -0.5
    L = MEM + SEG
    n_slots = H // G
    K1 = (H - TAIL_HEADS) * E
    CH = D // NCH
    WO_CH = H * E // nD
    X0 = S - 2 * QR * n_pairs
    assert X0 % PAIR == 0 and X0 // PAIR - 1 >= LAG and X0 < S
    RING = (X0 + PAIR) // 2
    assert RING % 16 == 0 and NK % G == 0
    assert G == 2 and n_slots == 16 and nF == 28 and nD == 8
    assert (H - TAIL_HEADS) // G - 1 < n_slots - 2

    WO_SEM = 3 * NCH
    B_SEM, X0_SEM, XM_SEM, X1_SEM, MEM_SEM, OUT_SEM = (WO_SEM + nD + i for i in range(6))
    XA = X0 + 2 * QR
    XB = X0 + 2 * QR * (LAG + 1)

    def kernel(x_hbm, mem0_hbm, wq_hbm, wk_hbm, wv_hbm, wo_hbm, w1_hbm, w2_hbm, w3_hbm, w4_hbm,
               out_hbm,
               raw, w_t, wo_raw, wo_t, w1_t, w2_t, w3_t, w4_t,
               x_v, out_v, mem0_v, xn0, ah_buf, lq_e, lq_o, lb_e, lb_o, sv, ob, wacc,
               h_buf, a1_buf, y_buf, z_buf, sems):

        def rows_copy(src, dst, start, size, sem):
            return pltpu.make_async_copy(src.at[pl.ds(start, size)], dst.at[pl.ds(start, size)], sems.at[sem])

        def raw_copy(i, c):
            src = (wq_hbm, wk_hbm, wv_hbm)[i]
            return rows_copy(src, raw.at[i], c * CH, CH, i * NCH + c)

        def wo_copy(j):
            return rows_copy(wo_hbm, wo_raw, j * WO_CH, WO_CH, WO_SEM + j)

        def mlp_weight_copies():
            return [pltpu.make_async_copy(src.at[:, pl.ds(j * 128, 128)], dst.at[j], sems.at[B_SEM])
                    for src, dst, n in ((w1_hbm, w1_t, nD), (w2_hbm, w2_t, nD),
                                        (w3_hbm, w3_t, nF), (w4_hbm, w4_t, nD))
                    for j in range(n)]

        def x_head_copy():
            return rows_copy(x_hbm, x_v, 0, XA, X0_SEM)

        def x_mid_copy():
            return rows_copy(x_hbm, x_v, XA, XB - XA, XM_SEM)

        def x_rest_copy():
            return rows_copy(x_hbm, x_v, XB, S - XB, X1_SEM)

        def mem_copy():
            return pltpu.make_async_copy(mem0_hbm, mem0_v, sems.at[MEM_SEM])

        def out_copy(c):
            return rows_copy(out_v, out_hbm, pl.multiple_of(c * PAIR, PAIR), PAIR, OUT_SEM)

        def relayout_part(i, b, h0, nh):
            x = raw[i, pl.ds(pl.multiple_of(b * 16, 16), 16), pl.ds(h0, nh), :]
            x = _as_u32(x).reshape(8, 2, nh // 2, E)
            ev, od = x[:, 0], x[:, 1]
            lo = jnp.swapaxes((ev & 0xFFFF) | (od << 16), 0, 1)
            hi = jnp.swapaxes((ev >> 16) | (od & jnp.uint32(0xFFFF0000)), 0, 1)
            rows = pl.ds(pl.multiple_of(b * 8, 8), 8)
            for p in range(nh // 2):
                w_t[i, h0 + 2 * p, rows, :] = lo[p]
                w_t[i, h0 + 2 * p + 1, rows, :] = hi[p]

        def relayout_block(i, b):
            relayout_part(i, b, 0, H)

        def wo_finish():
            for j in range(nD):
                wo_copy(j).wait()

                def body(b, carry):
                    r = j * WO_CH + b * 256
                    for m in range(4):
                        blk = wo_raw[pl.ds(pl.multiple_of(r + m * 64, 64), 64), :]
                        for n in range(nD):
                            wo_t[n, pl.ds(pl.multiple_of((r + m * 64) // 2, 32), 32), :] = _as_u32(
                                blk[:, n * 128:(n + 1) * 128])
                    return carry
                jax.lax.fori_loop(0, WO_CH // 256, body, 0)
            x_mid_copy().wait()

        def store_xn(t):
            xn = _ln(x_v[pl.ds(pl.multiple_of(t * PAIR, PAIR), PAIR), :].astype(F32))
            lb_e[pl.ds(0, 4), :] = _as_u32(xn[32:40].astype(BF))
            lb_e[pl.ds(4, 4), :] = _as_u32(xn[0:8].astype(BF))
            lb_e[pl.ds(8, 8), :] = _as_u32(xn[8:24].astype(BF))
            lb_e[pl.ds(16, 4), :] = _as_u32(xn[24:32].astype(BF))
            lb_o[pl.ds(0, 8), :] = _as_u32(xn[40:56].astype(BF))
            lb_o[pl.ds(8, 4), :] = _as_u32(xn[56:64].astype(BF))
            xq = _ln(x_v[pl.ds(pl.multiple_of(X0 + t * 2 * QR, 16), 2 * QR), :].astype(F32))
            lq_e[pl.ds(0, 8), :] = _as_u32(xq[0:16].astype(BF))
            lq_e[pl.ds(8, 4), :] = _as_u32(xq[16:24].astype(BF))
            for n in range(3):
                lq_o[pl.ds(4 * n, 4), :] = _as_u32(xq[24 + 8 * n:32 + 8 * n].astype(BF))

        def prologue():
            x_head_copy().start()
            mem_copy().start()
            for i in range(3):
                for c in range(NCH):
                    raw_copy(i, c).start()
            for j in range(nD):
                wo_copy(j).start()
            x_mid_copy().start()
            h_buf[pl.ds(0, HALO), :] = jnp.zeros((HALO, D), F32)
            h_buf[pl.ds(HALO + S, HALO), :] = jnp.zeros((HALO, D), F32)
            x_head_copy().wait()
            mem_copy().wait()
            lb_e[pl.ds(20, 4), :] = _as_u32(mem0_v[...])
            lq_e[pl.ds(12, 4), :] = _as_u32(mem0_v[...])

            def ln_body(b, carry):
                rows = x_v[pl.ds(pl.multiple_of(b * 64, 64), 64), :].astype(F32)
                xn0[pl.ds(pl.multiple_of(b * 32, 32), 32), :] = _as_u32(_ln(rows).astype(BF))
                return carry
            jax.lax.fori_loop(0, X0 // 64, ln_body, 0)

            with jax.named_scope("sc_wq"):
                def q_chunk(c, carry):
                    dst = raw.at[0, pl.ds(c * CH, CH)]
                    pltpu.make_async_copy(dst, dst, sems.at[c]).wait()

                    def q_body(b, carry):
                        relayout_block(0, b)
                        return carry
                    return jax.lax.fori_loop(c * (CH // 16), (c + 1) * (CH // 16), q_body, carry)
                jax.lax.fori_loop(0, NCH, q_chunk, 0)

            HP = 2
            per_head = 2 * (D // 16) // H
            it_per_chunk = H // HP // (2 * NCH)
            assert it_per_chunk * HP * per_head * 16 == CH

            def kv_body(it, carry):
                i = 1 + it // (H // HP // 2)

                @pl.when(it % it_per_chunk == 0)
                def _():
                    n = it // it_per_chunk
                    dst = raw.at[i, pl.ds((n % NCH) * CH, CH)]
                    pltpu.make_async_copy(dst, dst, sems.at[NCH + n]).wait()
                NPC = 8
                rows = X0 // 2 // NPC
                for k in range(HP):
                    h = it * HP + k
                    for n in range(NPC):
                        q = _dot(_as_bf(xn0[pl.ds(n * rows, rows), :]), _as_bf(w_t[0, h]))
                        ah_buf[pl.ds(n * rows, rows), pl.ds(pl.multiple_of(h * E, E), E)] = _as_u32(q.astype(BF))
                        relayout_part(i, (h % (H // 2)) * per_head + n // 2, (n % 2) * (H // 2), H // 2)
                return carry
            with jax.named_scope("sc_kv"):
                jax.lax.fori_loop(0, H // HP, kv_body, 0)

            def k_body(h, carry):
                rows = X0 // 2 // 4
                for n in range(4):
                    k = _dot(_as_bf(xn0[pl.ds(n * rows, rows), :]), _as_bf(w_t[1, h]))
                    ah_buf[pl.ds(n * rows, rows), pl.ds(pl.multiple_of((H + h) * E, E), E)] = _as_u32(k.astype(BF))
                return carry
            with jax.named_scope("sc_kb"):
                jax.lax.fori_loop(0, NK, k_body, 0)

            for c in mlp_weight_copies():
                c.start()
            x_rest_copy().start()

        def mlp_pre(c):
            a1_buf[pl.ds(0, 2 * HALO), :] = a1_buf[pl.ds(PAIR, 2 * HALO), :]
            y = _ln(h_buf[pl.ds(pl.multiple_of(c * PAIR + HALO, 8), PAIR + HALO), :])
            y_buf[...] = y[0:PAIR]
            z_buf[...] = _as_u32(_ln(y[HALO:]).astype(BF))

        def mlp_prologue():
            for c in mlp_weight_copies():
                c.wait()
            z = _ln(_ln(h_buf[pl.ds(0, 2 * HALO), :])).astype(BF)
            tok = jax.lax.broadcasted_iota(jnp.int32, (2 * HALO, 128), 0) - HALO
            for j in range(nD):
                a1_buf[pl.ds(PAIR, 2 * HALO), pl.ds(j * 128, 128)] = jnp.where(
                    tok >= 0, _gelu(_dot(z, w1_t[j])), 0.0)
            mlp_pre(0)

        def attention_jobs(t):
            row = jax.lax.broadcasted_iota(jnp.int32, (G * L, G * L), 0)
            col = jax.lax.broadcasted_iota(jnp.int32, (G * L, G * L), 1)

            def head_of(r):
                return jnp.where(r < G * SEG, r // SEG, (r - G * SEG) // MEM)
            mask = (head_of(row) == head_of(col)) & ((col >= G * SEG) | (row >= G * SEG) | (col <= row))
            x0 = t * PAIR
            h0 = x0 + HALO

            def step_jobs(even):
                lb = lb_e if even else lb_o
                st = {}

                lq = lq_e if even else lq_o
                def ring(r, mult):
                    return pl.multiple_of(jax.lax.rem(r, RING), mult)
                a_new = X0 // 2 + t * QR
                a_use = ring(t * SEG + (0 if even else SEG // 2), 16)

                def ahead(mat, h, col, slot):
                    cs, cb = pl.ds(h * E, E), pl.ds(col * E, E)
                    r = _dot(_as_bf(lq[...]), _as_bf(w_t[mat, h]))
                    if even:
                        ah_buf[pl.ds(ring(a_new, 8), 8), cb] = _as_u32(r[0:16].astype(BF))
                        sv[slot, :, cs] = r[16:24]
                    else:
                        ah_buf[pl.ds(ring(a_new + 8, 8), 8), cb] = _as_u32(
                            jnp.concatenate([sv[slot, :, cs], r[0:8]], axis=0).astype(BF))
                        ah_buf[pl.ds(ring(a_new + 16, 8), 8), cb] = _as_u32(r[8:24].astype(BF))
                    return _as_bf(ah_buf[pl.ds(a_use, SEG // 2), cb]), r[QR:QR + MEM]

                def in_step(mat, h, slot):
                    cs = pl.ds(h * E, E)
                    r = _dot(_as_bf(lb[...]), _as_bf(w_t[mat, h]))
                    if even:
                        sv[slot, :, cs] = r[0:8]
                        return [r[8:40]], r[40:48]
                    return [sv[slot, :, cs], r[0:24]], r[24:32]

                def stack(parts):
                    xs, ms = [p[0] for p in parts], [p[1] for p in parts]
                    if isinstance(xs[0], list):
                        return jnp.concatenate(xs[0] + xs[1] + ms, axis=0).astype(BF)
                    return jnp.concatenate(xs + [jnp.concatenate(ms, axis=0).astype(BF)], axis=0)

                def j_qkv(g, i):
                    def run():
                        h = g * G + i
                        parts = st.setdefault(('parts', g), [[], [], []])
                        parts[0].append(ahead(0, h, h, 2))
                        parts[1].append(ahead(1, h, H + h, 0) if h < NK else in_step(1, h, 0))
                        parts[2].append(in_step(2, h, 1))
                        if i == G - 1:
                            st['qkv', g] = [stack(p) for p in st.pop(('parts', g))]
                    return run

                def j_scores(g):
                    def run():
                        q, k, v = st.pop(('qkv', g))
                        s = jax.lax.dot_general(q, k, (((1,), (1,)), ((), ())),
                                                preferred_element_type=F32)
                        s = jnp.where(mask, s, -1000000000.0 / scale)
                        m = jnp.max(s, axis=-1, keepdims=True)
                        p = jnp.exp2((s - m) * (scale * LOG2E))
                        l = jnp.sum(p, axis=-1, keepdims=True)
                        r0 = pl.reciprocal(l, approx=True)
                        p = p * (r0 * (2.0 - l * r0))
                        st['p', g] = (p.astype(BF), v)
                    return run

                def j_pv(g):
                    def run():
                        p, v = st.pop(('p', g))
                        o2 = _dot(p, v)
                        for i, h in enumerate(range(g * G, (g + 1) * G)):
                            ox = o2[i * SEG:(i + 1) * SEG]
                            om = o2[G * SEG + i * MEM:G * SEG + (i + 1) * MEM]
                            cs = pl.ds(h * E, E)
                            if even:
                                ob[pl.ds(16, 4), cs] = _as_u32(ox[0:8].astype(BF))
                                ob[pl.ds(0, 16), cs] = _as_u32(
                                    jnp.concatenate([ox[8:32], om], axis=0).astype(BF))
                            else:
                                ob[pl.ds(20, 4), cs] = _as_u32(ox[0:8].astype(BF))
                                ob[pl.ds(24, 16), cs] = _as_u32(
                                    jnp.concatenate([ox[8:32], om], axis=0).astype(BF))
                    return run

                rows = pl.ds(0, 16) if even else pl.ds(16, 24)
                nrows = 32 if even else 48

                def j_wo1(j):
                    def run():
                        lhs = _as_bf(ob[rows, pl.ds(0, K1)])
                        wacc[pl.ds(0, nrows), pl.ds(j * 128, 128)] = _dot(
                            lhs, _as_bf(wo_t[j, pl.ds(0, K1 // 2), :]))
                    return run

                def j_wo2(j):
                    def run():
                        lhs = _as_bf(ob[rows, pl.ds(K1, H * E - K1)])
                        r = wacc[pl.ds(0, nrows), pl.ds(j * 128, 128)] + _dot(
                            lhs, _as_bf(wo_t[j, pl.ds(K1 // 2, (H * E - K1) // 2), :]))
                        cs = pl.ds(j * 128, 128)
                        xs = x_v[pl.ds(pl.multiple_of(x0, PAIR), PAIR), cs].astype(F32)
                        if even:
                            mem = _as_u32(r[24:32].astype(BF))
                            lb_o[pl.ds(12, 4), cs] = mem
                            lq_o[pl.ds(12, 4), cs] = mem
                            h_buf[pl.ds(pl.multiple_of(h0 + 8, 8), 24), cs] = xs[8:32] + r[0:24]
                        else:
                            mem = _as_u32(r[40:48].astype(BF))
                            lb_e[pl.ds(20, 4), cs] = mem
                            lq_e[pl.ds(12, 4), cs] = mem
                            h_buf[pl.ds(pl.multiple_of(h0, 8), 8), cs] = xs[0:8] + r[0:8]
                            h_buf[pl.ds(pl.multiple_of(h0 + 32, 8), 32), cs] = xs[32:64] + r[8:40]
                    return run

                last = n_slots - 1
                jobs = []
                for g in range(n_slots):
                    for i in range(G):
                        jobs.append((('qkv', g, i), j_qkv(g, i)))
                    if g >= 1:
                        jobs.append((('s', g - 1), j_scores(g - 1)))
                    if g >= 2:
                        jobs.append((('pv', g - 2), j_pv(g - 2)))
                wo1 = [(('wo1', j), j_wo1(j)) for j in range(nD)]
                jobs += (wo1[0:3] + [(('s', last), j_scores(last)), (('pv', last - 1), j_pv(last - 1))]
                         + wo1[3:6] + [(('pv', last), j_pv(last))] + wo1[6:8])
                jobs += [(('wo2', j), j_wo2(j)) for j in range(nD)]
                return jobs

            def j_next_xn():
                store_xn(jnp.minimum(t + 1, n_pairs - 1))

            return step_jobs(True), step_jobs(False), j_next_xn

        after_qkv = ('s', n_slots - 2)

        def mlp_jobs(c):
            r0 = pl.multiple_of(c * PAIR, PAIR)
            st = {}

            def j_pre_next():
                mlp_pre(jnp.minimum(c + 1, n_pairs - 1))

            def j_w1(j):
                def run():
                    tok = jax.lax.broadcasted_iota(jnp.int32, (PAIR, 128), 0) + (r0 + HALO)
                    a = _gelu(_dot(_as_bf(z_buf[...]), w1_t[j]))
                    a1_buf[pl.ds(2 * HALO, PAIR), pl.ds(j * 128, 128)] = jnp.where(tok < S, a, 0.0)
                return run

            def j_shift():
                cq = D // 4
                st['g'] = jnp.concatenate([
                    a1_buf[pl.ds(HALO - 1, PAIR), pl.ds(0 * cq, cq)],
                    a1_buf[pl.ds(HALO + 1, PAIR), pl.ds(1 * cq, cq)],
                    a1_buf[pl.ds(HALO - 2, PAIR), pl.ds(2 * cq, cq)],
                    a1_buf[pl.ds(HALO + 2, PAIR), pl.ds(3 * cq, cq)]], axis=1).astype(BF)

            def j_w2(j):
                def run():
                    st['x1', j] = y_buf[:, pl.ds(j * 128, 128)] + _dot(st['g'], w2_t[j])
                return run

            def j_ln3():
                x1 = jnp.concatenate([st['x1', j] for j in range(nD)], axis=1)
                st['z1'] = _ln(x1).astype(BF)

            def j_w3(j):
                def run():
                    st['a3', j] = _gelu(_dot(st['z1'], w3_t[j])).astype(BF)
                return run

            def j_cat():
                st['a3'] = jnp.concatenate([st.pop(('a3', j)) for j in range(nF)], axis=1)

            def j_w4(j):
                def run():
                    cs = pl.ds(j * 128, 128)
                    hh = h_buf[pl.ds(pl.multiple_of(r0 + HALO, 8), PAIR), cs]
                    out_v[pl.ds(r0, PAIR), cs] = (
                        hh + (st['x1', j] + _dot(st['a3'], w4_t[j]))).astype(out_v.dtype)
                return run

            return dict(pre_next=j_pre_next, w1=[j_w1(j) for j in range(nD)], shift=j_shift,
                        w2=[j_w2(j) for j in range(nD)], ln3=j_ln3,
                        w3=[j_w3(j) for j in range(nF)], cat=j_cat,
                        w4=[j_w4(j) for j in range(nD)])

        def attention_only(t, carry):
            ej, oj, j_next_xn = attention_jobs(t)

            def j_wo_wait():
                with jax.named_scope("sc_wo_finish"):
                    pl.when(t == 0)(wo_finish)
            _run(_interleave(ej, {after_qkv: [j_wo_wait]}) + _interleave(oj, {after_qkv: [j_next_xn]}))
            return carry

        def fused(t, carry):
            @pl.when(t == LAG)
            def _():
                x_rest_copy().wait()

            @pl.when(t > LAG)
            def _():
                out_copy(t - LAG - 1).start()

            ej, oj, j_next_xn = attention_jobs(t)
            b = mlp_jobs(t - LAG)
            w3, w4 = b['w3'], b['w4']
            fe, fo = {}, {}

            def put(d, label, *jobs):
                d.setdefault(label, []).extend(jobs)
            for i in range(nD):
                put(fe, ('qkv', 2 + i // 2, i % 2), b['w1'][i])
                put(fe, ('qkv', 8 + i // 2, i % 2), b['w2'][i])
            put(fe, ('qkv', 6, 0), b['shift'])
            put(fe, ('qkv', 12, 0), b['ln3'])
            put(fe, ('qkv', 15, 0), w3[0])
            put(fe, 'end', *w3[1:4])
            put(fo, ('qkv', 0, 1), b['pre_next'])
            for k in range(4, nF):
                put(fo, ('qkv', 1 + (k - 4) // 2, (k - 4) % 2), w3[k])
            put(fo, ('qkv', 13, 0), b['cat'])
            put(fo, ('qkv', 14, 0), w4[0])
            put(fo, ('qkv', 15, 0), w4[1])
            put(fo, after_qkv, j_next_xn)
            put(fo, ('s', n_slots - 1), w4[2])
            put(fo, 'end', *w4[3:])
            with jax.named_scope("sc_fused_body"):
                _run(_interleave(ej, fe) + _interleave(oj, fo))
            return carry

        def mlp_only(c, carry):
            out_copy(c - 1).start()
            b = mlp_jobs(c)
            _run(b['w1'] + [b['shift']] + b['w2'] + [b['ln3'], b['pre_next']] + b['w3'] + [b['cat']] + b['w4'])
            return carry

        with jax.named_scope("sc_prologue"):
            prologue()
            store_xn(0)
        with jax.named_scope("sc_a_only"):
            jax.lax.fori_loop(0, LAG, attention_only, 0)
        with jax.named_scope("sc_mlp_prologue"):
            mlp_prologue()
        with jax.named_scope("sc_fused"):
            jax.lax.fori_loop(LAG, n_pairs, fused, 0)
        with jax.named_scope("sc_b_tail"):
            jax.lax.fori_loop(n_pairs - LAG, n_pairs, mlp_only, 0)
        out_copy(n_pairs - 1).start()
        pltpu.make_async_copy(out_v, out_hbm, sems.at[OUT_SEM]).wait()

    return kernel, WO_SEM + nD + 6, X0, RING


@functools.partial(jax.jit, static_argnames=("A_seg_len",))
def pallas_sequential_preLN__memory_aug_recurrent_mem_tr__mixer_s_mlp__prompt_kernel(
    A_x, A_mem0, A_Wq, A_Wk, A_Wv, A_Wo, A_seg_len, B_x, B_w1, B_w2, B_w3, B_w4,
):
    _, S, D = A_x.shape
    H, E = A_Wq.shape[1], A_Wq.shape[2]
    F = B_w3.shape[1]
    assert A_seg_len == SEG and A_mem0.shape[1] == MEM and S % PAIR == 0
    nD, nF = D // 128, F // 128

    x = A_x.reshape(S, D)
    mem0 = A_mem0.reshape(MEM, D)
    wo = A_Wo.reshape(H * E, D)

    kernel, n_sems, x0, ring = _make_kernel(S, D, H, E, F)
    any_spec = pl.BlockSpec(memory_space=pl.ANY)
    out = pl.pallas_call(
        kernel,
        in_specs=[any_spec] * 10,
        out_specs=any_spec,
        out_shape=jax.ShapeDtypeStruct((S, D), A_x.dtype),
        scratch_shapes=[
            pltpu.VMEM((3, D, H, E), BF),
            pltpu.VMEM((3, H, D // 2, E), U32),
            pltpu.VMEM((H * E, D), BF),
            pltpu.VMEM((nD, H * E // 2, 128), U32),
            pltpu.VMEM((nD, D, 128), BF),
            pltpu.VMEM((nD, D, 128), BF),
            pltpu.VMEM((nF, D, 128), BF),
            pltpu.VMEM((nD, F, 128), BF),
            pltpu.VMEM((S, D), BF),
            pltpu.VMEM((S, D), BF),
            pltpu.VMEM((MEM, D), BF),
            pltpu.VMEM((x0 // 2, D), U32),
            pltpu.VMEM((ring, (H + NK) * E), U32),
            pltpu.VMEM((16, D), U32),
            pltpu.VMEM((16, D), U32),
            pltpu.VMEM((24, D), U32),
            pltpu.VMEM((16, D), U32),
            pltpu.VMEM((3, 8, H * E), F32),
            pltpu.VMEM((40, H * E), U32),
            pltpu.VMEM((48, D), F32),
            pltpu.VMEM((S + 2 * HALO, D), F32),
            pltpu.VMEM((PAIR + 2 * HALO, D), F32),
            pltpu.VMEM((PAIR, D), F32),
            pltpu.VMEM((PAIR // 2, D), U32),
            pltpu.SemaphoreType.DMA((n_sems,)),
        ],
        compiler_params=pltpu.CompilerParams(
            vmem_limit_bytes=124 * 1024 * 1024,
            disable_bounds_checks=True,
        ),
    )(x, mem0, A_Wq, A_Wk, A_Wv, wo, B_w1, B_w2, B_w3, B_w4)
    return out.reshape(1, S, D)
```

```python
import functools

import jax
import jax.numpy as jnp
from jax.experimental import pallas as pl
from jax.experimental.pallas import tpu as pltpu

BF = jnp.bfloat16
F32 = jnp.float32
U32 = jnp.uint32

SEG = 32
MEM = 8
PAIR = 2 * SEG
LAG = 3
HALO = 8
G = 2
TAIL_HEADS = 6
QR = 24
NK = 10
NCH = 8
LN_EPS = 1e-5
LOG2E = 1.4426950408889634


def _ln(x):
    m = jnp.mean(x, axis=-1, keepdims=True)
    xc = x - m
    v = jnp.mean(xc * xc, axis=-1, keepdims=True)
    return xc * jax.lax.rsqrt(v + LN_EPS)


_dot = functools.partial(jnp.dot, preferred_element_type=F32)


def _gelu(x):
    return jax.nn.gelu(x, approximate=True)


def _as_bf(x_u32):
    return pltpu.bitcast(x_u32, BF)


def _as_u32(x_bf):
    return pltpu.bitcast(x_bf, U32)


def _interleave(main, fill):
    fill = dict(fill)
    out = []
    for label, job in main:
        out.extend(fill.pop(label, []))
        out.append(job)
    out.extend(fill.pop('end', []))
    assert not fill, fill
    return out


def _run(jobs):
    for job in jobs:
        job()


def _make_kernel(S, D, H, E, F):
    n_pairs = S // PAIR
    nD = D // 128
    nF = F // 128
    scale = float(E) ** -0.5
    L = MEM + SEG
    n_slots = H // G
    K1 = (H - TAIL_HEADS) * E
    CH = D // NCH
    WO_CH = H * E // nD
    X0 = S - 2 * QR * n_pairs
    assert X0 % PAIR == 0 and X0 // PAIR - 1 >= LAG and X0 < S
    RING = (X0 + PAIR) // 2
    assert RING % 16 == 0 and NK % G == 0
    assert G == 2 and n_slots == 16 and nF == 28 and nD == 8
    assert (H - TAIL_HEADS) // G - 1 < n_slots - 2

    WO_SEM = 3 * NCH
    B_SEM, X0_SEM, XM_SEM, X1_SEM, MEM_SEM, OUT_SEM = (WO_SEM + nD + i for i in range(6))
    XA = X0 + 2 * QR
    XB = X0 + 2 * QR * (LAG + 1)

    def kernel(x_hbm, mem0_hbm, wq_hbm, wk_hbm, wv_hbm, wo_hbm, w1_hbm, w2_hbm, w3_hbm, w4_hbm,
               out_hbm,
               raw, w_t, wo_raw, wo_t, w1_t, w2_t, w3_t, w4_t,
               x_v, out_v, mem0_v, xn0, ah_buf, lq_e, lq_o, lb_e, lb_o, sv, ob, wacc,
               h_buf, a1_buf, y_buf, z_buf, sems):

        def rows_copy(src, dst, start, size, sem):
            return pltpu.make_async_copy(src.at[pl.ds(start, size)], dst.at[pl.ds(start, size)], sems.at[sem])

        def raw_copy(i, c):
            src = (wq_hbm, wk_hbm, wv_hbm)[i]
            return rows_copy(src, raw.at[i], c * CH, CH, i * NCH + c)

        def wo_copy(j):
            return rows_copy(wo_hbm, wo_raw, j * WO_CH, WO_CH, WO_SEM + j)

        def mlp_weight_copies():
            return [pltpu.make_async_copy(src.at[:, pl.ds(j * 128, 128)], dst.at[j], sems.at[B_SEM])
                    for src, dst, n in ((w1_hbm, w1_t, nD), (w2_hbm, w2_t, nD),
                                        (w3_hbm, w3_t, nF), (w4_hbm, w4_t, nD))
                    for j in range(n)]

        def x_head_copy():
            return rows_copy(x_hbm, x_v, 0, XA, X0_SEM)

        def x_mid_copy():
            return rows_copy(x_hbm, x_v, XA, XB - XA, XM_SEM)

        def x_rest_copy():
            return rows_copy(x_hbm, x_v, XB, S - XB, X1_SEM)

        def mem_copy():
            return pltpu.make_async_copy(mem0_hbm, mem0_v, sems.at[MEM_SEM])

        def out_copy(c):
            return rows_copy(out_v, out_hbm, pl.multiple_of(c * PAIR, PAIR), PAIR, OUT_SEM)

        def relayout_part(i, b, h0, nh):
            x = raw[i, pl.ds(pl.multiple_of(b * 16, 16), 16), pl.ds(h0, nh), :]
            x = _as_u32(x).reshape(8, 2, nh // 2, E)
            ev, od = x[:, 0], x[:, 1]
            lo = jnp.swapaxes((ev & 0xFFFF) | (od << 16), 0, 1)
            hi = jnp.swapaxes((ev >> 16) | (od & jnp.uint32(0xFFFF0000)), 0, 1)
            rows = pl.ds(pl.multiple_of(b * 8, 8), 8)
            for p in range(nh // 2):
                w_t[i, h0 + 2 * p, rows, :] = lo[p]
                w_t[i, h0 + 2 * p + 1, rows, :] = hi[p]

        def relayout_block(i, b):
            relayout_part(i, b, 0, H)

        def wo_finish():
            def chunk(j, carry):
                dst = wo_raw.at[pl.ds(j * WO_CH, WO_CH)]
                pltpu.make_async_copy(dst, dst, sems.at[WO_SEM + j]).wait()

                def body(b, carry):
                    r = j * WO_CH + b * 256
                    for m in range(4):
                        blk = wo_raw[pl.ds(pl.multiple_of(r + m * 64, 64), 64), :]
                        for n in range(nD):
                            wo_t[n, pl.ds(pl.multiple_of((r + m * 64) // 2, 32), 32), :] = _as_u32(
                                blk[:, n * 128:(n + 1) * 128])
                    return carry
                return jax.lax.fori_loop(0, WO_CH // 256, body, carry)
            jax.lax.fori_loop(0, nD, chunk, 0)
            x_mid_copy().wait()

        def store_xn(t):
            xn = _ln(x_v[pl.ds(pl.multiple_of(t * PAIR, PAIR), PAIR), :].astype(F32))
            lb_e[pl.ds(0, 4), :] = _as_u32(xn[32:40].astype(BF))
            lb_e[pl.ds(4, 4), :] = _as_u32(xn[0:8].astype(BF))
            lb_e[pl.ds(8, 8), :] = _as_u32(xn[8:24].astype(BF))
            lb_e[pl.ds(16, 4), :] = _as_u32(xn[24:32].astype(BF))
            lb_o[pl.ds(0, 8), :] = _as_u32(xn[40:56].astype(BF))
            lb_o[pl.ds(8, 4), :] = _as_u32(xn[56:64].astype(BF))
            xq = _ln(x_v[pl.ds(pl.multiple_of(X0 + t * 2 * QR, 16), 2 * QR), :].astype(F32))
            lq_e[pl.ds(0, 8), :] = _as_u32(xq[0:16].astype(BF))
            lq_e[pl.ds(8, 4), :] = _as_u32(xq[16:24].astype(BF))
            for n in range(3):
                lq_o[pl.ds(4 * n, 4), :] = _as_u32(xq[24 + 8 * n:32 + 8 * n].astype(BF))

        def prologue():
            x_head_copy().start()
            mem_copy().start()
            for i in range(3):
                for c in range(NCH):
                    raw_copy(i, c).start()
            for j in range(nD):
                wo_copy(j).start()
            x_mid_copy().start()

            assert CH == 128 and NK <= nD * (S // X0)

            def acc_at(j):
                if isinstance(j, int):
                    return pl.ds((j // nD) * X0, X0), pl.ds((j % nD) * 128, 128)
                return (pl.ds(pl.multiple_of((j // nD) * X0, X0), X0),
                        pl.ds(pl.multiple_of((j % nD) * 128, 128), 128))

            def zero_acc(j, carry):
                h_buf[acc_at(j)] = jnp.zeros((X0, 128), F32)
                return carry
            jax.lax.fori_loop(0, NK, zero_acc, 0)
            x_head_copy().wait()
            mem_copy().wait()
            lb_e[pl.ds(20, 4), :] = _as_u32(mem0_v[...])
            lq_e[pl.ds(12, 4), :] = _as_u32(mem0_v[...])

            def ln_body(b, carry):
                rows = x_v[pl.ds(pl.multiple_of(b * 64, 64), 64), :].astype(F32)
                xn0[pl.ds(pl.multiple_of(b * 32, 32), 32), :] = _as_u32(_ln(rows).astype(BF))
                return carry
            jax.lax.fori_loop(0, X0 // 64, ln_body, 0)

            def wait_raw(i, c):
                dst = raw.at[i, pl.ds(c * CH, CH)]
                pltpu.make_async_copy(dst, dst, sems.at[i * NCH + c]).wait()

            def q_tile(j, c):
                lhs = _as_bf(xn0[:, pl.ds(pl.multiple_of(c * 128, 128), 128)])
                return _dot(lhs, _as_bf(w_t[0, j, pl.ds(pl.multiple_of(c * 64, 64), 64), :]))

            def first_chunk(b, carry):
                relayout_block(0, b)
                return carry

            def q_chunk(c, carry):
                @pl.when(c + 1 < NCH)
                def _():
                    wait_raw(0, c + 1)
                nxt = jnp.minimum(c + 1, NCH - 1)
                n_items = 2 * (CH // 16)
                done = 0
                for j in range(NK):
                    h_buf[acc_at(j)] = h_buf[acc_at(j)] + q_tile(j, c)
                    upto = (j + 1) * n_items // NK
                    for m in range(done, upto):
                        relayout_part(0, nxt * (CH // 16) + m // 2, (m % 2) * (H // 2), H // 2)
                    done = upto
                return carry

            def q_cast(j, carry):
                ah_buf[pl.ds(0, X0 // 2), pl.ds(pl.multiple_of(j * E, E), E)] = _as_u32(
                    h_buf[acc_at(j)].astype(BF))
                return carry
            with jax.named_scope("sc_wq"):
                wait_raw(0, 0)
                jax.lax.fori_loop(0, CH // 16, first_chunk, 0)
                jax.lax.fori_loop(0, NCH, q_chunk, 0)
                jax.lax.fori_loop(0, NK, q_cast, 0)
            h_buf[pl.ds(0, HALO), :] = jnp.zeros((HALO, D), F32)
            h_buf[pl.ds(HALO + S, HALO), :] = jnp.zeros((HALO, D), F32)

            HP = 2
            per_head = 2 * (D // 16) // H
            it_per_chunk = H // HP // (2 * NCH)
            assert it_per_chunk * HP * per_head * 16 == CH and H - NK >= H // 2

            def kv_body(it, carry):
                i = 1 + it // (H // HP // 2)

                @pl.when(it % it_per_chunk == 0)
                def _():
                    wait_raw(i, (it // it_per_chunk) % NCH)
                NPC = 8
                rows = X0 // 2 // NPC
                for k in range(HP):
                    m = it * HP + k
                    is_k = m >= H - NK
                    mat = jnp.where(is_k, 1, 0)
                    h = jnp.where(is_k, m - (H - NK), m + NK)
                    col = jnp.where(is_k, H + h, h)
                    for n in range(NPC):
                        r = _dot(_as_bf(xn0[pl.ds(n * rows, rows), :]), _as_bf(w_t[mat, h]))
                        ah_buf[pl.ds(n * rows, rows), pl.ds(pl.multiple_of(col * E, E), E)] = _as_u32(r.astype(BF))
                        relayout_part(i, (m % (H // 2)) * per_head + n // 2, (n % 2) * (H // 2), H // 2)
                return carry
            with jax.named_scope("sc_kv"):
                jax.lax.fori_loop(0, H // HP, kv_body, 0)

            for c in mlp_weight_copies():
                c.start()
            x_rest_copy().start()

        def mlp_pre(c):
            a1_buf[pl.ds(0, 2 * HALO), :] = a1_buf[pl.ds(PAIR, 2 * HALO), :]
            y = _ln(h_buf[pl.ds(pl.multiple_of(c * PAIR + HALO, 8), PAIR + HALO), :])
            y_buf[...] = y[0:PAIR]
            z_buf[...] = _as_u32(_ln(y[HALO:]).astype(BF))

        def mlp_prologue():
            for c in mlp_weight_copies():
                c.wait()
            z = _ln(_ln(h_buf[pl.ds(0, 2 * HALO), :])).astype(BF)
            tok = jax.lax.broadcasted_iota(jnp.int32, (2 * HALO, 128), 0) - HALO

            for j in range(nD):
                a1_buf[pl.ds(PAIR, 2 * HALO), pl.ds(j * 128, 128)] = jnp.where(
                    tok >= 0, _gelu(_dot(z, w1_t[j])), 0.0)
            mlp_pre(0)

        def attention_jobs(t):
            row = jax.lax.broadcasted_iota(jnp.int32, (G * L, G * L), 0)
            col = jax.lax.broadcasted_iota(jnp.int32, (G * L, G * L), 1)

            def head_of(r):
                return jnp.where(r < G * SEG, r // SEG, (r - G * SEG) // MEM)
            mask = (head_of(row) == head_of(col)) & ((col >= G * SEG) | (row >= G * SEG) | (col <= row))
            x0 = t * PAIR
            h0 = x0 + HALO

            def step_jobs(even):
                lb = lb_e if even else lb_o
                st = {}

                lq = lq_e if even else lq_o
                def ring(r, mult):
                    return pl.multiple_of(jax.lax.rem(r, RING), mult)
                a_new = X0 // 2 + t * QR
                a_use = ring(t * SEG + (0 if even else SEG // 2), 16)

                def ahead(mat, h, col, slot):
                    cs, cb = pl.ds(h * E, E), pl.ds(col * E, E)
                    r = _dot(_as_bf(lq[...]), _as_bf(w_t[mat, h]))
                    if even:
                        ah_buf[pl.ds(ring(a_new, 8), 8), cb] = _as_u32(r[0:16].astype(BF))
                        sv[slot, :, cs] = r[16:24]
                    else:
                        ah_buf[pl.ds(ring(a_new + 8, 8), 8), cb] = _as_u32(
                            jnp.concatenate([sv[slot, :, cs], r[0:8]], axis=0).astype(BF))
                        ah_buf[pl.ds(ring(a_new + 16, 8), 8), cb] = _as_u32(r[8:24].astype(BF))
                    return _as_bf(ah_buf[pl.ds(a_use, SEG // 2), cb]), r[QR:QR + MEM]

                def in_step(mat, h, slot):
                    cs = pl.ds(h * E, E)
                    r = _dot(_as_bf(lb[...]), _as_bf(w_t[mat, h]))
                    if even:
                        sv[slot, :, cs] = r[0:8]
                        return [r[8:40]], r[40:48]
                    return [sv[slot, :, cs], r[0:24]], r[24:32]

                def stack(parts):
                    xs, ms = [p[0] for p in parts], [p[1] for p in parts]
                    if isinstance(xs[0], list):
                        return jnp.concatenate(xs[0] + xs[1] + ms, axis=0).astype(BF)
                    return jnp.concatenate(xs + [jnp.concatenate(ms, axis=0).astype(BF)], axis=0)

                def j_qkv(g, i):
                    def run():
                        h = g * G + i
                        parts = st.setdefault(('parts', g), [[], [], []])
                        parts[0].append(ahead(0, h, h, 2))
                        parts[1].append(ahead(1, h, H + h, 0) if h < NK else in_step(1, h, 0))
                        parts[2].append(in_step(2, h, 1))
                        if i == G - 1:
                            st['qkv', g] = [stack(p) for p in st.pop(('parts', g))]
                    return run

                def j_scores(g):
                    def run():
                        q, k, v = st.pop(('qkv', g))
                        s = jax.lax.dot_general(q, k, (((1,), (1,)), ((), ())),
                                                preferred_element_type=F32)
                        s = jnp.where(mask, s, -1000000000.0 / scale)
                        m = jnp.max(s, axis=-1, keepdims=True)
                        p = jnp.exp2((s - m) * (scale * LOG2E))
                        l = jnp.sum(p, axis=-1, keepdims=True)
                        r0 = pl.reciprocal(l, approx=True)
                        p = p * (r0 * (2.0 - l * r0))
                        st['p', g] = (p.astype(BF), v)
                    return run

                def j_pv(g):
                    def run():
                        p, v = st.pop(('p', g))
                        o2 = _dot(p, v)
                        for i, h in enumerate(range(g * G, (g + 1) * G)):
                            ox = o2[i * SEG:(i + 1) * SEG]
                            om = o2[G * SEG + i * MEM:G * SEG + (i + 1) * MEM]
                            cs = pl.ds(h * E, E)
                            if even:
                                ob[pl.ds(16, 4), cs] = _as_u32(ox[0:8].astype(BF))
                                ob[pl.ds(0, 16), cs] = _as_u32(
                                    jnp.concatenate([ox[8:32], om], axis=0).astype(BF))
                            else:
                                ob[pl.ds(20, 4), cs] = _as_u32(ox[0:8].astype(BF))
                                ob[pl.ds(24, 16), cs] = _as_u32(
                                    jnp.concatenate([ox[8:32], om], axis=0).astype(BF))
                    return run

                rows = pl.ds(0, 16) if even else pl.ds(16, 24)
                nrows = 32 if even else 48

                def j_wo1(j):
                    def run():
                        lhs = _as_bf(ob[rows, pl.ds(0, K1)])
                        wacc[pl.ds(0, nrows), pl.ds(j * 128, 128)] = _dot(
                            lhs, _as_bf(wo_t[j, pl.ds(0, K1 // 2), :]))
                    return run

                def j_wo2(j):
                    def run():
                        lhs = _as_bf(ob[rows, pl.ds(K1, H * E - K1)])
                        r = wacc[pl.ds(0, nrows), pl.ds(j * 128, 128)] + _dot(
                            lhs, _as_bf(wo_t[j, pl.ds(K1 // 2, (H * E - K1) // 2), :]))
                        cs = pl.ds(j * 128, 128)
                        xs = x_v[pl.ds(pl.multiple_of(x0, PAIR), PAIR), cs].astype(F32)
                        if even:
                            mem = _as_u32(r[24:32].astype(BF))
                            lb_o[pl.ds(12, 4), cs] = mem
                            lq_o[pl.ds(12, 4), cs] = mem
                            h_buf[pl.ds(pl.multiple_of(h0 + 8, 8), 24), cs] = xs[8:32] + r[0:24]
                        else:
                            mem = _as_u32(r[40:48].astype(BF))
                            lb_e[pl.ds(20, 4), cs] = mem
                            lq_e[pl.ds(12, 4), cs] = mem
                            h_buf[pl.ds(pl.multiple_of(h0, 8), 8), cs] = xs[0:8] + r[0:8]
                            h_buf[pl.ds(pl.multiple_of(h0 + 32, 8), 32), cs] = xs[32:64] + r[8:40]
                    return run

                last = n_slots - 1
                jobs = []
                for g in range(n_slots):
                    for i in range(G):
                        jobs.append((('qkv', g, i), j_qkv(g, i)))
                    if g >= 1:
                        jobs.append((('s', g - 1), j_scores(g - 1)))
                    if g >= 2:
                        jobs.append((('pv', g - 2), j_pv(g - 2)))
                wo1 = [(('wo1', j), j_wo1(j)) for j in range(nD)]
                jobs += (wo1[0:3] + [(('s', last), j_scores(last)), (('pv', last - 1), j_pv(last - 1))]
                         + wo1[3:6] + [(('pv', last), j_pv(last))] + wo1[6:8])
                jobs += [(('wo2', j), j_wo2(j)) for j in range(nD)]
                return jobs

            def j_next_xn():
                store_xn(jnp.minimum(t + 1, n_pairs - 1))

            return step_jobs(True), step_jobs(False), j_next_xn

        after_qkv = ('s', n_slots - 2)

        def mlp_jobs(c):
            r0 = pl.multiple_of(c * PAIR, PAIR)
            st = {}

            def j_pre_next():
                mlp_pre(jnp.minimum(c + 1, n_pairs - 1))

            def j_w1(j):
                def run():
                    tok = jax.lax.broadcasted_iota(jnp.int32, (PAIR, 128), 0) + (r0 + HALO)
                    a = _gelu(_dot(_as_bf(z_buf[...]), w1_t[j]))
                    a1_buf[pl.ds(2 * HALO, PAIR), pl.ds(j * 128, 128)] = jnp.where(tok < S, a, 0.0)
                return run

            def j_shift():
                cq = D // 4
                st['g'] = jnp.concatenate([
                    a1_buf[pl.ds(HALO - 1, PAIR), pl.ds(0 * cq, cq)],
                    a1_buf[pl.ds(HALO + 1, PAIR), pl.ds(1 * cq, cq)],
                    a1_buf[pl.ds(HALO - 2, PAIR), pl.ds(2 * cq, cq)],
                    a1_buf[pl.ds(HALO + 2, PAIR), pl.ds(3 * cq, cq)]], axis=1).astype(BF)

            def j_w2(j):
                def run():
                    st['x1', j] = y_buf[:, pl.ds(j * 128, 128)] + _dot(st['g'], w2_t[j])
                return run

            def j_ln3():
                x1 = jnp.concatenate([st['x1', j] for j in range(nD)], axis=1)
                st['z1'] = _ln(x1).astype(BF)

            def j_w3(j):
                def run():
                    st['a3', j] = _gelu(_dot(st['z1'], w3_t[j])).astype(BF)
                return run

            def j_cat():
                st['a3'] = jnp.concatenate([st.pop(('a3', j)) for j in range(nF)], axis=1)

            def j_w4(j):
                def run():
                    cs = pl.ds(j * 128, 128)
                    hh = h_buf[pl.ds(pl.multiple_of(r0 + HALO, 8), PAIR), cs]
                    out_v[pl.ds(r0, PAIR), cs] = (
                        hh + (st['x1', j] + _dot(st['a3'], w4_t[j]))).astype(out_v.dtype)
                return run

            return dict(pre_next=j_pre_next, w1=[j_w1(j) for j in range(nD)], shift=j_shift,
                        w2=[j_w2(j) for j in range(nD)], ln3=j_ln3,
                        w3=[j_w3(j) for j in range(nF)], cat=j_cat,
                        w4=[j_w4(j) for j in range(nD)])

        def attention_only(t, carry):
            ej, oj, j_next_xn = attention_jobs(t)

            def j_wo_wait():
                with jax.named_scope("sc_wo_finish"):
                    pl.when(t == 0)(wo_finish)
            _run(_interleave(ej, {after_qkv: [j_wo_wait]}) + _interleave(oj, {after_qkv: [j_next_xn]}))
            return carry

        def fused(t, carry):
            @pl.when(t == LAG)
            def _():
                x_rest_copy().wait()

            @pl.when(t > LAG)
            def _():
                out_copy(t - LAG - 1).start()

            ej, oj, j_next_xn = attention_jobs(t)
            b = mlp_jobs(t - LAG)
            w3, w4 = b['w3'], b['w4']
            fe, fo = {}, {}

            def put(d, label, *jobs):
                d.setdefault(label, []).extend(jobs)
            for i in range(nD):
                put(fe, ('qkv', 2 + i // 2, i % 2), b['w1'][i])
                put(fe, ('qkv', 8 + i // 2, i % 2), b['w2'][i])
            put(fe, ('qkv', 6, 0), b['shift'])
            put(fe, ('qkv', 12, 0), b['ln3'])
            put(fe, ('qkv', 15, 0), w3[0])
            put(fe, 'end', *w3[1:4])
            put(fo, ('qkv', 0, 1), b['pre_next'])
            for k in range(4, nF):
                put(fo, ('qkv', 1 + (k - 4) // 2, (k - 4) % 2), w3[k])
            put(fo, ('qkv', 13, 0), b['cat'])
            put(fo, ('qkv', 14, 0), w4[0])
            put(fo, ('qkv', 15, 0), w4[1])
            put(fo, after_qkv, j_next_xn)
            put(fo, ('s', n_slots - 1), w4[2])
            put(fo, 'end', *w4[3:])
            with jax.named_scope("sc_fused_body"):
                _run(_interleave(ej, fe) + _interleave(oj, fo))
            return carry

        def mlp_only(c, carry):
            out_copy(c - 1).start()
            b = mlp_jobs(c)
            _run(b['w1'] + [b['shift']] + b['w2'] + [b['ln3'], b['pre_next']] + b['w3'] + [b['cat']] + b['w4'])
            return carry

        with jax.named_scope("sc_prologue"):
            prologue()
            store_xn(0)
        with jax.named_scope("sc_a_only"):
            jax.lax.fori_loop(0, LAG, attention_only, 0)
        with jax.named_scope("sc_mlp_prologue"):
            mlp_prologue()
        with jax.named_scope("sc_fused"):
            jax.lax.fori_loop(LAG, n_pairs, fused, 0)
        with jax.named_scope("sc_b_tail"):
            jax.lax.fori_loop(n_pairs - LAG, n_pairs, mlp_only, 0)
        out_copy(n_pairs - 1).start()
        pltpu.make_async_copy(out_v, out_hbm, sems.at[OUT_SEM]).wait()

    return kernel, WO_SEM + nD + 6, X0, RING


@functools.partial(jax.jit, static_argnames=("A_seg_len",))
def pallas_sequential_preLN__memory_aug_recurrent_mem_tr__mixer_s_mlp__prompt_kernel(
    A_x, A_mem0, A_Wq, A_Wk, A_Wv, A_Wo, A_seg_len, B_x, B_w1, B_w2, B_w3, B_w4,
):
    _, S, D = A_x.shape
    H, E = A_Wq.shape[1], A_Wq.shape[2]
    F = B_w3.shape[1]
    assert A_seg_len == SEG and A_mem0.shape[1] == MEM and S % PAIR == 0
    nD, nF = D // 128, F // 128

    x = A_x.reshape(S, D)
    mem0 = A_mem0.reshape(MEM, D)
    wo = A_Wo.reshape(H * E, D)

    kernel, n_sems, x0, ring = _make_kernel(S, D, H, E, F)
    any_spec = pl.BlockSpec(memory_space=pl.ANY)
    out = pl.pallas_call(
        kernel,
        in_specs=[any_spec] * 10,
        out_specs=any_spec,
        out_shape=jax.ShapeDtypeStruct((S, D), A_x.dtype),
        scratch_shapes=[
            pltpu.VMEM((3, D, H, E), BF),
            pltpu.VMEM((3, H, D // 2, E), U32),
            pltpu.VMEM((H * E, D), BF),
            pltpu.VMEM((nD, H * E // 2, 128), U32),
            pltpu.VMEM((nD, D, 128), BF),
            pltpu.VMEM((nD, D, 128), BF),
            pltpu.VMEM((nF, D, 128), BF),
            pltpu.VMEM((nD, F, 128), BF),
            pltpu.VMEM((S, D), BF),
            pltpu.VMEM((S, D), BF),
            pltpu.VMEM((MEM, D), BF),
            pltpu.VMEM((x0 // 2, D), U32),
            pltpu.VMEM((ring, (H + NK) * E), U32),
            pltpu.VMEM((16, D), U32),
            pltpu.VMEM((16, D), U32),
            pltpu.VMEM((24, D), U32),
            pltpu.VMEM((16, D), U32),
            pltpu.VMEM((3, 8, H * E), F32),
            pltpu.VMEM((40, H * E), U32),
            pltpu.VMEM((48, D), F32),
            pltpu.VMEM((S + 2 * HALO, D), F32),
            pltpu.VMEM((PAIR + 2 * HALO, D), F32),
            pltpu.VMEM((PAIR, D), F32),
            pltpu.VMEM((PAIR // 2, D), U32),
            pltpu.SemaphoreType.DMA((n_sems,)),
        ],
        compiler_params=pltpu.CompilerParams(
            vmem_limit_bytes=124 * 1024 * 1024,
            disable_bounds_checks=True,
        ),
    )(x, mem0, A_Wq, A_Wk, A_Wv, wo, B_w1, B_w2, B_w3, B_w4)
    return out.reshape(1, S, D)
```

```python
import functools

import jax
import jax.numpy as jnp
from jax.experimental import pallas as pl
from jax.experimental.pallas import tpu as pltpu

BF = jnp.bfloat16
F32 = jnp.float32
U32 = jnp.uint32

SEG = 32
MEM = 8
PAIR = 2 * SEG
LAG = 3
HALO = 8
G = 2
TAIL_HEADS = 6
QR = 24
NK = 10
NCH = 8
LN_EPS = 1e-5
LOG2E = 1.4426950408889634


def _ln(x):
    m = jnp.mean(x, axis=-1, keepdims=True)
    xc = x - m
    v = jnp.mean(xc * xc, axis=-1, keepdims=True)
    return xc * jax.lax.rsqrt(v + LN_EPS)


_dot = functools.partial(jnp.dot, preferred_element_type=F32)


def _gelu(x):
    return jax.nn.gelu(x, approximate=True)


def _as_bf(x_u32):
    return pltpu.bitcast(x_u32, BF)


def _as_u32(x_bf):
    return pltpu.bitcast(x_bf, U32)


def _interleave(main, fill):
    fill = dict(fill)
    out = []
    for label, job in main:
        out.extend(fill.pop(label, []))
        out.append(job)
    out.extend(fill.pop('end', []))
    assert not fill, fill
    return out


def _run(jobs):
    for job in jobs:
        job()


def _make_kernel(S, D, H, E, F):
    n_pairs = S // PAIR
    nD = D // 128
    nF = F // 128
    scale = float(E) ** -0.5
    L = MEM + SEG
    n_slots = H // G
    K1 = (H - TAIL_HEADS) * E
    CH = D // NCH
    WO_CH = H * E // nD
    X0 = S - 2 * QR * n_pairs
    assert X0 % PAIR == 0 and X0 // PAIR - 1 >= LAG and X0 < S
    RING = (X0 + PAIR) // 2
    assert RING % 16 == 0 and NK % G == 0
    assert G == 2 and n_slots == 16 and nF == 28 and nD == 8
    assert (H - TAIL_HEADS) // G - 1 < n_slots - 2

    WO_SEM = 3 * NCH
    B_SEM, X0_SEM, XM_SEM, X1_SEM, MEM_SEM, OUT_SEM = (WO_SEM + nD + i for i in range(6))
    XA = X0 + 2 * QR
    XB = X0 + 2 * QR * (LAG + 1)

    def kernel(x_hbm, mem0_hbm, wq_hbm, wk_hbm, wv_hbm, wo_hbm, w1_hbm, w2_hbm, w3_hbm, w4_hbm,
               out_hbm,
               raw, w_t, wo_raw, wo_t, w1_t, w2_t, w3_t, w4_t,
               x_v, out_v, mem0_v, xn0, ah_buf, lq_e, lq_o, lb_e, lb_o, sv, ob, wacc,
               h_buf, a1_buf, y_buf, z_buf, sems):

        def rows_copy(src, dst, start, size, sem):
            return pltpu.make_async_copy(src.at[pl.ds(start, size)], dst.at[pl.ds(start, size)], sems.at[sem])

        def raw_copy(i, c):
            src = (wq_hbm, wk_hbm, wv_hbm)[i]
            return rows_copy(src, raw.at[i], c * CH, CH, i * NCH + c)

        def wo_copy(j):
            return rows_copy(wo_hbm, wo_raw, j * WO_CH, WO_CH, WO_SEM + j)

        def mlp_weight_copies():
            return [pltpu.make_async_copy(src.at[:, pl.ds(j * 128, 128)], dst.at[j], sems.at[B_SEM])
                    for src, dst, n in ((w1_hbm, w1_t, nD), (w2_hbm, w2_t, nD),
                                        (w3_hbm, w3_t, nF), (w4_hbm, w4_t, nD))
                    for j in range(n)]

        def x_head_copy():
            return rows_copy(x_hbm, x_v, 0, XA, X0_SEM)

        def x_mid_copy():
            return rows_copy(x_hbm, x_v, XA, XB - XA, XM_SEM)

        def x_rest_copy():
            return rows_copy(x_hbm, x_v, XB, S - XB, X1_SEM)

        def mem_copy():
            return pltpu.make_async_copy(mem0_hbm, mem0_v, sems.at[MEM_SEM])

        def out_copy(c):
            return rows_copy(out_v, out_hbm, pl.multiple_of(c * PAIR, PAIR), PAIR, OUT_SEM)

        def relayout_part(i, b, h0, nh):
            x = raw[i, pl.ds(pl.multiple_of(b * 16, 16), 16), pl.ds(h0, nh), :]
            x = _as_u32(x).reshape(8, 2, nh // 2, E)
            ev, od = x[:, 0], x[:, 1]
            lo = jnp.swapaxes((ev & 0xFFFF) | (od << 16), 0, 1)
            hi = jnp.swapaxes((ev >> 16) | (od & jnp.uint32(0xFFFF0000)), 0, 1)
            rows = pl.ds(pl.multiple_of(b * 8, 8), 8)
            for p in range(nh // 2):
                w_t[i, h0 + 2 * p, rows, :] = lo[p]
                w_t[i, h0 + 2 * p + 1, rows, :] = hi[p]

        def relayout_block(i, b):
            relayout_part(i, b, 0, H)

        def wo_finish():
            def chunk(j, carry):
                dst = wo_raw.at[pl.ds(j * WO_CH, WO_CH)]
                pltpu.make_async_copy(dst, dst, sems.at[WO_SEM + j]).wait()

                def body(b, carry):
                    r = j * WO_CH + b * 256
                    for m in range(4):
                        blk = wo_raw[pl.ds(pl.multiple_of(r + m * 64, 64), 64), :]
                        for n in range(nD):
                            wo_t[n, pl.ds(pl.multiple_of((r + m * 64) // 2, 32), 32), :] = _as_u32(
                                blk[:, n * 128:(n + 1) * 128])
                    return carry
                return jax.lax.fori_loop(0, WO_CH // 256, body, carry)
            jax.lax.fori_loop(0, nD, chunk, 0)
            x_mid_copy().wait()

        def store_xn(t, even):
            x0 = pl.multiple_of(t * PAIR, PAIR)
            q0 = pl.multiple_of(X0 + t * 2 * QR, 16)
            if even:
                xn = _ln(x_v[pl.ds(x0, 40), :].astype(F32))
                lb_e[pl.ds(0, 4), :] = _as_u32(xn[32:40].astype(BF))
                lb_e[pl.ds(4, 4), :] = _as_u32(xn[0:8].astype(BF))
                lb_e[pl.ds(8, 8), :] = _as_u32(xn[8:24].astype(BF))
                lb_e[pl.ds(16, 4), :] = _as_u32(xn[24:32].astype(BF))
                xq = _ln(x_v[pl.ds(q0, QR), :].astype(F32))
                lq_e[pl.ds(0, 8), :] = _as_u32(xq[0:16].astype(BF))
                lq_e[pl.ds(8, 4), :] = _as_u32(xq[16:24].astype(BF))
            else:
                xn = _ln(x_v[pl.ds(x0 + 40, 24), :].astype(F32))
                lb_o[pl.ds(0, 8), :] = _as_u32(xn[0:16].astype(BF))
                lb_o[pl.ds(8, 4), :] = _as_u32(xn[16:24].astype(BF))
                xq = _ln(x_v[pl.ds(q0 + QR, QR), :].astype(F32))
                for n in range(3):
                    lq_o[pl.ds(4 * n, 4), :] = _as_u32(xq[8 * n:8 * n + 8].astype(BF))

        def prologue():
            x_head_copy().start()
            mem_copy().start()
            for i in range(3):
                for c in range(NCH):
                    raw_copy(i, c).start()
            for j in range(nD):
                wo_copy(j).start()
            x_mid_copy().start()

            assert CH == 128 and NK <= nD * (S // X0)

            def acc_at(j):
                if isinstance(j, int):
                    return pl.ds((j // nD) * X0, X0), pl.ds((j % nD) * 128, 128)
                return (pl.ds(pl.multiple_of((j // nD) * X0, X0), X0),
                        pl.ds(pl.multiple_of((j % nD) * 128, 128), 128))

            def zero_acc(j, carry):
                h_buf[acc_at(j)] = jnp.zeros((X0, 128), F32)
                return carry
            jax.lax.fori_loop(0, NK, zero_acc, 0)
            x_head_copy().wait()
            mem_copy().wait()
            lb_e[pl.ds(20, 4), :] = _as_u32(mem0_v[...])
            lq_e[pl.ds(12, 4), :] = _as_u32(mem0_v[...])

            def ln_body(b, carry):
                rows = x_v[pl.ds(pl.multiple_of(b * 64, 64), 64), :].astype(F32)
                xn0[pl.ds(pl.multiple_of(b * 32, 32), 32), :] = _as_u32(_ln(rows).astype(BF))
                return carry
            jax.lax.fori_loop(0, X0 // 64, ln_body, 0)

            def wait_raw(i, c):
                dst = raw.at[i, pl.ds(c * CH, CH)]
                pltpu.make_async_copy(dst, dst, sems.at[i * NCH + c]).wait()

            def q_tile(j, c):
                lhs = _as_bf(xn0[:, pl.ds(pl.multiple_of(c * 128, 128), 128)])
                return _dot(lhs, _as_bf(w_t[0, j, pl.ds(pl.multiple_of(c * 64, 64), 64), :]))

            def first_chunk(b, carry):
                relayout_block(0, b)
                return carry

            def q_chunk(c, carry):
                @pl.when(c + 1 < NCH)
                def _():
                    wait_raw(0, c + 1)
                nxt = jnp.minimum(c + 1, NCH - 1)
                n_items = 2 * (CH // 16)
                done = 0
                for j in range(NK):
                    h_buf[acc_at(j)] = h_buf[acc_at(j)] + q_tile(j, c)
                    upto = (j + 1) * n_items // NK
                    for m in range(done, upto):
                        relayout_part(0, nxt * (CH // 16) + m // 2, (m % 2) * (H // 2), H // 2)
                    done = upto
                return carry

            def q_cast(j, carry):
                ah_buf[pl.ds(0, X0 // 2), pl.ds(pl.multiple_of(j * E, E), E)] = _as_u32(
                    h_buf[acc_at(j)].astype(BF))
                return carry
            with jax.named_scope("sc_wq"):
                wait_raw(0, 0)
                jax.lax.fori_loop(0, CH // 16, first_chunk, 0)
                jax.lax.fori_loop(0, NCH, q_chunk, 0)
                jax.lax.fori_loop(0, NK, q_cast, 0)
            h_buf[pl.ds(0, HALO), :] = jnp.zeros((HALO, D), F32)
            h_buf[pl.ds(HALO + S, HALO), :] = jnp.zeros((HALO, D), F32)

            HP = 2
            per_head = 2 * (D // 16) // H
            it_per_chunk = H // HP // (2 * NCH)
            assert it_per_chunk * HP * per_head * 16 == CH and H - NK >= H // 2

            def kv_body(it, carry):
                i = 1 + it // (H // HP // 2)

                @pl.when(it % it_per_chunk == 0)
                def _():
                    wait_raw(i, (it // it_per_chunk) % NCH)
                NPC = 8
                rows = X0 // 2 // NPC
                for k in range(HP):
                    m = it * HP + k
                    is_k = m >= H - NK
                    mat = jnp.where(is_k, 1, 0)
                    h = jnp.where(is_k, m - (H - NK), m + NK)
                    col = jnp.where(is_k, H + h, h)
                    for n in range(NPC):
                        r = _dot(_as_bf(xn0[pl.ds(n * rows, rows), :]), _as_bf(w_t[mat, h]))
                        ah_buf[pl.ds(n * rows, rows), pl.ds(pl.multiple_of(col * E, E), E)] = _as_u32(r.astype(BF))
                        relayout_part(i, (m % (H // 2)) * per_head + n // 2, (n % 2) * (H // 2), H // 2)
                return carry
            with jax.named_scope("sc_kv"):
                jax.lax.fori_loop(0, H // HP, kv_body, 0)

            for c in mlp_weight_copies():
                c.start()
            x_rest_copy().start()

        def mlp_pre(c):
            a1_buf[pl.ds(0, 2 * HALO), :] = a1_buf[pl.ds(PAIR, 2 * HALO), :]
            y = _ln(h_buf[pl.ds(pl.multiple_of(c * PAIR + HALO, 8), PAIR + HALO), :])
            y_buf[...] = y[0:PAIR]
            z_buf[...] = _as_u32(_ln(y[HALO:]).astype(BF))

        def mlp_prologue():
            for c in mlp_weight_copies():
                c.wait()
            z = _ln(_ln(h_buf[pl.ds(0, 2 * HALO), :])).astype(BF)
            tok = jax.lax.broadcasted_iota(jnp.int32, (2 * HALO, 128), 0) - HALO

            for j in range(nD):
                a1_buf[pl.ds(PAIR, 2 * HALO), pl.ds(j * 128, 128)] = jnp.where(
                    tok >= 0, _gelu(_dot(z, w1_t[j])), 0.0)
            mlp_pre(0)

        def attention_jobs(t):
            row = jax.lax.broadcasted_iota(jnp.int32, (G * L, G * L), 0)
            col = jax.lax.broadcasted_iota(jnp.int32, (G * L, G * L), 1)

            def head_of(r):
                return jnp.where(r < G * SEG, r // SEG, (r - G * SEG) // MEM)
            mask = (head_of(row) == head_of(col)) & ((col >= G * SEG) | (row >= G * SEG) | (col <= row))
            x0 = t * PAIR
            h0 = x0 + HALO

            def step_jobs(even):
                lb = lb_e if even else lb_o
                st = {}

                lq = lq_e if even else lq_o
                def ring(r, mult):
                    return pl.multiple_of(jax.lax.rem(r, RING), mult)
                a_new = X0 // 2 + t * QR
                a_use = ring(t * SEG + (0 if even else SEG // 2), 16)

                def ahead(mat, h, col, slot):
                    cs, cb = pl.ds(h * E, E), pl.ds(col * E, E)
                    r = _dot(_as_bf(lq[...]), _as_bf(w_t[mat, h]))
                    if even:
                        ah_buf[pl.ds(ring(a_new, 8), 8), cb] = _as_u32(r[0:16].astype(BF))
                        sv[slot, :, cs] = r[16:24]
                    else:
                        ah_buf[pl.ds(ring(a_new + 8, 8), 8), cb] = _as_u32(
                            jnp.concatenate([sv[slot, :, cs], r[0:8]], axis=0).astype(BF))
                        ah_buf[pl.ds(ring(a_new + 16, 8), 8), cb] = _as_u32(r[8:24].astype(BF))
                    return _as_bf(ah_buf[pl.ds(a_use, SEG // 2), cb]), r[QR:QR + MEM]

                def in_step(mat, h, slot):
                    cs = pl.ds(h * E, E)
                    r = _dot(_as_bf(lb[...]), _as_bf(w_t[mat, h]))
                    if even:
                        sv[slot, :, cs] = r[0:8]
                        return [r[8:40]], r[40:48]
                    return [sv[slot, :, cs], r[0:24]], r[24:32]

                def stack(parts):
                    xs, ms = [p[0] for p in parts], [p[1] for p in parts]
                    if isinstance(xs[0], list):
                        return jnp.concatenate(xs[0] + xs[1] + ms, axis=0).astype(BF)
                    return jnp.concatenate(xs + [jnp.concatenate(ms, axis=0).astype(BF)], axis=0)

                def j_qkv(g, i):
                    def run():
                        h = g * G + i
                        parts = st.setdefault(('parts', g), [[], [], []])
                        parts[0].append(ahead(0, h, h, 2))
                        parts[1].append(ahead(1, h, H + h, 0) if h < NK else in_step(1, h, 0))
                        parts[2].append(in_step(2, h, 1))
                        if i == G - 1:
                            st['qkv', g] = [stack(p) for p in st.pop(('parts', g))]
                    return run

                def j_scores(g):
                    def run():
                        q, k, v = st.pop(('qkv', g))
                        s = jax.lax.dot_general(q, k, (((1,), (1,)), ((), ())),
                                                preferred_element_type=F32)
                        s = jnp.where(mask, s, -1000000000.0 / scale)
                        m = jnp.max(s, axis=-1, keepdims=True)
                        p = jnp.exp2((s - m) * (scale * LOG2E))
                        l = jnp.sum(p, axis=-1, keepdims=True)
                        r0 = pl.reciprocal(l, approx=True)
                        p = p * (r0 * (2.0 - l * r0))
                        st['p', g] = (p.astype(BF), v)
                    return run

                def j_pv(g):
                    def run():
                        p, v = st.pop(('p', g))
                        o2 = _dot(p, v)
                        for i, h in enumerate(range(g * G, (g + 1) * G)):
                            ox = o2[i * SEG:(i + 1) * SEG]
                            om = o2[G * SEG + i * MEM:G * SEG + (i + 1) * MEM]
                            cs = pl.ds(h * E, E)
                            if even:
                                ob[pl.ds(16, 4), cs] = _as_u32(ox[0:8].astype(BF))
                                ob[pl.ds(0, 16), cs] = _as_u32(
                                    jnp.concatenate([ox[8:32], om], axis=0).astype(BF))
                            else:
                                ob[pl.ds(20, 4), cs] = _as_u32(ox[0:8].astype(BF))
                                ob[pl.ds(24, 16), cs] = _as_u32(
                                    jnp.concatenate([ox[8:32], om], axis=0).astype(BF))
                    return run

                rows = pl.ds(0, 16) if even else pl.ds(16, 24)
                nrows = 32 if even else 48

                def j_wo1(j):
                    def run():
                        lhs = _as_bf(ob[rows, pl.ds(0, K1)])
                        wacc[pl.ds(0, nrows), pl.ds(j * 128, 128)] = _dot(
                            lhs, _as_bf(wo_t[j, pl.ds(0, K1 // 2), :]))
                    return run

                def j_wo2(j):
                    def run():
                        lhs = _as_bf(ob[rows, pl.ds(K1, H * E - K1)])
                        r = wacc[pl.ds(0, nrows), pl.ds(j * 128, 128)] + _dot(
                            lhs, _as_bf(wo_t[j, pl.ds(K1 // 2, (H * E - K1) // 2), :]))
                        cs = pl.ds(j * 128, 128)
                        xs = x_v[pl.ds(pl.multiple_of(x0, PAIR), PAIR), cs].astype(F32)
                        if even:
                            mem = _as_u32(r[24:32].astype(BF))
                            lb_o[pl.ds(12, 4), cs] = mem
                            lq_o[pl.ds(12, 4), cs] = mem
                            h_buf[pl.ds(pl.multiple_of(h0 + 8, 8), 24), cs] = xs[8:32] + r[0:24]
                        else:
                            mem = _as_u32(r[40:48].astype(BF))
                            lb_e[pl.ds(20, 4), cs] = mem
                            lq_e[pl.ds(12, 4), cs] = mem
                            h_buf[pl.ds(pl.multiple_of(h0, 8), 8), cs] = xs[0:8] + r[0:8]
                            h_buf[pl.ds(pl.multiple_of(h0 + 32, 8), 32), cs] = xs[32:64] + r[8:40]
                    return run

                last = n_slots - 1
                jobs = []
                for g in range(n_slots):
                    for i in range(G):
                        jobs.append((('qkv', g, i), j_qkv(g, i)))
                    if g >= 1:
                        jobs.append((('s', g - 1), j_scores(g - 1)))
                    if g >= 2:
                        jobs.append((('pv', g - 2), j_pv(g - 2)))
                wo1 = [(('wo1', j), j_wo1(j)) for j in range(nD)]
                jobs += (wo1[0:3] + [(('s', last), j_scores(last)), (('pv', last - 1), j_pv(last - 1))]
                         + wo1[3:6] + [(('pv', last), j_pv(last))] + wo1[6:8])
                jobs += [(('wo2', j), j_wo2(j)) for j in range(nD)]
                return jobs

            def j_next_xn(even):
                return lambda: store_xn(jnp.minimum(t + 1, n_pairs - 1), even)

            return step_jobs(True), step_jobs(False), j_next_xn

        after_qkv = ('s', n_slots - 2)

        def mlp_jobs(c):
            r0 = pl.multiple_of(c * PAIR, PAIR)
            st = {}

            def j_pre_next():
                mlp_pre(jnp.minimum(c + 1, n_pairs - 1))

            def j_w1(j):
                def run():
                    tok = jax.lax.broadcasted_iota(jnp.int32, (PAIR, 128), 0) + (r0 + HALO)
                    a = _gelu(_dot(_as_bf(z_buf[...]), w1_t[j]))
                    a1_buf[pl.ds(2 * HALO, PAIR), pl.ds(j * 128, 128)] = jnp.where(tok < S, a, 0.0)
                return run

            def j_shift():
                cq = D // 4
                st['g'] = jnp.concatenate([
                    a1_buf[pl.ds(HALO - 1, PAIR), pl.ds(0 * cq, cq)],
                    a1_buf[pl.ds(HALO + 1, PAIR), pl.ds(1 * cq, cq)],
                    a1_buf[pl.ds(HALO - 2, PAIR), pl.ds(2 * cq, cq)],
                    a1_buf[pl.ds(HALO + 2, PAIR), pl.ds(3 * cq, cq)]], axis=1).astype(BF)

            def j_w2(j):
                def run():
                    st['x1', j] = y_buf[:, pl.ds(j * 128, 128)] + _dot(st['g'], w2_t[j])
                return run

            def j_ln3():
                x1 = jnp.concatenate([st['x1', j] for j in range(nD)], axis=1)
                st['z1'] = _ln(x1).astype(BF)

            def j_w3(j):
                def run():
                    st['a3', j] = _gelu(_dot(st['z1'], w3_t[j])).astype(BF)
                return run

            def j_cat():
                st['a3'] = jnp.concatenate([st.pop(('a3', j)) for j in range(nF)], axis=1)

            def j_w4(j):
                def run():
                    cs = pl.ds(j * 128, 128)
                    hh = h_buf[pl.ds(pl.multiple_of(r0 + HALO, 8), PAIR), cs]
                    out_v[pl.ds(r0, PAIR), cs] = (
                        hh + (st['x1', j] + _dot(st['a3'], w4_t[j]))).astype(out_v.dtype)
                return run

            return dict(pre_next=j_pre_next, w1=[j_w1(j) for j in range(nD)], shift=j_shift,
                        w2=[j_w2(j) for j in range(nD)], ln3=j_ln3,
                        w3=[j_w3(j) for j in range(nF)], cat=j_cat,
                        w4=[j_w4(j) for j in range(nD)])

        def attention_only(t, carry):
            ej, oj, j_next_xn = attention_jobs(t)

            def j_wo_wait():
                with jax.named_scope("sc_wo_finish"):
                    pl.when(t == 0)(wo_finish)
            _run(_interleave(ej, {after_qkv: [j_wo_wait]})
                 + _interleave(oj, {('qkv', 4, 0): [j_next_xn(True)], after_qkv: [j_next_xn(False)]}))
            return carry

        def fused(t, carry):
            @pl.when(t == LAG)
            def _():
                x_rest_copy().wait()

            @pl.when(t > LAG)
            def _():
                out_copy(t - LAG - 1).start()

            ej, oj, j_next_xn = attention_jobs(t)
            b = mlp_jobs(t - LAG)
            w3, w4 = b['w3'], b['w4']
            fe, fo = {}, {}

            def put(d, label, *jobs):
                d.setdefault(label, []).extend(jobs)
            for i in range(nD):
                put(fe, ('qkv', 2 + i // 2, i % 2), b['w1'][i])
                put(fe, ('qkv', 8 + i // 2, i % 2), b['w2'][i])
            put(fe, ('qkv', 6, 0), b['shift'])
            put(fe, ('qkv', 12, 0), b['ln3'])
            put(fe, ('qkv', 15, 0), w3[0])
            put(fe, 'end', *w3[1:4])
            put(fo, ('qkv', 0, 1), b['pre_next'])
            for k in range(4, nF):
                put(fo, ('qkv', 1 + (k - 4) // 2, (k - 4) % 2), w3[k])
            put(fo, ('qkv', 13, 0), b['cat'])
            put(fo, ('qkv', 14, 0), w4[0])
            put(fo, ('qkv', 15, 0), w4[1])
            put(fo, ('qkv', 4, 0), j_next_xn(True))
            put(fo, after_qkv, j_next_xn(False))
            put(fo, ('s', n_slots - 1), w4[2])
            put(fo, 'end', *w4[3:])
            with jax.named_scope("sc_fused_body"):
                _run(_interleave(ej, fe) + _interleave(oj, fo))
            return carry

        def mlp_only(c, carry):
            out_copy(c - 1).start()
            b = mlp_jobs(c)
            _run(b['w1'] + [b['shift']] + b['w2'] + [b['ln3'], b['pre_next']] + b['w3'] + [b['cat']] + b['w4'])
            return carry

        with jax.named_scope("sc_prologue"):
            prologue()
            store_xn(0, True)
            store_xn(0, False)
        with jax.named_scope("sc_a_only"):
            jax.lax.fori_loop(0, LAG, attention_only, 0)
        with jax.named_scope("sc_mlp_prologue"):
            mlp_prologue()
        with jax.named_scope("sc_fused"):
            jax.lax.fori_loop(LAG, n_pairs, fused, 0)
        with jax.named_scope("sc_b_tail"):
            jax.lax.fori_loop(n_pairs - LAG, n_pairs, mlp_only, 0)
        out_copy(n_pairs - 1).start()
        pltpu.make_async_copy(out_v, out_hbm, sems.at[OUT_SEM]).wait()

    return kernel, WO_SEM + nD + 6, X0, RING


@functools.partial(jax.jit, static_argnames=("A_seg_len",))
def pallas_sequential_preLN__memory_aug_recurrent_mem_tr__mixer_s_mlp__prompt_kernel(
    A_x, A_mem0, A_Wq, A_Wk, A_Wv, A_Wo, A_seg_len, B_x, B_w1, B_w2, B_w3, B_w4,
):
    _, S, D = A_x.shape
    H, E = A_Wq.shape[1], A_Wq.shape[2]
    F = B_w3.shape[1]
    assert A_seg_len == SEG and A_mem0.shape[1] == MEM and S % PAIR == 0
    nD, nF = D // 128, F // 128

    x = A_x.reshape(S, D)
    mem0 = A_mem0.reshape(MEM, D)
    wo = A_Wo.reshape(H * E, D)

    kernel, n_sems, x0, ring = _make_kernel(S, D, H, E, F)
    any_spec = pl.BlockSpec(memory_space=pl.ANY)
    out = pl.pallas_call(
        kernel,
        in_specs=[any_spec] * 10,
        out_specs=any_spec,
        out_shape=jax.ShapeDtypeStruct((S, D), A_x.dtype),
        scratch_shapes=[
            pltpu.VMEM((3, D, H, E), BF),
            pltpu.VMEM((3, H, D // 2, E), U32),
            pltpu.VMEM((H * E, D), BF),
            pltpu.VMEM((nD, H * E // 2, 128), U32),
            pltpu.VMEM((nD, D, 128), BF),
            pltpu.VMEM((nD, D, 128), BF),
            pltpu.VMEM((nF, D, 128), BF),
            pltpu.VMEM((nD, F, 128), BF),
            pltpu.VMEM((S, D), BF),
            pltpu.VMEM((S, D), BF),
            pltpu.VMEM((MEM, D), BF),
            pltpu.VMEM((x0 // 2, D), U32),
            pltpu.VMEM((ring, (H + NK) * E), U32),
            pltpu.VMEM((16, D), U32),
            pltpu.VMEM((16, D), U32),
            pltpu.VMEM((24, D), U32),
            pltpu.VMEM((16, D), U32),
            pltpu.VMEM((3, 8, H * E), F32),
            pltpu.VMEM((40, H * E), U32),
            pltpu.VMEM((48, D), F32),
            pltpu.VMEM((S + 2 * HALO, D), F32),
            pltpu.VMEM((PAIR + 2 * HALO, D), F32),
            pltpu.VMEM((PAIR, D), F32),
            pltpu.VMEM((PAIR // 2, D), U32),
            pltpu.SemaphoreType.DMA((n_sems,)),
        ],
        compiler_params=pltpu.CompilerParams(
            vmem_limit_bytes=124 * 1024 * 1024,
            disable_bounds_checks=True,
        ),
    )(x, mem0, A_Wq, A_Wk, A_Wv, wo, B_w1, B_w2, B_w3, B_w4)
    return out.reshape(1, S, D)
```

```python
import functools

import jax
import jax.numpy as jnp
from jax.experimental import pallas as pl
from jax.experimental.pallas import tpu as pltpu

BF = jnp.bfloat16
F32 = jnp.float32
U32 = jnp.uint32

SEG = 32
MEM = 8
PAIR = 2 * SEG
LAG = 3
HALO = 8
G = 2
TAIL_HEADS = 6
QR = 24
NK = 14
QPC = 4
NCH = 8
LN_EPS = 1e-5
LOG2E = 1.4426950408889634


def _ln(x):
    m = jnp.mean(x, axis=-1, keepdims=True)
    xc = x - m
    v = jnp.mean(xc * xc, axis=-1, keepdims=True)
    return xc * jax.lax.rsqrt(v + LN_EPS)


_dot = functools.partial(jnp.dot, preferred_element_type=F32)


def _gelu(x):
    return jax.nn.gelu(x, approximate=True)


def _as_bf(x_u32):
    return pltpu.bitcast(x_u32, BF)


def _as_u32(x_bf):
    return pltpu.bitcast(x_bf, U32)


def _interleave(main, fill):
    fill = dict(fill)
    out = []
    for label, job in main:
        out.extend(fill.pop(label, []))
        out.append(job)
    out.extend(fill.pop('end', []))
    assert not fill, fill
    return out


def _run(jobs):
    for job in jobs:
        job()


def _make_kernel(S, D, H, E, F):
    n_pairs = S // PAIR
    nD = D // 128
    nF = F // 128
    scale = float(E) ** -0.5
    L = MEM + SEG
    n_slots = H // G
    K1 = (H - TAIL_HEADS) * E
    CH = D // NCH
    WO_CH = H * E // nD
    X0 = S - 2 * QR * n_pairs
    assert X0 % PAIR == 0 and X0 // PAIR - 1 >= LAG and X0 < S
    RING = (X0 + PAIR) // 2
    assert RING % 16 == 0 and NK % G == 0
    assert G == 2 and n_slots == 16 and nF == 28 and nD == 8
    assert (H - TAIL_HEADS) // G - 1 < n_slots - 2

    WO_SEM = 3 * NCH
    B_SEM, X0_SEM, XM_SEM, X1_SEM, MEM_SEM, OUT_SEM = (WO_SEM + nD + i for i in range(6))
    XA = X0 + 2 * QR
    XB = X0 + 2 * QR * (LAG + 1)

    def kernel(x_hbm, mem0_hbm, wq_hbm, wk_hbm, wv_hbm, wo_hbm, w1_hbm, w2_hbm, w3_hbm, w4_hbm,
               out_hbm,
               raw, w_t, wo_raw, wo_t, w1_t, w2_t, w3_t, w4_t,
               x_v, out_v, mem0_v, xn0, ah_buf, lq_e, lq_o, lb_e, lb_o, sv, ob, wacc,
               h_buf, a1_buf, y_buf, z_buf, sems):

        def rows_copy(src, dst, start, size, sem):
            return pltpu.make_async_copy(src.at[pl.ds(start, size)], dst.at[pl.ds(start, size)], sems.at[sem])

        def raw_copy(i, c):
            src = (wq_hbm, wk_hbm, wv_hbm)[i]
            return rows_copy(src, raw.at[i], c * CH, CH, i * NCH + c)

        def wo_copy(j):
            return rows_copy(wo_hbm, wo_raw, j * WO_CH, WO_CH, WO_SEM + j)

        def mlp_weight_copies():
            return [pltpu.make_async_copy(src.at[:, pl.ds(j * 128, 128)], dst.at[j], sems.at[B_SEM])
                    for src, dst, n in ((w1_hbm, w1_t, nD), (w2_hbm, w2_t, nD),
                                        (w3_hbm, w3_t, nF), (w4_hbm, w4_t, nD))
                    for j in range(n)]

        def x_head_copy():
            return rows_copy(x_hbm, x_v, 0, XA, X0_SEM)

        def x_mid_copy():
            return rows_copy(x_hbm, x_v, XA, XB - XA, XM_SEM)

        def x_rest_copy():
            return rows_copy(x_hbm, x_v, XB, S - XB, X1_SEM)

        def mem_copy():
            return pltpu.make_async_copy(mem0_hbm, mem0_v, sems.at[MEM_SEM])

        def out_copy(c):
            return rows_copy(out_v, out_hbm, pl.multiple_of(c * PAIR, PAIR), PAIR, OUT_SEM)

        def relayout_part(i, b, h0, nh):
            x = raw[i, pl.ds(pl.multiple_of(b * 16, 16), 16), pl.ds(h0, nh), :]
            x = _as_u32(x).reshape(8, 2, nh // 2, E)
            ev, od = x[:, 0], x[:, 1]
            lo = jnp.swapaxes((ev & 0xFFFF) | (od << 16), 0, 1)
            hi = jnp.swapaxes((ev >> 16) | (od & jnp.uint32(0xFFFF0000)), 0, 1)
            rows = pl.ds(pl.multiple_of(b * 8, 8), 8)
            for p in range(nh // 2):
                w_t[i, h0 + 2 * p, rows, :] = lo[p]
                w_t[i, h0 + 2 * p + 1, rows, :] = hi[p]

        def relayout_block(i, b):
            relayout_part(i, b, 0, H)

        def wo_finish():
            def chunk(j, carry):
                dst = wo_raw.at[pl.ds(j * WO_CH, WO_CH)]
                pltpu.make_async_copy(dst, dst, sems.at[WO_SEM + j]).wait()

                def body(b, carry):
                    r = j * WO_CH + b * 256
                    for m in range(4):
                        blk = wo_raw[pl.ds(pl.multiple_of(r + m * 64, 64), 64), :]
                        for n in range(nD):
                            wo_t[n, pl.ds(pl.multiple_of((r + m * 64) // 2, 32), 32), :] = _as_u32(
                                blk[:, n * 128:(n + 1) * 128])
                    return carry
                return jax.lax.fori_loop(0, WO_CH // 256, body, carry)
            jax.lax.fori_loop(0, nD, chunk, 0)
            x_mid_copy().wait()

        def store_xn(t, even):
            x0 = pl.multiple_of(t * PAIR, PAIR)
            q0 = pl.multiple_of(X0 + t * 2 * QR, 16)
            if even:
                xn = _ln(x_v[pl.ds(x0, 40), :].astype(F32))
                lb_e[pl.ds(0, 4), :] = _as_u32(xn[32:40].astype(BF))
                lb_e[pl.ds(4, 4), :] = _as_u32(xn[0:8].astype(BF))
                lb_e[pl.ds(8, 8), :] = _as_u32(xn[8:24].astype(BF))
                lb_e[pl.ds(16, 4), :] = _as_u32(xn[24:32].astype(BF))
                xq = _ln(x_v[pl.ds(q0, QR), :].astype(F32))
                lq_e[pl.ds(0, 8), :] = _as_u32(xq[0:16].astype(BF))
                lq_e[pl.ds(8, 4), :] = _as_u32(xq[16:24].astype(BF))
            else:
                xn = _ln(x_v[pl.ds(x0 + 40, 24), :].astype(F32))
                lb_o[pl.ds(0, 8), :] = _as_u32(xn[0:16].astype(BF))
                lb_o[pl.ds(8, 4), :] = _as_u32(xn[16:24].astype(BF))
                xq = _ln(x_v[pl.ds(q0 + QR, QR), :].astype(F32))
                for n in range(3):
                    lq_o[pl.ds(4 * n, 4), :] = _as_u32(xq[8 * n:8 * n + 8].astype(BF))

        def prologue():
            x_head_copy().start()
            mem_copy().start()
            for i in range(3):
                for c in range(NCH):
                    raw_copy(i, c).start()
            for j in range(nD):
                wo_copy(j).start()
            x_mid_copy().start()

            assert CH == 128 and NK <= nD * (S // X0)

            def acc_at(j):
                if isinstance(j, int):
                    return pl.ds((j // nD) * X0, X0), pl.ds((j % nD) * 128, 128)
                return (pl.ds(pl.multiple_of((j // nD) * X0, X0), X0),
                        pl.ds(pl.multiple_of((j % nD) * 128, 128), 128))

            def zero_acc(j, carry):
                h_buf[acc_at(j)] = jnp.zeros((X0, 128), F32)
                return carry
            jax.lax.fori_loop(0, NK, zero_acc, 0)
            x_head_copy().wait()
            mem_copy().wait()
            lb_e[pl.ds(20, 4), :] = _as_u32(mem0_v[...])
            lq_e[pl.ds(12, 4), :] = _as_u32(mem0_v[...])

            def ln_body(b, carry):
                rows = x_v[pl.ds(pl.multiple_of(b * 64, 64), 64), :].astype(F32)
                xn0[pl.ds(pl.multiple_of(b * 32, 32), 32), :] = _as_u32(_ln(rows).astype(BF))
                return carry
            jax.lax.fori_loop(0, X0 // 64, ln_body, 0)

            def wait_raw(i, c):
                dst = raw.at[i, pl.ds(c * CH, CH)]
                pltpu.make_async_copy(dst, dst, sems.at[i * NCH + c]).wait()

            def q_tile(j, c):
                lhs = _as_bf(xn0[:, pl.ds(pl.multiple_of(c * 128, 128), 128)])
                return _dot(lhs, _as_bf(w_t[0, j, pl.ds(pl.multiple_of(c * 64, 64), 64), :]))

            def first_chunk(b, carry):
                relayout_block(0, b)
                return carry

            def q_chunk(c, carry):
                @pl.when(c + 1 < NCH)
                def _():
                    wait_raw(0, c + 1)
                nxt = jnp.minimum(c + 1, NCH - 1)
                n_items = 2 * (CH // 16)
                done = 0
                rows = X0 // QPC
                for j in range(NK):
                    for n in range(QPC):
                        at = (pl.ds((j // nD) * X0 + n * rows, rows), pl.ds((j % nD) * 128, 128))
                        lhs = _as_bf(xn0[pl.ds(n * rows // 2, rows // 2), pl.ds(pl.multiple_of(c * 128, 128), 128)])
                        h_buf[at] = h_buf[at] + _dot(
                            lhs, _as_bf(w_t[0, j, pl.ds(pl.multiple_of(c * 64, 64), 64), :]))
                        upto = (j * QPC + n + 1) * n_items // (NK * QPC)
                        for m in range(done, upto):
                            relayout_part(0, nxt * (CH // 16) + m // 2, (m % 2) * (H // 2), H // 2)
                        done = upto
                return carry

            def q_cast(j, carry):
                ah_buf[pl.ds(0, X0 // 2), pl.ds(pl.multiple_of(j * E, E), E)] = _as_u32(
                    h_buf[acc_at(j)].astype(BF))
                return carry
            with jax.named_scope("sc_wq"):
                wait_raw(0, 0)
                jax.lax.fori_loop(0, CH // 16, first_chunk, 0)
                jax.lax.fori_loop(0, NCH, q_chunk, 0)
                jax.lax.fori_loop(0, NK, q_cast, 0)
            h_buf[pl.ds(0, HALO), :] = jnp.zeros((HALO, D), F32)
            h_buf[pl.ds(HALO + S, HALO), :] = jnp.zeros((HALO, D), F32)

            HP = 2
            per_head = 2 * (D // 16) // H
            it_per_chunk = H // HP // (2 * NCH)
            assert it_per_chunk * HP * per_head * 16 == CH and H - NK >= H // 2

            def kv_body(it, carry):
                i = 1 + it // (H // HP // 2)

                @pl.when(it % it_per_chunk == 0)
                def _():
                    wait_raw(i, (it // it_per_chunk) % NCH)
                NPC = 8
                rows = X0 // 2 // NPC
                for k in range(HP):
                    m = it * HP + k
                    is_k = m >= H - NK
                    mat = jnp.where(is_k, 1, 0)
                    h = jnp.where(is_k, m - (H - NK), m + NK)
                    col = jnp.where(is_k, H + h, h)
                    for n in range(NPC):
                        r = _dot(_as_bf(xn0[pl.ds(n * rows, rows), :]), _as_bf(w_t[mat, h]))
                        ah_buf[pl.ds(n * rows, rows), pl.ds(pl.multiple_of(col * E, E), E)] = _as_u32(r.astype(BF))
                        relayout_part(i, (m % (H // 2)) * per_head + n // 2, (n % 2) * (H // 2), H // 2)
                return carry
            with jax.named_scope("sc_kv"):
                jax.lax.fori_loop(0, H // HP, kv_body, 0)

            for c in mlp_weight_copies():
                c.start()
            x_rest_copy().start()

        def mlp_pre(c):
            a1_buf[pl.ds(0, 2 * HALO), :] = a1_buf[pl.ds(PAIR, 2 * HALO), :]
            y = _ln(h_buf[pl.ds(pl.multiple_of(c * PAIR + HALO, 8), PAIR + HALO), :])
            y_buf[...] = y[0:PAIR]
            z_buf[...] = _as_u32(_ln(y[HALO:]).astype(BF))

        def mlp_prologue():
            for c in mlp_weight_copies():
                c.wait()
            z = _ln(_ln(h_buf[pl.ds(0, 2 * HALO), :])).astype(BF)
            tok = jax.lax.broadcasted_iota(jnp.int32, (2 * HALO, 128), 0) - HALO

            for j in range(nD):
                a1_buf[pl.ds(PAIR, 2 * HALO), pl.ds(j * 128, 128)] = jnp.where(
                    tok >= 0, _gelu(_dot(z, w1_t[j])), 0.0)
            mlp_pre(0)

        def attention_jobs(t):
            row = jax.lax.broadcasted_iota(jnp.int32, (G * L, G * L), 0)
            col = jax.lax.broadcasted_iota(jnp.int32, (G * L, G * L), 1)

            def head_of(r):
                return jnp.where(r < G * SEG, r // SEG, (r - G * SEG) // MEM)
            mask = (head_of(row) == head_of(col)) & ((col >= G * SEG) | (row >= G * SEG) | (col <= row))
            x0 = t * PAIR
            h0 = x0 + HALO

            def step_jobs(even):
                lb = lb_e if even else lb_o
                st = {}

                lq = lq_e if even else lq_o
                def ring(r, mult):
                    return pl.multiple_of(jax.lax.rem(r, RING), mult)
                a_new = X0 // 2 + t * QR
                a_use = ring(t * SEG + (0 if even else SEG // 2), 16)

                def ahead(mat, h, col, slot):
                    cs, cb = pl.ds(h * E, E), pl.ds(col * E, E)
                    r = _dot(_as_bf(lq[...]), _as_bf(w_t[mat, h]))
                    if even:
                        ah_buf[pl.ds(ring(a_new, 8), 8), cb] = _as_u32(r[0:16].astype(BF))
                        sv[slot, :, cs] = r[16:24]
                    else:
                        ah_buf[pl.ds(ring(a_new + 8, 8), 8), cb] = _as_u32(
                            jnp.concatenate([sv[slot, :, cs], r[0:8]], axis=0).astype(BF))
                        ah_buf[pl.ds(ring(a_new + 16, 8), 8), cb] = _as_u32(r[8:24].astype(BF))
                    return _as_bf(ah_buf[pl.ds(a_use, SEG // 2), cb]), r[QR:QR + MEM]

                def in_step(mat, h, slot):
                    cs = pl.ds(h * E, E)
                    r = _dot(_as_bf(lb[...]), _as_bf(w_t[mat, h]))
                    if even:
                        sv[slot, :, cs] = r[0:8]
                        return [r[8:40]], r[40:48]
                    return [sv[slot, :, cs], r[0:24]], r[24:32]

                def stack(parts):
                    xs, ms = [p[0] for p in parts], [p[1] for p in parts]
                    if isinstance(xs[0], list):
                        return jnp.concatenate(xs[0] + xs[1] + ms, axis=0).astype(BF)
                    return jnp.concatenate(xs + [jnp.concatenate(ms, axis=0).astype(BF)], axis=0)

                def j_qkv(g, i):
                    def run():
                        h = g * G + i
                        parts = st.setdefault(('parts', g), [[], [], []])
                        parts[0].append(ahead(0, h, h, 2))
                        parts[1].append(ahead(1, h, H + h, 0) if h < NK else in_step(1, h, 0))
                        parts[2].append(in_step(2, h, 1))
                        if i == G - 1:
                            st['qkv', g] = [stack(p) for p in st.pop(('parts', g))]
                    return run

                def j_scores(g):
                    def run():
                        q, k, v = st.pop(('qkv', g))
                        s = jax.lax.dot_general(q, k, (((1,), (1,)), ((), ())),
                                                preferred_element_type=F32)
                        s = jnp.where(mask, s, -1000000000.0 / scale)
                        m = jnp.max(s, axis=-1, keepdims=True)
                        p = jnp.exp2((s - m) * (scale * LOG2E))
                        l = jnp.sum(p, axis=-1, keepdims=True)
                        r0 = pl.reciprocal(l, approx=True)
                        p = p * (r0 * (2.0 - l * r0))
                        st['p', g] = (p.astype(BF), v)
                    return run

                def j_pv(g):
                    def run():
                        p, v = st.pop(('p', g))
                        o2 = _dot(p, v)
                        for i, h in enumerate(range(g * G, (g + 1) * G)):
                            ox = o2[i * SEG:(i + 1) * SEG]
                            om = o2[G * SEG + i * MEM:G * SEG + (i + 1) * MEM]
                            cs = pl.ds(h * E, E)
                            if even:
                                ob[pl.ds(16, 4), cs] = _as_u32(ox[0:8].astype(BF))
                                ob[pl.ds(0, 16), cs] = _as_u32(
                                    jnp.concatenate([ox[8:32], om], axis=0).astype(BF))
                            else:
                                ob[pl.ds(20, 4), cs] = _as_u32(ox[0:8].astype(BF))
                                ob[pl.ds(24, 16), cs] = _as_u32(
                                    jnp.concatenate([ox[8:32], om], axis=0).astype(BF))
                    return run

                rows = pl.ds(0, 16) if even else pl.ds(16, 24)
                nrows = 32 if even else 48

                def j_wo1(j):
                    def run():
                        lhs = _as_bf(ob[rows, pl.ds(0, K1)])
                        wacc[pl.ds(0, nrows), pl.ds(j * 128, 128)] = _dot(
                            lhs, _as_bf(wo_t[j, pl.ds(0, K1 // 2), :]))
                    return run

                def j_wo2(j):
                    def run():
                        lhs = _as_bf(ob[rows, pl.ds(K1, H * E - K1)])
                        r = wacc[pl.ds(0, nrows), pl.ds(j * 128, 128)] + _dot(
                            lhs, _as_bf(wo_t[j, pl.ds(K1 // 2, (H * E - K1) // 2), :]))
                        cs = pl.ds(j * 128, 128)
                        xs = x_v[pl.ds(pl.multiple_of(x0, PAIR), PAIR), cs].astype(F32)
                        if even:
                            mem = _as_u32(r[24:32].astype(BF))
                            lb_o[pl.ds(12, 4), cs] = mem
                            lq_o[pl.ds(12, 4), cs] = mem
                            h_buf[pl.ds(pl.multiple_of(h0 + 8, 8), 24), cs] = xs[8:32] + r[0:24]
                        else:
                            mem = _as_u32(r[40:48].astype(BF))
                            lb_e[pl.ds(20, 4), cs] = mem
                            lq_e[pl.ds(12, 4), cs] = mem
                            h_buf[pl.ds(pl.multiple_of(h0, 8), 8), cs] = xs[0:8] + r[0:8]
                            h_buf[pl.ds(pl.multiple_of(h0 + 32, 8), 32), cs] = xs[32:64] + r[8:40]
                    return run

                last = n_slots - 1
                jobs = []
                for g in range(n_slots):
                    for i in range(G):
                        jobs.append((('qkv', g, i), j_qkv(g, i)))
                    if g >= 1:
                        jobs.append((('s', g - 1), j_scores(g - 1)))
                    if g >= 2:
                        jobs.append((('pv', g - 2), j_pv(g - 2)))
                wo1 = [(('wo1', j), j_wo1(j)) for j in range(nD)]
                jobs += (wo1[0:3] + [(('s', last), j_scores(last)), (('pv', last - 1), j_pv(last - 1))]
                         + wo1[3:6] + [(('pv', last), j_pv(last))] + wo1[6:8])
                jobs += [(('wo2', j), j_wo2(j)) for j in range(nD)]
                return jobs

            def j_next_xn(even):
                return lambda: store_xn(jnp.minimum(t + 1, n_pairs - 1), even)

            return step_jobs(True), step_jobs(False), j_next_xn

        after_qkv = ('s', n_slots - 2)

        def mlp_jobs(c):
            r0 = pl.multiple_of(c * PAIR, PAIR)
            st = {}

            def j_pre_next():
                mlp_pre(jnp.minimum(c + 1, n_pairs - 1))

            def j_w1(j):
                def run():
                    tok = jax.lax.broadcasted_iota(jnp.int32, (PAIR, 128), 0) + (r0 + HALO)
                    a = _gelu(_dot(_as_bf(z_buf[...]), w1_t[j]))
                    a1_buf[pl.ds(2 * HALO, PAIR), pl.ds(j * 128, 128)] = jnp.where(tok < S, a, 0.0)
                return run

            def j_shift():
                cq = D // 4
                st['g'] = jnp.concatenate([
                    a1_buf[pl.ds(HALO - 1, PAIR), pl.ds(0 * cq, cq)],
                    a1_buf[pl.ds(HALO + 1, PAIR), pl.ds(1 * cq, cq)],
                    a1_buf[pl.ds(HALO - 2, PAIR), pl.ds(2 * cq, cq)],
                    a1_buf[pl.ds(HALO + 2, PAIR), pl.ds(3 * cq, cq)]], axis=1).astype(BF)

            def j_w2(j):
                def run():
                    st['x1', j] = y_buf[:, pl.ds(j * 128, 128)] + _dot(st['g'], w2_t[j])
                return run

            def j_ln3():
                x1 = jnp.concatenate([st['x1', j] for j in range(nD)], axis=1)
                st['z1'] = _ln(x1).astype(BF)

            def j_w3(j):
                def run():
                    st['a3', j] = _gelu(_dot(st['z1'], w3_t[j])).astype(BF)
                return run

            def j_cat():
                st['a3'] = jnp.concatenate([st.pop(('a3', j)) for j in range(nF)], axis=1)

            def j_w4(j):
                def run():
                    cs = pl.ds(j * 128, 128)
                    hh = h_buf[pl.ds(pl.multiple_of(r0 + HALO, 8), PAIR), cs]
                    out_v[pl.ds(r0, PAIR), cs] = (
                        hh + (st['x1', j] + _dot(st['a3'], w4_t[j]))).astype(out_v.dtype)
                return run

            return dict(pre_next=j_pre_next, w1=[j_w1(j) for j in range(nD)], shift=j_shift,
                        w2=[j_w2(j) for j in range(nD)], ln3=j_ln3,
                        w3=[j_w3(j) for j in range(nF)], cat=j_cat,
                        w4=[j_w4(j) for j in range(nD)])

        def attention_only(t, carry):
            ej, oj, j_next_xn = attention_jobs(t)

            def j_wo_wait():
                with jax.named_scope("sc_wo_finish"):
                    pl.when(t == 0)(wo_finish)
            _run(_interleave(ej, {after_qkv: [j_wo_wait]})
                 + _interleave(oj, {('qkv', 4, 0): [j_next_xn(True)], after_qkv: [j_next_xn(False)]}))
            return carry

        def fused(t, carry):
            @pl.when(t == LAG)
            def _():
                x_rest_copy().wait()

            @pl.when(t > LAG)
            def _():
                out_copy(t - LAG - 1).start()

            ej, oj, j_next_xn = attention_jobs(t)
            b = mlp_jobs(t - LAG)
            w3, w4 = b['w3'], b['w4']
            fe, fo = {}, {}

            def put(d, label, *jobs):
                d.setdefault(label, []).extend(jobs)
            for i in range(nD):
                put(fe, ('qkv', 2 + i // 2, i % 2), b['w1'][i])
                put(fe, ('qkv', 8 + i // 2, i % 2), b['w2'][i])
            put(fe, ('qkv', 6, 0), b['shift'])
            put(fe, ('qkv', 12, 0), b['ln3'])
            put(fe, ('qkv', 15, 0), w3[0])
            put(fe, 'end', *w3[1:4])
            put(fo, ('qkv', 0, 1), b['pre_next'])
            for k in range(4, nF):
                put(fo, ('qkv', 1 + (k - 4) // 2, (k - 4) % 2), w3[k])
            put(fo, ('qkv', 13, 0), b['cat'])
            put(fo, ('qkv', 14, 0), w4[0])
            put(fo, ('qkv', 15, 0), w4[1])
            put(fo, ('qkv', 4, 0), j_next_xn(True))
            put(fo, after_qkv, j_next_xn(False))
            put(fo, ('s', n_slots - 1), w4[2])
            put(fo, 'end', *w4[3:])
            with jax.named_scope("sc_fused_body"):
                _run(_interleave(ej, fe) + _interleave(oj, fo))
            return carry

        def mlp_only(c, carry):
            out_copy(c - 1).start()
            b = mlp_jobs(c)
            _run(b['w1'] + [b['shift']] + b['w2'] + [b['ln3'], b['pre_next']] + b['w3'] + [b['cat']] + b['w4'])
            return carry

        with jax.named_scope("sc_prologue"):
            prologue()
            store_xn(0, True)
            store_xn(0, False)
        with jax.named_scope("sc_a_only"):
            jax.lax.fori_loop(0, LAG, attention_only, 0)
        with jax.named_scope("sc_mlp_prologue"):
            mlp_prologue()
        with jax.named_scope("sc_fused"):
            jax.lax.fori_loop(LAG, n_pairs, fused, 0)
        with jax.named_scope("sc_b_tail"):
            jax.lax.fori_loop(n_pairs - LAG, n_pairs, mlp_only, 0)
        out_copy(n_pairs - 1).start()
        pltpu.make_async_copy(out_v, out_hbm, sems.at[OUT_SEM]).wait()

    return kernel, WO_SEM + nD + 6, X0, RING


@functools.partial(jax.jit, static_argnames=("A_seg_len",))
def pallas_sequential_preLN__memory_aug_recurrent_mem_tr__mixer_s_mlp__prompt_kernel(
    A_x, A_mem0, A_Wq, A_Wk, A_Wv, A_Wo, A_seg_len, B_x, B_w1, B_w2, B_w3, B_w4,
):
    _, S, D = A_x.shape
    H, E = A_Wq.shape[1], A_Wq.shape[2]
    F = B_w3.shape[1]
    assert A_seg_len == SEG and A_mem0.shape[1] == MEM and S % PAIR == 0
    nD, nF = D // 128, F // 128

    x = A_x.reshape(S, D)
    mem0 = A_mem0.reshape(MEM, D)
    wo = A_Wo.reshape(H * E, D)

    kernel, n_sems, x0, ring = _make_kernel(S, D, H, E, F)
    any_spec = pl.BlockSpec(memory_space=pl.ANY)
    out = pl.pallas_call(
        kernel,
        in_specs=[any_spec] * 10,
        out_specs=any_spec,
        out_shape=jax.ShapeDtypeStruct((S, D), A_x.dtype),
        scratch_shapes=[
            pltpu.VMEM((3, D, H, E), BF),
            pltpu.VMEM((3, H, D // 2, E), U32),
            pltpu.VMEM((H * E, D), BF),
            pltpu.VMEM((nD, H * E // 2, 128), U32),
            pltpu.VMEM((nD, D, 128), BF),
            pltpu.VMEM((nD, D, 128), BF),
            pltpu.VMEM((nF, D, 128), BF),
            pltpu.VMEM((nD, F, 128), BF),
            pltpu.VMEM((S, D), BF),
            pltpu.VMEM((S, D), BF),
            pltpu.VMEM((MEM, D), BF),
            pltpu.VMEM((x0 // 2, D), U32),
            pltpu.VMEM((ring, (H + NK) * E), U32),
            pltpu.VMEM((16, D), U32),
            pltpu.VMEM((16, D), U32),
            pltpu.VMEM((24, D), U32),
            pltpu.VMEM((16, D), U32),
            pltpu.VMEM((3, 8, H * E), F32),
            pltpu.VMEM((40, H * E), U32),
            pltpu.VMEM((48, D), F32),
            pltpu.VMEM((S + 2 * HALO, D), F32),
            pltpu.VMEM((PAIR + 2 * HALO, D), F32),
            pltpu.VMEM((PAIR, D), F32),
            pltpu.VMEM((PAIR // 2, D), U32),
            pltpu.SemaphoreType.DMA((n_sems,)),
        ],
        compiler_params=pltpu.CompilerParams(
            vmem_limit_bytes=124 * 1024 * 1024,
            disable_bounds_checks=True,
        ),
    )(x, mem0, A_Wq, A_Wk, A_Wv, wo, B_w1, B_w2, B_w3, B_w4)
    return out.reshape(1, S, D)
```

```python
import functools

import jax
import jax.numpy as jnp
from jax.experimental import pallas as pl
from jax.experimental.pallas import tpu as pltpu

BF = jnp.bfloat16
F32 = jnp.float32
U32 = jnp.uint32

SEG = 32
MEM = 8
PAIR = 2 * SEG
LAG = 3
HALO = 8
G = 2
TAIL_HEADS = 6
QR = 24
NK = 16
QPC = 4
NCH = 8
LN_EPS = 1e-5
LOG2E = 1.4426950408889634


def _ln(x):
    m = jnp.mean(x, axis=-1, keepdims=True)
    xc = x - m
    v = jnp.mean(xc * xc, axis=-1, keepdims=True)
    return xc * jax.lax.rsqrt(v + LN_EPS)


_dot = functools.partial(jnp.dot, preferred_element_type=F32)


def _gelu(x):
    return jax.nn.gelu(x, approximate=True)


def _as_bf(x_u32):
    return pltpu.bitcast(x_u32, BF)


def _as_u32(x_bf):
    return pltpu.bitcast(x_bf, U32)


def _interleave(main, fill):
    fill = dict(fill)
    out = []
    for label, job in main:
        out.extend(fill.pop(label, []))
        out.append(job)
    out.extend(fill.pop('end', []))
    assert not fill, fill
    return out


def _run(jobs):
    for job in jobs:
        job()


def _make_kernel(S, D, H, E, F):
    n_pairs = S // PAIR
    nD = D // 128
    nF = F // 128
    scale = float(E) ** -0.5
    L = MEM + SEG
    n_slots = H // G
    K1 = (H - TAIL_HEADS) * E
    CH = D // NCH
    WO_CH = H * E // nD
    X0 = S - 2 * QR * n_pairs
    assert X0 % PAIR == 0 and X0 // PAIR - 1 >= LAG and X0 < S
    RING = (X0 + PAIR) // 2
    assert RING % 16 == 0 and NK % G == 0
    assert G == 2 and n_slots == 16 and nF == 28 and nD == 8
    assert (H - TAIL_HEADS) // G - 1 < n_slots - 2

    WO_SEM = 3 * NCH
    B_SEM, X0_SEM, XM_SEM, X1_SEM, MEM_SEM, OUT_SEM = (WO_SEM + nD + i for i in range(6))
    XA = X0 + 2 * QR
    XB = X0 + 2 * QR * (LAG + 1)

    def kernel(x_hbm, mem0_hbm, wq_hbm, wk_hbm, wv_hbm, wo_hbm, w1_hbm, w2_hbm, w3_hbm, w4_hbm,
               out_hbm,
               raw, w_t, wo_raw, wo_t, w1_t, w2_t, w3_t, w4_t,
               x_v, out_v, mem0_v, xn0, ah_buf, lq_e, lq_o, lb_e, lb_o, sv, ob, wacc,
               h_buf, a1_buf, y_buf, z_buf, sems):

        def rows_copy(src, dst, start, size, sem):
            return pltpu.make_async_copy(src.at[pl.ds(start, size)], dst.at[pl.ds(start, size)], sems.at[sem])

        def raw_copy(i, c):
            src = (wq_hbm, wk_hbm, wv_hbm)[i]
            return rows_copy(src, raw.at[i], c * CH, CH, i * NCH + c)

        def wo_copy(j):
            return rows_copy(wo_hbm, wo_raw, j * WO_CH, WO_CH, WO_SEM + j)

        def mlp_weight_copies():
            return [pltpu.make_async_copy(src.at[:, pl.ds(j * 128, 128)], dst.at[j], sems.at[B_SEM])
                    for src, dst, n in ((w1_hbm, w1_t, nD), (w2_hbm, w2_t, nD),
                                        (w3_hbm, w3_t, nF), (w4_hbm, w4_t, nD))
                    for j in range(n)]

        def x_head_copy():
            return rows_copy(x_hbm, x_v, 0, XA, X0_SEM)

        def x_mid_copy():
            return rows_copy(x_hbm, x_v, XA, XB - XA, XM_SEM)

        def x_rest_copy():
            return rows_copy(x_hbm, x_v, XB, S - XB, X1_SEM)

        def mem_copy():
            return pltpu.make_async_copy(mem0_hbm, mem0_v, sems.at[MEM_SEM])

        def out_copy(c):
            return rows_copy(out_v, out_hbm, pl.multiple_of(c * PAIR, PAIR), PAIR, OUT_SEM)

        def relayout_part(i, b, h0, nh):
            x = raw[i, pl.ds(pl.multiple_of(b * 16, 16), 16), pl.ds(h0, nh), :]
            x = _as_u32(x).reshape(8, 2, nh // 2, E)
            ev, od = x[:, 0], x[:, 1]
            lo = jnp.swapaxes((ev & 0xFFFF) | (od << 16), 0, 1)
            hi = jnp.swapaxes((ev >> 16) | (od & jnp.uint32(0xFFFF0000)), 0, 1)
            rows = pl.ds(pl.multiple_of(b * 8, 8), 8)
            for p in range(nh // 2):
                w_t[i, h0 + 2 * p, rows, :] = lo[p]
                w_t[i, h0 + 2 * p + 1, rows, :] = hi[p]

        def relayout_block(i, b):
            relayout_part(i, b, 0, H)

        def wo_finish():
            def chunk(j, carry):
                dst = wo_raw.at[pl.ds(j * WO_CH, WO_CH)]
                pltpu.make_async_copy(dst, dst, sems.at[WO_SEM + j]).wait()

                def body(b, carry):
                    r = j * WO_CH + b * 256
                    for m in range(4):
                        blk = wo_raw[pl.ds(pl.multiple_of(r + m * 64, 64), 64), :]
                        for n in range(nD):
                            wo_t[n, pl.ds(pl.multiple_of((r + m * 64) // 2, 32), 32), :] = _as_u32(
                                blk[:, n * 128:(n + 1) * 128])
                    return carry
                return jax.lax.fori_loop(0, WO_CH // 256, body, carry)
            jax.lax.fori_loop(0, nD, chunk, 0)
            x_mid_copy().wait()

        def store_xn(t, even):
            x0 = pl.multiple_of(t * PAIR, PAIR)
            q0 = pl.multiple_of(X0 + t * 2 * QR, 16)
            if even:
                xn = _ln(x_v[pl.ds(x0, 40), :].astype(F32))
                lb_e[pl.ds(0, 4), :] = _as_u32(xn[32:40].astype(BF))
                lb_e[pl.ds(4, 4), :] = _as_u32(xn[0:8].astype(BF))
                lb_e[pl.ds(8, 8), :] = _as_u32(xn[8:24].astype(BF))
                lb_e[pl.ds(16, 4), :] = _as_u32(xn[24:32].astype(BF))
                xq = _ln(x_v[pl.ds(q0, QR), :].astype(F32))
                lq_e[pl.ds(0, 8), :] = _as_u32(xq[0:16].astype(BF))
                lq_e[pl.ds(8, 4), :] = _as_u32(xq[16:24].astype(BF))
            else:
                xn = _ln(x_v[pl.ds(x0 + 40, 24), :].astype(F32))
                lb_o[pl.ds(0, 8), :] = _as_u32(xn[0:16].astype(BF))
                lb_o[pl.ds(8, 4), :] = _as_u32(xn[16:24].astype(BF))
                xq = _ln(x_v[pl.ds(q0 + QR, QR), :].astype(F32))
                for n in range(3):
                    lq_o[pl.ds(4 * n, 4), :] = _as_u32(xq[8 * n:8 * n + 8].astype(BF))

        def prologue():
            x_head_copy().start()
            mem_copy().start()
            for i in range(3):
                for c in range(NCH):
                    raw_copy(i, c).start()
            for j in range(nD):
                wo_copy(j).start()
            x_mid_copy().start()

            assert CH == 128 and NK <= nD * (S // X0)

            def acc_at(j):
                if isinstance(j, int):
                    return pl.ds((j // nD) * X0, X0), pl.ds((j % nD) * 128, 128)
                return (pl.ds(pl.multiple_of((j // nD) * X0, X0), X0),
                        pl.ds(pl.multiple_of((j % nD) * 128, 128), 128))

            def zero_acc(j, carry):
                h_buf[acc_at(j)] = jnp.zeros((X0, 128), F32)
                return carry
            jax.lax.fori_loop(0, NK, zero_acc, 0)
            x_head_copy().wait()
            mem_copy().wait()
            lb_e[pl.ds(20, 4), :] = _as_u32(mem0_v[...])
            lq_e[pl.ds(12, 4), :] = _as_u32(mem0_v[...])

            def ln_body(b, carry):
                rows = x_v[pl.ds(pl.multiple_of(b * 64, 64), 64), :].astype(F32)
                xn0[pl.ds(pl.multiple_of(b * 32, 32), 32), :] = _as_u32(_ln(rows).astype(BF))
                return carry
            jax.lax.fori_loop(0, X0 // 64, ln_body, 0)

            def wait_raw(i, c):
                dst = raw.at[i, pl.ds(c * CH, CH)]
                pltpu.make_async_copy(dst, dst, sems.at[i * NCH + c]).wait()

            def q_tile(j, c):
                lhs = _as_bf(xn0[:, pl.ds(pl.multiple_of(c * 128, 128), 128)])
                return _dot(lhs, _as_bf(w_t[0, j, pl.ds(pl.multiple_of(c * 64, 64), 64), :]))

            def first_chunk(b, carry):
                relayout_block(0, b)
                return carry

            def q_chunk(c, carry):
                @pl.when(c + 1 < NCH)
                def _():
                    wait_raw(0, c + 1)
                nxt = jnp.minimum(c + 1, NCH - 1)
                n_items = 2 * (CH // 16)
                done = 0
                rows = X0 // QPC
                for n in range(QPC):
                    lhs = _as_bf(xn0[pl.ds(n * rows // 2, rows // 2), pl.ds(pl.multiple_of(c * 128, 128), 128)])
                    for j in range(NK):
                        at = (pl.ds((j // nD) * X0 + n * rows, rows), pl.ds((j % nD) * 128, 128))
                        h_buf[at] = h_buf[at] + _dot(
                            lhs, _as_bf(w_t[0, j, pl.ds(pl.multiple_of(c * 64, 64), 64), :]))
                        upto = (n * NK + j + 1) * n_items // (NK * QPC)
                        for m in range(done, upto):
                            relayout_part(0, nxt * (CH // 16) + m // 2, (m % 2) * (H // 2), H // 2)
                        done = upto
                return carry

            def q_cast(j, carry):
                ah_buf[pl.ds(0, X0 // 2), pl.ds(pl.multiple_of(j * E, E), E)] = _as_u32(
                    h_buf[acc_at(j)].astype(BF))
                return carry
            with jax.named_scope("sc_wq"):
                wait_raw(0, 0)
                jax.lax.fori_loop(0, CH // 16, first_chunk, 0)
                jax.lax.fori_loop(0, NCH, q_chunk, 0)
                jax.lax.fori_loop(0, NK, q_cast, 0)
            h_buf[pl.ds(0, HALO), :] = jnp.zeros((HALO, D), F32)
            h_buf[pl.ds(HALO + S, HALO), :] = jnp.zeros((HALO, D), F32)

            HP = 2
            per_head = 2 * (D // 16) // H
            it_per_chunk = H // HP // (2 * NCH)
            assert it_per_chunk * HP * per_head * 16 == CH and H - NK >= H // 2

            def kv_body(it, carry):
                i = 1 + it // (H // HP // 2)

                @pl.when(it % it_per_chunk == 0)
                def _():
                    wait_raw(i, (it // it_per_chunk) % NCH)
                NPC = 8
                rows = X0 // 2 // NPC
                for k in range(HP):
                    m = it * HP + k
                    is_k = m >= H - NK
                    mat = jnp.where(is_k, 1, 0)
                    h = jnp.where(is_k, m - (H - NK), m + NK)
                    col = jnp.where(is_k, H + h, h)
                    for n in range(NPC):
                        r = _dot(_as_bf(xn0[pl.ds(n * rows, rows), :]), _as_bf(w_t[mat, h]))
                        ah_buf[pl.ds(n * rows, rows), pl.ds(pl.multiple_of(col * E, E), E)] = _as_u32(r.astype(BF))
                        relayout_part(i, (m % (H // 2)) * per_head + n // 2, (n % 2) * (H // 2), H // 2)
                return carry
            with jax.named_scope("sc_kv"):
                jax.lax.fori_loop(0, H // HP, kv_body, 0)

            for c in mlp_weight_copies():
                c.start()
            x_rest_copy().start()

        def mlp_pre(c):
            a1_buf[pl.ds(0, 2 * HALO), :] = a1_buf[pl.ds(PAIR, 2 * HALO), :]
            y = _ln(h_buf[pl.ds(pl.multiple_of(c * PAIR + HALO, 8), PAIR + HALO), :])
            y_buf[...] = y[0:PAIR]
            z_buf[...] = _as_u32(_ln(y[HALO:]).astype(BF))

        def mlp_prologue():
            for c in mlp_weight_copies():
                c.wait()
            z = _ln(_ln(h_buf[pl.ds(0, 2 * HALO), :])).astype(BF)
            tok = jax.lax.broadcasted_iota(jnp.int32, (2 * HALO, 128), 0) - HALO

            for j in range(nD):
                a1_buf[pl.ds(PAIR, 2 * HALO), pl.ds(j * 128, 128)] = jnp.where(
                    tok >= 0, _gelu(_dot(z, w1_t[j])), 0.0)
            mlp_pre(0)

        def attention_jobs(t):
            row = jax.lax.broadcasted_iota(jnp.int32, (G * L, G * L), 0)
            col = jax.lax.broadcasted_iota(jnp.int32, (G * L, G * L), 1)

            def head_of(r):
                return jnp.where(r < G * SEG, r // SEG, (r - G * SEG) // MEM)
            mask = (head_of(row) == head_of(col)) & ((col >= G * SEG) | (row >= G * SEG) | (col <= row))
            x0 = t * PAIR
            h0 = x0 + HALO

            def step_jobs(even):
                lb = lb_e if even else lb_o
                st = {}

                lq = lq_e if even else lq_o
                def ring(r, mult):
                    return pl.multiple_of(jax.lax.rem(r, RING), mult)
                a_new = X0 // 2 + t * QR
                a_use = ring(t * SEG + (0 if even else SEG // 2), 16)

                def ahead(mat, h, col, slot):
                    cs, cb = pl.ds(h * E, E), pl.ds(col * E, E)
                    r = _dot(_as_bf(lq[...]), _as_bf(w_t[mat, h]))
                    if even:
                        ah_buf[pl.ds(ring(a_new, 8), 8), cb] = _as_u32(r[0:16].astype(BF))
                        sv[slot, :, cs] = r[16:24]
                    else:
                        ah_buf[pl.ds(ring(a_new + 8, 8), 8), cb] = _as_u32(
                            jnp.concatenate([sv[slot, :, cs], r[0:8]], axis=0).astype(BF))
                        ah_buf[pl.ds(ring(a_new + 16, 8), 8), cb] = _as_u32(r[8:24].astype(BF))
                    return _as_bf(ah_buf[pl.ds(a_use, SEG // 2), cb]), r[QR:QR + MEM]

                def in_step(mat, h, slot):
                    cs = pl.ds(h * E, E)
                    r = _dot(_as_bf(lb[...]), _as_bf(w_t[mat, h]))
                    if even:
                        sv[slot, :, cs] = r[0:8]
                        return [r[8:40]], r[40:48]
                    return [sv[slot, :, cs], r[0:24]], r[24:32]

                def stack(parts):
                    xs, ms = [p[0] for p in parts], [p[1] for p in parts]
                    if isinstance(xs[0], list):
                        return jnp.concatenate(xs[0] + xs[1] + ms, axis=0).astype(BF)
                    return jnp.concatenate(xs + [jnp.concatenate(ms, axis=0).astype(BF)], axis=0)

                def j_qkv(g, i):
                    def run():
                        h = g * G + i
                        parts = st.setdefault(('parts', g), [[], [], []])
                        parts[0].append(ahead(0, h, h, 2))
                        parts[1].append(ahead(1, h, H + h, 0) if h < NK else in_step(1, h, 0))
                        parts[2].append(in_step(2, h, 1))
                        if i == G - 1:
                            st['qkv', g] = [stack(p) for p in st.pop(('parts', g))]
                    return run

                def j_scores(g):
                    def run():
                        q, k, v = st.pop(('qkv', g))
                        s = jax.lax.dot_general(q, k, (((1,), (1,)), ((), ())),
                                                preferred_element_type=F32)
                        s = jnp.where(mask, s, -1000000000.0 / scale)
                        m = jnp.max(s, axis=-1, keepdims=True)
                        p = jnp.exp2((s - m) * (scale * LOG2E))
                        l = jnp.sum(p, axis=-1, keepdims=True)
                        r0 = pl.reciprocal(l, approx=True)
                        p = p * (r0 * (2.0 - l * r0))
                        st['p', g] = (p.astype(BF), v)
                    return run

                def j_pv(g):
                    def run():
                        p, v = st.pop(('p', g))
                        o2 = _dot(p, v)
                        for i, h in enumerate(range(g * G, (g + 1) * G)):
                            ox = o2[i * SEG:(i + 1) * SEG]
                            om = o2[G * SEG + i * MEM:G * SEG + (i + 1) * MEM]
                            cs = pl.ds(h * E, E)
                            if even:
                                ob[pl.ds(16, 4), cs] = _as_u32(ox[0:8].astype(BF))
                                ob[pl.ds(0, 16), cs] = _as_u32(
                                    jnp.concatenate([ox[8:32], om], axis=0).astype(BF))
                            else:
                                ob[pl.ds(20, 4), cs] = _as_u32(ox[0:8].astype(BF))
                                ob[pl.ds(24, 16), cs] = _as_u32(
                                    jnp.concatenate([ox[8:32], om], axis=0).astype(BF))
                    return run

                rows = pl.ds(0, 16) if even else pl.ds(16, 24)
                nrows = 32 if even else 48

                def j_wo1(j):
                    def run():
                        lhs = _as_bf(ob[rows, pl.ds(0, K1)])
                        wacc[pl.ds(0, nrows), pl.ds(j * 128, 128)] = _dot(
                            lhs, _as_bf(wo_t[j, pl.ds(0, K1 // 2), :]))
                    return run

                def j_wo2(j):
                    def run():
                        lhs = _as_bf(ob[rows, pl.ds(K1, H * E - K1)])
                        r = wacc[pl.ds(0, nrows), pl.ds(j * 128, 128)] + _dot(
                            lhs, _as_bf(wo_t[j, pl.ds(K1 // 2, (H * E - K1) // 2), :]))
                        cs = pl.ds(j * 128, 128)
                        xs = x_v[pl.ds(pl.multiple_of(x0, PAIR), PAIR), cs].astype(F32)
                        if even:
                            mem = _as_u32(r[24:32].astype(BF))
                            lb_o[pl.ds(12, 4), cs] = mem
                            lq_o[pl.ds(12, 4), cs] = mem
                            h_buf[pl.ds(pl.multiple_of(h0 + 8, 8), 24), cs] = xs[8:32] + r[0:24]
                        else:
                            mem = _as_u32(r[40:48].astype(BF))
                            lb_e[pl.ds(20, 4), cs] = mem
                            lq_e[pl.ds(12, 4), cs] = mem
                            h_buf[pl.ds(pl.multiple_of(h0, 8), 8), cs] = xs[0:8] + r[0:8]
                            h_buf[pl.ds(pl.multiple_of(h0 + 32, 8), 32), cs] = xs[32:64] + r[8:40]
                    return run

                last = n_slots - 1
                jobs = []
                for g in range(n_slots):
                    for i in range(G):
                        jobs.append((('qkv', g, i), j_qkv(g, i)))
                    if g >= 1:
                        jobs.append((('s', g - 1), j_scores(g - 1)))
                    if g >= 2:
                        jobs.append((('pv', g - 2), j_pv(g - 2)))
                wo1 = [(('wo1', j), j_wo1(j)) for j in range(nD)]
                jobs += (wo1[0:3] + [(('s', last), j_scores(last)), (('pv', last - 1), j_pv(last - 1))]
                         + wo1[3:6] + [(('pv', last), j_pv(last))] + wo1[6:8])
                jobs += [(('wo2', j), j_wo2(j)) for j in range(nD)]
                return jobs

            def j_next_xn(even):
                return lambda: store_xn(jnp.minimum(t + 1, n_pairs - 1), even)

            return step_jobs(True), step_jobs(False), j_next_xn

        after_qkv = ('s', n_slots - 2)

        def mlp_jobs(c):
            r0 = pl.multiple_of(c * PAIR, PAIR)
            st = {}

            def j_pre_next():
                mlp_pre(jnp.minimum(c + 1, n_pairs - 1))

            def j_w1(j):
                def run():
                    tok = jax.lax.broadcasted_iota(jnp.int32, (PAIR, 128), 0) + (r0 + HALO)
                    a = _gelu(_dot(_as_bf(z_buf[...]), w1_t[j]))
                    a1_buf[pl.ds(2 * HALO, PAIR), pl.ds(j * 128, 128)] = jnp.where(tok < S, a, 0.0)
                return run

            def j_shift():
                cq = D // 4
                st['g'] = jnp.concatenate([
                    a1_buf[pl.ds(HALO - 1, PAIR), pl.ds(0 * cq, cq)],
                    a1_buf[pl.ds(HALO + 1, PAIR), pl.ds(1 * cq, cq)],
                    a1_buf[pl.ds(HALO - 2, PAIR), pl.ds(2 * cq, cq)],
                    a1_buf[pl.ds(HALO + 2, PAIR), pl.ds(3 * cq, cq)]], axis=1).astype(BF)

            def j_w2(j):
                def run():
                    st['x1', j] = y_buf[:, pl.ds(j * 128, 128)] + _dot(st['g'], w2_t[j])
                return run

            def j_ln3():
                x1 = jnp.concatenate([st['x1', j] for j in range(nD)], axis=1)
                st['z1'] = _ln(x1).astype(BF)

            def j_w3(j):
                def run():
                    st['a3', j] = _gelu(_dot(st['z1'], w3_t[j])).astype(BF)
                return run

            def j_cat():
                st['a3'] = jnp.concatenate([st.pop(('a3', j)) for j in range(nF)], axis=1)

            def j_w4(j):
                def run():
                    cs = pl.ds(j * 128, 128)
                    hh = h_buf[pl.ds(pl.multiple_of(r0 + HALO, 8), PAIR), cs]
                    out_v[pl.ds(r0, PAIR), cs] = (
                        hh + (st['x1', j] + _dot(st['a3'], w4_t[j]))).astype(out_v.dtype)
                return run

            return dict(pre_next=j_pre_next, w1=[j_w1(j) for j in range(nD)], shift=j_shift,
                        w2=[j_w2(j) for j in range(nD)], ln3=j_ln3,
                        w3=[j_w3(j) for j in range(nF)], cat=j_cat,
                        w4=[j_w4(j) for j in range(nD)])

        def attention_only(t, carry):
            ej, oj, j_next_xn = attention_jobs(t)

            def j_wo_wait():
                with jax.named_scope("sc_wo_finish"):
                    pl.when(t == 0)(wo_finish)
            _run(_interleave(ej, {after_qkv: [j_wo_wait]})
                 + _interleave(oj, {('qkv', 4, 0): [j_next_xn(True)], after_qkv: [j_next_xn(False)]}))
            return carry

        def fused(t, carry):
            @pl.when(t == LAG)
            def _():
                x_rest_copy().wait()

            @pl.when(t > LAG)
            def _():
                out_copy(t - LAG - 1).start()

            ej, oj, j_next_xn = attention_jobs(t)
            b = mlp_jobs(t - LAG)
            w3, w4 = b['w3'], b['w4']
            fe, fo = {}, {}

            def put(d, label, *jobs):
                d.setdefault(label, []).extend(jobs)
            for i in range(nD):
                put(fe, ('qkv', 2 + i // 2, i % 2), b['w1'][i])
                put(fe, ('qkv', 8 + i // 2, i % 2), b['w2'][i])
            put(fe, ('qkv', 6, 0), b['shift'])
            put(fe, ('qkv', 12, 0), b['ln3'])
            put(fe, ('qkv', 15, 0), w3[0])
            put(fe, 'end', *w3[1:4])
            put(fo, ('qkv', 0, 1), b['pre_next'])
            for k in range(4, nF):
                put(fo, ('qkv', 1 + (k - 4) // 2, (k - 4) % 2), w3[k])
            put(fo, ('qkv', 13, 0), b['cat'])
            put(fo, ('qkv', 14, 0), w4[0])
            put(fo, ('qkv', 15, 0), w4[1])
            put(fo, ('qkv', 4, 0), j_next_xn(True))
            put(fo, after_qkv, j_next_xn(False))
            put(fo, ('s', n_slots - 1), w4[2])
            put(fo, 'end', *w4[3:])
            with jax.named_scope("sc_fused_body"):
                _run(_interleave(ej, fe) + _interleave(oj, fo))
            return carry

        def mlp_only(c, carry):
            out_copy(c - 1).start()
            b = mlp_jobs(c)
            _run(b['w1'] + [b['shift']] + b['w2'] + [b['ln3'], b['pre_next']] + b['w3'] + [b['cat']] + b['w4'])
            return carry

        with jax.named_scope("sc_prologue"):
            prologue()
            store_xn(0, True)
            store_xn(0, False)
        with jax.named_scope("sc_a_only"):
            jax.lax.fori_loop(0, LAG, attention_only, 0)
        with jax.named_scope("sc_mlp_prologue"):
            mlp_prologue()
        with jax.named_scope("sc_fused"):
            jax.lax.fori_loop(LAG, n_pairs, fused, 0)
        with jax.named_scope("sc_b_tail"):
            jax.lax.fori_loop(n_pairs - LAG, n_pairs, mlp_only, 0)
        out_copy(n_pairs - 1).start()
        pltpu.make_async_copy(out_v, out_hbm, sems.at[OUT_SEM]).wait()

    return kernel, WO_SEM + nD + 6, X0, RING


@functools.partial(jax.jit, static_argnames=("A_seg_len",))
def pallas_sequential_preLN__memory_aug_recurrent_mem_tr__mixer_s_mlp__prompt_kernel(
    A_x, A_mem0, A_Wq, A_Wk, A_Wv, A_Wo, A_seg_len, B_x, B_w1, B_w2, B_w3, B_w4,
):
    _, S, D = A_x.shape
    H, E = A_Wq.shape[1], A_Wq.shape[2]
    F = B_w3.shape[1]
    assert A_seg_len == SEG and A_mem0.shape[1] == MEM and S % PAIR == 0
    nD, nF = D // 128, F // 128

    x = A_x.reshape(S, D)
    mem0 = A_mem0.reshape(MEM, D)
    wo = A_Wo.reshape(H * E, D)

    kernel, n_sems, x0, ring = _make_kernel(S, D, H, E, F)
    any_spec = pl.BlockSpec(memory_space=pl.ANY)
    out = pl.pallas_call(
        kernel,
        in_specs=[any_spec] * 10,
        out_specs=any_spec,
        out_shape=jax.ShapeDtypeStruct((S, D), A_x.dtype),
        scratch_shapes=[
            pltpu.VMEM((3, D, H, E), BF),
            pltpu.VMEM((3, H, D // 2, E), U32),
            pltpu.VMEM((H * E, D), BF),
            pltpu.VMEM((nD, H * E // 2, 128), U32),
            pltpu.VMEM((nD, D, 128), BF),
            pltpu.VMEM((nD, D, 128), BF),
            pltpu.VMEM((nF, D, 128), BF),
            pltpu.VMEM((nD, F, 128), BF),
            pltpu.VMEM((S, D), BF),
            pltpu.VMEM((S, D), BF),
            pltpu.VMEM((MEM, D), BF),
            pltpu.VMEM((x0 // 2, D), U32),
            pltpu.VMEM((ring, (H + NK) * E), U32),
            pltpu.VMEM((16, D), U32),
            pltpu.VMEM((16, D), U32),
            pltpu.VMEM((24, D), U32),
            pltpu.VMEM((16, D), U32),
            pltpu.VMEM((3, 8, H * E), F32),
            pltpu.VMEM((40, H * E), U32),
            pltpu.VMEM((48, D), F32),
            pltpu.VMEM((S + 2 * HALO, D), F32),
            pltpu.VMEM((PAIR + 2 * HALO, D), F32),
            pltpu.VMEM((PAIR, D), F32),
            pltpu.VMEM((PAIR // 2, D), U32),
            pltpu.SemaphoreType.DMA((n_sems,)),
        ],
        compiler_params=pltpu.CompilerParams(
            vmem_limit_bytes=124 * 1024 * 1024,
            disable_bounds_checks=True,
        ),
    )(x, mem0, A_Wq, A_Wk, A_Wv, wo, B_w1, B_w2, B_w3, B_w4)
    return out.reshape(1, S, D)
```

```python
import functools

import jax
import jax.numpy as jnp
from jax.experimental import pallas as pl
from jax.experimental.pallas import tpu as pltpu

BF = jnp.bfloat16
F32 = jnp.float32
U32 = jnp.uint32

SEG = 32
MEM = 8
PAIR = 2 * SEG
LAG = 3
HALO = 8
G = 2
TAIL_HEADS = 6
QR = 24
NK = 16
QPC = 4
KVP = 8
NCH = 8
LN_EPS = 1e-5
LOG2E = 1.4426950408889634


def _ln(x):
    m = jnp.mean(x, axis=-1, keepdims=True)
    xc = x - m
    v = jnp.mean(xc * xc, axis=-1, keepdims=True)
    return xc * jax.lax.rsqrt(v + LN_EPS)


_dot = functools.partial(jnp.dot, preferred_element_type=F32)


def _gelu(x):
    return jax.nn.gelu(x, approximate=True)


def _as_bf(x_u32):
    return pltpu.bitcast(x_u32, BF)


def _as_u32(x_bf):
    return pltpu.bitcast(x_bf, U32)


def _interleave(main, fill):
    fill = dict(fill)
    out = []
    for label, job in main:
        out.extend(fill.pop(label, []))
        out.append(job)
    out.extend(fill.pop('end', []))
    assert not fill, fill
    return out


def _run(jobs):
    for job in jobs:
        job()


def _make_kernel(S, D, H, E, F):
    n_pairs = S // PAIR
    nD = D // 128
    nF = F // 128
    scale = float(E) ** -0.5
    L = MEM + SEG
    n_slots = H // G
    K1 = (H - TAIL_HEADS) * E
    CH = D // NCH
    WO_CH = H * E // nD
    X0 = S - 2 * QR * n_pairs
    assert X0 % PAIR == 0 and X0 // PAIR - 1 >= LAG and X0 < S
    RING = (X0 + PAIR) // 2
    assert RING % 16 == 0 and NK % G == 0
    assert G == 2 and n_slots == 16 and nF == 28 and nD == 8
    assert (H - TAIL_HEADS) // G - 1 < n_slots - 2

    WO_SEM = 3 * NCH
    B_SEM, X0_SEM, XM_SEM, X1_SEM, MEM_SEM, OUT_SEM = (WO_SEM + nD + i for i in range(6))
    XA = X0 + 2 * QR
    XB = X0 + 2 * QR * (LAG + 1)

    def kernel(x_hbm, mem0_hbm, wq_hbm, wk_hbm, wv_hbm, wo_hbm, w1_hbm, w2_hbm, w3_hbm, w4_hbm,
               out_hbm,
               raw, w_t, wo_raw, wo_t, w1_t, w2_t, w3_t, w4_t,
               x_v, out_v, mem0_v, xn0, ah_buf, lq_e, lq_o, lb_e, lb_o, sv, ob, wacc,
               h_buf, a1_buf, y_buf, z_buf, sems):

        def rows_copy(src, dst, start, size, sem):
            return pltpu.make_async_copy(src.at[pl.ds(start, size)], dst.at[pl.ds(start, size)], sems.at[sem])

        def raw_copy(i, c):
            src = (wq_hbm, wk_hbm, wv_hbm)[i]
            return rows_copy(src, raw.at[i], c * CH, CH, i * NCH + c)

        def wo_copy(j):
            return rows_copy(wo_hbm, wo_raw, j * WO_CH, WO_CH, WO_SEM + j)

        def mlp_weight_copies():
            return [pltpu.make_async_copy(src.at[:, pl.ds(j * 128, 128)], dst.at[j], sems.at[B_SEM])
                    for src, dst, n in ((w1_hbm, w1_t, nD), (w2_hbm, w2_t, nD),
                                        (w3_hbm, w3_t, nF), (w4_hbm, w4_t, nD))
                    for j in range(n)]

        def x_head_copy():
            return rows_copy(x_hbm, x_v, 0, XA, X0_SEM)

        def x_mid_copy():
            return rows_copy(x_hbm, x_v, XA, XB - XA, XM_SEM)

        def x_rest_copy():
            return rows_copy(x_hbm, x_v, XB, S - XB, X1_SEM)

        def mem_copy():
            return pltpu.make_async_copy(mem0_hbm, mem0_v, sems.at[MEM_SEM])

        def out_copy(c):
            return rows_copy(out_v, out_hbm, pl.multiple_of(c * PAIR, PAIR), PAIR, OUT_SEM)

        def relayout_part(i, b, h0, nh):
            x = raw[i, pl.ds(pl.multiple_of(b * 16, 16), 16), pl.ds(h0, nh), :]
            x = _as_u32(x).reshape(8, 2, nh // 2, E)
            ev, od = x[:, 0], x[:, 1]
            lo = jnp.swapaxes((ev & 0xFFFF) | (od << 16), 0, 1)
            hi = jnp.swapaxes((ev >> 16) | (od & jnp.uint32(0xFFFF0000)), 0, 1)
            rows = pl.ds(pl.multiple_of(b * 8, 8), 8)
            for p in range(nh // 2):
                w_t[i, h0 + 2 * p, rows, :] = lo[p]
                w_t[i, h0 + 2 * p + 1, rows, :] = hi[p]

        def relayout_block(i, b):
            relayout_part(i, b, 0, H)

        def wo_finish():
            def chunk(j, carry):
                dst = wo_raw.at[pl.ds(j * WO_CH, WO_CH)]
                pltpu.make_async_copy(dst, dst, sems.at[WO_SEM + j]).wait()

                def body(b, carry):
                    r = j * WO_CH + b * 256
                    for m in range(4):
                        blk = wo_raw[pl.ds(pl.multiple_of(r + m * 64, 64), 64), :]
                        for n in range(nD):
                            wo_t[n, pl.ds(pl.multiple_of((r + m * 64) // 2, 32), 32), :] = _as_u32(
                                blk[:, n * 128:(n + 1) * 128])
                    return carry
                return jax.lax.fori_loop(0, WO_CH // 256, body, carry)
            jax.lax.fori_loop(0, nD, chunk, 0)
            x_mid_copy().wait()

        def store_xn(t, even):
            x0 = pl.multiple_of(t * PAIR, PAIR)
            q0 = pl.multiple_of(X0 + t * 2 * QR, 16)
            if even:
                xn = _ln(x_v[pl.ds(x0, 40), :].astype(F32))
                lb_e[pl.ds(0, 4), :] = _as_u32(xn[32:40].astype(BF))
                lb_e[pl.ds(4, 4), :] = _as_u32(xn[0:8].astype(BF))
                lb_e[pl.ds(8, 8), :] = _as_u32(xn[8:24].astype(BF))
                lb_e[pl.ds(16, 4), :] = _as_u32(xn[24:32].astype(BF))
                xq = _ln(x_v[pl.ds(q0, QR), :].astype(F32))
                lq_e[pl.ds(0, 8), :] = _as_u32(xq[0:16].astype(BF))
                lq_e[pl.ds(8, 4), :] = _as_u32(xq[16:24].astype(BF))
            else:
                xn = _ln(x_v[pl.ds(x0 + 40, 24), :].astype(F32))
                lb_o[pl.ds(0, 8), :] = _as_u32(xn[0:16].astype(BF))
                lb_o[pl.ds(8, 4), :] = _as_u32(xn[16:24].astype(BF))
                xq = _ln(x_v[pl.ds(q0 + QR, QR), :].astype(F32))
                for n in range(3):
                    lq_o[pl.ds(4 * n, 4), :] = _as_u32(xq[8 * n:8 * n + 8].astype(BF))

        def prologue():
            x_head_copy().start()
            mem_copy().start()
            for i in range(3):
                for c in range(NCH):
                    raw_copy(i, c).start()
            for j in range(nD):
                wo_copy(j).start()
            x_mid_copy().start()

            assert CH == 128 and NK <= nD * (S // X0)

            def acc_at(j):
                if isinstance(j, int):
                    return pl.ds((j // nD) * X0, X0), pl.ds((j % nD) * 128, 128)
                return (pl.ds(pl.multiple_of((j // nD) * X0, X0), X0),
                        pl.ds(pl.multiple_of((j % nD) * 128, 128), 128))

            def zero_acc(j, carry):
                h_buf[acc_at(j)] = jnp.zeros((X0, 128), F32)
                return carry
            jax.lax.fori_loop(0, NK, zero_acc, 0)
            x_head_copy().wait()
            mem_copy().wait()
            lb_e[pl.ds(20, 4), :] = _as_u32(mem0_v[...])
            lq_e[pl.ds(12, 4), :] = _as_u32(mem0_v[...])

            def ln_body(b, carry):
                rows = x_v[pl.ds(pl.multiple_of(b * 64, 64), 64), :].astype(F32)
                xn0[pl.ds(pl.multiple_of(b * 32, 32), 32), :] = _as_u32(_ln(rows).astype(BF))
                return carry
            jax.lax.fori_loop(0, X0 // 64, ln_body, 0)

            def wait_raw(i, c):
                dst = raw.at[i, pl.ds(c * CH, CH)]
                pltpu.make_async_copy(dst, dst, sems.at[i * NCH + c]).wait()

            def first_chunk(b, carry):
                relayout_block(0, b)
                return carry

            def q_chunk(c, carry):
                @pl.when(c + 1 < NCH)
                def _():
                    wait_raw(0, c + 1)
                nxt = jnp.minimum(c + 1, NCH - 1)
                n_items = 2 * (CH // 16)
                done = 0
                rows = X0 // QPC
                for n in range(QPC):
                    lhs = _as_bf(xn0[pl.ds(n * rows // 2, rows // 2), pl.ds(pl.multiple_of(c * 128, 128), 128)])
                    for j in range(NK):
                        at = (pl.ds((j // nD) * X0 + n * rows, rows), pl.ds((j % nD) * 128, 128))
                        h_buf[at] = h_buf[at] + _dot(
                            lhs, _as_bf(w_t[0, j, pl.ds(pl.multiple_of(c * 64, 64), 64), :]))
                        upto = (n * NK + j + 1) * n_items // (NK * QPC)
                        for m in range(done, upto):
                            relayout_part(0, nxt * (CH // 16) + m // 2, (m % 2) * (H // 2), H // 2)
                        done = upto
                return carry

            def q_cast(j):
                ah_buf[pl.ds(0, X0 // 2), pl.ds(pl.multiple_of(j * E, E), E)] = _as_u32(
                    h_buf[acc_at(j)].astype(BF))
            wait_raw(0, 0)
            jax.lax.fori_loop(0, CH // 16, first_chunk, 0)
            jax.lax.fori_loop(0, NCH, q_chunk, 0)

            HP = 2
            per_head = 2 * (D // 16) // H
            it_per_chunk = H // HP // (2 * NCH)
            assert it_per_chunk * HP * per_head * 16 == CH and H - NK >= H // 2

            def kv_body(it, carry):
                i = 1 + it // (H // HP // 2)

                @pl.when(it % it_per_chunk == 0)
                def _():
                    wait_raw(i, (it // it_per_chunk) % NCH)
                NPC = KVP
                rows = X0 // 2 // NPC
                for k in range(HP):
                    m = it * HP + k
                    is_k = m >= H - NK
                    mat = jnp.where(is_k, 1, 0)
                    h = jnp.where(is_k, m - (H - NK), m + NK)
                    col = jnp.where(is_k, H + h, h)
                    for n in range(NPC):
                        r = _dot(_as_bf(xn0[pl.ds(n * rows, rows), :]), _as_bf(w_t[mat, h]))
                        ah_buf[pl.ds(n * rows, rows), pl.ds(pl.multiple_of(col * E, E), E)] = _as_u32(r.astype(BF))
                        for q in range(n * 8 // NPC, (n + 1) * 8 // NPC):
                            relayout_part(i, (m % (H // 2)) * per_head + q // 2, (q % 2) * (H // 2), H // 2)
                    if k == 1:
                        q_cast(it)
                return carry
            assert NK == H // HP
            for c in mlp_weight_copies():
                c.start()
            x_rest_copy().start()
            jax.lax.fori_loop(0, H // HP, kv_body, 0)
            h_buf[pl.ds(0, HALO), :] = jnp.zeros((HALO, D), F32)
            h_buf[pl.ds(HALO + S, HALO), :] = jnp.zeros((HALO, D), F32)

        def mlp_pre(c):
            a1_buf[pl.ds(0, 2 * HALO), :] = a1_buf[pl.ds(PAIR, 2 * HALO), :]
            y = _ln(h_buf[pl.ds(pl.multiple_of(c * PAIR + HALO, 8), PAIR + HALO), :])
            y_buf[...] = y[0:PAIR]
            z_buf[...] = _as_u32(_ln(y[HALO:]).astype(BF))

        def mlp_prologue():
            for c in mlp_weight_copies():
                c.wait()
            z = _ln(_ln(h_buf[pl.ds(0, 2 * HALO), :])).astype(BF)
            tok = jax.lax.broadcasted_iota(jnp.int32, (2 * HALO, 128), 0) - HALO

            for j in range(nD):
                a1_buf[pl.ds(PAIR, 2 * HALO), pl.ds(j * 128, 128)] = jnp.where(
                    tok >= 0, _gelu(_dot(z, w1_t[j])), 0.0)
            mlp_pre(0)

        def attention_jobs(t):
            row = jax.lax.broadcasted_iota(jnp.int32, (G * L, G * L), 0)
            col = jax.lax.broadcasted_iota(jnp.int32, (G * L, G * L), 1)

            def head_of(r):
                return jnp.where(r < G * SEG, r // SEG, (r - G * SEG) // MEM)
            mask = (head_of(row) == head_of(col)) & ((col >= G * SEG) | (row >= G * SEG) | (col <= row))
            x0 = t * PAIR
            h0 = x0 + HALO

            def step_jobs(even):
                lb = lb_e if even else lb_o
                st = {}

                lq = lq_e if even else lq_o
                def ring(r, mult):
                    return pl.multiple_of(jax.lax.rem(r, RING), mult)
                a_new = X0 // 2 + t * QR
                a_use = ring(t * SEG + (0 if even else SEG // 2), 16)

                def ahead(mat, h, col, slot):
                    cs, cb = pl.ds(h * E, E), pl.ds(col * E, E)
                    r = _dot(_as_bf(lq[...]), _as_bf(w_t[mat, h]))
                    if even:
                        ah_buf[pl.ds(ring(a_new, 8), 8), cb] = _as_u32(r[0:16].astype(BF))
                        sv[slot, :, cs] = r[16:24]
                    else:
                        ah_buf[pl.ds(ring(a_new + 8, 8), 8), cb] = _as_u32(
                            jnp.concatenate([sv[slot, :, cs], r[0:8]], axis=0).astype(BF))
                        ah_buf[pl.ds(ring(a_new + 16, 8), 8), cb] = _as_u32(r[8:24].astype(BF))
                    return _as_bf(ah_buf[pl.ds(a_use, SEG // 2), cb]), r[QR:QR + MEM]

                def in_step(mat, h, slot):
                    cs = pl.ds(h * E, E)
                    r = _dot(_as_bf(lb[...]), _as_bf(w_t[mat, h]))
                    if even:
                        sv[slot, :, cs] = r[0:8]
                        return [r[8:40]], r[40:48]
                    return [sv[slot, :, cs], r[0:24]], r[24:32]

                def stack(parts):
                    xs, ms = [p[0] for p in parts], [p[1] for p in parts]
                    if isinstance(xs[0], list):
                        return jnp.concatenate(xs[0] + xs[1] + ms, axis=0).astype(BF)
                    return jnp.concatenate(xs + [jnp.concatenate(ms, axis=0).astype(BF)], axis=0)

                def j_qkv(g, i):
                    def run():
                        h = g * G + i
                        parts = st.setdefault(('parts', g), [[], [], []])
                        parts[0].append(ahead(0, h, h, 2))
                        parts[1].append(ahead(1, h, H + h, 0) if h < NK else in_step(1, h, 0))
                        parts[2].append(in_step(2, h, 1))
                        if i == G - 1:
                            st['qkv', g] = [stack(p) for p in st.pop(('parts', g))]
                    return run

                def j_scores(g):
                    def run():
                        q, k, v = st.pop(('qkv', g))
                        s = jax.lax.dot_general(q, k, (((1,), (1,)), ((), ())),
                                                preferred_element_type=F32)
                        s = jnp.where(mask, s, -1000000000.0 / scale)
                        m = jnp.max(s, axis=-1, keepdims=True)
                        p = jnp.exp2((s - m) * (scale * LOG2E))
                        l = jnp.sum(p, axis=-1, keepdims=True)
                        r0 = pl.reciprocal(l, approx=True)
                        p = p * (r0 * (2.0 - l * r0))
                        st['p', g] = (p.astype(BF), v)
                    return run

                def j_pv(g):
                    def run():
                        p, v = st.pop(('p', g))
                        o2 = _dot(p, v)
                        for i, h in enumerate(range(g * G, (g + 1) * G)):
                            ox = o2[i * SEG:(i + 1) * SEG]
                            om = o2[G * SEG + i * MEM:G * SEG + (i + 1) * MEM]
                            cs = pl.ds(h * E, E)
                            if even:
                                ob[pl.ds(16, 4), cs] = _as_u32(ox[0:8].astype(BF))
                                ob[pl.ds(0, 16), cs] = _as_u32(
                                    jnp.concatenate([ox[8:32], om], axis=0).astype(BF))
                            else:
                                ob[pl.ds(20, 4), cs] = _as_u32(ox[0:8].astype(BF))
                                ob[pl.ds(24, 16), cs] = _as_u32(
                                    jnp.concatenate([ox[8:32], om], axis=0).astype(BF))
                    return run

                rows = pl.ds(0, 16) if even else pl.ds(16, 24)
                nrows = 32 if even else 48

                def j_wo1(j):
                    def run():
                        lhs = _as_bf(ob[rows, pl.ds(0, K1)])
                        wacc[pl.ds(0, nrows), pl.ds(j * 128, 128)] = _dot(
                            lhs, _as_bf(wo_t[j, pl.ds(0, K1 // 2), :]))
                    return run

                def j_wo2(j):
                    def run():
                        lhs = _as_bf(ob[rows, pl.ds(K1, H * E - K1)])
                        r = wacc[pl.ds(0, nrows), pl.ds(j * 128, 128)] + _dot(
                            lhs, _as_bf(wo_t[j, pl.ds(K1 // 2, (H * E - K1) // 2), :]))
                        cs = pl.ds(j * 128, 128)
                        xs = x_v[pl.ds(pl.multiple_of(x0, PAIR), PAIR), cs].astype(F32)
                        if even:
                            mem = _as_u32(r[24:32].astype(BF))
                            lb_o[pl.ds(12, 4), cs] = mem
                            lq_o[pl.ds(12, 4), cs] = mem
                            h_buf[pl.ds(pl.multiple_of(h0 + 8, 8), 24), cs] = xs[8:32] + r[0:24]
                        else:
                            mem = _as_u32(r[40:48].astype(BF))
                            lb_e[pl.ds(20, 4), cs] = mem
                            lq_e[pl.ds(12, 4), cs] = mem
                            h_buf[pl.ds(pl.multiple_of(h0, 8), 8), cs] = xs[0:8] + r[0:8]
                            h_buf[pl.ds(pl.multiple_of(h0 + 32, 8), 32), cs] = xs[32:64] + r[8:40]
                    return run

                last = n_slots - 1
                jobs = []
                for g in range(n_slots):
                    for i in range(G):
                        jobs.append((('qkv', g, i), j_qkv(g, i)))
                    if g >= 1:
                        jobs.append((('s', g - 1), j_scores(g - 1)))
                    if g >= 2:
                        jobs.append((('pv', g - 2), j_pv(g - 2)))
                wo1 = [(('wo1', j), j_wo1(j)) for j in range(nD)]
                jobs += (wo1[0:3] + [(('s', last), j_scores(last)), (('pv', last - 1), j_pv(last - 1))]
                         + wo1[3:6] + [(('pv', last), j_pv(last))] + wo1[6:8])
                jobs += [(('wo2', j), j_wo2(j)) for j in range(nD)]
                return jobs

            def j_next_xn(even):
                return lambda: store_xn(jnp.minimum(t + 1, n_pairs - 1), even)

            return step_jobs(True), step_jobs(False), j_next_xn

        after_qkv = ('s', n_slots - 2)

        def mlp_jobs(c):
            r0 = pl.multiple_of(c * PAIR, PAIR)
            st = {}

            def j_pre_next():
                mlp_pre(jnp.minimum(c + 1, n_pairs - 1))

            def j_w1(j):
                def run():
                    tok = jax.lax.broadcasted_iota(jnp.int32, (PAIR, 128), 0) + (r0 + HALO)
                    a = _gelu(_dot(_as_bf(z_buf[...]), w1_t[j]))
                    a1_buf[pl.ds(2 * HALO, PAIR), pl.ds(j * 128, 128)] = jnp.where(tok < S, a, 0.0)
                return run

            def j_shift():
                cq = D // 4
                st['g'] = jnp.concatenate([
                    a1_buf[pl.ds(HALO - 1, PAIR), pl.ds(0 * cq, cq)],
                    a1_buf[pl.ds(HALO + 1, PAIR), pl.ds(1 * cq, cq)],
                    a1_buf[pl.ds(HALO - 2, PAIR), pl.ds(2 * cq, cq)],
                    a1_buf[pl.ds(HALO + 2, PAIR), pl.ds(3 * cq, cq)]], axis=1).astype(BF)

            def j_w2(j):
                def run():
                    st['x1', j] = y_buf[:, pl.ds(j * 128, 128)] + _dot(st['g'], w2_t[j])
                return run

            def j_ln3():
                x1 = jnp.concatenate([st['x1', j] for j in range(nD)], axis=1)
                st['z1'] = _ln(x1).astype(BF)

            def j_w3(j):
                def run():
                    st['a3', j] = _gelu(_dot(st['z1'], w3_t[j])).astype(BF)
                return run

            def j_cat():
                st['a3'] = jnp.concatenate([st.pop(('a3', j)) for j in range(nF)], axis=1)

            def j_w4(j):
                def run():
                    cs = pl.ds(j * 128, 128)
                    hh = h_buf[pl.ds(pl.multiple_of(r0 + HALO, 8), PAIR), cs]
                    out_v[pl.ds(r0, PAIR), cs] = (
                        hh + (st['x1', j] + _dot(st['a3'], w4_t[j]))).astype(out_v.dtype)
                return run

            return dict(pre_next=j_pre_next, w1=[j_w1(j) for j in range(nD)], shift=j_shift,
                        w2=[j_w2(j) for j in range(nD)], ln3=j_ln3,
                        w3=[j_w3(j) for j in range(nF)], cat=j_cat,
                        w4=[j_w4(j) for j in range(nD)])

        def attention_only(t, carry):
            ej, oj, j_next_xn = attention_jobs(t)

            def j_wo_wait():
                pl.when(t == 0)(wo_finish)
            _run(_interleave(ej, {after_qkv: [j_wo_wait]})
                 + _interleave(oj, {('qkv', 4, 0): [j_next_xn(True)], after_qkv: [j_next_xn(False)]}))
            return carry

        def fused(t, carry):
            @pl.when(t == LAG)
            def _():
                x_rest_copy().wait()

            @pl.when(t > LAG)
            def _():
                out_copy(t - LAG - 1).start()

            ej, oj, j_next_xn = attention_jobs(t)
            b = mlp_jobs(t - LAG)
            w3, w4 = b['w3'], b['w4']
            fe, fo = {}, {}

            def put(d, label, *jobs):
                d.setdefault(label, []).extend(jobs)
            for i in range(nD):
                put(fe, ('qkv', 2 + i // 2, i % 2), b['w1'][i])
                put(fe, ('qkv', 8 + i // 2, i % 2), b['w2'][i])
            put(fe, ('qkv', 6, 0), b['shift'])
            put(fe, ('qkv', 12, 0), b['ln3'])
            put(fe, ('qkv', 15, 0), w3[0])
            put(fe, 'end', *w3[1:4])
            put(fo, ('qkv', 0, 1), b['pre_next'])
            for k in range(4, nF):
                put(fo, ('qkv', 1 + (k - 4) // 2, (k - 4) % 2), w3[k])
            put(fo, ('qkv', 13, 0), b['cat'])
            put(fo, ('qkv', 14, 0), w4[0])
            put(fo, ('qkv', 15, 0), w4[1])
            put(fo, ('qkv', 4, 0), j_next_xn(True))
            put(fo, after_qkv, j_next_xn(False))
            put(fo, ('s', n_slots - 1), w4[2])
            put(fo, 'end', *w4[3:])
            _run(_interleave(ej, fe) + _interleave(oj, fo))
            return carry

        def mlp_only(c, carry):
            out_copy(c - 1).start()
            b = mlp_jobs(c)
            _run(b['w1'] + [b['shift']] + b['w2'] + [b['ln3'], b['pre_next']] + b['w3'] + [b['cat']] + b['w4'])
            return carry

        prologue()
        store_xn(0, True)
        store_xn(0, False)
        jax.lax.fori_loop(0, LAG, attention_only, 0)
        mlp_prologue()
        jax.lax.fori_loop(LAG, n_pairs, fused, 0)
        jax.lax.fori_loop(n_pairs - LAG, n_pairs, mlp_only, 0)
        out_copy(n_pairs - 1).start()
        pltpu.make_async_copy(out_v, out_hbm, sems.at[OUT_SEM]).wait()

    return kernel, WO_SEM + nD + 6, X0, RING


@functools.partial(jax.jit, static_argnames=("A_seg_len",))
def pallas_sequential_preLN__memory_aug_recurrent_mem_tr__mixer_s_mlp__prompt_kernel(
    A_x, A_mem0, A_Wq, A_Wk, A_Wv, A_Wo, A_seg_len, B_x, B_w1, B_w2, B_w3, B_w4,
):
    _, S, D = A_x.shape
    H, E = A_Wq.shape[1], A_Wq.shape[2]
    F = B_w3.shape[1]
    assert A_seg_len == SEG and A_mem0.shape[1] == MEM and S % PAIR == 0
    nD, nF = D // 128, F // 128

    x = A_x.reshape(S, D)
    mem0 = A_mem0.reshape(MEM, D)
    wo = A_Wo.reshape(H * E, D)

    kernel, n_sems, x0, ring = _make_kernel(S, D, H, E, F)
    any_spec = pl.BlockSpec(memory_space=pl.ANY)
    out = pl.pallas_call(
        kernel,
        in_specs=[any_spec] * 10,
        out_specs=any_spec,
        out_shape=jax.ShapeDtypeStruct((S, D), A_x.dtype),
        scratch_shapes=[
            pltpu.VMEM((3, D, H, E), BF),
            pltpu.VMEM((3, H, D // 2, E), U32),
            pltpu.VMEM((H * E, D), BF),
            pltpu.VMEM((nD, H * E // 2, 128), U32),
            pltpu.VMEM((nD, D, 128), BF),
            pltpu.VMEM((nD, D, 128), BF),
            pltpu.VMEM((nF, D, 128), BF),
            pltpu.VMEM((nD, F, 128), BF),
            pltpu.VMEM((S, D), BF),
            pltpu.VMEM((S, D), BF),
            pltpu.VMEM((MEM, D), BF),
            pltpu.VMEM((x0 // 2, D), U32),
            pltpu.VMEM((ring, (H + NK) * E), U32),
            pltpu.VMEM((16, D), U32),
            pltpu.VMEM((16, D), U32),
            pltpu.VMEM((24, D), U32),
            pltpu.VMEM((16, D), U32),
            pltpu.VMEM((3, 8, H * E), F32),
            pltpu.VMEM((40, H * E), U32),
            pltpu.VMEM((48, D), F32),
            pltpu.VMEM((S + 2 * HALO, D), F32),
            pltpu.VMEM((PAIR + 2 * HALO, D), F32),
            pltpu.VMEM((PAIR, D), F32),
            pltpu.VMEM((PAIR // 2, D), U32),
            pltpu.SemaphoreType.DMA((n_sems,)),
        ],
        compiler_params=pltpu.CompilerParams(
            vmem_limit_bytes=124 * 1024 * 1024,
            disable_bounds_checks=True,
        ),
    )(x, mem0, A_Wq, A_Wk, A_Wv, wo, B_w1, B_w2, B_w3, B_w4)
    return out.reshape(1, S, D)
```
